```python
import jax
import jax.numpy as jnp

def _softmax(x, axis=-1):
    return jax.nn.softmax(x, axis=axis)

def _gelu(x):
    return jax.nn.gelu(x, approximate=True)

def _silu(x):
    return jax.nn.silu(x)

def _sigmoid(x):
    return jax.nn.sigmoid(x)

def _layernorm(x, axis=-1, eps=1e-05):
    m = jnp.mean(x, axis=axis, keepdims=True)
    v = jnp.var(x, axis=axis, keepdims=True)
    return (x - m) / jnp.sqrt(v + eps)

def _scatter_add(tgt, idx, src, axis=0):
    return tgt.at[idx].add(src)

def _segment_sum(src, seg, n):
    return jax.ops.segment_sum(src, seg, n)

class _Rng:

    def __init__(self, key):
        self._k = key

    def _next(self):
        self._k, sub = jax.random.split(self._k)
        return sub

    def normal(self, shape):
        return jax.random.normal(self._next(), shape, dtype=jnp.bfloat16)

    def randint(self, lo, hi, shape):
        return jax.random.randint(self._next(), shape, lo, hi, dtype=jnp.int32)

    def uniform(self, shape, lo=0.0, hi=1.0):
        return jax.random.uniform(self._next(), shape, jnp.bfloat16, lo, hi)

    def permutation(self, n):
        return jax.random.permutation(self._next(), n)
kernel_name = 'parallel_sum__memory_aug_recurrent_mem_tr__mixer_s_mlp__prompt'

def setup_inputs():
    _rng = _Rng(jax.random.key(int.from_bytes(__import__("os").urandom(4), "little")))
    _w = lambda a: (lambda t: t.astype(jnp.bfloat16) if jnp.issubdtype(t.dtype, jnp.floating) else t)(jnp.asarray(a))

    def _A_setup():
        B, S, Dm = (1, 2048, 1024)
        H, Dh = (32, 128)
        M, seg = (8, 32)
        seg = min(seg, S)
        S = S // seg * seg
        return {'x': _w((lambda *s: _rng.normal(s) * 0.05)(B, S, Dm)), 'mem0': _w((lambda *s: _rng.normal(s) * 0.05)(B, M, Dm)), 'Wq': _w((lambda *s: _rng.normal(s) * 0.05)(Dm, H, Dh) * Dm ** (-0.5)), 'Wk': _w((lambda *s: _rng.normal(s) * 0.05)(Dm, H, Dh) * Dm ** (-0.5)), 'Wv': _w((lambda *s: _rng.normal(s) * 0.05)(Dm, H, Dh) * Dm ** (-0.5)), 'Wo': _w((lambda *s: _rng.normal(s) * 0.05)(H, Dh, Dm) * (H * Dh) ** (-0.5)), 'seg_len': seg}
    _A_in = _A_setup()

    def _B_setup():
        B, S, D, F = (1, 2048, 1024, 3584)
        return {'x': _w((lambda *s: _rng.normal(s) * 0.05)(B, S, D)), 'w1': _w((lambda *s: _rng.normal(s) * 0.05)(D, D) * D ** (-0.5)), 'w2': _w((lambda *s: _rng.normal(s) * 0.05)(D, D) * D ** (-0.5)), 'w3': _w((lambda *s: _rng.normal(s) * 0.05)(D, F) * D ** (-0.5)), 'w4': _w((lambda *s: _rng.normal(s) * 0.05)(F, D) * F ** (-0.5))}
    _B_in = _B_setup()
    return {'A_x': _A_in['x'], 'A_mem0': _A_in['mem0'], 'A_Wq': _A_in['Wq'], 'A_Wk': _A_in['Wk'], 'A_Wv': _A_in['Wv'], 'A_Wo': _A_in['Wo'], 'A_seg_len': _A_in['seg_len'], 'B_x': _B_in['x'], 'B_w1': _B_in['w1'], 'B_w2': _B_in['w2'], 'B_w3': _B_in['w3'], 'B_w4': _B_in['w4']}

def reference(A_x, A_mem0, A_Wq, A_Wk, A_Wv, A_Wo, A_seg_len, B_x, B_w1, B_w2, B_w3, B_w4):

    def _A_ref(x, mem0, Wq, Wk, Wv, Wo, seg_len):
        B, S, Dm = x.shape
        H, Dh = (Wq.shape[1], Wq.shape[2])
        M = mem0.shape[1]
        scale = Dh ** (-0.5)
        n_seg = S // seg_len
        L = M + seg_len
        idx = jnp.arange(L)
        mask = (idx[:, None] < M) | (idx[:, None] >= idx[None, :])
        mem = mem0
        outs = []
        for s in range(n_seg):
            xs = x[:, s * seg_len:(s + 1) * seg_len, :].copy()
            h = jnp.concatenate([mem, xs], axis=1)
            q = jnp.einsum('btd,dhe->bhte', h, Wq)
            k = jnp.einsum('btd,dhe->bhte', h, Wk)
            v = jnp.einsum('btd,dhe->bhte', h, Wv)
            scores = jnp.einsum('bhqe,bhke->bhqk', q, k) * scale
            scores = jnp.where(mask[None, None], scores, -1000000000.0)
            p = _softmax(scores, axis=-1)
            o = jnp.einsum('bhqk,bhke->bhqe', p, v)
            o = jnp.einsum('bhte,hed->btd', o, Wo)
            mem = o[:, :M, :].copy()
            outs.append(o[:, M:, :])
        return jnp.concatenate(outs, axis=1)

    def _B_ref(x, w1, w2, w3, w4):
        B, S, D = x.shape
        h = _gelu(_layernorm(x, axis=-1) @ w1)
        c = D // 4
        g0 = jnp.pad(h[:, :, 0 * c:1 * c], ((0, 0), (1, 0), (0, 0)))[:, :S, :]
        g1 = jnp.pad(h[:, :, 1 * c:2 * c], ((0, 0), (0, 1), (0, 0)))[:, 1:, :]
        g2 = jnp.pad(h[:, :, 2 * c:3 * c], ((0, 0), (2, 0), (0, 0)))[:, :S, :]
        g3 = jnp.pad(h[:, :, 3 * c:], ((0, 0), (0, 2), (0, 0)))[:, 2:, :]
        hs = jnp.concatenate([g0, g1, g2, g3], axis=-1) @ w2
        x1 = x + hs
        h2 = _gelu(_layernorm(x1, axis=-1) @ w3) @ w4
        return x1 + h2
    x = A_x
    xn = _layernorm(x, axis=-1)
    return x + _A_ref(xn, A_mem0, A_Wq, A_Wk, A_Wv, A_Wo, A_seg_len) + _B_ref(xn, B_w1, B_w2, B_w3, B_w4)
```

```python
import functools

import jax
import jax.numpy as jnp
import numpy as np
from jax import lax
import jax.experimental.pallas as pl
import jax.experimental.pallas.tpu as pltpu

F32 = jnp.float32
BF16 = jnp.bfloat16
U32 = jnp.uint32

_EPS = 1e-5
_NEG = -1e9
_GELU_C = float(np.sqrt(2.0 / np.pi))

TM = 256


def _dot(a, b):
    return lax.dot_general(a, b, (((1,), (0,)), ((), ())), preferred_element_type=F32)


def _dot_nt(a, b):
    return lax.dot_general(a, b, (((1,), (1,)), ((), ())), preferred_element_type=F32)


def _bf(words):
    return pltpu.bitcast(words, BF16)


def _ln(x):
    inv_n = 1.0 / x.shape[-1]
    xc = x - jnp.sum(x, axis=-1, keepdims=True) * inv_n
    var = jnp.sum(xc * xc, axis=-1, keepdims=True) * inv_n
    return xc * lax.rsqrt(var + _EPS)


def _gelu(x):
    inner = x * (_GELU_C + (_GELU_C * 0.044715) * (x * x))
    hx = 0.5 * x
    return hx + hx * jnp.tanh(inner)


def _kernel(x_hbm, mem0_ref, wq_hbm, wk_hbm, wv_hbm, wo_hbm, w1_hbm, w2_hbm, w3_hbm, w4_hbm,
            out_hbm,
            x_v, xn_v, h_v, part_v, x1_v, l3_v, u_v, out_v,
            wqkv_v, wo_v, w1_v, w2_v, w3_v, w4_v,
            sem_x, sem_w, sem_qkv, sem_out, *, seg):
    S, D = x_hbm.shape
    H, Dh = wq_hbm.shape[1], wq_hbm.shape[2]
    M = mem0_ref.shape[0]
    FF = w3_hbm.shape[1]
    HP = H // 2
    L = M + seg
    n_blk = S // TM
    n_seg = S // seg
    per_blk = 3 * HP // n_blk
    pairs_per_blk = HP // n_blk

    def x_copy(i):
        rows = pl.ds(pl.multiple_of(i * TM, TM), TM)
        return pltpu.make_async_copy(x_hbm.at[rows], x_v.at[rows], sem_x.at[i])

    w_copy = [
        pltpu.make_async_copy(hbm.bitcast(U32), vmem, sem_w.at[n])
        for n, (hbm, vmem) in enumerate(
            ((w1_hbm, w1_v), (w2_hbm, w2_v), (w3_hbm, w3_v), (w4_hbm, w4_v), (wo_hbm, wo_v)))
    ]

    def qkv_copies(i):
        cps = []
        for m, hbm in enumerate((wq_hbm, wk_hbm, wv_hbm)):
            for j in range(pairs_per_blk):
                hp = i * pairs_per_blk + j
                cps.append(pltpu.make_async_copy(
                    hbm.bitcast(U32).at[:, hp, :],
                    wqkv_v.at[m, hp].reshape(D, Dh),
                    sem_qkv.at[i]))
        return cps

    def out_copy(s):
        rows = pl.ds(pl.multiple_of(s * seg, seg), seg)
        return pltpu.make_async_copy(out_v.at[rows], out_hbm.at[rows], sem_out)

    x_copy(0).start()
    w_copy[0].start()
    for i in range(1, n_blk):
        x_copy(i).start()
    w_copy[1].start()
    for c in qkv_copies(0):
        c.start()
    w_copy[2].start()

    h_v[0:8, :] = jnp.zeros((8, D), F32)
    h_v[S + 8:S + 16, :] = jnp.zeros((8, D), F32)

    def norm_block(i):
        rows = pl.ds(pl.multiple_of(i * TM, TM), TM)
        xn = _ln(x_v[rows, :].astype(F32)).astype(BF16).astype(F32)
        xn_v[rows, :] = xn
        l3_v[i % 2] = _ln(xn).astype(BF16)

    def h_block(i):
        h = _gelu(_dot(l3_v[i % 2], _bf(w1_v[...])))
        h_v[pl.ds(pl.multiple_of(i * TM + 8, 8), TM), :] = h

    x_copy(0).wait()
    norm_block(0)
    w_copy[0].wait()

    def b1_body(i, _):
        x_copy(i + 1).wait()
        h_block(i)
        norm_block(i + 1)
        return 0

    lax.fori_loop(0, n_blk - 1, b1_body, 0)
    w_copy[3].start()
    h_block(n_blk - 1)

    c4 = D // 4

    def mix_block(i):
        base = pl.multiple_of(i * TM, TM)
        parts = []
        for g, shift in enumerate((-1, 1, -2, 2)):
            win = h_v[pl.ds(base, TM + 16), g * c4:(g + 1) * c4]
            parts.append(win[8 + shift:8 + shift + TM].astype(BF16))
        hs = _dot(jnp.concatenate(parts, axis=1), _bf(w2_v[...]))
        rows = pl.ds(base, TM)
        x1 = xn_v[rows, :] + hs
        part_v[rows, :] = x1 + x_v[rows, :].astype(F32)
        l3_v[i % 2] = _ln(x1).astype(BF16)

    def up_block(i):
        u_v[...] = _gelu(_dot(l3_v[i % 2], _bf(w3_v[...]))).astype(BF16)

    def down_block(i):
        rows = pl.ds(pl.multiple_of(i * TM, TM), TM)
        part_v[rows, :] += _dot(u_v[...], _bf(w4_v[...]))

    def relayout(i):
        for m in range(3):
            for j in range(pairs_per_blk):
                slab = wqkv_v.at[m, i * pairs_per_blk + j]
                a = slab[...].reshape(D, Dh)
                lo = pltpu.bitcast(a << 16, F32).astype(BF16)
                hi = pltpu.bitcast(a & jnp.uint32(0xFFFF0000), F32).astype(BF16)
                slab[:, 0] = pltpu.bitcast(lo, U32).reshape(D // 16, 8, Dh)
                slab[:, 1] = pltpu.bitcast(hi, U32).reshape(D // 16, 8, Dh)

    w_copy[1].wait()
    mix_block(0)
    w_copy[2].wait()
    w_copy[3].wait()
    w_copy[4].start()

    def b2_body(i, _):
        for c in qkv_copies(i + 1):
            c.start()
        for c in qkv_copies(i):
            c.wait()
        up_block(i)
        mix_block(i + 1)
        relayout(i)
        down_block(i)
        return 0

    lax.fori_loop(0, n_blk - 1, b2_body, 0)
    for c in qkv_copies(n_blk - 1):
        c.wait()
    up_block(n_blk - 1)
    relayout(n_blk - 1)
    down_block(n_blk - 1)
    w_copy[4].wait()

    scale = float(Dh) ** -0.5
    row = lax.broadcasted_iota(jnp.int32, (2 * L, 2 * L), 0)
    col = lax.broadcasted_iota(jnp.int32, (2 * L, 2 * L), 1)
    r_in = jnp.where(row >= L, row - L, row)
    c_in = jnp.where(col >= L, col - L, col)
    same_head = (row >= L) == (col >= L)
    keep = same_head & ((r_in < M) | (r_in >= c_in))
    fill = jnp.where(same_head, _NEG, -jnp.inf).astype(F32)

    G = 2
    n_grp = HP // G

    def project(h, hp):
        res = []
        for m in range(3):
            res.append(jnp.concatenate(
                [_dot(h, _bf(wqkv_v[m, hp, :, j].reshape(D // 2, Dh))) for j in range(2)], axis=0))
        return res

    def scores(q, k):
        s = jnp.where(keep, _dot_nt(q, k.astype(BF16)) * scale, fill)
        e = jnp.exp(s - jnp.max(s, axis=-1, keepdims=True))
        return e, 1.0 / jnp.sum(e, axis=-1, keepdims=True)

    def attend(e, inv, v):
        o = _dot(e, v.astype(BF16)) * inv
        return [o[:L], o[L:]]

    def a_body(s, mem):
        rows = pl.ds(pl.multiple_of(s * seg, seg), seg)
        h = jnp.concatenate([mem, xn_v[rows, :]], axis=0)
        qkv, prob, heads = {}, {}, {}
        acc = None
        for t in range(n_grp + 3):
            if t < n_grp:
                qkv[t] = [project(h, t * G + j) for j in range(G)]
            g = t - 3
            if 0 <= g < n_grp:
                w = _bf(wo_v[g * G * Dh:(g + 1) * G * Dh, :])
                y = _dot(jnp.concatenate(heads.pop(g), axis=1), w)
                acc = y if acc is None else acc + y
            g = t - 2
            if 0 <= g < n_grp:
                heads[g] = []
                for (e, inv), (_, _, v) in zip(prob.pop(g), qkv.pop(g)):
                    heads[g] += attend(e, inv, v)
            g = t - 1
            if 0 <= g < n_grp:
                prob[g] = [scores(q, k) for q, k, _ in qkv[g]]
        out_v[rows, :] = (part_v[rows, :] + acc[M:]).astype(BF16)
        out_copy(s).start()
        return acc[:M]

    lax.fori_loop(0, n_seg, a_body, mem0_ref[...].astype(F32))
    pltpu.make_async_copy(out_v, out_hbm, sem_out).wait()


@functools.partial(jax.jit, static_argnames=("A_seg_len",))
def pallas_parallel_sum__memory_aug_recurrent_mem_tr__mixer_s_mlp__prompt_kernel(
    A_x: jax.Array,
    A_mem0: jax.Array,
    A_Wq: jax.Array,
    A_Wk: jax.Array,
    A_Wv: jax.Array,
    A_Wo: jax.Array,
    A_seg_len: int,
    B_x: jax.Array,
    B_w1: jax.Array,
    B_w2: jax.Array,
    B_w3: jax.Array,
    B_w4: jax.Array,
):
    del B_x
    B, S, D = A_x.shape
    assert B == 1
    H, Dh = A_Wq.shape[1], A_Wq.shape[2]
    M = A_mem0.shape[1]
    FF = B_w3.shape[1]
    n_blk = S // TM

    hbm = pl.BlockSpec(memory_space=pl.ANY)
    out = pl.pallas_call(
        functools.partial(_kernel, seg=int(A_seg_len)),
        out_shape=jax.ShapeDtypeStruct((S, D), A_x.dtype),
        in_specs=[hbm, pl.BlockSpec(memory_space=pltpu.VMEM)] + [hbm] * 8,
        out_specs=hbm,
        scratch_shapes=[
            pltpu.VMEM((S, D), BF16),
            pltpu.VMEM((S, D), F32),
            pltpu.VMEM((S + 16, D), F32),
            pltpu.VMEM((S, D), F32),
            pltpu.VMEM((TM, D), F32),
            pltpu.VMEM((2, TM, D), BF16),
            pltpu.VMEM((TM, FF), BF16),
            pltpu.VMEM((S, D), BF16),
            pltpu.VMEM((3, H // 2, D // 16, 2, 8, Dh), U32),
            pltpu.VMEM((H * Dh // 2, D), U32),
            pltpu.VMEM((D // 2, D), U32),
            pltpu.VMEM((D // 2, D), U32),
            pltpu.VMEM((D // 2, FF), U32),
            pltpu.VMEM((FF // 2, D), U32),
            pltpu.SemaphoreType.DMA((n_blk,)),
            pltpu.SemaphoreType.DMA((5,)),
            pltpu.SemaphoreType.DMA((n_blk,)),
            pltpu.SemaphoreType.DMA,
        ],
        compiler_params=pltpu.CompilerParams(vmem_limit_bytes=120 * 1024 * 1024),
    )(A_x.reshape(S, D), A_mem0.reshape(M, D), A_Wq, A_Wk, A_Wv, A_Wo.reshape(H * Dh, D),
      B_w1, B_w2, B_w3, B_w4)
    return out.reshape(B, S, D)
```

```python
import functools

import jax
import jax.numpy as jnp
import numpy as np
from jax import lax
import jax.experimental.pallas as pl
import jax.experimental.pallas.tpu as pltpu

F32 = jnp.float32
BF16 = jnp.bfloat16
U32 = jnp.uint32

_EPS = 1e-5
_NEG = -1e9
_GELU_C = float(np.sqrt(2.0 / np.pi))

TM = 512
RS = 128
RC = 16
WC = 32
AC = 16
LANE = 128
G = 2
PERIOD = 4
LHS_DT = BF16
SKIP_A = False
SKIP_B = False


def _dot(a, b):
    return lax.dot_general(a, b, (((1,), (0,)), ((), ())), preferred_element_type=F32)


def _dot_nt(a, b):
    return lax.dot_general(a, b, (((1,), (1,)), ((), ())), preferred_element_type=F32)


def _bf(words):
    return pltpu.bitcast(words, BF16)


def _words(x):
    return pltpu.bitcast(x.astype(BF16), U32)


def _at(start, n, align=None):
    return pl.ds(start if isinstance(start, int) else pl.multiple_of(start, align or n), n)


def _ln(x):
    inv_n = 1.0 / x.shape[-1]
    xc = x - jnp.sum(x, axis=-1, keepdims=True) * inv_n
    var = jnp.sum(xc * xc, axis=-1, keepdims=True) * inv_n
    return xc * lax.rsqrt(var + _EPS)


def _gelu(x):
    inner = x * (_GELU_C + (_GELU_C * 0.044715) * (x * x))
    hx = 0.5 * x
    return hx + hx * jnp.tanh(inner)


def _lhs7(a11, a12, a21, a22):
    return (a11 + a22, a21 + a22, a11, a22, a11 + a12, a21 - a11, a12 - a22)


def _rhs5(b11, b12, b21, b22):
    return (b11 + b22, b12 - b22, b21 - b11, b11 + b12, b21 + b22)


_SUM_SLOT = {0: 0, 2: 1, 3: 2, 5: 3, 6: 4}


def _combine(m):
    return (m[0] + m[3] - m[4] + m[6], m[2] + m[4], m[1] + m[3], m[0] - m[1] + m[2] + m[5])


def _weave(main, side):
    out, k = [], 0
    for i, t in enumerate(main):
        out.append(t)
        while k < len(side) and (k + 1) * len(main) <= (i + 1) * len(side):
            out.append(side[k])
            k += 1
    return out


def _run(tasks):
    for t in tasks:
        t()


class _Matmul:
    def __init__(self, quad, kh, pairs, sums_ref, acc_ref, turn):
        self.quad, self.kh, self.pairs = quad, kh, pairs
        self.sums, self.acc, self.turn = sums_ref, acc_ref, turn

    def slot(self, j):
        return self.sums.at[0 if j == 0 else 1 + j % 2]

    def prep(self, j):
        def chunk(r):
            quads = [_bf(self.quad(a, c, j, r, WC)).astype(F32) for a in range(2) for c in range(2)]
            for n, v in enumerate(_rhs5(*quads)):
                self.slot(j)[r:r + WC, n * LANE:(n + 1) * LANE] = _words(v)
        return [functools.partial(chunk, r) for r in range(0, self.kh, WC)]

    def tasks(self, lhs_ref, emit, tail, after):
        out = []
        for j in range(self.pairs):
            def step(c, r, i, j=j):
                if i in _SUM_SLOT:
                    w = self.slot(j)[:, _SUM_SLOT[i] * LANE:(_SUM_SLOT[i] + 1) * LANE]
                else:
                    w = self.quad(i // 4, i // 4, j, 0, self.kh)
                c[i][...] = _dot(_bf(lhs_ref.at[i][r // 2:(r + RS) // 2, :]), _bf(w))

            def finish(c, j, r, k):
                emit(j, r + k, _combine([q[k:k + RC, :] for q in c]))

            steps = []
            for r in range(0, TM // 2, RS):
                c = [self.acc.at[self.turn[0] % 2, q] for q in range(7)]
                self.turn[0] += 1
                steps += _weave([functools.partial(step, c, r, i) for i in range(7)], tail)
                tail = [functools.partial(finish, c, j, r, k) for k in range(0, RS, RC)]
            out += _weave(steps, self.prep(j + 1) if j + 1 < self.pairs else after)
        return out, tail


def _kernel(x_hbm, mem0_ref, wq_hbm, wk_hbm, wv_hbm, wo_hbm, w1_hbm, w2_hbm, w3_hbm, w4_hbm,
            out_hbm,
            x_v, part_v, wqkv_v, wo_v, w3_v, w4_v, l3_v, s3_v, acc_v,
            sem_x, sem_w, sem_a, sem_out, *, seg):
    S, D = x_hbm.shape
    H, Dh = wq_hbm.shape[2], wq_hbm.shape[3]
    M = mem0_ref.shape[0]
    FF = w3_hbm.shape[1]
    HP = H // 2
    L = M + seg
    R = TM // 2
    n_blk = S // TM
    n_it = 2 * n_blk
    n_grp = HP // G
    assert n_grp == n_it
    grows = G * Dh

    def copy(hbm, vmem, sem, rows=slice(None)):
        return pltpu.make_async_copy(hbm.bitcast(U32).at[rows], vmem.at[rows], sem)

    def attn_copies(g):
        copies = [copy(wo_hbm, wo_v, sem_a.at[g], _at(g * grows, grows))]
        for m, hbm in enumerate((wq_hbm, wk_hbm, wv_hbm)):
            for j in range(G):
                hp = g * G + j
                for par in range(2):
                    copies.append(pltpu.make_async_copy(
                        hbm.bitcast(U32).at[:, par, hp, :], wqkv_v.at[m * H + 2 * hp + par], sem_a.at[g]))
        return copies

    def x_rows(r0, n):
        return _bf(x_v[_at(r0 // 2, n // 2), :]).astype(F32)

    def store_lhs(ref, r, top, bot):
        k = top.shape[1] // 2
        for n, v in enumerate(_lhs7(top[:, :k], top[:, k:], bot[:, :k], bot[:, k:])):
            ref.at[n][_at(r // 2, RC // 2), :] = _words(v)

    turn = [0]

    def up_matmul(f):
        def quad(a, c, j, r, n):
            r += a * (D // 4)
            return w3_v[r:r + n, _at(c * (FF // 2) + f * (FF // 4) + j * LANE, LANE)]
        return _Matmul(quad, D // 4, FF // 4 // LANE, s3_v, acc_v, turn)

    def norm3_tasks(i, r0, n):
        def chunk(r):
            store_lhs(l3_v.at[i % 2], r0 + r,
                      *[_ln(part_v[_at(i * TM + half + r0 + r, RC), :]) for half in (0, R)])
        return [functools.partial(chunk, r) for r in range(0, n, RC)]

    w3_copy, w4_copy = copy(w3_hbm, w3_v, sem_w.at[2]), copy(w4_hbm, w4_v, sem_w.at[3])

    def mixing(h_v, w1_v, w2_v, l1_v, l2_v, s1_v, s2_v):
        w1_copy, w2_copy = copy(w1_hbm, w1_v, sem_w.at[0]), copy(w2_hbm, w2_v, sem_w.at[1])
        x_copy = [copy(x_hbm, x_v, sem_x.at[i], _at(i * R, R)) for i in range(n_blk)]

        def cols(j, c):
            return slice(c * (D // 2) + j * LANE, c * (D // 2) + (j + 1) * LANE)

        def square(w, sums):
            def quad(a, c, j, r, n):
                r += a * (D // 4)
                return w[r:r + n, cols(j, c)]
            return _Matmul(quad, D // 4, D // 2 // LANE, sums, acc_v, turn)

        mm1, mm2 = square(w1_v, s1_v), square(w2_v, s2_v)
        tail = []

        def norm1_tasks(i):
            def chunk(r):
                halves = []
                for half in (0, R):
                    r0 = i * TM + half + r
                    xn = _ln(x_rows(r0, RC))
                    part_v[r0:r0 + RC, :] = xn
                    halves.append(_ln(xn))
                store_lhs(l1_v.at[i % 2], r, *halves)
            return [functools.partial(chunk, r) for r in range(0, R, RC)]

        def h_tasks(i):
            def emit(j, r, quad):
                for q, v in enumerate(quad):
                    r0 = 8 + i * TM + (q // 2) * R + r
                    h_v[r0:r0 + RC, cols(j, q % 2)] = _gelu(v)
            return mm1.tasks(l1_v.at[i % 2], emit, list(tail), [])

        def shifted(r0):
            c4 = D // 4
            parts = []
            for g, shift in enumerate((-1, 1, -2, 2)):
                c = slice(g * c4, (g + 1) * c4)
                if shift < 0:
                    parts.append(pltpu.roll(h_v[r0:r0 + RC + 8, c], -shift, 0)[8:])
                else:
                    parts.append(pltpu.roll(h_v[r0 + 8:r0 + RC + 16, c], RC + 8 - shift, 0)[:RC])
            return jnp.concatenate(parts, axis=1)

        def shift_tasks(i):
            def chunk(r):
                store_lhs(l2_v.at[i % 2], r, *[shifted(i * TM + half + r) for half in (0, R)])
            return [functools.partial(chunk, r) for r in range(0, R, RC)]

        def mix_tasks(i):
            def emit(j, r, quad):
                for q, v in enumerate(quad):
                    r0 = i * TM + (q // 2) * R + r
                    part_v[r0:r0 + RC, cols(j, q % 2)] += v
            return mm2.tasks(l2_v.at[i % 2], emit, list(tail), [])

        def stage(tasks, side):
            main, last = tasks
            _run(main[:16] + _weave(main[16:], side))
            tail[:] = last

        def third(hbm, vmem, n, k):
            rows = vmem.shape[0] // 2
            copy(hbm, vmem, sem_w.at[n], _at(k * rows, rows)).start()

        with jax.named_scope("pro"):
            x_copy[0].start()
            w1_copy.start()
            x_copy[1].start()
            x_copy[2].start()
            h_v[0:8, :] = jnp.zeros((8, D), F32)
            h_v[S + 8:S + 16, :] = jnp.zeros((8, D), F32)
            x_copy[0].wait()
            _run(norm1_tasks(0))
            w1_copy.wait()
            _run(mm1.prep(0))
            x_copy[1].wait()
        with jax.named_scope("b1"):
            x_copy[3].start()
            w2_copy.start()
            stage(h_tasks(0), norm1_tasks(1))
            x_copy[2].wait()
            third(w3_hbm, w3_v, 2, 0)
            stage(h_tasks(1), norm1_tasks(2))
            x_copy[3].wait()
            w2_copy.wait()
            third(w3_hbm, w3_v, 2, 1)
            stage(h_tasks(2), norm1_tasks(3) + mm2.prep(0))
            stage(h_tasks(3), shift_tasks(0))
            third(w4_hbm, w4_v, 3, 0)
            stage(mix_tasks(0), shift_tasks(1))
            third(w4_hbm, w4_v, 3, 1)
            stage(mix_tasks(1), shift_tasks(2))
            w3_copy.wait()
            for c in attn_copies(0):
                c.start()
            stage(mix_tasks(2), shift_tasks(3))
            stage(mix_tasks(3), norm3_tasks(0, 0, R) + up_matmul(0).prep(0))
            _run(tail)

    if not SKIP_B:
        pl.run_scoped(
            mixing,
            pltpu.VMEM((S + 16, D), F32),
            pltpu.VMEM((D // 2, D), U32),
            pltpu.VMEM((D // 2, D), U32),
            pltpu.VMEM((2, 7, R // 2, D // 2), U32),
            pltpu.VMEM((2, 7, R // 2, D // 2), U32),
            pltpu.VMEM((3, D // 4, 5 * LANE), U32),
            pltpu.VMEM((3, D // 4, 5 * LANE), U32),
        )

    def channel_mlp(sq_v, so_v, u_v, s4_v):
        def attn_weight_tasks(g):
            def qkv(m, j, r):
                slab = m * HP + g * G + j
                even, odd = wqkv_v.at[2 * slab], wqkv_v.at[2 * slab + 1]
                quads = []
                for rr in (r, r + D // 4):
                    a, b = even[rr:rr + AC, :], odd[rr:rr + AC, :]
                    h0 = (a & jnp.uint32(0xFFFF)) | (b << 16)
                    h1 = (a >> 16) | (b & jnp.uint32(0xFFFF0000))
                    even[rr:rr + AC, :] = h0
                    odd[rr:rr + AC, :] = h1
                    quads += [_bf(h0).astype(F32), _bf(h1).astype(F32)]
                for n, v in enumerate(_rhs5(*quads)):
                    sq_v.at[slab][r:r + AC, n * LANE:(n + 1) * LANE] = _words(v)

            def out(r):
                quads = [_bf(wo_v[_at(g * grows + a * (grows // 2) + r, 8), c * (D // 2):(c + 1) * (D // 2)]
                             ).astype(F32) for a in range(2) for c in range(2)]
                for n, v in enumerate(_rhs5(*quads)):
                    so_v.at[g][r:r + 8, n * (D // 2):(n + 1) * (D // 2)] = _words(v)

            return ([functools.partial(qkv, m, j, r) for m in range(3) for j in range(G)
                     for r in range(0, D // 4, AC)]
                    + [functools.partial(out, r) for r in range(0, grows // 2, 8)])

        w4_copy.wait()

        def body(it, _):
            i, f = it // 2, it % 2

            @pl.when(it + 1 < n_it)
            def _():
                for c in attn_copies(it + 1):
                    c.start()

            for c in attn_copies(it):
                c.wait()

            def quad4(a, c, j, r, n):
                lanes = slice(c * (D // 2) + j * LANE, c * (D // 2) + (j + 1) * LANE)
                return w4_v[_at(a * (FF // 4) + f * (FF // 8) + r, n, WC), lanes]

            mm3 = up_matmul(f)
            mm4 = _Matmul(quad4, FF // 8, D // 2 // LANE, s4_v, acc_v, turn)

            def emit_up(j, r, quad):
                for n, v in enumerate(_lhs7(*[_gelu(q) for q in quad])):
                    u_v.at[n][r // 2:(r + RC) // 2, j * LANE:(j + 1) * LANE] = _words(v)

            def emit_down(j, r, quad):
                for q, v in enumerate(quad):
                    c0 = (q % 2) * (D // 2) + j * LANE
                    part_v[_at(i * TM + (q // 2) * R + r, RC), c0:c0 + LANE] += v

            up, last = mm3.tasks(l3_v.at[i % 2], emit_up, [], [])
            down, end = mm4.tasks(u_v, emit_down, last, up_matmul(1 - f).prep(0))
            nxt = jnp.where(i + 1 < n_blk, i + 1, i - 1)
            side = attn_weight_tasks(it)
            cut = len(side) // 3
            _run(_weave(_weave(up, mm4.prep(0)), side[:cut]))
            _run(_weave(_weave(down, norm3_tasks(nxt, f * (R // 2), R // 2)), side[cut:]))
            _run(end)
            return 0

        with jax.named_scope("b2"):
            lax.fori_loop(0, n_it, body, 0)

    def recurrence(sq_v, so_v, own_v, lhs_v, next_v, hq_v, ho_v):
        scale = float(Dh) ** -0.5
        own = seg - 8
        row = lax.broadcasted_iota(jnp.int32, (2 * L, 2 * L), 0)
        col = lax.broadcasted_iota(jnp.int32, (2 * L, 2 * L), 1)
        r_in = jnp.where(row >= L, row - L, row)
        c_in = jnp.where(col >= L, col - L, col)
        same_head = (row >= L) == (col >= L)
        keep = same_head & ((r_in < M) | (r_in >= c_in))
        fill = jnp.where(same_head, _NEG, -jnp.inf).astype(F32)

        def load_own(s):
            own_v[...] = _ln(x_rows(s * seg, seg)[:own])

        def load_held(s, q):
            next_v[8 * q:8 * q + 8, :] = _ln(x_rows(s * seg + seg - 16, 16)[8:])

        def scores(q, k):
            s = jnp.where(keep, _dot_nt(q, k.astype(BF16)) * scale, fill)
            e = jnp.exp(s - jnp.max(s, axis=-1, keepdims=True))
            return e, 1.0 / jnp.sum(e, axis=-1, keepdims=True)

        def step(s, r, mem):
            first = isinstance(r, int) and r == 0
            last = isinstance(r, int) and r == PERIOD - 1
            top = jnp.concatenate([mem, own_v[...]], axis=0)
            if first:
                bot = next_v[...]
                k = D // 2
                for n, v in enumerate(_lhs7(top[:, :k], top[:, k:], bot[:, :k], bot[:, k:])):
                    lhs_v.at[n][...] = _words(v)
            top = top.astype(LHS_DT)

            def project(hp):
                res = []
                for m in range(3):
                    h0 = m * H + 2 * hp
                    if first:
                        prods = []
                        for i in range(7):
                            if i in _SUM_SLOT:
                                w = sq_v.at[m * HP + hp][:, _SUM_SLOT[i] * LANE:(_SUM_SLOT[i] + 1) * LANE]
                            else:
                                w = wqkv_v[h0 + i // 4, (i // 4) * (D // 4):(i // 4 + 1) * (D // 4), :]
                            prods.append(_dot(_bf(lhs_v.at[i][...]), _bf(w)))
                        c11, c12, c21, c22 = _combine(prods)
                        hq_v[h0], hq_v[h0 + 1] = c21[8:], c22[8:]
                        res.append(jnp.concatenate([c11, c21[:8], c12, c22[:8]], axis=0))
                    else:
                        parts = []
                        for j in range(2):
                            parts += [_dot(top, _bf(wqkv_v[h0 + j])), hq_v[h0 + j, _at(8 * (r - 1), 8), :]]
                        res.append(jnp.concatenate(parts, axis=0))
                return res

            def merge(g, heads, acc):
                tops = jnp.concatenate([o[:L - 8] for o in heads], axis=1)
                held = jnp.concatenate([o[L - 8:] for o in heads], axis=1)
                lanes = slice(2 * g * grows, 2 * (g + 1) * grows)
                if last:
                    bots = jnp.concatenate([ho_v[:, lanes], held], axis=0)
                    lhs = _lhs7(tops[:, :grows], tops[:, grows:], bots[:, :grows], bots[:, grows:])
                    y = []
                    for i in range(7):
                        if i in _SUM_SLOT:
                            w = so_v.at[g][:, _SUM_SLOT[i] * (D // 2):(_SUM_SLOT[i] + 1) * (D // 2)]
                        else:
                            r0 = g * grows + (i // 4) * (grows // 2)
                            w = wo_v[r0:r0 + grows // 2, (i // 4) * (D // 2):(i // 4 + 1) * (D // 2)]
                        y.append(_dot(lhs[i].astype(LHS_DT), _bf(w)))
                else:
                    ho_v[_at(8 * r, 8), lanes] = held
                    y = [_dot(tops.astype(LHS_DT), _bf(wo_v[g * grows:(g + 1) * grows, :]))]
                return y if acc is None else [a + b for a, b in zip(acc, y)]

            qkv, prob, heads = {}, {}, {}
            acc = None
            for t in range(n_grp + 3):
                if t < n_grp:
                    qkv[t] = [project(t * G + j) for j in range(G)]
                if 0 <= t - 3 < n_grp:
                    acc = merge(t - 3, heads.pop(t - 3), acc)
                if 0 <= t - 2 < n_grp:
                    heads[t - 2] = []
                    for (e, inv), (_, _, v) in zip(prob.pop(t - 2), qkv.pop(t - 2)):
                        o = _dot(e, v.astype(BF16)) * inv
                        heads[t - 2] += [o[:L], o[L:]]
                if 0 <= t - 1 < n_grp:
                    prob[t - 1] = [scores(q, k) for q, k, _ in qkv[t - 1]]
                if last and 1 <= t <= PERIOD:
                    load_held(jnp.minimum(s + t, S // seg - 1), t - 1)
                if t == n_grp - 1:
                    load_own(jnp.minimum(s + 1, S // seg - 1))
            if last:
                c11, c12, c21, c22 = _combine(acc)
                y, y_held = jnp.concatenate([c11, c12], axis=1), jnp.concatenate([c21, c22], axis=1)
            else:
                y = acc[0]
            base = x_rows(s * seg, seg) + part_v[_at(s * seg, seg), :]
            x_v[_at(s * (seg // 2), 8), :] = _words(base[:16] + y[M:M + 16])
            part_v[_at(s * seg + 16, 16), :] = jnp.concatenate([base[16:24] + y[M + 16:], base[24:]], axis=0)
            if last:
                for q in range(PERIOD):
                    r0 = (s - (PERIOD - 1) + q) * seg + 16
                    rest = part_v[_at(r0, 16), :]
                    x_v[_at(r0 // 2, 8), :] = _words(jnp.concatenate(
                        [rest[:8], rest[8:] + y_held[8 * q:8 * q + 8]], axis=0))
            return y[:M]

        def period(p, mem):
            s = p * PERIOD
            mem = step(s, 0, mem)
            mem = lax.fori_loop(1, PERIOD - 1, lambda r, mem: step(s + r, r, mem), mem)
            mem = step(s + PERIOD - 1, PERIOD - 1, mem)
            rows = _at(s * (seg // 2), PERIOD * seg // 2)
            pltpu.make_async_copy(x_v.at[rows], out_hbm.bitcast(U32).at[rows], sem_out).start()
            return mem

        load_own(0)
        for q in range(PERIOD):
            load_held(q, q)
        with jax.named_scope("aloop"):
            lax.fori_loop(0, S // seg // PERIOD, period, mem0_ref[...].astype(F32))

    def rest(sq_v, so_v):
        if not SKIP_B:
            pl.run_scoped(
                functools.partial(channel_mlp, sq_v, so_v),
                pltpu.VMEM((7, R // 2, FF // 4), U32),
                pltpu.VMEM((3, FF // 8, 5 * LANE), U32),
            )
        if SKIP_A:
            x_v[0:8, :] = sq_v[5, 0:8, 0:LANE].repeat(8, 1) + so_v[5, 0:8, 0:D] + pltpu.bitcast(part_v[0:8, :], U32)
            pltpu.make_async_copy(x_v, out_hbm.bitcast(U32), sem_out).start()
            return
        pl.run_scoped(
            functools.partial(recurrence, sq_v, so_v),
            pltpu.VMEM((seg - 8, D), F32),
            pltpu.VMEM((7, (L - 8) // 2, D // 2), U32),
            pltpu.VMEM((8 * PERIOD, D), F32),
            pltpu.VMEM((3 * H, 8 * (PERIOD - 1), Dh), F32),
            pltpu.VMEM((8 * (PERIOD - 1), H * Dh), F32),
        )

    pl.run_scoped(
        rest,
        pltpu.VMEM((3 * HP, D // 4, 5 * LANE), U32),
        pltpu.VMEM((n_grp, grows // 2, 5 * (D // 2)), U32),
    )
    pltpu.make_async_copy(x_v, out_hbm.bitcast(U32), sem_out).wait()


@functools.partial(jax.jit, static_argnames=("A_seg_len",))
def pallas_parallel_sum__memory_aug_recurrent_mem_tr__mixer_s_mlp__prompt_kernel(
    A_x, A_mem0, A_Wq, A_Wk, A_Wv, A_Wo, A_seg_len, B_x, B_w1, B_w2, B_w3, B_w4):
    del B_x
    B, S, D = A_x.shape
    assert B == 1
    H, Dh = A_Wq.shape[1], A_Wq.shape[2]
    M = A_mem0.shape[1]
    FF = B_w3.shape[1]
    n_blk = S // TM

    hbm = pl.BlockSpec(memory_space=pl.ANY)
    out = pl.pallas_call(
        functools.partial(_kernel, seg=int(A_seg_len)),
        out_shape=jax.ShapeDtypeStruct((S, D), A_x.dtype),
        in_specs=[hbm, pl.BlockSpec(memory_space=pltpu.VMEM)] + [hbm] * 8,
        out_specs=hbm,
        scratch_shapes=[
            pltpu.VMEM((S // 2, D), U32),
            pltpu.VMEM((S, D), F32),
            pltpu.VMEM((3 * H, D // 2, Dh), U32),
            pltpu.VMEM((H * Dh // 2, D), U32),
            pltpu.VMEM((D // 2, FF), U32),
            pltpu.VMEM((FF // 2, D), U32),
            pltpu.VMEM((2, 7, TM // 4, D // 2), U32),
            pltpu.VMEM((3, D // 4, 5 * LANE), U32),
            pltpu.VMEM((2, 7, RS, LANE), F32),
            pltpu.SemaphoreType.DMA((n_blk,)),
            pltpu.SemaphoreType.DMA((4,)),
            pltpu.SemaphoreType.DMA((2 * n_blk,)),
            pltpu.SemaphoreType.DMA,
        ],
        compiler_params=pltpu.CompilerParams(vmem_limit_bytes=126 * 1024 * 1024),
    )(A_x.reshape(S, D), A_mem0.reshape(M, D),
      A_Wq.reshape(D // 2, 2, H, Dh), A_Wk.reshape(D // 2, 2, H, Dh), A_Wv.reshape(D // 2, 2, H, Dh),
      A_Wo.reshape(H * Dh, D), B_w1, B_w2, B_w3, B_w4)
    return out.reshape(B, S, D)
```

```python
import functools

import jax
import jax.numpy as jnp
import numpy as np
from jax import lax
import jax.experimental.pallas as pl
import jax.experimental.pallas.tpu as pltpu

F32 = jnp.float32
BF16 = jnp.bfloat16
U32 = jnp.uint32

_EPS = 1e-5
_NEG = -1e9
_GELU_C = float(np.sqrt(2.0 / np.pi))

LANE = 128
TM = 512
RC = 16
AC = 8
G = 2
PERIOD = 4
LAG = 4
CUT = 0.6
LHS_DT = BF16
SKIP_B1 = False
SKIP_B2 = False
SKIP_A = False


def _dot(a, b):
    return lax.dot_general(a, b, (((1,), (0,)), ((), ())), preferred_element_type=F32)


def _dot_nt(a, b):
    return lax.dot_general(a, b, (((1,), (1,)), ((), ())), preferred_element_type=F32)


def _bf(words):
    return pltpu.bitcast(words, BF16)


def _words(x):
    return pltpu.bitcast(x.astype(BF16), U32)


def _at(start, n, align=None):
    return pl.ds(start if isinstance(start, int) else pl.multiple_of(start, align or n), n)


def _ln(x):
    inv_n = 1.0 / x.shape[-1]
    xc = x - jnp.sum(x, axis=-1, keepdims=True) * inv_n
    var = jnp.sum(xc * xc, axis=-1, keepdims=True) * inv_n
    return xc * lax.rsqrt(var + _EPS)


def _gelu(x):
    inner = x * (_GELU_C + (_GELU_C * 0.044715) * (x * x))
    hx = 0.5 * x
    return hx + hx * jnp.tanh(inner)


def _lhs7(a11, a12, a21, a22):
    return (a11 + a22, a21 + a22, a11, a22, a11 + a12, a21 - a11, a12 - a22)


def _rhs(i, b):
    if i in (1, 4):
        return b(i // 4, i // 4)
    p, q, sign = {0: ((0, 0), (1, 1), 1), 2: ((0, 1), (1, 1), -1), 3: ((1, 0), (0, 0), -1),
                  5: ((0, 0), (0, 1), 1), 6: ((1, 0), (1, 1), 1)}[i]
    p, q = b(*p).astype(F32), b(*q).astype(F32)
    return (p + q if sign > 0 else p - q).astype(BF16)


_STORED = (0, 2, 3, 5, 6)


def _combine(m):
    return (m[0] + m[3] - m[4] + m[6], m[2] + m[4], m[1] + m[3], m[0] - m[1] + m[2] + m[5])


def _weave(main, side):
    out, k = [], 0
    for i, task in enumerate(main):
        out.append(task)
        while k < len(side) and (k + 1) * len(main) <= (i + 1) * len(side):
            out.append(side[k])
            k += 1
    return out


def _run(tasks):
    for task in tasks:
        task()


def _finish_tasks(acc, emit):
    def finish(r):
        emit(r, _combine([pltpu.bitcast(ref[r0 + r:r0 + r + RC, c0:c0 + LANE], F32) for ref, r0, c0 in acc]))
    return [functools.partial(finish, r) for r in range(0, TM // 2, RC)]


def _matmul_tasks(lhs, quad, pairs, next_acc, emit, tail):
    def product(acc, j, i):
        ref, r0, c0 = acc[i]
        ref[r0:r0 + TM // 2, c0:c0 + LANE] = pltpu.bitcast(
            _dot(lhs(i), _rhs(i, functools.partial(quad, j))), U32)

    out = []
    for j in range(pairs):
        acc = next_acc()
        out += _weave([functools.partial(product, acc, j, i) for i in (1, 0, 2, 3, 4, 5, 6)], tail)
        tail = _finish_tasks(acc, functools.partial(emit, j))
    return out, tail


def _kernel(x_hbm, mem0_ref, wq_hbm, wk_hbm, wv_hbm, wo_hbm, w1_hbm, w2_hbm, w3_hbm, w4_hbm,
            out_hbm,
            x_v, part_v, wqkv_v, wo_v, w3_v, w4_v, l3_v,
            sem_x, sem_w1, sem_w, sem_a, sem_out, *, seg):
    S, D = x_hbm.shape
    H, Dh = wq_hbm.shape[2], wq_hbm.shape[3]
    M = mem0_ref.shape[0]
    FF = w3_hbm.shape[1]
    HP = H // 2
    L = M + seg
    R = TM // 2
    n_blk = S // TM
    n_seg = S // seg
    n_grp = HP // G
    assert n_grp == 2 * n_blk
    grows = G * Dh

    def copy(hbm, vmem, sem, *idx):
        return pltpu.make_async_copy(hbm.bitcast(U32).at[idx], vmem.at[idx], sem)

    def attn_copies(g):
        copies = [copy(wo_hbm, wo_v, sem_a.at[g], _at(g * grows, grows))]
        for m, hbm in enumerate((wq_hbm, wk_hbm, wv_hbm)):
            for j in range(G):
                hp = g * G + j
                for par in range(2):
                    copies.append(pltpu.make_async_copy(
                        hbm.bitcast(U32).at[:, par, hp, :], wqkv_v.at[m * H + 2 * hp + par], sem_a.at[g]))
        return copies

    def half_copy(hbm, vmem, n, k):
        rows = vmem.shape[0] // 2
        return copy(hbm, vmem, sem_w.at[n], _at(k * rows, rows))

    def x_rows(r0, n):
        return _bf(x_v[_at(r0 // 2, n // 2), :]).astype(F32)

    def cols(j, c):
        return slice(c * (D // 2) + j * LANE, c * (D // 2) + (j + 1) * LANE)

    def mixing(h_v, w1_v, w2_v, l1_v, l2_v, acc_v):
        pairs = D // 2 // LANE
        w1_copies = [[copy(w1_hbm, w1_v, sem_w1.at[j], slice(None), cols(j, c)) for c in range(2)]
                     for j in range(pairs)]
        w2_copy = copy(w2_hbm, w2_v, sem_w.at[0], slice(None))
        first = [[copy(x_hbm, x_v, sem_x.at[n_blk + k], _at(half + k * R // 8, R // 8))
                  for half in (0, R // 2)] for k in range(4)]
        x_copy = {i: copy(x_hbm, x_v, sem_x.at[i], _at(i * R, R)) for i in range(1, n_blk)}
        state = {"turn": 0, "tail": []}

        def next_acc():
            state["turn"] += 1
            return [(acc_v.at[state["turn"] % 2, i], 0, 0) for i in range(7)]

        def lhs_tasks(ref, rows):
            def chunk(r):
                top, bot = rows(r), rows(R + r)
                k = D // 2
                for n, v in enumerate(_lhs7(top[:, :k], top[:, k:], bot[:, :k], bot[:, k:])):
                    ref.at[n][r // 2:(r + RC) // 2, :] = _words(v)
            return [functools.partial(chunk, r) for r in range(0, R, RC)]

        def norm1(i):
            def rows(r):
                r0 = i * TM + r
                xn = _ln(x_rows(r0, RC))
                part_v[r0:r0 + RC, :] = xn
                return _ln(xn)
            return lhs_tasks(l1_v.at[i % 2], rows)

        def shift(i):
            def rows(r):
                r0 = i * TM + r
                parts = []
                for g, by in enumerate((-1, 1, -2, 2)):
                    c = slice(g * D // 4, (g + 1) * D // 4)
                    if by < 0:
                        parts.append(pltpu.roll(h_v[r0:r0 + RC + 8, c], -by, 0)[8:])
                    else:
                        parts.append(pltpu.roll(h_v[r0 + 8:r0 + RC + 16, c], RC + 8 - by, 0)[:RC])
                return jnp.concatenate(parts, axis=1)
            return lhs_tasks(l2_v.at[i % 2], rows)

        def norm3(i):
            return lhs_tasks(l3_v.at[i], lambda r: _ln(part_v[i * TM + r:i * TM + r + RC, :]))

        def stage(i, second, side, waits=()):
            lhs, w = (l2_v, w2_v) if second else (l1_v, w1_v)

            def emit(j, r, quads):
                for q, v in enumerate(quads):
                    r0 = i * TM + (q // 2) * R + r
                    if second:
                        part_v[r0:r0 + RC, cols(j, q % 2)] += v
                    else:
                        h_v[8 + r0:8 + r0 + RC, cols(j, q % 2)] = _gelu(v)

            main, state["tail"] = _matmul_tasks(
                lambda n: _bf(lhs.at[i % 2, n][...]),
                lambda j, a, c: _bf(w[a * (D // 4):(a + 1) * (D // 4), cols(j, c)]),
                pairs, next_acc, emit, state["tail"])
            n = 7 + R // RC
            if waits:
                main = main[:7] + waits[0] + main[7:7 + n] + waits[1] + main[7 + n:7 + 2 * n] + waits[2] + main[7 + 2 * n:]
            _run(main[:n] + _weave(main[n:], side))

        with jax.named_scope("pro"):
            for c in sum(first, []) + sum(w1_copies[:2], []) + [x_copy[1]] + sum(w1_copies[2:], []) + [x_copy[2]]:
                c.start()
            h_v[0:8, :] = jnp.zeros((8, D), F32)
            h_v[S + 8:S + 16, :] = jnp.zeros((8, D), F32)
            todo = norm1(0)
            for k in range(4):
                for c in first[k]:
                    c.wait()
                _run(todo[k * len(todo) // 4:(k + 1) * len(todo) // 4])
            for c in w1_copies[0]:
                c.wait()
        with jax.named_scope("b1"):
            waits = [[c.wait for c in cs] for cs in w1_copies[1:]]
            waits[0].append(x_copy[1].wait)
            x_copy[3].start()
            w2_copy.start()
            stage(0, False, norm1(1), waits)
            x_copy[2].wait()
            half_copy(w3_hbm, w3_v, 1, 0).start()
            stage(1, False, norm1(2))
            x_copy[3].wait()
            half_copy(w3_hbm, w3_v, 1, 1).start()
            stage(2, False, norm1(3))
            w2_copy.wait()
            stage(3, False, shift(0))
            half_copy(w4_hbm, w4_v, 2, 0).start()
            stage(0, True, shift(1))
            half_copy(w4_hbm, w4_v, 2, 1).start()
            stage(1, True, _weave(shift(2), norm3(0)))
            for c in attn_copies(0):
                c.start()
            stage(2, True, _weave(shift(3), norm3(1)))
            stage(3, True, norm3(2))
            _run(state["tail"] + norm3(3))

    if SKIP_B1:
        for c in [half_copy(w3_hbm, w3_v, 1, 0), half_copy(w3_hbm, w3_v, 1, 1), half_copy(w4_hbm, w4_v, 2, 0),
                  half_copy(w4_hbm, w4_v, 2, 1)] + attn_copies(0):
            c.start()
    else:
        pl.run_scoped(
            mixing,
            pltpu.VMEM((S + 16, D), F32),
            pltpu.VMEM((D // 2, D), U32),
            pltpu.VMEM((D // 2, D), U32),
            pltpu.VMEM((2, 7, R // 2, D // 2), U32),
            pltpu.VMEM((2, 7, R // 2, D // 2), U32),
            pltpu.VMEM((2, 7, R, LANE), U32),
        )
    for k in range(2):
        half_copy(w3_hbm, w3_v, 1, k).wait()
        half_copy(w4_hbm, w4_v, 2, k).wait()

    def channel_mlp(sums_v, u_v):
        up_pairs, down_pairs = FF // 4 // LANE, D // 2 // LANE

        def acc(slot):
            return [(sums_v.at[4 * HP + n // 5], 0, (n % 5) * LANE) for n in range(7 * slot, 7 * slot + 7)]

        def attn_weight_tasks(g):
            def store(slab, r, quads):
                for n, i in enumerate(_STORED):
                    sums_v.at[slab][r:r + AC, n * LANE:(n + 1) * LANE] = pltpu.bitcast(
                        _rhs(i, lambda a, c: quads[2 * a + c]), U32)

            def qkv(m, j, r):
                slab = m * HP + g * G + j
                even, odd = wqkv_v.at[2 * slab], wqkv_v.at[2 * slab + 1]
                quads = []
                for rr in (r, r + D // 4):
                    a, b = even[rr:rr + AC, :], odd[rr:rr + AC, :]
                    h0 = (a & jnp.uint32(0xFFFF)) | (b << 16)
                    h1 = (a >> 16) | (b & jnp.uint32(0xFFFF0000))
                    even[rr:rr + AC, :] = h0
                    odd[rr:rr + AC, :] = h1
                    quads += [_bf(h0), _bf(h1)]
                store(slab, r, quads)

            def out(j, r):
                store(3 * HP + 2 * g + j // 2, r + (j % 2) * (grows // 2),
                      [_bf(wo_v[_at(g * grows + a * (grows // 2) + r, AC), cols(j, c)])
                       for a in range(2) for c in range(2)])

            return ([functools.partial(qkv, m, j, r) for m in range(3) for j in range(G)
                     for r in range(0, D // 4, AC)]
                    + [functools.partial(out, j, r) for j in range(down_pairs)
                       for r in range(0, grows // 2, AC)])

        def emit_up(j, r, quads):
            for n, v in enumerate(_lhs7(*[_gelu(q) for q in quads])):
                u_v.at[n][r // 2:(r + RC) // 2, j * LANE:(j + 1) * LANE] = _words(v)

        def emit_down(i, j, r, quads):
            for q, v in enumerate(quads):
                part_v[_at(i * TM + (q // 2) * R + r, RC), cols(j, q % 2)] += v

        def last_epilogue(i):
            return _finish_tasks(acc(2), functools.partial(emit_down, i, down_pairs - 1))

        for ref, r0, c0 in acc(2):
            ref[r0:r0 + R, c0:c0 + LANE] = jnp.zeros((R, LANE), U32)

        def body(it, _):
            i, f = it // 2, it % 2

            @pl.when(it + 1 < n_grp)
            def _():
                for c in attn_copies(it + 1):
                    c.start()

            for c in attn_copies(it):
                c.wait()
            slots = [n % 2 for n in range(up_pairs + down_pairs - 1)] + [2]
            next_acc = lambda: acc(slots.pop(0))
            up, tail = _matmul_tasks(
                lambda n: _bf(l3_v.at[i, n][...]),
                lambda j, a, c: _bf(w3_v[a * (D // 4):(a + 1) * (D // 4),
                                         _at(c * (FF // 2) + f * (FF // 4) + j * LANE, LANE)]),
                up_pairs, next_acc, emit_up, last_epilogue(jnp.maximum(it - 1, 0) // 2))
            down, _ = _matmul_tasks(
                lambda n: _bf(u_v.at[n][...]),
                lambda j, a, c: _bf(w4_v[_at(a * (FF // 4) + f * (FF // 8), FF // 8, 64), cols(j, c)]),
                down_pairs, next_acc, functools.partial(emit_down, i), [])
            side = attn_weight_tasks(it)
            cut = int(len(side) * CUT)
            _run(_weave(up, side[:cut]) + tail + _weave(down, side[cut:]))
            return 0

        with jax.named_scope("b2"):
            lax.fori_loop(0, n_grp, body, 0)
            _run(last_epilogue(n_blk - 1))

    def recurrence(sums_v, own_v, lhs_v, next_v, hq_v, ho_v):
        scale = float(Dh) ** -0.5
        own = seg - 8
        row = lax.broadcasted_iota(jnp.int32, (2 * L, 2 * L), 0)
        col = lax.broadcasted_iota(jnp.int32, (2 * L, 2 * L), 1)
        r_in = jnp.where(row >= L, row - L, row)
        c_in = jnp.where(col >= L, col - L, col)
        same_head = (row >= L) == (col >= L)
        keep = same_head & ((r_in < M) | (r_in >= c_in))
        fill = jnp.where(same_head, _NEG, -jnp.inf).astype(F32)

        def load_own(s):
            own_v[...] = _ln(x_rows(s * seg, seg)[:own])

        def load_held(s, q):
            next_v[8 * q:8 * q + 8, :] = _ln(x_rows(s * seg + seg - 16, 16)[8:])

        def scores(q, k):
            s = jnp.where(keep, _dot_nt(q, k.astype(BF16)) * scale, fill)
            e = jnp.exp(s - jnp.max(s, axis=-1, keepdims=True))
            return e, 1.0 / jnp.sum(e, axis=-1, keepdims=True)

        def stored(slab, i, rows=slice(None)):
            n = _STORED.index(i)
            return sums_v.at[slab][rows, n * LANE:(n + 1) * LANE]

        def step(s, r, mem):
            first = isinstance(r, int) and r == 0
            last = isinstance(r, int) and r == PERIOD - 1
            top = jnp.concatenate([mem, own_v[...]], axis=0)
            if first:
                bot, k = next_v[...], D // 2
                for n, v in enumerate(_lhs7(top[:, :k], top[:, k:], bot[:, :k], bot[:, k:])):
                    lhs_v.at[n][...] = _words(v)
            top = top.astype(LHS_DT)

            def project(hp):
                res = []
                for m in range(3):
                    h0 = m * H + 2 * hp
                    if first:
                        prods = []
                        for i in range(7):
                            if i in _STORED:
                                w = stored(m * HP + hp, i)
                            else:
                                w = wqkv_v[h0 + i // 4, (i // 4) * (D // 4):(i // 4 + 1) * (D // 4), :]
                            prods.append(_dot(_bf(lhs_v.at[i][...]), _bf(w)))
                        c11, c12, c21, c22 = _combine(prods)
                        hq_v[h0], hq_v[h0 + 1] = c21[8:], c22[8:]
                        res.append(jnp.concatenate([c11, c21[:8], c12, c22[:8]], axis=0))
                    else:
                        parts = []
                        for j in range(2):
                            parts += [_dot(top, _bf(wqkv_v[h0 + j])), hq_v[h0 + j, _at(8 * (r - 1), 8), :]]
                        res.append(jnp.concatenate(parts, axis=0))
                return res

            def merge(g, heads, acc):
                tops = jnp.concatenate([o[:L - 8] for o in heads], axis=1)
                held = jnp.concatenate([o[L - 8:] for o in heads], axis=1)
                lanes = slice(2 * g * grows, 2 * (g + 1) * grows)
                if last:
                    bots = jnp.concatenate([ho_v[:, lanes], held], axis=0)
                    lhs = _lhs7(tops[:, :grows], tops[:, grows:], bots[:, :grows], bots[:, grows:])
                    y, n = [], grows // 2
                    for i in range(7):
                        if i in _STORED:
                            w = jnp.concatenate(
                                [stored(3 * HP + 2 * g + j // 2, i, slice((j % 2) * n, (j % 2 + 1) * n))
                                 for j in range(D // 2 // LANE)], axis=1)
                        else:
                            r0, c0 = g * grows + (i // 4) * n, (i // 4) * (D // 2)
                            w = wo_v[r0:r0 + n, c0:c0 + D // 2]
                        y.append(_dot(lhs[i].astype(LHS_DT), _bf(w)))
                else:
                    ho_v[_at(8 * r, 8), lanes] = held
                    y = [_dot(tops.astype(LHS_DT), _bf(wo_v[g * grows:(g + 1) * grows, :]))]
                return y if acc is None else [a + b for a, b in zip(acc, y)]

            qkv, prob, heads = {}, {}, {}
            acc, done = None, 0
            for t in range(n_grp + 3):
                if t < n_grp:
                    qkv[t] = [project(t * G + j) for j in range(G)]
                upto = {n_grp + 1: n_grp - 2, n_grp + 2: n_grp}.get(t, t - LAG + 1)
                while done < upto:
                    acc = merge(done, heads.pop(done), acc)
                    done += 1
                if 0 <= t - 2 < n_grp:
                    heads[t - 2] = []
                    for (e, inv), (_, _, v) in zip(prob.pop(t - 2), qkv.pop(t - 2)):
                        o = _dot(e, v.astype(BF16)) * inv
                        heads[t - 2] += [o[:L], o[L:]]
                if 0 <= t - 1 < n_grp:
                    prob[t - 1] = [scores(q, k) for q, k, _ in qkv[t - 1]]
                if last and 1 <= t <= PERIOD:
                    load_held(jnp.minimum(s + t, n_seg - 1), t - 1)
                if t == n_grp - 1:
                    load_own(jnp.minimum(s + 1, n_seg - 1))
            if last:
                c11, c12, c21, c22 = _combine(acc)
                y, y_held = jnp.concatenate([c11, c12], axis=1), jnp.concatenate([c21, c22], axis=1)
            else:
                y = acc[0]
            base = x_rows(s * seg, seg) + part_v[_at(s * seg, seg), :]
            x_v[_at(s * (seg // 2), 8), :] = _words(base[:16] + y[M:M + 16])
            part_v[_at(s * seg + 16, 16), :] = jnp.concatenate([base[16:24] + y[M + 16:], base[24:]], axis=0)
            if last:
                for q in range(PERIOD):
                    r0 = (s - (PERIOD - 1) + q) * seg + 16
                    rest = part_v[_at(r0, 16), :]
                    x_v[_at(r0 // 2, 8), :] = _words(jnp.concatenate(
                        [rest[:8], rest[8:] + y_held[8 * q:8 * q + 8]], axis=0))
            return y[:M]

        def period(p, mem):
            s = p * PERIOD
            mem = step(s, 0, mem)
            mem = lax.fori_loop(1, PERIOD - 1, lambda r, mem: step(s + r, r, mem), mem)
            mem = step(s + PERIOD - 1, PERIOD - 1, mem)
            rows = _at(s * (seg // 2), PERIOD * seg // 2)
            pltpu.make_async_copy(x_v.at[rows], out_hbm.bitcast(U32).at[rows], sem_out).start()
            return mem

        load_own(0)
        for q in range(PERIOD):
            load_held(q, q)
        with jax.named_scope("aloop"):
            lax.fori_loop(0, n_seg // PERIOD, period, mem0_ref[...].astype(F32))

    def rest(sums_v):
        if not SKIP_B2:
            pl.run_scoped(functools.partial(channel_mlp, sums_v), pltpu.VMEM((7, R // 2, FF // 4), U32))
        if SKIP_A:
            x_v[0:8, :] = jnp.concatenate([sums_v[5, 0:8, 0:512]] * 2, axis=1) + l3_v[n_blk - 1, 3, 0:8, 0:1]
            pltpu.make_async_copy(x_v, out_hbm.bitcast(U32), sem_out).start()
            return
        pl.run_scoped(
            functools.partial(recurrence, sums_v),
            pltpu.VMEM((seg - 8, D), F32),
            pltpu.VMEM((7, (L - 8) // 2, D // 2), U32),
            pltpu.VMEM((8 * PERIOD, D), F32),
            pltpu.VMEM((3 * H, 8 * (PERIOD - 1), Dh), F32),
            pltpu.VMEM((8 * (PERIOD - 1), H * Dh), F32),
        )

    pl.run_scoped(rest, pltpu.VMEM((4 * HP + 5, D // 4, 5 * LANE), U32))
    pltpu.make_async_copy(x_v, out_hbm.bitcast(U32), sem_out).wait()


@functools.partial(jax.jit, static_argnames=("A_seg_len",))
def pallas_parallel_sum__memory_aug_recurrent_mem_tr__mixer_s_mlp__prompt_kernel(
    A_x: jax.Array,
    A_mem0: jax.Array,
    A_Wq: jax.Array,
    A_Wk: jax.Array,
    A_Wv: jax.Array,
    A_Wo: jax.Array,
    A_seg_len: int,
    B_x: jax.Array,
    B_w1: jax.Array,
    B_w2: jax.Array,
    B_w3: jax.Array,
    B_w4: jax.Array,
):
    del B_x
    B, S, D = A_x.shape
    H, Dh = A_Wq.shape[1], A_Wq.shape[2]
    M = A_mem0.shape[1]
    FF = B_w3.shape[1]
    assert (B, M, A_seg_len) == (1, 8, 32)
    n_blk = S // TM

    hbm = pl.BlockSpec(memory_space=pl.ANY)
    out = pl.pallas_call(
        functools.partial(_kernel, seg=A_seg_len),
        out_shape=jax.ShapeDtypeStruct((S, D), A_x.dtype),
        in_specs=[hbm, pl.BlockSpec(memory_space=pltpu.VMEM)] + [hbm] * 8,
        out_specs=hbm,
        scratch_shapes=[
            pltpu.VMEM((S // 2, D), U32),
            pltpu.VMEM((S, D), F32),
            pltpu.VMEM((3 * H, D // 2, Dh), U32),
            pltpu.VMEM((H * Dh // 2, D), U32),
            pltpu.VMEM((D // 2, FF), U32),
            pltpu.VMEM((FF // 2, D), U32),
            pltpu.VMEM((n_blk, 7, TM // 4, D // 2), U32),
            pltpu.SemaphoreType.DMA((n_blk + 4,)),
            pltpu.SemaphoreType.DMA((D // 2 // LANE,)),
            pltpu.SemaphoreType.DMA((3,)),
            pltpu.SemaphoreType.DMA((2 * n_blk,)),
            pltpu.SemaphoreType.DMA,
        ],
        compiler_params=pltpu.CompilerParams(
            vmem_limit_bytes=126 * 1024 * 1024, disable_bounds_checks=True),
    )(A_x.reshape(S, D), A_mem0.reshape(M, D),
      A_Wq.reshape(D // 2, 2, H, Dh), A_Wk.reshape(D // 2, 2, H, Dh), A_Wv.reshape(D // 2, 2, H, Dh),
      A_Wo.reshape(H * Dh, D), B_w1, B_w2, B_w3, B_w4)
    return out.reshape(B, S, D)
```

```python
import functools

import jax
import jax.numpy as jnp
import numpy as np
from jax import lax
import jax.experimental.pallas as pl
import jax.experimental.pallas.tpu as pltpu

F32 = jnp.float32
BF16 = jnp.bfloat16
U32 = jnp.uint32

_EPS = 1e-5
_NEG = -1e9
_GELU_C = float(np.sqrt(2.0 / np.pi))

LANE = 128
TM = 512
RC = 16
AC = 32
G = 2
PERIOD = 4
LAG = 5
CUT = 1.0
HEAD = 23
FOOT = 8
LHS_DT = BF16
KEEP = True
PIN1 = False
UNROLL = False
SPLIT = 0
S1 = False
ALLSPLIT = False
LN2 = True
OPQ = True
EARLY = 1
SKIP_B1 = False
SKIP_B2 = False
SKIP_A = False


def _dot(a, b):
    return lax.dot_general(a, b, (((1,), (0,)), ((), ())), preferred_element_type=F32)


def _dot_nt(a, b):
    return lax.dot_general(a, b, (((1,), (1,)), ((), ())), preferred_element_type=F32)


def _bf(words):
    return pltpu.bitcast(words, BF16)


def _words(x):
    return pltpu.bitcast(x.astype(BF16), U32)


def _at(start, n, align=None):
    return pl.ds(start if isinstance(start, int) else pl.multiple_of(start, align or n), n)


def _ln(x):
    inv_n = 1.0 / x.shape[-1]
    xc = x - jnp.sum(x, axis=-1, keepdims=True) * inv_n
    var = jnp.sum(xc * xc, axis=-1, keepdims=True) * inv_n
    return xc * lax.rsqrt(var + _EPS)


def _gelu(x):
    inner = x * (_GELU_C + (_GELU_C * 0.044715) * (x * x))
    hx = 0.5 * x
    return hx + hx * jnp.tanh(inner)


def _lhs7(a11, a12, a21, a22):
    return (a11 + a22, a21 + a22, a11, a22, a11 + a12, a21 - a11, a12 - a22)


def _rhs(i, b):
    if i in (1, 4):
        return b(i // 4, i // 4)
    p, q, sign = {0: ((0, 0), (1, 1), 1), 2: ((0, 1), (1, 1), -1), 3: ((1, 0), (0, 0), -1),
                  5: ((0, 0), (0, 1), 1), 6: ((1, 0), (1, 1), 1)}[i]
    p, q = b(*p).astype(F32), b(*q).astype(F32)
    return (p + q if sign > 0 else p - q).astype(BF16)


_STORED = (0, 2, 3, 5, 6)


def _combine(m):
    return (m[0] + m[3] - m[4] + m[6], m[2] + m[4], m[1] + m[3], m[0] - m[1] + m[2] + m[5])


def _weave(main, side):
    out, k = [], 0
    for i, task in enumerate(main):
        out.append(task)
        while k < len(side) and (k + 1) * len(main) <= (i + 1) * len(side):
            out.append(side[k])
            k += 1
    return out


def _run(tasks):
    for task in tasks:
        task()


def _finish_tasks(acc, emit):
    def finish(r):
        emit(r, _combine([pltpu.bitcast(ref[r0 + r:r0 + r + RC, c0:c0 + LANE], F32) for ref, r0, c0 in acc]))
    return [functools.partial(finish, r) for r in range(0, TM // 2, RC)]


def _matmul_tasks(lhs, rhs, pairs, next_acc, emit, tail):
    def product(acc, j, i):
        ref, r0, c0 = acc[i]
        ref[r0:r0 + TM // 2, c0:c0 + LANE] = pltpu.bitcast(
            _dot(lhs(i), rhs(j, i)), U32)

    out = []
    for j in range(pairs):
        acc = next_acc()
        out += _weave([functools.partial(product, acc, j, i) for i in (1, 0, 2, 3, 4, 5, 6)], tail)
        tail = _finish_tasks(acc, functools.partial(emit, j))
    return out, tail


def _kernel(x_hbm, mem0_ref, wq_hbm, wk_hbm, wv_hbm, wo_hbm, w1_hbm, w2_hbm, w3_hbm, w4_hbm,
            out_hbm,
            x_v, part_v, wqkv_v, wo_v, w3_v, w4_v, l3_v, raw_v,
            sem_x, sem_w1, sem_w, sem_a, sem_out, *, seg):
    S, D = x_hbm.shape
    H, Dh = wq_hbm.shape[2], wq_hbm.shape[3]
    M = mem0_ref.shape[0]
    FF = w3_hbm.shape[1]
    HP = H // 2
    L = M + seg
    R = TM // 2
    n_blk = S // TM
    n_seg = S // seg
    n_grp = HP // G
    assert n_grp == 2 * n_blk
    grows = G * Dh

    class part:
        @staticmethod
        def get(r0, n, c=slice(None)):
            return part_v[_at(r0, n, 8), c]

        @staticmethod
        def set(r0, v, c=slice(None)):
            part_v[_at(r0, v.shape[0], 8), c] = v

    def copy(hbm, vmem, sem, *idx):
        return pltpu.make_async_copy(hbm.bitcast(U32).at[idx], vmem.at[idx], sem)

    slabs = 4 * G

    def attn_copies(g):
        rows = _at(g * grows, grows)
        copies = [copy(wo_hbm, wo_v, sem_a.at[g], rows)]
        base = g % 2 * slabs
        for m, hbm in enumerate((wq_hbm, wk_hbm, wv_hbm)):
            for j in range(G):
                for par in range(2):
                    copies.append(pltpu.make_async_copy(
                        hbm.bitcast(U32).at[:, par, g * G + j, :],
                        raw_v.at[base + m * G + j, :, par * LANE:(par + 1) * LANE], sem_a.at[g]))
        for n in range(4):
            copies.append(pltpu.make_async_copy(
                wo_hbm.bitcast(U32).at[rows, n * D // 4:(n + 1) * D // 4],
                raw_v.at[base + 3 * G + n // 2, (n % 2) * grows:(n % 2 + 1) * grows], sem_a.at[g]))
        return copies

    def half_copy(hbm, vmem, n, k):
        rows = vmem.shape[0] // 2
        return copy(hbm, vmem, sem_w.at[n], _at(k * rows, rows))

    def x_rows(r0, n):
        return _bf(x_v[_at(r0 // 2, n // 2), :]).astype(F32)

    def cols(j, c):
        return slice(c * (D // 2) + j * LANE, c * (D // 2) + (j + 1) * LANE)

    def mixing(h_v, w1_v, w2_v, l1_v, l2_v, s1_v, s2_v, acc_v):
        zero = pl.semaphore_read(sem_out)
        pairs = D // 2 // LANE
        w1_copies = [[copy(w1_hbm, w1_v, sem_w1.at[j], slice(None), cols(j, c)) for c in range(2)]
                     for j in range(pairs)]
        w2_copy = copy(w2_hbm, w2_v, sem_w.at[0], slice(None))
        first = [[copy(x_hbm, x_v, sem_x.at[n_blk + k], _at(half + k * R // 8, R // 8))
                  for half in (0, R // 2)] for k in range(4)]
        x_copy = {i: copy(x_hbm, x_v, sem_x.at[i], _at(i * R, R)) for i in range(1, n_blk)}
        state = {"turn": 0, "tail": []}

        def next_acc():
            state["turn"] += 1
            return [(acc_v.at[state["turn"] % 2 * 7 + i], 0, 0) for i in range(7)]

        def lhs_tasks(ref, rows):
            def chunk(r):
                top, bot = rows(r), rows(R + r)
                k = D // 2
                for n, v in enumerate(_lhs7(top[:, :k], top[:, k:], bot[:, :k], bot[:, k:])):
                    ref.at[n][r // 2:(r + RC) // 2, :] = _words(v)
                if PIN1:
                    acc_v[14 + zero, 0:8, :] = ref[zero, 0:8, 0:LANE]
            return [functools.partial(chunk, r) for r in range(0, R, RC)]

        def norm1(i):
            def rows(r):
                r0 = i * TM + r
                x = x_rows(r0, RC)
                if LN2:
                    xc = x - jnp.sum(x, axis=-1, keepdims=True) * (1.0 / D)
                    var = jnp.sum(xc * xc, axis=-1, keepdims=True) * (1.0 / D)
                    inv = lax.rsqrt(var + _EPS)
                    xn = xc * inv
                    part.set(r0, xn)
                    return xn * lax.rsqrt(var * inv * inv + _EPS)
                xn = _ln(x)
                part.set(r0, xn)
                return _ln(xn)
            return lhs_tasks(l1_v.at[i % 2], rows)

        def shift(i):
            def rows(r):
                r0 = i * TM + r
                parts = []
                for g, by in enumerate((-1, 1, -2, 2)):
                    c = slice(g * D // 4, (g + 1) * D // 4)
                    if by < 0:
                        parts.append(pltpu.roll(h_v[r0:r0 + RC + 8, c], -by, 0)[8:])
                    else:
                        parts.append(pltpu.roll(h_v[r0 + 8:r0 + RC + 16, c], RC + 8 - by, 0)[:RC])
                return jnp.concatenate(parts, axis=1)
            return lhs_tasks(l2_v.at[i % 2], rows)

        def norm3(i):
            return lhs_tasks(l3_v.at[i], lambda r: _ln(part.get(i * TM + r, RC)))

        def stage(i, second, early, side, waits=()):
            if EARLY == 0:
                side = early + side
            lhs, w = (l2_v, w2_v) if second else (l1_v, w1_v)

            def emit(j, r, quads):
                for q, v in enumerate(quads):
                    r0 = i * TM + (q // 2) * R + r
                    if second:
                        part.set(r0, part.get(r0, RC, cols(j, q % 2)) + v, cols(j, q % 2))
                    else:
                        h_v[8 + r0:8 + r0 + RC, cols(j, q % 2)] = _gelu(v)

            zo = zero if OPQ else 0

            def rhs(j, n):
                kept = (s2_v if second else s1_v).at[j + i * zo]
                lanes = _at(_STORED.index(n) * LANE, LANE) if n in _STORED else None
                if KEEP and lanes and i > 0:
                    return _bf(kept[:, lanes])
                v = _rhs(n, lambda a, c: _bf(w[_at(a * (D // 4) + i * zo, D // 4), cols(j, c)]))
                if KEEP and lanes:
                    kept[:, lanes] = pltpu.bitcast(v, U32)
                return v

            main, state["tail"] = _matmul_tasks(
                lambda n: _bf(lhs.at[i % 2, n][...]),
                rhs,
                pairs, next_acc, emit, state["tail"])
            n = 7 + R // RC
            if waits:
                main = main[:7] + waits[0] + main[7:7 + n] + waits[1] + main[7 + n:7 + 2 * n] + waits[2] + main[7 + 2 * n:]
            if i == 0 and not second or EARLY == 0:
                _run(main[:n] + _weave(main[n:], side))
            else:
                k = len(early)
                _run(_weave(main[:n], early) + _weave(main[n:], side))

        with jax.named_scope("pro"):
            for c in sum(first, []) + sum(w1_copies[:2], []) + [x_copy[1]] + sum(w1_copies[2:], []) + [x_copy[2]]:
                c.start()
            h_v[0:8, :] = jnp.zeros((8, D), F32)
            h_v[S + 8:S + 16, :] = jnp.zeros((8, D), F32)
            todo = norm1(0)
            for k in range(4):
                for c in first[k]:
                    c.wait()
                _run(todo[k * len(todo) // 4:(k + 1) * len(todo) // 4])
            for c in w1_copies[0]:
                c.wait()
        with jax.named_scope("b1"):
            waits = [[c.wait for c in cs] for cs in w1_copies[1:]]
            waits[0].append(x_copy[1].wait)
            x_copy[3].start()
            w2_copy.start()
            stage(0, False, [], norm1(1), waits)
            x_copy[2].wait()
            half_copy(w3_hbm, w3_v, 1, 0).start()
            stage(1, False, norm1(2)[:4], norm1(2)[4:])
            x_copy[3].wait()
            half_copy(w3_hbm, w3_v, 1, 1).start()
            stage(2, False, norm1(3)[:4], norm1(3)[4:])
            w2_copy.wait()
            stage(3, False, shift(0)[:4], shift(0)[4:])
            half_copy(w4_hbm, w4_v, 2, 0).start()
            stage(0, True, shift(1)[:4], shift(1)[4:])
            half_copy(w4_hbm, w4_v, 2, 1).start()
            stage(1, True, shift(2)[:8], _weave(norm3(0), shift(2)[8:]))
            for c in attn_copies(0):
                c.start()
            stage(2, True, shift(3)[:8], _weave(norm3(1), shift(3)[8:]))
            stage(3, True, [], norm3(2))
            _run(state["tail"] + norm3(3))

    if SKIP_B1:
        for c in [half_copy(w3_hbm, w3_v, 1, 0), half_copy(w3_hbm, w3_v, 1, 1), half_copy(w4_hbm, w4_v, 2, 0),
                  half_copy(w4_hbm, w4_v, 2, 1)] + attn_copies(0):
            c.start()
    else:
        pl.run_scoped(
            mixing,
            pltpu.VMEM((S + 16, D), F32),
            pltpu.VMEM((D // 2, D), U32),
            pltpu.VMEM((D // 2, D), U32),
            pltpu.VMEM((2, 7, R // 2, D // 2), U32),
            pltpu.VMEM((2, 7, R // 2, D // 2), U32),
            pltpu.VMEM((D // 2 // LANE, D // 4, 5 * LANE), U32),
            pltpu.VMEM((D // 2 // LANE, D // 4, 5 * LANE), U32),
            pltpu.VMEM((15, R, LANE), U32),
        )
    for k in range(2):
        half_copy(w3_hbm, w3_v, 1, k).wait()
        half_copy(w4_hbm, w4_v, 2, k).wait()

    def channel_mlp(sums_v, u_v):
        up_pairs, down_pairs = FF // 4 // LANE, D // 2 // LANE

        def acc(slot):
            return [(raw_v.at[2 * slabs + n // 4], (n % 2) * R, (n // 2 % 2) * LANE) for n in range(7 * slot, 7 * slot + 7)]

        def attn_weight_tasks(g):
            def store(slab, r, quads):
                for n, i in enumerate(_STORED):
                    sums_v.at[slab][r:r + AC, n * LANE:(n + 1) * LANE] = pltpu.bitcast(
                        _rhs(i, lambda a, c: quads[2 * a + c]), U32)

            def qkv(m, j, r):
                slab = m * HP + g * G + j
                src = raw_v.at[g % 2 * slabs + m * G + j]
                quads = []
                for rr in (r, r + D // 4):
                    a, b = src[rr:rr + AC, :LANE], src[rr:rr + AC, LANE:]
                    h0 = (a & jnp.uint32(0xFFFF)) | (b << 16)
                    h1 = (a >> 16) | (b & jnp.uint32(0xFFFF0000))
                    wqkv_v[2 * slab, rr:rr + AC, :] = h0
                    wqkv_v[2 * slab + 1, rr:rr + AC, :] = h1
                    quads += [_bf(h0), _bf(h1)]
                store(slab, r, quads)

            def out(j, r):
                quads = []
                for a in range(2):
                    for n in (j, j + down_pairs):
                        r0, c0 = (n // 2 % 2) * grows + a * (grows // 2) + r, (n % 2) * LANE
                        quads.append(_bf(raw_v.at[g % 2 * slabs + 3 * G + n // 4][r0:r0 + AC, c0:c0 + LANE]))
                store(3 * HP + 2 * g + j // 2, r + (j % 2) * (grows // 2), quads)

            return ([functools.partial(qkv, m, j, r) for m in range(3) for j in range(G)
                     for r in range(0, D // 4, AC)]
                    + [functools.partial(out, j, r) for j in range(down_pairs)
                       for r in range(0, grows // 2, AC)])

        def emit_up(j, r, quads):
            for n, v in enumerate(_lhs7(*[_gelu(q) for q in quads])):
                u_v.at[n][r // 2:(r + RC) // 2, j * LANE:(j + 1) * LANE] = _words(v)

        def emit_down(i, j, r, quads):
            for q, v in enumerate(quads):
                r0 = i * TM + (q // 2) * R + r
                part.set(r0, part.get(r0, RC, cols(j, q % 2)) + v, cols(j, q % 2))

        def last_epilogue(i):
            return _finish_tasks(acc(2), functools.partial(emit_down, i, down_pairs - 1))

        for ref, r0, c0 in acc(2):
            ref[r0:r0 + R, c0:c0 + LANE] = jnp.zeros((R, LANE), U32)

        def body(it, _):
            i, f = it // 2, it % 2

            @pl.when(it + 1 < n_grp)
            def _():
                for c in attn_copies(it + 1):
                    c.start()

            for c in attn_copies(it):
                c.wait()
            slots = [n % 2 for n in range(up_pairs + down_pairs - 1)] + [2]
            next_acc = lambda: acc(slots.pop(0))
            up, tail = _matmul_tasks(
                lambda n: _bf(l3_v.at[i, n][...]),
                lambda j, n: _rhs(n, lambda a, c: _bf(
                    w3_v[a * (D // 4):(a + 1) * (D // 4), _at(c * (FF // 2) + f * (FF // 4) + j * LANE, LANE)])),
                up_pairs, next_acc, emit_up, last_epilogue(jnp.maximum(it - 1, 0) // 2))
            down, _ = _matmul_tasks(
                lambda n: _bf(u_v.at[n][...]),
                lambda j, n: _rhs(n, lambda a, c: _bf(
                    w4_v[_at(a * (FF // 4) + f * (FF // 8), FF // 8, 64), cols(j, c)])),
                down_pairs, next_acc, functools.partial(emit_down, i), [])
            side = attn_weight_tasks(it)
            cut = int(len(side) * CUT)
            _run(up[:HEAD] + _weave(up[HEAD:], side[:cut]) + tail + _weave(down[:len(down) - FOOT], side[cut:]) + down[len(down) - FOOT:])
            return 0

        with jax.named_scope("b2"):
            lax.fori_loop(0, n_grp, body, 0)
            _run(last_epilogue(n_blk - 1))

    def recurrence(sums_v, own_v, lhs_v, next_v, hq_v, ho_v):
        scale = float(Dh) ** -0.5
        own = seg - 8
        row = lax.broadcasted_iota(jnp.int32, (2 * L, 2 * L), 0)
        col = lax.broadcasted_iota(jnp.int32, (2 * L, 2 * L), 1)
        r_in = jnp.where(row >= L, row - L, row)
        c_in = jnp.where(col >= L, col - L, col)
        same_head = (row >= L) == (col >= L)
        keep = same_head & ((r_in < M) | (r_in >= c_in))
        fill = jnp.where(same_head, _NEG, -jnp.inf).astype(F32)

        def load_own(s):
            own_v[...] = _ln(x_rows(s * seg, seg)[:own])

        def load_held(s, q):
            next_v[8 * q:8 * q + 8, :] = _ln(x_rows(s * seg + seg - 16, 16)[8:])

        def load_lhs(mem):
            top, bot, k = jnp.concatenate([mem, own_v[...]], axis=0), next_v[...], D // 2
            for n, v in enumerate(_lhs7(top[:, :k], top[:, k:], bot[:, :k], bot[:, k:])):
                lhs_v.at[n][...] = _words(v)

        def by_head(split, dot, a, b):
            return jnp.concatenate([dot(a[:L], b), dot(a[L:], b)], axis=0) if split else dot(a, b)

        def scores(split, q, k):
            s = jnp.where(keep, by_head(split, _dot_nt, q, k.astype(BF16)) * scale, fill)
            e = jnp.exp(s - jnp.max(s, axis=-1, keepdims=True))
            return e, 1.0 / jnp.sum(e, axis=-1, keepdims=True)

        def stored(slab, i, rows=slice(None)):
            n = _STORED.index(i)
            return sums_v.at[slab][rows, n * LANE:(n + 1) * LANE]

        def step(s, r, mem):
            first = isinstance(r, int) and r == 0
            last = isinstance(r, int) and r == PERIOD - 1
            top = None if first else jnp.concatenate([mem, own_v[...]], axis=0)
            early = {} if first else {
                h: _dot(top[:, :D // 2].astype(BF16), _bf(wqkv_v[h, :D // 4, :])) for h in (0, 1, H, H + 1, 2 * H)[:SPLIT]}

            def plain(h):
                if h in early:
                    return early[h] + _dot(top[:, D // 2:].astype(BF16), _bf(wqkv_v[h, D // 4:, :]))
                return _dot(top.astype(BF16), _bf(wqkv_v[h]))

            def project(hp):
                res = []
                for m in range(3):
                    h0 = m * H + 2 * hp
                    if first:
                        prods = []
                        for i in range(7):
                            if i in _STORED:
                                w = stored(m * HP + hp, i)
                            else:
                                w = wqkv_v[h0 + i // 4, (i // 4) * (D // 4):(i // 4 + 1) * (D // 4), :]
                            prods.append(_dot(_bf(lhs_v.at[i][...]), _bf(w)))
                        c11, c12, c21, c22 = _combine(prods)
                        hq_v[h0], hq_v[h0 + 1] = c21[8:], c22[8:]
                        res.append(jnp.concatenate([c11, c21[:8], c12, c22[:8]], axis=0))
                    else:
                        parts = []
                        for j in range(2):
                            parts += [plain(h0 + j), hq_v[h0 + j, _at(8 * (r - 1), 8), :]]
                        res.append(jnp.concatenate(parts, axis=0))
                return res

            def merge(g, heads, acc):
                tops = jnp.concatenate([o[:L - 8] for o in heads], axis=1)
                held = jnp.concatenate([o[L - 8:] for o in heads], axis=1)
                lanes = slice(2 * g * grows, 2 * (g + 1) * grows)
                if last:
                    bots = jnp.concatenate([ho_v[:, lanes], held], axis=0)
                    lhs = _lhs7(tops[:, :grows], tops[:, grows:], bots[:, :grows], bots[:, grows:])
                    y, n = [None] * 7, grows // 2
                    for i in (0, 3, 4, 6, 2, 1, 5):
                        if i in _STORED:
                            w = jnp.concatenate(
                                [stored(3 * HP + 2 * g + j // 2, i, slice((j % 2) * n, (j % 2 + 1) * n))
                                 for j in range(D // 2 // LANE)], axis=1)
                        else:
                            r0, c0 = g * grows + (i // 4) * n, (i // 4) * (D // 2)
                            w = wo_v[r0:r0 + n, c0:c0 + D // 2]
                        y[i] = _dot(lhs[i].astype(LHS_DT), _bf(w))
                else:
                    ho_v[_at(8 * r, 8), lanes] = held
                    y = [_dot(tops.astype(LHS_DT), _bf(wo_v[g * grows:(g + 1) * grows, :]))]
                return y if acc is None else [a + b for a, b in zip(acc, y)]

            qkv, prob, heads = {}, {}, {}
            acc, done = None, 0
            for t in range(n_grp + 3):
                if t < n_grp:
                    qkv[t] = [project(t * G + j) for j in range(G)]
                upto = {n_grp + 1: n_grp - 2, n_grp + 2: n_grp}.get(t, t - LAG + 1)
                while done < upto:
                    acc = merge(done, heads.pop(done), acc)
                    done += 1
                if 0 <= t - 2 < n_grp:
                    heads[t - 2] = []
                    for (e, inv), (_, _, v) in zip(prob.pop(t - 2), qkv.pop(t - 2)):
                        o = by_head(S1 and t - 2 == n_grp - 1 or ALLSPLIT, _dot, e, v.astype(BF16)) * inv
                        heads[t - 2] += [o[:L], o[L:]]
                if 0 <= t - 1 < n_grp:
                    prob[t - 1] = [scores(S1 and t == 1 or ALLSPLIT, q, k) for q, k, _ in qkv[t - 1]]
                if last and 1 <= t <= PERIOD:
                    load_held(jnp.minimum(s + t, n_seg - 1), t - 1)
                if t == n_grp - 1:
                    load_own(jnp.minimum(s + 1, n_seg - 1))
            if last:
                c11, c12, c21, c22 = _combine(acc)
                load_lhs(jnp.concatenate([c11[:M], c12[:M]], axis=1))
                y, y_held = jnp.concatenate([c11, c12], axis=1), jnp.concatenate([c21, c22], axis=1)
            else:
                y = acc[0]
            base = x_rows(s * seg, seg) + part.get(s * seg, seg)
            x_v[_at(s * (seg // 2), 8), :] = _words(base[:16] + y[M:M + 16])
            part.set(s * seg + 16, jnp.concatenate([base[16:24] + y[M + 16:], base[24:]], axis=0))
            if last:
                for q in range(PERIOD):
                    r0 = (s - (PERIOD - 1) + q) * seg + 16
                    rest = part.get(r0, 16)
                    x_v[_at(r0 // 2, 8), :] = _words(jnp.concatenate(
                        [rest[:8], rest[8:] + y_held[8 * q:8 * q + 8]], axis=0))
            return y[:M]

        def period(p, _):
            s = p * PERIOD
            mem = step(s, 0, None)
            if UNROLL:
                for r in range(1, PERIOD - 1):
                    mem = step(s + r, r, mem)
            else:
                mem = lax.fori_loop(1, PERIOD - 1, lambda r, mem: step(s + r, r, mem), mem)
            mem = step(s + PERIOD - 1, PERIOD - 1, mem)
            rows = _at(s * (seg // 2), PERIOD * seg // 2)
            pltpu.make_async_copy(x_v.at[rows], out_hbm.bitcast(U32).at[rows], sem_out).start()
            return 0

        load_own(0)
        for q in range(PERIOD):
            load_held(q, q)
        load_lhs(mem0_ref[...].astype(F32))
        with jax.named_scope("aloop"):
            lax.fori_loop(0, n_seg // PERIOD, period, 0)

    def rest(sums_v):
        if not SKIP_B2:
            pl.run_scoped(functools.partial(channel_mlp, sums_v), pltpu.VMEM((7, R // 2, FF // 4), U32))
        if SKIP_A:
            x_v[0:8, :] = jnp.concatenate([sums_v[5, 0:8, 0:512]] * 2, axis=1) + l3_v[pl.semaphore_read(sem_out), 3, 0:8, 0:1] + wqkv_v[7, 0:8, 0:1]
            pltpu.make_async_copy(x_v, out_hbm.bitcast(U32), sem_out).start()
            return
        pl.run_scoped(
            functools.partial(recurrence, sums_v),
            pltpu.VMEM((seg - 8, D), F32),
            pltpu.VMEM((7, (L - 8) // 2, D // 2), U32),
            pltpu.VMEM((8 * PERIOD, D), F32),
            pltpu.VMEM((3 * H, 8 * (PERIOD - 1), Dh), F32),
            pltpu.VMEM((8 * (PERIOD - 1), H * Dh), F32),
        )

    pl.run_scoped(rest, pltpu.VMEM((4 * HP, D // 4, 5 * LANE), U32))
    pltpu.make_async_copy(x_v, out_hbm.bitcast(U32), sem_out).wait()


@functools.partial(jax.jit, static_argnames=("A_seg_len",))
def pallas_parallel_sum__memory_aug_recurrent_mem_tr__mixer_s_mlp__prompt_kernel(
    A_x: jax.Array,
    A_mem0: jax.Array,
    A_Wq: jax.Array,
    A_Wk: jax.Array,
    A_Wv: jax.Array,
    A_Wo: jax.Array,
    A_seg_len: int,
    B_x: jax.Array,
    B_w1: jax.Array,
    B_w2: jax.Array,
    B_w3: jax.Array,
    B_w4: jax.Array,
):
    del B_x
    B, S, D = A_x.shape
    H, Dh = A_Wq.shape[1], A_Wq.shape[2]
    M = A_mem0.shape[1]
    FF = B_w3.shape[1]
    assert (B, M, A_seg_len) == (1, 8, 32)
    n_blk = S // TM

    hbm = pl.BlockSpec(memory_space=pl.ANY)
    out = pl.pallas_call(
        functools.partial(_kernel, seg=A_seg_len),
        out_shape=jax.ShapeDtypeStruct((S, D), A_x.dtype),
        in_specs=[hbm, pl.BlockSpec(memory_space=pltpu.VMEM)] + [hbm] * 8,
        out_specs=hbm,
        scratch_shapes=[
            pltpu.VMEM((S // 2, D), U32), pltpu.VMEM((S, D), F32),
            pltpu.VMEM((3 * H, D // 2, Dh), U32),
            pltpu.VMEM((H * Dh // 2, D), U32),
            pltpu.VMEM((D // 2, FF), U32),
            pltpu.VMEM((FF // 2, D), U32),
            pltpu.VMEM((n_blk, 7, TM // 4, D // 2), U32),
            pltpu.VMEM((8 * G + 6, D // 2, 2 * LANE), U32),
            pltpu.SemaphoreType.DMA((n_blk + 4,)),
            pltpu.SemaphoreType.DMA((D // 2 // LANE,)),
            pltpu.SemaphoreType.DMA((3,)),
            pltpu.SemaphoreType.DMA((2 * n_blk,)),
            pltpu.SemaphoreType.DMA,
        ],
        compiler_params=pltpu.CompilerParams(
            vmem_limit_bytes=126 * 1024 * 1024, disable_bounds_checks=True),
    )(A_x.reshape(S, D), A_mem0.reshape(M, D),
      A_Wq.reshape(D // 2, 2, H, Dh), A_Wk.reshape(D // 2, 2, H, Dh), A_Wv.reshape(D // 2, 2, H, Dh),
      A_Wo.reshape(H * Dh, D), B_w1, B_w2, B_w3, B_w4)
    return out.reshape(B, S, D)
```

```python
import functools

import jax
import jax.numpy as jnp
import numpy as np
from jax import lax
import jax.experimental.pallas as pl
import jax.experimental.pallas.tpu as pltpu

F32 = jnp.float32
BF16 = jnp.bfloat16
U32 = jnp.uint32

_EPS = 1e-5
_NEG = -1e9
_GELU_C = float(np.sqrt(2.0 / np.pi))

LANE = 128
TM = 512
UNIT = 64
RC = 16
AC = 32
G = 2
PERIOD = 4
LAG = 5
CUT = 1.0
HEAD = 23
FOOT = 8
LHS_DT = BF16
KEEP = True
PIN1 = False
UNROLL = False
SPLIT = 0
S1 = False
ALLSPLIT = False
LN2 = True
OPQ = True
OP3 = True
OPS = False
TWO = False
ORDER = 1
E1 = 24
PIN3 = False
EARLY = 1
SKIP_B1 = False
SKIP_B2 = False
SKIP_A = False


def _dot(a, b):
    return lax.dot_general(a, b, (((1,), (0,)), ((), ())), preferred_element_type=F32)


def _dot_nt(a, b):
    return lax.dot_general(a, b, (((1,), (1,)), ((), ())), preferred_element_type=F32)


def _bf(words):
    return pltpu.bitcast(words, BF16)


def _words(x):
    return pltpu.bitcast(x.astype(BF16), U32)


def _at(start, n, align=None):
    return pl.ds(start if isinstance(start, int) else pl.multiple_of(start, align or n), n)


def _ln(x):
    inv_n = 1.0 / x.shape[-1]
    xc = x - jnp.sum(x, axis=-1, keepdims=True) * inv_n
    var = jnp.sum(xc * xc, axis=-1, keepdims=True) * inv_n
    return xc * lax.rsqrt(var + _EPS)


def _gelu(x):
    inner = x * (_GELU_C + (_GELU_C * 0.044715) * (x * x))
    hx = 0.5 * x
    return hx + hx * jnp.tanh(inner)


def _lhs7(a11, a12, a21, a22):
    return (a11 + a22, a21 + a22, a11, a22, a11 + a12, a21 - a11, a12 - a22)


def _rhs(i, b):
    if i in (1, 4):
        return b(i // 4, i // 4)
    p, q, sign = {0: ((0, 0), (1, 1), 1), 2: ((0, 1), (1, 1), -1), 3: ((1, 0), (0, 0), -1),
                  5: ((0, 0), (0, 1), 1), 6: ((1, 0), (1, 1), 1)}[i]
    p, q = b(*p).astype(F32), b(*q).astype(F32)
    return (p + q if sign > 0 else p - q).astype(BF16)


_STORED = (0, 2, 3, 5, 6)


def _combine(m):
    return (m[0] + m[3] - m[4] + m[6], m[2] + m[4], m[1] + m[3], m[0] - m[1] + m[2] + m[5])


def _weave(main, side):
    out, k = [], 0
    for i, task in enumerate(main):
        out.append(task)
        while k < len(side) and (k + 1) * len(main) <= (i + 1) * len(side):
            out.append(side[k])
            k += 1
    return out


def _run(tasks):
    for task in tasks:
        task()


def _finish_tasks(acc, emit):
    def finish(r):
        emit(r, _combine([pltpu.bitcast(ref[r0 + r:r0 + r + RC, c0:c0 + LANE], F32) for ref, r0, c0 in acc]))
    return [functools.partial(finish, r) for r in range(0, TM // 2, RC)]


def _matmul_tasks(lhs, rhs, pairs, next_acc, emit, tail):
    def product(acc, j, i):
        ref, r0, c0 = acc[i]
        ref[r0:r0 + TM // 2, c0:c0 + LANE] = pltpu.bitcast(
            _dot(lhs(i), rhs(j, i)), U32)

    out = []
    for j in range(pairs):
        acc = next_acc()
        out += _weave([functools.partial(product, acc, j, i) for i in (1, 0, 2, 3, 4, 5, 6)], tail)
        tail = _finish_tasks(acc, functools.partial(emit, j))
    return out, tail


def _kernel(x_hbm, mem0_ref, wq_hbm, wk_hbm, wv_hbm, wo_hbm, w1_hbm, w2_hbm, w3_hbm, w4_hbm,
            out_hbm,
            x_v, part_v, wqkv_v, wo_v, w3_v, w4_v, l3_v, raw_v,
            sem_x, sem_w1, sem_w, sem_a, sem_out, *, seg):
    S, D = x_hbm.shape
    H, Dh = wq_hbm.shape[2], wq_hbm.shape[3]
    M = mem0_ref.shape[0]
    FF = w3_hbm.shape[1]
    HP = H // 2
    L = M + seg
    R = TM // 2
    n_blk = S // TM
    n_seg = S // seg
    n_grp = HP // G
    assert n_grp == 2 * n_blk
    grows = G * Dh

    class part:
        @staticmethod
        def get(r0, n, c=slice(None)):
            return part_v[_at(r0, n, 8), c]

        @staticmethod
        def set(r0, v, c=slice(None)):
            part_v[_at(r0, v.shape[0], 8), c] = v

    def copy(hbm, vmem, sem, *idx):
        return pltpu.make_async_copy(hbm.bitcast(U32).at[idx], vmem.at[idx], sem)

    slabs = 4 * G

    def attn_copies(g):
        rows = _at(g * grows, grows)
        copies = [copy(wo_hbm, wo_v, sem_a.at[g], rows)]
        base = g % 2 * slabs
        for m, hbm in enumerate((wq_hbm, wk_hbm, wv_hbm)):
            for j in range(G):
                for par in range(2):
                    copies.append(pltpu.make_async_copy(
                        hbm.bitcast(U32).at[:, par, g * G + j, :],
                        raw_v.at[base + m * G + j, :, par * LANE:(par + 1) * LANE], sem_a.at[g]))
        for n in range(4):
            copies.append(pltpu.make_async_copy(
                wo_hbm.bitcast(U32).at[rows, n * D // 4:(n + 1) * D // 4],
                raw_v.at[base + 3 * G + n // 2, (n % 2) * grows:(n % 2 + 1) * grows], sem_a.at[g]))
        return copies

    def half_copy(hbm, vmem, n, k):
        rows = vmem.shape[0] // 2
        return copy(hbm, vmem, sem_w.at[n], _at(k * rows, rows))

    def x_rows(r0, n):
        return _bf(x_v[_at(r0 // 2, n // 2), :]).astype(F32)

    def cols(j, c):
        return slice(c * (D // 2) + j * LANE, c * (D // 2) + (j + 1) * LANE)

    def mixing(h_v, w1_v, w2_v, s1_v, s2_v, lhs_v, tmp_v):
        pairs = D // 2 // LANE
        units = TM // UNIT
        n_unit = S // UNIT
        half = UNIT // 2

        def w_copies(n, hbm, vmem, j):
            return [copy(hbm, vmem, sem_w1.at[n, j], slice(None), _at(c * (D // 2) + j * LANE, LANE))
                    for c in range(2)]

        def x_copy(i):
            return copy(x_hbm, x_v, sem_x.at[i], _at(i * R, R))

        def quad(w, j, a, c, r=0, n=D // 4):
            return _bf(w[a * (D // 4) + r:a * (D // 4) + r + n, _at(c * (D // 2) + j * LANE, LANE)])

        def prepare(w, sums, j, r, size):
            for n, i in enumerate(_STORED):
                sums.at[j][r:r + size, n * LANE:(n + 1) * LANE] = pltpu.bitcast(
                    _rhs(i, lambda a, c: quad(w, j, a, c, r, size)), U32)

        def store_lhs(ref, r, rows, size=UNIT):
            k = D // 2
            for q in range(0, size // 2, RC):
                top, bot = rows(q), rows(size // 2 + q)
                for n, v in enumerate(_lhs7(top[:, :k], top[:, k:], bot[:, :k], bot[:, k:])):
                    ref.at[n][(r + q) // 2:(r + q + RC) // 2, :] = _words(v)

        def norm1(r0, ref, size=UNIT):
            def rows(r):
                x = x_rows(r0 + r, RC)
                xc = x - jnp.sum(x, axis=-1, keepdims=True) * (1.0 / D)
                var = jnp.sum(xc * xc, axis=-1, keepdims=True) * (1.0 / D)
                inv = lax.rsqrt(var + _EPS)
                xn = xc * inv
                part_v[_at(r0 + r, RC), :] = xn
                return xn * lax.rsqrt(var * inv * inv + _EPS)
            store_lhs(ref, 0, rows, size)

        def shift(u, slot):
            def rows(r):
                r0 = u * UNIT + r
                parts = []
                for g, by in enumerate((-1, 1, -2, 2)):
                    c = slice(g * D // 4, (g + 1) * D // 4)
                    if by < 0:
                        parts.append(pltpu.roll(h_v[_at(r0, RC + 8, 8), c], -by, 0)[8:])
                    else:
                        parts.append(pltpu.roll(h_v[_at(r0 + 8, RC + 8, 8), c], RC + 8 - by, 0)[:RC])
                return jnp.concatenate(parts, axis=1)
            store_lhs(lhs_v.at[slot], 0, rows)

        def norm3(i, k):
            store_lhs(l3_v.at[i], k * half, lambda r: _ln(part_v[_at(i * TM + k * UNIT + r, RC), :]))

        def matmul(w, sums, lhs, emit, arriving=None):
            for j in range(pairs):
                if arriving:
                    for c in arriving(j):
                        c.wait()
                prods = [None] * 7
                for n in (1, 0, 2, 3, 4, 5, 6):
                    if n not in _STORED:
                        rhs = quad(w, j, n // 4, n // 4)
                    else:
                        lanes = _at(_STORED.index(n) * LANE, LANE)
                        if arriving:
                            rhs = _rhs(n, functools.partial(quad, w, j))
                            sums.at[j][:, lanes] = pltpu.bitcast(rhs, U32)
                        else:
                            rhs = _bf(sums.at[j][:, lanes])
                    prods[n] = _dot(_bf(lhs.at[n][...]), rhs)
                for q, v in enumerate(_combine(prods)):
                    emit((q // 2) * v.shape[0], cols(j, q % 2), v)

        def emit_h(r0, r, c, v):
            h_v[_at(8 + r0 + r, v.shape[0], 8), c] = _gelu(v)

        def h_body(i, _):
            @pl.when(i + 2 < n_blk)
            def _():
                x_copy(i + 2).start()

            for c in w_copies(1, w2_hbm, w2_v, i):
                c.start()
            w3_copy(i).start()
            x_copy(i).wait()
            for c in w_copies(1, w2_hbm, w2_v, i - 1):
                c.wait()
            norm1(i * TM, lhs_v.at[0])
            for k in range(units):
                r0 = i * TM + k * UNIT
                if k + 1 < units:
                    norm1(r0 + UNIT, lhs_v.at[(k + 1) % 2])
                matmul(w1_v, s1_v, lhs_v.at[k % 2], functools.partial(emit_h, r0))
                prepare(w2_v, s2_v, i - 1, k * (D // 4 // units), D // 4 // units)
            return 0

        def mix_body(i, _):
            copy(w4_hbm, w4_v, sem_w.at[2], _at(i * (FF // 2 // n_blk), FF // 2 // n_blk)).start()

            @pl.when(i == 1)
            def _():
                for c in attn_copies(0):
                    c.start()

            norm3(jnp.maximum(i - 1, 0), units - 1)
            for k in range(units):
                u = i * units + k
                shift(jnp.minimum(u + 1, n_unit - 1), (k + 1) % 2)

                def emit(r, c, v):
                    part_v[_at(u * UNIT + r, half), c] += v
                matmul(w2_v, s2_v, lhs_v.at[k % 2], emit)
                if k + 1 < units:
                    norm3(i, k)
            return 0

        def w3_copy(i):
            return copy(w3_hbm, w3_v, sem_w.at[1], _at(i * (D // 2 // n_blk), D // 2 // n_blk))

        with jax.named_scope("pro"):
            first = [copy(x_hbm, x_v, sem, _at(k * R // 2, R // 2)) for k, sem in enumerate((sem_w.at[0], sem_x.at[0]))]
            w1_copies = functools.partial(w_copies, 0, w1_hbm, w1_v)
            for c in ([first[0]] + w1_copies(0) + w1_copies(1) + [first[1]] + w1_copies(2) + w1_copies(3)
                      + [x_copy(1)] + w_copies(1, w2_hbm, w2_v, 0) + [x_copy(2), w3_copy(0)]):
                c.start()
            h_v[0:8, :] = jnp.zeros((8, D), F32)
            h_v[S + 8:S + 16, :] = jnp.zeros((8, D), F32)
            first[0].wait()
            norm1(0, tmp_v.at[0], R)
            matmul(w1_v, s1_v, tmp_v.at[0], functools.partial(emit_h, 0),
                   lambda j: w1_copies(j) + [first[1]] * (j == 2))
            norm1(R, tmp_v.at[1], R)
            matmul(w1_v, s1_v, tmp_v.at[1], functools.partial(emit_h, R))
        with jax.named_scope("b1"):
            lax.fori_loop(1, n_blk, h_body, 0)
            shift(0, 0)
            for c in w_copies(1, w2_hbm, w2_v, pairs - 1):
                c.wait()
            for r in range(0, D // 4, AC):
                prepare(w2_v, s2_v, pairs - 1, r, AC)
            lax.fori_loop(0, n_blk, mix_body, 0)
            norm3(n_blk - 1, units - 1)

    if SKIP_B1:
        for c in [half_copy(w3_hbm, w3_v, 1, 0), half_copy(w3_hbm, w3_v, 1, 1), half_copy(w4_hbm, w4_v, 2, 0),
                  half_copy(w4_hbm, w4_v, 2, 1)] + attn_copies(0):
            c.start()
    else:
        pl.run_scoped(
            mixing,
            pltpu.VMEM((S + 16, D), F32),
            pltpu.VMEM((D // 2, D), U32),
            pltpu.VMEM((D // 2, D), U32),
            pltpu.VMEM((D // 2 // LANE, D // 4, 5 * LANE), U32),
            pltpu.VMEM((D // 2 // LANE, D // 4, 5 * LANE), U32),
            pltpu.VMEM((2, 7, UNIT // 4, D // 2), U32),
            pltpu.VMEM((2, 7, R // 4, D // 2), U32),
        )
    for k in range(2):
        half_copy(w3_hbm, w3_v, 1, k).wait()
        half_copy(w4_hbm, w4_v, 2, k).wait()

    def channel_mlp(sums_v, u_v):
        up_pairs, down_pairs = FF // 4 // LANE, D // 2 // LANE

        def acc(slot):
            return [(raw_v.at[2 * slabs + n // 4], (n % 2) * R, (n // 2 % 2) * LANE) for n in range(7 * slot, 7 * slot + 7)]

        def attn_weight_tasks(g):
            def store(slab, r, quads):
                for n, i in enumerate(_STORED):
                    sums_v.at[slab][r:r + AC, n * LANE:(n + 1) * LANE] = pltpu.bitcast(
                        _rhs(i, lambda a, c: quads[2 * a + c]), U32)

            def qkv(m, j, r):
                slab = m * HP + g * G + j
                src = raw_v.at[g % 2 * slabs + m * G + j]
                quads = []
                for rr in (r, r + D // 4):
                    a, b = src[rr:rr + AC, :LANE], src[rr:rr + AC, LANE:]
                    h0 = (a & jnp.uint32(0xFFFF)) | (b << 16)
                    h1 = (a >> 16) | (b & jnp.uint32(0xFFFF0000))
                    wqkv_v[2 * slab, rr:rr + AC, :] = h0
                    wqkv_v[2 * slab + 1, rr:rr + AC, :] = h1
                    quads += [_bf(h0), _bf(h1)]
                store(slab, r, quads)

            def out(j, r):
                quads = []
                for a in range(2):
                    for n in (j, j + down_pairs):
                        r0, c0 = (n // 2 % 2) * grows + a * (grows // 2) + r, (n % 2) * LANE
                        quads.append(_bf(raw_v.at[g % 2 * slabs + 3 * G + n // 4][r0:r0 + AC, c0:c0 + LANE]))
                store(3 * HP + 2 * g + j // 2, r + (j % 2) * (grows // 2), quads)

            return ([functools.partial(qkv, m, j, r) for m in range(3) for j in range(G)
                     for r in range(0, D // 4, AC)]
                    + [functools.partial(out, j, r) for j in range(down_pairs)
                       for r in range(0, grows // 2, AC)])

        def emit_up(j, r, quads):
            for n, v in enumerate(_lhs7(*[_gelu(q) for q in quads])):
                u_v.at[n][r // 2:(r + RC) // 2, j * LANE:(j + 1) * LANE] = _words(v)

        def emit_down(i, j, r, quads):
            for q, v in enumerate(quads):
                r0 = i * TM + r // (UNIT // 2) * UNIT + (q // 2) * (UNIT // 2) + r % (UNIT // 2)
                part_v[_at(r0, RC), cols(j, q % 2)] += v

        def last_epilogue(i):
            return _finish_tasks(acc(2), functools.partial(emit_down, i, down_pairs - 1))

        for ref, r0, c0 in acc(2):
            ref[r0:r0 + R, c0:c0 + LANE] = jnp.zeros((R, LANE), U32)

        def body(it, _):
            i, f = it // 2, it % 2

            @pl.when(it + 1 < n_grp)
            def _():
                for c in attn_copies(it + 1):
                    c.start()

            for c in attn_copies(it):
                c.wait()
            slots = [n % 2 for n in range(up_pairs + down_pairs - 1)] + [2]
            next_acc = lambda: acc(slots.pop(0))
            up, tail = _matmul_tasks(
                lambda n: _bf(l3_v.at[i, n][...]),
                lambda j, n: _rhs(n, lambda a, c: _bf(
                    w3_v[a * (D // 4):(a + 1) * (D // 4), _at(c * (FF // 2) + f * (FF // 4) + j * LANE, LANE)])),
                up_pairs, next_acc, emit_up, last_epilogue(jnp.maximum(it - 1, 0) // 2))
            down, _ = _matmul_tasks(
                lambda n: _bf(u_v.at[n][...]),
                lambda j, n: _rhs(n, lambda a, c: _bf(
                    w4_v[_at(a * (FF // 4) + f * (FF // 8), FF // 8, 64), cols(j, c)])),
                down_pairs, next_acc, functools.partial(emit_down, i), [])
            side = attn_weight_tasks(it)
            cut = int(len(side) * CUT)
            _run(up[:HEAD] + _weave(up[HEAD:], side[:cut]) + tail + _weave(down[:len(down) - FOOT], side[cut:]) + down[len(down) - FOOT:])
            return 0

        with jax.named_scope("b2"):
            lax.fori_loop(0, n_grp, body, 0)
            _run(last_epilogue(n_blk - 1))

    def recurrence(sums_v, own_v, lhs_v, next_v, hq_v, ho_v):
        scale = float(Dh) ** -0.5
        own = seg - 8
        row = lax.broadcasted_iota(jnp.int32, (2 * L, 2 * L), 0)
        col = lax.broadcasted_iota(jnp.int32, (2 * L, 2 * L), 1)
        r_in = jnp.where(row >= L, row - L, row)
        c_in = jnp.where(col >= L, col - L, col)
        same_head = (row >= L) == (col >= L)
        keep = same_head & ((r_in < M) | (r_in >= c_in))
        fill = jnp.where(same_head, _NEG, -jnp.inf).astype(F32)

        def load_own(s):
            own_v[...] = _ln(x_rows(s * seg, seg)[:own])

        def load_held(s, q):
            next_v[8 * q:8 * q + 8, :] = _ln(x_rows(s * seg + seg - 16, 16)[8:])

        def load_lhs(mem):
            top, bot, k = jnp.concatenate([mem, own_v[...]], axis=0), next_v[...], D // 2
            for n, v in enumerate(_lhs7(top[:, :k], top[:, k:], bot[:, :k], bot[:, k:])):
                lhs_v.at[n][...] = _words(v)

        def by_head(split, dot, a, b):
            return jnp.concatenate([dot(a[:L], b), dot(a[L:], b)], axis=0) if split else dot(a, b)

        def scores(split, q, k):
            s = jnp.where(keep, by_head(split, _dot_nt, q, k.astype(BF16)) * scale, fill)
            e = jnp.exp(s - jnp.max(s, axis=-1, keepdims=True))
            return e, 1.0 / jnp.sum(e, axis=-1, keepdims=True)

        def stored(slab, i, rows=slice(None)):
            n = _STORED.index(i)
            return sums_v.at[slab][rows, n * LANE:(n + 1) * LANE]

        def step(s, r, mem):
            first = isinstance(r, int) and r == 0
            last = isinstance(r, int) and r == PERIOD - 1
            top = None if first else jnp.concatenate([mem, own_v[...]], axis=0)
            early = {} if first else {
                h: _dot(top[:, :D // 2].astype(BF16), _bf(wqkv_v[h, :D // 4, :])) for h in (0, 1, H, H + 1, 2 * H)[:SPLIT]}

            def plain(h):
                if h in early:
                    return early[h] + _dot(top[:, D // 2:].astype(BF16), _bf(wqkv_v[h, D // 4:, :]))
                return _dot(top.astype(BF16), _bf(wqkv_v[h]))

            def project(hp):
                res = []
                for m in range(3):
                    h0 = m * H + 2 * hp
                    if first:
                        prods = []
                        for i in range(7):
                            if i in _STORED:
                                w = stored(m * HP + hp, i)
                            else:
                                w = wqkv_v[h0 + i // 4, (i // 4) * (D // 4):(i // 4 + 1) * (D // 4), :]
                            prods.append(_dot(_bf(lhs_v.at[i][...]), _bf(w)))
                        c11, c12, c21, c22 = _combine(prods)
                        hq_v[h0], hq_v[h0 + 1] = c21[8:], c22[8:]
                        res.append(jnp.concatenate([c11, c21[:8], c12, c22[:8]], axis=0))
                    else:
                        parts = []
                        for j in range(2):
                            parts += [plain(h0 + j), hq_v[h0 + j, _at(8 * (r - 1), 8), :]]
                        res.append(jnp.concatenate(parts, axis=0))
                return res

            def merge(g, heads, acc):
                tops = jnp.concatenate([o[:L - 8] for o in heads], axis=1)
                held = jnp.concatenate([o[L - 8:] for o in heads], axis=1)
                lanes = slice(2 * g * grows, 2 * (g + 1) * grows)
                if last:
                    bots = jnp.concatenate([ho_v[:, lanes], held], axis=0)
                    lhs = _lhs7(tops[:, :grows], tops[:, grows:], bots[:, :grows], bots[:, grows:])
                    y, n = [None] * 7, grows // 2
                    for i in (0, 3, 4, 6, 2, 1, 5):
                        if i in _STORED:
                            w = jnp.concatenate(
                                [stored(3 * HP + 2 * g + j // 2, i, slice((j % 2) * n, (j % 2 + 1) * n))
                                 for j in range(D // 2 // LANE)], axis=1)
                        else:
                            r0, c0 = g * grows + (i // 4) * n, (i // 4) * (D // 2)
                            w = wo_v[r0:r0 + n, c0:c0 + D // 2]
                        y[i] = _dot(lhs[i].astype(LHS_DT), _bf(w))
                else:
                    ho_v[_at(8 * r, 8), lanes] = held
                    y = [_dot(tops.astype(LHS_DT), _bf(wo_v[g * grows:(g + 1) * grows, :]))]
                return y if acc is None else [a + b for a, b in zip(acc, y)]

            qkv, prob, heads = {}, {}, {}
            acc, done = None, 0
            for t in range(n_grp + 3):
                if t < n_grp:
                    qkv[t] = [project(t * G + j) for j in range(G)]
                upto = {n_grp + 1: n_grp - 2, n_grp + 2: n_grp}.get(t, t - LAG + 1)
                while done < upto:
                    acc = merge(done, heads.pop(done), acc)
                    done += 1
                if 0 <= t - 2 < n_grp:
                    heads[t - 2] = []
                    for (e, inv), (_, _, v) in zip(prob.pop(t - 2), qkv.pop(t - 2)):
                        o = by_head(S1 and t - 2 == n_grp - 1 or ALLSPLIT, _dot, e, v.astype(BF16)) * inv
                        heads[t - 2] += [o[:L], o[L:]]
                if 0 <= t - 1 < n_grp:
                    prob[t - 1] = [scores(S1 and t == 1 or ALLSPLIT, q, k) for q, k, _ in qkv[t - 1]]
                if last and 1 <= t <= PERIOD:
                    load_held(jnp.minimum(s + t, n_seg - 1), t - 1)
                if t == n_grp - 1:
                    load_own(jnp.minimum(s + 1, n_seg - 1))
            if last:
                c11, c12, c21, c22 = _combine(acc)
                load_lhs(jnp.concatenate([c11[:M], c12[:M]], axis=1))
                y, y_held = jnp.concatenate([c11, c12], axis=1), jnp.concatenate([c21, c22], axis=1)
            else:
                y = acc[0]
            base = x_rows(s * seg, seg) + part.get(s * seg, seg)
            x_v[_at(s * (seg // 2), 8), :] = _words(base[:16] + y[M:M + 16])
            part.set(s * seg + 16, jnp.concatenate([base[16:24] + y[M + 16:], base[24:]], axis=0))
            if last:
                for q in range(PERIOD):
                    r0 = (s - (PERIOD - 1) + q) * seg + 16
                    rest = part.get(r0, 16)
                    x_v[_at(r0 // 2, 8), :] = _words(jnp.concatenate(
                        [rest[:8], rest[8:] + y_held[8 * q:8 * q + 8]], axis=0))
            return y[:M]

        def period(p, _):
            s = p * PERIOD
            mem = step(s, 0, None)
            if UNROLL:
                for r in range(1, PERIOD - 1):
                    mem = step(s + r, r, mem)
            else:
                mem = lax.fori_loop(1, PERIOD - 1, lambda r, mem: step(s + r, r, mem), mem)
            mem = step(s + PERIOD - 1, PERIOD - 1, mem)
            rows = _at(s * (seg // 2), PERIOD * seg // 2)
            pltpu.make_async_copy(x_v.at[rows], out_hbm.bitcast(U32).at[rows], sem_out).start()
            return 0

        load_own(0)
        for q in range(PERIOD):
            load_held(q, q)
        load_lhs(mem0_ref[...].astype(F32))
        with jax.named_scope("aloop"):
            lax.fori_loop(0, n_seg // PERIOD, period, 0)

    def rest(sums_v):
        if not SKIP_B2:
            pl.run_scoped(functools.partial(channel_mlp, sums_v), pltpu.VMEM((7, R // 2, FF // 4), U32))
        if SKIP_A:
            x_v[0:8, :] = jnp.concatenate([sums_v[5, 0:8, 0:512]] * 2, axis=1) + l3_v[pl.semaphore_read(sem_out), 3, 0:8, 0:1] + wqkv_v[7, 0:8, 0:1]
            pltpu.make_async_copy(x_v, out_hbm.bitcast(U32), sem_out).start()
            return
        pl.run_scoped(
            functools.partial(recurrence, sums_v),
            pltpu.VMEM((seg - 8, D), F32),
            pltpu.VMEM((7, (L - 8) // 2, D // 2), U32),
            pltpu.VMEM((8 * PERIOD, D), F32),
            pltpu.VMEM((3 * H, 8 * (PERIOD - 1), Dh), F32),
            pltpu.VMEM((8 * (PERIOD - 1), H * Dh), F32),
        )

    pl.run_scoped(rest, pltpu.VMEM((4 * HP, D // 4, 5 * LANE), U32))
    pltpu.make_async_copy(x_v, out_hbm.bitcast(U32), sem_out).wait()


@functools.partial(jax.jit, static_argnames=("A_seg_len",))
def pallas_parallel_sum__memory_aug_recurrent_mem_tr__mixer_s_mlp__prompt_kernel(
    A_x: jax.Array,
    A_mem0: jax.Array,
    A_Wq: jax.Array,
    A_Wk: jax.Array,
    A_Wv: jax.Array,
    A_Wo: jax.Array,
    A_seg_len: int,
    B_x: jax.Array,
    B_w1: jax.Array,
    B_w2: jax.Array,
    B_w3: jax.Array,
    B_w4: jax.Array,
):
    del B_x
    B, S, D = A_x.shape
    H, Dh = A_Wq.shape[1], A_Wq.shape[2]
    M = A_mem0.shape[1]
    FF = B_w3.shape[1]
    assert (B, M, A_seg_len) == (1, 8, 32)
    n_blk = S // TM

    hbm = pl.BlockSpec(memory_space=pl.ANY)
    out = pl.pallas_call(
        functools.partial(_kernel, seg=A_seg_len),
        out_shape=jax.ShapeDtypeStruct((S, D), A_x.dtype),
        in_specs=[hbm, pl.BlockSpec(memory_space=pltpu.VMEM)] + [hbm] * 8,
        out_specs=hbm,
        scratch_shapes=[
            pltpu.VMEM((S // 2, D), U32), pltpu.VMEM((S, D), F32),
            pltpu.VMEM((3 * H, D // 2, Dh), U32),
            pltpu.VMEM((H * Dh // 2, D), U32),
            pltpu.VMEM((D // 2, FF), U32),
            pltpu.VMEM((FF // 2, D), U32),
            pltpu.VMEM((n_blk, 7, TM // 4, D // 2), U32),
            pltpu.VMEM((8 * G + 6, D // 2, 2 * LANE), U32),
            pltpu.SemaphoreType.DMA((n_blk,)),
            pltpu.SemaphoreType.DMA((2, D // 2 // LANE)),
            pltpu.SemaphoreType.DMA((3,)),
            pltpu.SemaphoreType.DMA((2 * n_blk,)),
            pltpu.SemaphoreType.DMA,
        ],
        compiler_params=pltpu.CompilerParams(
            vmem_limit_bytes=126 * 1024 * 1024, disable_bounds_checks=True),
    )(A_x.reshape(S, D), A_mem0.reshape(M, D),
      A_Wq.reshape(D // 2, 2, H, Dh), A_Wk.reshape(D // 2, 2, H, Dh), A_Wv.reshape(D // 2, 2, H, Dh),
      A_Wo.reshape(H * Dh, D), B_w1, B_w2, B_w3, B_w4)
    return out.reshape(B, S, D)
```

```python
import functools

import jax
import jax.numpy as jnp
import numpy as np
from jax import lax
import jax.experimental.pallas as pl
import jax.experimental.pallas.tpu as pltpu

F32 = jnp.float32
BF16 = jnp.bfloat16
U32 = jnp.uint32

_EPS = 1e-5
_NEG = -1e9
_LOG2E = float(np.log2(np.e))
_GELU_C = float(np.sqrt(2.0 / np.pi))

LANE = 128
TM = 512
UNIT = 64
RC = 16
AC = 32
G = 2
PERIOD = 4
LAG = 5
CUT = 1.0
HEAD = 23
FOOT = 8
LHS_DT = BF16
KEEP = True
PIN1 = False
UNROLL = True
SPLIT = 4
S1 = True
UP0 = 4
UP1 = 5
WIDE = False
RCP = True
PRE = False
S1T = (1,)
P1T = (7,)
ALLSPLIT = False
LN2 = True
OPQ = True
OP3 = True
OPS = False
TWO = False
ORDER = 1
E1 = 24
PIN3 = False
EARLY = 1
SKIP_B1 = False
SKIP_B2 = False
SKIP_A = False


def _dot(a, b):
    return lax.dot_general(a, b, (((1,), (0,)), ((), ())), preferred_element_type=F32)


def _dot_nt(a, b):
    return lax.dot_general(a, b, (((1,), (1,)), ((), ())), preferred_element_type=F32)


def _bf(words):
    return pltpu.bitcast(words, BF16)


def _words(x):
    return pltpu.bitcast(x.astype(BF16), U32)


def _at(start, n, align=None):
    return pl.ds(start if isinstance(start, int) else pl.multiple_of(start, align or n), n)


def _ln(x):
    inv_n = 1.0 / x.shape[-1]
    xc = x - jnp.sum(x, axis=-1, keepdims=True) * inv_n
    var = jnp.sum(xc * xc, axis=-1, keepdims=True) * inv_n
    return xc * lax.rsqrt(var + _EPS)


def _gelu(x):
    inner = x * (_GELU_C + (_GELU_C * 0.044715) * (x * x))
    hx = 0.5 * x
    return hx + hx * jnp.tanh(inner)


def _lhs7(a11, a12, a21, a22):
    return (a11 + a22, a21 + a22, a11, a22, a11 + a12, a21 - a11, a12 - a22)


def _rhs(i, b):
    if i in (1, 4):
        return b(i // 4, i // 4)
    p, q, sign = {0: ((0, 0), (1, 1), 1), 2: ((0, 1), (1, 1), -1), 3: ((1, 0), (0, 0), -1),
                  5: ((0, 0), (0, 1), 1), 6: ((1, 0), (1, 1), 1)}[i]
    p, q = b(*p).astype(F32), b(*q).astype(F32)
    return (p + q if sign > 0 else p - q).astype(BF16)


_STORED = (0, 2, 3, 5, 6)


def _combine(m):
    return (m[0] + m[3] - m[4] + m[6], m[2] + m[4], m[1] + m[3], m[0] - m[1] + m[2] + m[5])


def _weave(main, side):
    out, k = [], 0
    for i, task in enumerate(main):
        out.append(task)
        while k < len(side) and (k + 1) * len(main) <= (i + 1) * len(side):
            out.append(side[k])
            k += 1
    return out


def _run(tasks):
    for task in tasks:
        task()


def _finish_tasks(acc, emit):
    def finish(r):
        emit(r, _combine([pltpu.bitcast(ref[r0 + r:r0 + r + RC, c0:c0 + LANE], F32) for ref, r0, c0 in acc]))
    return [functools.partial(finish, r) for r in range(0, TM // 2, RC)]


def _matmul_tasks(lhs, rhs, pairs, next_acc, emit, tail):
    def product(acc, j, i):
        ref, r0, c0 = acc[i]
        ref[r0:r0 + TM // 2, c0:c0 + LANE] = pltpu.bitcast(
            _dot(lhs(i), rhs(j, i)), U32)

    out = []
    for j in range(pairs):
        acc = next_acc()
        out += _weave([functools.partial(product, acc, j, i) for i in (1, 0, 2, 3, 4, 5, 6)], tail)
        tail = _finish_tasks(acc, functools.partial(emit, j))
    return out, tail


def _kernel(x_hbm, mem0_hbm, wq_hbm, wk_hbm, wv_hbm, wo_hbm, w1_hbm, w2_hbm, w3_hbm, w4_hbm,
            out_hbm,
            x_v, part_v, wqkv_v, wo_v, w3_v, w4_v, l3_v, raw_v, mem0_v,
            sem_x, sem_w1, sem_w, sem_a, sem_out, *, seg):
    S, D = x_hbm.shape
    H, Dh = wq_hbm.shape[2], wq_hbm.shape[3]
    M = mem0_hbm.shape[0]
    FF = w3_hbm.shape[1]
    HP = H // 2
    L = M + seg
    R = TM // 2
    n_blk = S // TM
    n_seg = S // seg
    n_grp = HP // G
    assert n_grp == 2 * n_blk
    grows = G * Dh

    class part:
        @staticmethod
        def get(r0, n, c=slice(None)):
            return part_v[_at(r0, n, 8), c]

        @staticmethod
        def set(r0, v, c=slice(None)):
            part_v[_at(r0, v.shape[0], 8), c] = v

    def copy(hbm, vmem, sem, *idx):
        return pltpu.make_async_copy(hbm.bitcast(U32).at[idx], vmem.at[idx], sem)

    slabs = 4 * G

    def attn_copies(g):
        rows = _at(g * grows, grows)
        copies = [copy(wo_hbm, wo_v, sem_a.at[g], rows)]
        base = g % 2 * slabs
        for m, hbm in enumerate((wq_hbm, wk_hbm, wv_hbm)):
            for j in range(G):
                for par in range(2):
                    copies.append(pltpu.make_async_copy(
                        hbm.bitcast(U32).at[:, par, g * G + j, :],
                        raw_v.at[base + m * G + j, :, par * LANE:(par + 1) * LANE], sem_a.at[g]))
        for n in range(4):
            copies.append(pltpu.make_async_copy(
                wo_hbm.bitcast(U32).at[rows, n * D // 4:(n + 1) * D // 4],
                raw_v.at[base + 3 * G + n // 2, (n % 2) * grows:(n % 2 + 1) * grows], sem_a.at[g]))
        return copies

    mem0_copy = pltpu.make_async_copy(mem0_hbm, mem0_v, sem_w.at[3])

    def half_copy(hbm, vmem, n, k):
        rows = vmem.shape[0] // 2
        return copy(hbm, vmem, sem_w.at[n], _at(k * rows, rows))

    def x_rows(r0, n):
        return _bf(x_v[_at(r0 // 2, n // 2), :]).astype(F32)

    def cols(j, c):
        return slice(c * (D // 2) + j * LANE, c * (D // 2) + (j + 1) * LANE)

    def mixing(h_v, w1_v, w2_v, s1_v, s2_v, lhs_v, tmp_v):
        pairs = D // 2 // LANE
        units = TM // UNIT
        n_unit = S // UNIT
        half = UNIT // 2

        def w_copies(n, hbm, vmem, j):
            return [copy(hbm, vmem, sem_w1.at[n, j], slice(None), _at(c * (D // 2) + j * LANE, LANE))
                    for c in range(2)]

        def x_copy(i):
            return copy(x_hbm, x_v, sem_x.at[i], _at(i * R, R))

        def quad(w, j, a, c, r=0, n=D // 4):
            return _bf(w[a * (D // 4) + r:a * (D // 4) + r + n, _at(c * (D // 2) + j * LANE, LANE)])

        def prepare(w, sums, j, r, size):
            for n, i in enumerate(_STORED):
                sums.at[j][r:r + size, n * LANE:(n + 1) * LANE] = pltpu.bitcast(
                    _rhs(i, lambda a, c: quad(w, j, a, c, r, size)), U32)

        def store_lhs(ref, r, rows, size=UNIT):
            k = D // 2
            for q in range(0, size // 2, RC):
                top, bot = rows(q), rows(size // 2 + q)
                for n, v in enumerate(_lhs7(top[:, :k], top[:, k:], bot[:, :k], bot[:, k:])):
                    ref.at[n][(r + q) // 2:(r + q + RC) // 2, :] = _words(v)

        def norm1(r0, ref, size=UNIT):
            def rows(r):
                x = x_rows(r0 + r, RC)
                xc = x - jnp.sum(x, axis=-1, keepdims=True) * (1.0 / D)
                var = jnp.sum(xc * xc, axis=-1, keepdims=True) * (1.0 / D)
                inv = lax.rsqrt(var + _EPS)
                xn = xc * inv
                part_v[_at(r0 + r, RC), :] = xn
                return xn * lax.rsqrt(var * inv * inv + _EPS)
            store_lhs(ref, 0, rows, size)

        def shift(u, slot):
            def rows(r):
                r0 = u * UNIT + r
                parts = []
                for g, by in enumerate((-1, 1, -2, 2)):
                    c = slice(g * D // 4, (g + 1) * D // 4)
                    if by < 0:
                        parts.append(pltpu.roll(h_v[_at(r0, RC + 8, 8), c], -by, 0)[8:])
                    else:
                        parts.append(pltpu.roll(h_v[_at(r0 + 8, RC + 8, 8), c], RC + 8 - by, 0)[:RC])
                return jnp.concatenate(parts, axis=1)
            store_lhs(lhs_v.at[slot], 0, rows)

        def norm3(i, k):
            store_lhs(l3_v.at[i], k * half, lambda r: _ln(part_v[_at(i * TM + k * UNIT + r, RC), :]))

        def matmul(w, sums, lhs, emit, arriving=None):
            for j in range(pairs):
                if arriving:
                    for c in arriving(j):
                        c.wait()
                prods = [None] * 7
                for n in (1, 0, 2, 3, 4, 5, 6):
                    if n not in _STORED:
                        rhs = quad(w, j, n // 4, n // 4)
                    else:
                        lanes = _at(_STORED.index(n) * LANE, LANE)
                        if arriving:
                            rhs = _rhs(n, functools.partial(quad, w, j))
                            sums.at[j][:, lanes] = pltpu.bitcast(rhs, U32)
                        else:
                            rhs = _bf(sums.at[j][:, lanes])
                    prods[n] = _dot(_bf(lhs.at[n][...]), rhs)
                for q, v in enumerate(_combine(prods)):
                    emit((q // 2) * v.shape[0], cols(j, q % 2), v)

        def emit_h(r0, r, c, v):
            h_v[_at(8 + r0 + r, v.shape[0], 8), c] = _gelu(v)

        def h_body(i, _):
            @pl.when(i + 2 < n_blk)
            def _():
                x_copy(i + 2).start()

            for c in w_copies(1, w2_hbm, w2_v, i):
                c.start()
            w3_copy(i).start()
            x_copy(i).wait()
            for c in w_copies(1, w2_hbm, w2_v, i - 1):
                c.wait()
            norm1(i * TM, lhs_v.at[0])
            for k in range(units):
                r0 = i * TM + k * UNIT
                if k + 1 < units:
                    norm1(r0 + UNIT, lhs_v.at[(k + 1) % 2])
                matmul(w1_v, s1_v, lhs_v.at[k % 2], functools.partial(emit_h, r0))
                prepare(w2_v, s2_v, i - 1, k * (D // 4 // units), D // 4 // units)
            return 0

        def mix_body(i, _):
            copy(w4_hbm, w4_v, sem_w.at[2], _at(i * (FF // 2 // n_blk), FF // 2 // n_blk)).start()

            @pl.when(i == 1)
            def _():
                for c in attn_copies(0):
                    c.start()

            norm3(jnp.maximum(i - 1, 0), units - 1)
            for k in range(units):
                u = i * units + k
                shift(jnp.minimum(u + 1, n_unit - 1), (k + 1) % 2)

                def emit(r, c, v):
                    part_v[_at(u * UNIT + r, half), c] += v
                matmul(w2_v, s2_v, lhs_v.at[k % 2], emit)
                if k + 1 < units:
                    norm3(i, k)
            return 0

        def w3_copy(i):
            return copy(w3_hbm, w3_v, sem_w.at[1], _at(i * (D // 2 // n_blk), D // 2 // n_blk))

        with jax.named_scope("pro"):
            first = [copy(x_hbm, x_v, sem, _at(k * R // 2, R // 2)) for k, sem in enumerate((sem_w.at[0], sem_x.at[0]))]
            w1_copies = functools.partial(w_copies, 0, w1_hbm, w1_v)
            for c in ([first[0]] + w1_copies(0) + w1_copies(1) + [first[1]] + w1_copies(2) + w1_copies(3)
                      + [x_copy(1)] + w_copies(1, w2_hbm, w2_v, 0) + [x_copy(2), w3_copy(0)]):
                c.start()
            h_v[0:8, :] = jnp.zeros((8, D), F32)
            h_v[S + 8:S + 16, :] = jnp.zeros((8, D), F32)
            first[0].wait()
            norm1(0, tmp_v.at[0], R)
            matmul(w1_v, s1_v, tmp_v.at[0], functools.partial(emit_h, 0),
                   lambda j: w1_copies(j) + [first[1]] * (j == 2))
            norm1(R, tmp_v.at[1], R)
            matmul(w1_v, s1_v, tmp_v.at[1], functools.partial(emit_h, R))
        with jax.named_scope("b1"):
            lax.fori_loop(1, n_blk, h_body, 0)
            shift(0, 0)
            for c in w_copies(1, w2_hbm, w2_v, pairs - 1):
                c.wait()
            for r in range(0, D // 4, AC):
                prepare(w2_v, s2_v, pairs - 1, r, AC)
            lax.fori_loop(0, n_blk, mix_body, 0)
            norm3(n_blk - 1, units - 1)

    if SKIP_B1:
        for c in [half_copy(w3_hbm, w3_v, 1, 0), half_copy(w3_hbm, w3_v, 1, 1), half_copy(w4_hbm, w4_v, 2, 0),
                  half_copy(w4_hbm, w4_v, 2, 1)] + attn_copies(0):
            c.start()
    else:
        pl.run_scoped(
            mixing,
            pltpu.VMEM((S + 16, D), F32),
            pltpu.VMEM((D // 2, D), U32),
            pltpu.VMEM((D // 2, D), U32),
            pltpu.VMEM((D // 2 // LANE, D // 4, 5 * LANE), U32),
            pltpu.VMEM((D // 2 // LANE, D // 4, 5 * LANE), U32),
            pltpu.VMEM((2, 7, UNIT // 4, D // 2), U32),
            pltpu.VMEM((2, 7, R // 4, D // 2), U32),
        )
    mem0_copy.start()
    for k in range(2):
        half_copy(w3_hbm, w3_v, 1, k).wait()
        half_copy(w4_hbm, w4_v, 2, k).wait()

    def channel_mlp(sums_v, u_v):
        up_pairs, down_pairs = FF // 4 // LANE, D // 2 // LANE

        def acc(slot):
            return [(raw_v.at[2 * slabs + n // 4], (n % 2) * R, (n // 2 % 2) * LANE) for n in range(7 * slot, 7 * slot + 7)]

        def attn_weight_tasks(g):
            def store(slab, r, quads):
                for n, i in enumerate(_STORED):
                    sums_v.at[slab][r:r + AC, n * LANE:(n + 1) * LANE] = pltpu.bitcast(
                        _rhs(i, lambda a, c: quads[2 * a + c]), U32)

            def qkv(m, j, r):
                slab = m * HP + g * G + j
                src = raw_v.at[g % 2 * slabs + m * G + j]
                quads = []
                for rr in (r, r + D // 4):
                    a, b = src[rr:rr + AC, :LANE], src[rr:rr + AC, LANE:]
                    h0 = (a & jnp.uint32(0xFFFF)) | (b << 16)
                    h1 = (a >> 16) | (b & jnp.uint32(0xFFFF0000))
                    wqkv_v[2 * slab, rr:rr + AC, :] = h0
                    wqkv_v[2 * slab + 1, rr:rr + AC, :] = h1
                    quads += [_bf(h0), _bf(h1)]
                store(slab, r, quads)

            def out(j, r):
                quads = []
                for a in range(2):
                    for n in (j, j + down_pairs):
                        r0, c0 = (n // 2 % 2) * grows + a * (grows // 2) + r, (n % 2) * LANE
                        quads.append(_bf(raw_v.at[g % 2 * slabs + 3 * G + n // 4][r0:r0 + AC, c0:c0 + LANE]))
                store(3 * HP + 2 * g + j // 2, r + (j % 2) * (grows // 2), quads)

            return ([functools.partial(qkv, m, j, r) for m in range(3) for j in range(G)
                     for r in range(0, D // 4, AC)]
                    + [functools.partial(out, j, r) for j in range(down_pairs)
                       for r in range(0, grows // 2, AC)])

        def emit_up(j, r, quads):
            for n, v in enumerate(_lhs7(*[_gelu(q) for q in quads])):
                u_v.at[n][r // 2:(r + RC) // 2, j * LANE:(j + 1) * LANE] = _words(v)

        def emit_down(i, j, r, quads):
            for q, v in enumerate(quads):
                r0 = i * TM + r // (UNIT // 2) * UNIT + (q // 2) * (UNIT // 2) + r % (UNIT // 2)
                part_v[_at(r0, RC), cols(j, q % 2)] += v

        def last_epilogue(i):
            return _finish_tasks(acc(2), functools.partial(emit_down, i, down_pairs - 1))

        for ref, r0, c0 in acc(2):
            ref[r0:r0 + R, c0:c0 + LANE] = jnp.zeros((R, LANE), U32)

        def body(it, _):
            i, f = it // 2, it % 2

            @pl.when(it + 1 < n_grp)
            def _():
                for c in attn_copies(it + 1):
                    c.start()

            for c in attn_copies(it):
                c.wait()
            slots = [n % 2 for n in range(up_pairs + down_pairs - 1)] + [2]
            next_acc = lambda: acc(slots.pop(0))
            up, tail = _matmul_tasks(
                lambda n: _bf(l3_v.at[i, n][...]),
                lambda j, n: _rhs(n, lambda a, c: _bf(
                    w3_v[a * (D // 4):(a + 1) * (D // 4), _at(c * (FF // 2) + f * (FF // 4) + j * LANE, LANE)])),
                up_pairs, next_acc, emit_up, last_epilogue(jnp.maximum(it - 1, 0) // 2))
            down, _ = _matmul_tasks(
                lambda n: _bf(u_v.at[n][...]),
                lambda j, n: _rhs(n, lambda a, c: _bf(
                    w4_v[_at(a * (FF // 4) + f * (FF // 8), FF // 8, 64), cols(j, c)])),
                down_pairs, next_acc, functools.partial(emit_down, i), [])
            side = attn_weight_tasks(it)
            cut = int(len(side) * CUT)
            _run(up[:HEAD] + _weave(up[HEAD:], side[:cut]) + tail + _weave(down[:len(down) - FOOT], side[cut:]) + down[len(down) - FOOT:])
            return 0

        with jax.named_scope("b2"):
            lax.fori_loop(0, n_grp, body, 0)
            _run(last_epilogue(n_blk - 1))

    def recurrence(sums_v, own_v, lhs_v, next_v, hq_v, ho_v):
        scale = float(Dh) ** -0.5
        own = seg - 8
        row = lax.broadcasted_iota(jnp.int32, (2 * L, LANE if WIDE else 2 * L), 0)
        col = lax.broadcasted_iota(jnp.int32, (2 * L, LANE if WIDE else 2 * L), 1)
        r_in = jnp.where(row >= L, row - L, row)
        c_in = jnp.where(col >= L, col - L, col)
        same_head = ((row >= L) == (col >= L)) & (col < 2 * L)
        keep = same_head & ((r_in < M) | (r_in >= c_in))
        fill = jnp.where(same_head, _NEG / scale, -jnp.inf).astype(F32)

        def load_own(s):
            own_v[...] = _ln(x_rows(s * seg, seg)[:own])

        def load_held(s, q):
            next_v[8 * q:8 * q + 8, :] = _ln(x_rows(s * seg + seg - 16, 16)[8:])

        def load_lhs(mem):
            top, bot, k = jnp.concatenate([mem, own_v[...]], axis=0), next_v[...], D // 2
            for n, v in enumerate(_lhs7(top[:, :k], top[:, k:], bot[:, :k], bot[:, k:])):
                lhs_v.at[n][...] = _words(v)

        def by_head(split, dot, a, b):
            return jnp.concatenate([dot(a[:L], b), dot(a[L:], b)], axis=0) if split else dot(a, b)

        def scores(split, q, k):
            s = jnp.where(keep, by_head(split, _dot_nt, q, widen(k)), fill)
            e = jnp.exp2((s - jnp.max(s, axis=-1, keepdims=True)) * (scale * _LOG2E))
            total = jnp.sum(e, axis=-1, keepdims=True)
            return e, pl.reciprocal(total, full_range=False) if RCP else 1.0 / total

        def widen(x):
            return (jnp.concatenate([x, x[:LANE - 2 * L]], axis=0) if WIDE else x).astype(BF16)

        def stored(slab, i, rows=slice(None)):
            n = _STORED.index(i)
            return sums_v.at[slab][rows, n * LANE:(n + 1) * LANE]

        def step(s, r, mem):
            first = isinstance(r, int) and r == 0
            last = isinstance(r, int) and r == PERIOD - 1
            top = None if first else jnp.concatenate([mem, own_v[...]], axis=0)
            early = {} if first else {
                h: _dot(top[:, :D // 2].astype(BF16), _bf(wqkv_v[h, :D // 4, :])) for h in (0, 1, H, H + 1, 2 * H)[:SPLIT]}

            def plain(h):
                if h in early:
                    return early[h] + _dot(top[:, D // 2:].astype(BF16), _bf(wqkv_v[h, D // 4:, :]))
                return _dot(top.astype(BF16), _bf(wqkv_v[h]))

            def project(hp):
                res = []
                for m in range(3):
                    h0 = m * H + 2 * hp
                    if first:
                        prods = []
                        for i in range(7):
                            if i in _STORED:
                                w = stored(m * HP + hp, i)
                            else:
                                w = wqkv_v[h0 + i // 4, (i // 4) * (D // 4):(i // 4 + 1) * (D // 4), :]
                            prods.append(_dot(_bf(lhs_v.at[i][...]), _bf(w)))
                        c11, c12, c21, c22 = _combine(prods)
                        hq_v[h0], hq_v[h0 + 1] = c21[8:], c22[8:]
                        res.append(jnp.concatenate([c11, c21[:8], c12, c22[:8]], axis=0))
                    else:
                        parts = []
                        for j in range(2):
                            parts += [plain(h0 + j), hq_v[h0 + j, _at(8 * (r - 1), 8), :]]
                        res.append(jnp.concatenate(parts, axis=0))
                return res

            def merge(g, heads, acc):
                tops = jnp.concatenate([o[:L - 8] for o in heads], axis=1)
                held = jnp.concatenate([o[L - 8:] for o in heads], axis=1)
                lanes = slice(2 * g * grows, 2 * (g + 1) * grows)
                if last:
                    bots = jnp.concatenate([ho_v[:, lanes], held], axis=0)
                    lhs = _lhs7(tops[:, :grows], tops[:, grows:], bots[:, :grows], bots[:, grows:])
                    y, n = [None] * 7, grows // 2
                    for i in (0, 3, 4, 6, 2, 1, 5):
                        if i in _STORED:
                            w = jnp.concatenate(
                                [stored(3 * HP + 2 * g + j // 2, i, slice((j % 2) * n, (j % 2 + 1) * n))
                                 for j in range(D // 2 // LANE)], axis=1)
                        else:
                            r0, c0 = g * grows + (i // 4) * n, (i // 4) * (D // 2)
                            w = wo_v[r0:r0 + n, c0:c0 + D // 2]
                        y[i] = _dot(lhs[i].astype(LHS_DT), _bf(w))
                else:
                    ho_v[_at(8 * r, 8), lanes] = held
                    y = [_dot(tops.astype(LHS_DT), _bf(wo_v[g * grows:(g + 1) * grows, :]))]
                return y if acc is None else [a + b for a, b in zip(acc, y)]

            qkv, prob, heads = {}, {}, {}
            acc, done = None, 0
            for t in range(n_grp + 3):
                if t < n_grp:
                    qkv[t] = [project(t * G + j) for j in range(G)]
                upto = {n_grp: UP0, n_grp + 1: UP1, n_grp + 2: n_grp}.get(t, t - LAG + 1)
                while done < upto:
                    acc = merge(done, heads.pop(done), acc)
                    done += 1
                if 0 <= t - 2 < n_grp:
                    heads[t - 2] = []
                    for (e, inv), (_, _, v) in zip(prob.pop(t - 2), qkv.pop(t - 2)):
                        split = S1 and t - 2 in P1T or ALLSPLIT
                        if PRE:
                            o = by_head(split, _dot, e * inv, widen(v))
                        else:
                            o = by_head(split, _dot, e, widen(v)) * inv
                        heads[t - 2] += [o[:L], o[L:]]
                if 0 <= t - 1 < n_grp:
                    prob[t - 1] = [scores(S1 and t in S1T or ALLSPLIT, q, k) for q, k, _ in qkv[t - 1]]
                if last and 1 <= t <= PERIOD:
                    load_held(jnp.minimum(s + t, n_seg - 1), t - 1)
                if t == n_grp - 1:
                    load_own(jnp.minimum(s + 1, n_seg - 1))
            if last:
                c11, c12, c21, c22 = _combine(acc)
                load_lhs(jnp.concatenate([c11[:M], c12[:M]], axis=1))
                y, y_held = jnp.concatenate([c11, c12], axis=1), jnp.concatenate([c21, c22], axis=1)
            else:
                y = acc[0]
            base = x_rows(s * seg, seg) + part.get(s * seg, seg)
            x_v[_at(s * (seg // 2), 8), :] = _words(base[:16] + y[M:M + 16])
            part.set(s * seg + 16, jnp.concatenate([base[16:24] + y[M + 16:], base[24:]], axis=0))
            if last:
                for q in range(PERIOD):
                    r0 = (s - (PERIOD - 1) + q) * seg + 16
                    rest = part.get(r0, 16)
                    x_v[_at(r0 // 2, 8), :] = _words(jnp.concatenate(
                        [rest[:8], rest[8:] + y_held[8 * q:8 * q + 8]], axis=0))
            return y[:M]

        def period(p, _):
            s = p * PERIOD
            mem = step(s, 0, None)
            if UNROLL:
                for r in range(1, PERIOD - 1):
                    mem = step(s + r, r, mem)
            else:
                mem = lax.fori_loop(1, PERIOD - 1, lambda r, mem: step(s + r, r, mem), mem)
            mem = step(s + PERIOD - 1, PERIOD - 1, mem)
            rows = _at(s * (seg // 2), PERIOD * seg // 2)
            pltpu.make_async_copy(x_v.at[rows], out_hbm.bitcast(U32).at[rows], sem_out).start()
            return 0

        load_own(0)
        for q in range(PERIOD):
            load_held(q, q)
        mem0_copy.wait()
        load_lhs(mem0_v[...].astype(F32))
        with jax.named_scope("aloop"):
            lax.fori_loop(0, n_seg // PERIOD, period, 0)

    def rest(sums_v):
        if not SKIP_B2:
            pl.run_scoped(functools.partial(channel_mlp, sums_v), pltpu.VMEM((7, R // 2, FF // 4), U32))
        if SKIP_A:
            x_v[0:8, :] = jnp.concatenate([sums_v[5, 0:8, 0:512]] * 2, axis=1) + l3_v[pl.semaphore_read(sem_out), 3, 0:8, 0:1] + wqkv_v[7, 0:8, 0:1]
            pltpu.make_async_copy(x_v, out_hbm.bitcast(U32), sem_out).start()
            return
        pl.run_scoped(
            functools.partial(recurrence, sums_v),
            pltpu.VMEM((seg - 8, D), F32),
            pltpu.VMEM((7, (L - 8) // 2, D // 2), U32),
            pltpu.VMEM((8 * PERIOD, D), F32),
            pltpu.VMEM((3 * H, 8 * (PERIOD - 1), Dh), F32),
            pltpu.VMEM((8 * (PERIOD - 1), H * Dh), F32),
        )

    pl.run_scoped(rest, pltpu.VMEM((4 * HP, D // 4, 5 * LANE), U32))
    pltpu.make_async_copy(x_v, out_hbm.bitcast(U32), sem_out).wait()


@functools.partial(jax.jit, static_argnames=("A_seg_len",))
def pallas_parallel_sum__memory_aug_recurrent_mem_tr__mixer_s_mlp__prompt_kernel(
    A_x: jax.Array,
    A_mem0: jax.Array,
    A_Wq: jax.Array,
    A_Wk: jax.Array,
    A_Wv: jax.Array,
    A_Wo: jax.Array,
    A_seg_len: int,
    B_x: jax.Array,
    B_w1: jax.Array,
    B_w2: jax.Array,
    B_w3: jax.Array,
    B_w4: jax.Array,
):
    del B_x
    B, S, D = A_x.shape
    H, Dh = A_Wq.shape[1], A_Wq.shape[2]
    M = A_mem0.shape[1]
    FF = B_w3.shape[1]
    assert (B, M, A_seg_len) == (1, 8, 32)
    n_blk = S // TM

    hbm = pl.BlockSpec(memory_space=pl.ANY)
    out = pl.pallas_call(
        functools.partial(_kernel, seg=A_seg_len),
        out_shape=jax.ShapeDtypeStruct((S, D), A_x.dtype),
        in_specs=[hbm] * 10,
        out_specs=hbm,
        scratch_shapes=[
            pltpu.VMEM((S // 2, D), U32), pltpu.VMEM((S, D), F32),
            pltpu.VMEM((3 * H, D // 2, Dh), U32),
            pltpu.VMEM((H * Dh // 2, D), U32),
            pltpu.VMEM((D // 2, FF), U32),
            pltpu.VMEM((FF // 2, D), U32),
            pltpu.VMEM((n_blk, 7, TM // 4, D // 2), U32),
            pltpu.VMEM((8 * G + 6, D // 2, 2 * LANE), U32),
            pltpu.VMEM((M, D), A_mem0.dtype),
            pltpu.SemaphoreType.DMA((n_blk,)),
            pltpu.SemaphoreType.DMA((2, D // 2 // LANE)),
            pltpu.SemaphoreType.DMA((4,)),
            pltpu.SemaphoreType.DMA((2 * n_blk,)),
            pltpu.SemaphoreType.DMA,
        ],
        compiler_params=pltpu.CompilerParams(
            vmem_limit_bytes=126 * 1024 * 1024, disable_bounds_checks=True),
    )(A_x.reshape(S, D), A_mem0.reshape(M, D),
      A_Wq.reshape(D // 2, 2, H, Dh), A_Wk.reshape(D // 2, 2, H, Dh), A_Wv.reshape(D // 2, 2, H, Dh),
      A_Wo.reshape(H * Dh, D), B_w1, B_w2, B_w3, B_w4)
    return out.reshape(B, S, D)
```

```python
import functools

import jax
import jax.numpy as jnp
import numpy as np
from jax import lax
import jax.experimental.pallas as pl
import jax.experimental.pallas.tpu as pltpu

F32 = jnp.float32
BF16 = jnp.bfloat16
U32 = jnp.uint32

_EPS = 1e-5
_NEG = -1e9
_LOG2E = float(np.log2(np.e))
_GELU_C = float(np.sqrt(2.0 / np.pi))

LANE = 128
TM = 512
UNIT = 64
RC = 16
AC = 8
WC = 32
FEN = 1
SUMONLY = False
SEP = True
PU = ()
REG = (0,)
DIRECT = False
LEAD = False
CARRY = False
G = 2
PERIOD = 4
LAG = 5
CUT = 0.6
HEAD = 1
FOOT = 1
LHS_DT = BF16
KEEP = True
PIN1 = False
UNROLL = True
SPLIT = 4
S1 = True
UP0 = 4
UP1 = 6
WIDE = False
RCP = True
PRE = False
S1T = (1,)
P1T = (7,)
ALLSPLIT = False
LN2 = True
OPQ = True
OP3 = True
OPS = False
TWO = False
ORDER = 1
E1 = 24
PIN3 = False
EARLY = 1
SKIP_B1 = False
SKIP_B2 = False
SKIP_A = False


def _dot(a, b):
    return lax.dot_general(a, b, (((1,), (0,)), ((), ())), preferred_element_type=F32)


def _dot_nt(a, b):
    return lax.dot_general(a, b, (((1,), (1,)), ((), ())), preferred_element_type=F32)


def _bf(words):
    return pltpu.bitcast(words, BF16)


def _words(x):
    return pltpu.bitcast(x.astype(BF16), U32)


def _at(start, n, align=None):
    return pl.ds(start if isinstance(start, int) else pl.multiple_of(start, align or n), n)


def _ln(x):
    inv_n = 1.0 / x.shape[-1]
    xc = x - jnp.sum(x, axis=-1, keepdims=True) * inv_n
    var = jnp.sum(xc * xc, axis=-1, keepdims=True) * inv_n
    return xc * lax.rsqrt(var + _EPS)


def _gelu(x):
    inner = x * (_GELU_C + (_GELU_C * 0.044715) * (x * x))
    hx = 0.5 * x
    return hx + hx * jnp.tanh(inner)


def _lhs7(a11, a12, a21, a22):
    return (a11 + a22, a21 + a22, a11, a22, a11 + a12, a21 - a11, a12 - a22)


def _rhs(i, b):
    if i in (1, 4):
        return b(i // 4, i // 4)
    p, q, sign = {0: ((0, 0), (1, 1), 1), 2: ((0, 1), (1, 1), -1), 3: ((1, 0), (0, 0), -1),
                  5: ((0, 0), (0, 1), 1), 6: ((1, 0), (1, 1), 1)}[i]
    p, q = b(*p).astype(F32), b(*q).astype(F32)
    return (p + q if sign > 0 else p - q).astype(BF16)


_STORED = (0, 2, 3, 5, 6)


def _combine(m):
    return (m[0] + m[3] - m[4] + m[6], m[2] + m[4], m[1] + m[3], m[0] - m[1] + m[2] + m[5])


def _hopcroft_kerr(p):
    own = {0: ((1, 2, 1), (2, 0, 1)), 1: ((2, 1, -1), (0, 2, 1)), 2: ((1, 1, 1), (0, 0, 1))}
    cross = {(0, 1): ((1, 0, 1, 0, 1, -1), (0, -1, 0, -1, 0, 1, -1), (-1, 0, 1, 0, 1, 0, 1)),
             (0, 2): ((2, 0, 1, 2, 1, 1), (-1, 0, 0, -1, 0, 1, -1), (0, -1, -1, 0, -1, 0, 1)),
             (1, 2): ((2, 1, -1, 2, 0, 1), (0, -1, -1, 0, 1, 0, 1), (1, 0, 0, -1, 0, 1, -1))}
    prods, diag, entry = [], {}, {}

    def product(left, out):
        prods.append((left, out))
        return len(prods) - 1

    def diagonal(idx, kind):
        diag[idx] = [product([(i, f, 1) for i in idx], [(i, g, 1) for i in idx]) for f, g, _ in own[kind]]

    def pair(a, ka, b, kb):
        if ka > kb:
            return pair(b, kb, a, ka)[::-1]
        (f0, f1, s, g0, g1, t), ab, ba = cross[ka, kb]
        diagonal(a + b, 3 - ka - kb)
        used = diag[a] + diag[b] + diag[a + b] + [product(
            [(i, f0, 1) for i in a] + [(i, f1, s) for i in b], [(i, g0, 1) for i in a] + [(i, g1, t) for i in b])]
        return dict(zip(used, ab)), dict(zip(used, ba))

    for i in range(p):
        diagonal((i,), i % 3)
        entry[i, i] = {r: sign for r, (_, _, sign) in zip(diag[i,], own[i % 3])}
    for j in range(p):
        for i in range(j):
            if i % 3 != j % 3:
                entry[i, j], entry[j, i] = pair((i,), i % 3, (j,), j % 3)
    for j in range(p):
        for i in range(j % 3, j, 3):
            k = i + 1
            both = (i, k) if (i, k) in diag else (k, i)
            entry[i, j], entry[j, i] = pair(both, 3 - i % 3 - k % 3, (j,), j % 3)
            for ij, kj in (((i, j), (k, j)), ((j, i), (j, k))):
                for r, c in entry[kj].items():
                    entry[ij][r] = entry[ij].get(r, 0) - c
    return [(left, [(i, j, c[r]) for (i, j), c in sorted(entry.items()) if c.get(r)], out)
            for r, (left, out) in enumerate(prods)]

P = 2 * G
_HK = _hopcroft_kerr(P)
_HK_STORED = [r for r, (_, weight, _) in enumerate(_HK) if len(weight) > 1]


def _signed_sum(terms):
    terms = sorted(terms, key=lambda t: -t[0])
    assert terms[0][0] > 0
    total = terms[0][1]
    for sign, value in terms[1:]:
        total = total + value if sign > 0 else total - value
    return total


def _hk_left(top, bot):
    k = top.shape[1] // P
    forms = [(t, b, t - b) for t, b in ((top[:, i * k:(i + 1) * k], bot[:, i * k:(i + 1) * k]) for i in range(P))]
    return [_signed_sum([(sign, forms[i][f]) for i, f, sign in left]) for left, _, _ in _HK]


def _hk_weights(block):
    wide = {(i, j): block(i, j).astype(F32) for i in range(P) for j in range(P)}
    return [_signed_sum([(sign, wide[i, j]) for i, j, sign in _HK[r][1]]) for r in _HK_STORED]


def _hk_matmul(left, block, stored, order, acc):
    acc = dict(acc)
    for r in order:
        _, weight, out = _HK[r]
        if r in _HK_STORED:
            flip, w = 1, stored(_HK_STORED.index(r))
        else:
            flip, w = weight[0][2], block(*weight[0][:2])
        m = _dot(left(r), w)
        for j, f, sign in out:
            if (j, f) in acc:
                acc[j, f] = acc[j, f] + m if sign * flip > 0 else acc[j, f] - m
            else:
                acc[j, f] = m if sign * flip > 0 else -m
    return acc


def _hk_result(acc):
    return ([acc[j, 0] + acc[j, 2] for j in range(P)], [acc[j, 1] + acc[j, 2] for j in range(P)])


def _weave(main, side):
    out, k = [], 0
    for i, task in enumerate(main):
        out.append(task)
        while k < len(side) and (k + 1) * len(main) <= (i + 1) * len(side):
            out.append(side[k])
            k += 1
    return out


def _run(tasks):
    for task in tasks:
        task()


def _finish_tasks(acc, emit):
    def finish(r):
        emit(r, _combine([pltpu.bitcast(ref[r0 + r:r0 + r + RC, c0:c0 + LANE], F32) for ref, r0, c0 in acc]))
    return [functools.partial(finish, r) for r in range(0, TM // 2, RC)]


def _matmul_tasks(lhs, rhs, pairs, next_acc, emit, tail):
    def product(acc, j, i):
        ref, r0, c0 = acc[i]
        ref[r0:r0 + TM // 2, c0:c0 + LANE] = pltpu.bitcast(
            _dot(lhs(i), rhs(j, i)), U32)

    out = []
    for j in range(pairs):
        acc = next_acc()
        out += _weave([functools.partial(product, acc, j, i) for i in (1, 0, 2, 3, 4, 5, 6)], tail)
        tail = _finish_tasks(acc, functools.partial(emit, j))
    return out, tail


def _kernel(x_hbm, mem0_hbm, wq_hbm, wk_hbm, wv_hbm, wo_hbm, w1_hbm, w2_hbm, w3_hbm, w4_hbm,
            out_hbm,
            x_v, part_v, wqkv_v, wo_v, w3_v, w4_v, l3_v, raw_v, mem0_v,
            sem_x, sem_w1, sem_w, sem_a, sem_out, *, seg):
    S, D = x_hbm.shape
    H, Dh = wq_hbm.shape[2], wq_hbm.shape[3]
    M = mem0_hbm.shape[0]
    FF = w3_hbm.shape[1]
    HP = H // 2
    L = M + seg
    R = TM // 2
    n_blk = S // TM
    n_seg = S // seg
    n_grp = HP // G
    assert n_grp == 2 * n_blk
    grows = G * Dh

    class part:
        @staticmethod
        def get(r0, n, c=slice(None)):
            return part_v[_at(r0, n, 8), c]

        @staticmethod
        def set(r0, v, c=slice(None)):
            part_v[_at(r0, v.shape[0], 8), c] = v

    def copy(hbm, vmem, sem, *idx):
        return pltpu.make_async_copy(hbm.bitcast(U32).at[idx], vmem.at[idx], sem)

    slabs = 4 * G

    def attn_copies(g):
        rows = _at(g * grows, grows)
        copies = [copy(wo_hbm, wo_v, sem_a.at[g], rows)]
        base = g % 2 * slabs
        for m, hbm in enumerate((wq_hbm, wk_hbm, wv_hbm)):
            for j in range(G):
                for par in range(2):
                    copies.append(pltpu.make_async_copy(
                        hbm.bitcast(U32).at[:, par, g * G + j, :],
                        raw_v.at[base + m * G + j, :, par * LANE:(par + 1) * LANE], sem_a.at[g]))
        for n in range(4):
            copies.append(pltpu.make_async_copy(
                wo_hbm.bitcast(U32).at[rows, n * D // 4:(n + 1) * D // 4],
                raw_v.at[base + 3 * G + n // 2, (n % 2) * grows:(n % 2 + 1) * grows], sem_a.at[g]))
        return copies

    mem0_copy = pltpu.make_async_copy(mem0_hbm, mem0_v, sem_w.at[3])

    def half_copy(hbm, vmem, n, k):
        rows = vmem.shape[0] // 2
        return copy(hbm, vmem, sem_w.at[n], _at(k * rows, rows))

    def x_rows(r0, n):
        return _bf(x_v[_at(r0 // 2, n // 2), :]).astype(F32)

    def cols(j, c):
        return slice(c * (D // 2) + j * LANE, c * (D // 2) + (j + 1) * LANE)

    def mixing(h_v, w1_v, w2_v, s1_v, s2_v, lhs_v, tmp_v):
        pairs = D // 2 // LANE
        units = TM // UNIT
        n_unit = S // UNIT
        half = UNIT // 2

        def w_copies(n, hbm, vmem, j):
            return [copy(hbm, vmem, sem_w1.at[n, j], slice(None), _at(c * (D // 2) + j * LANE, LANE))
                    for c in range(2)]

        def x_copy(i):
            return copy(x_hbm, x_v, sem_x.at[i], _at(i * R, R))

        def quad(w, j, a, c, r=0, n=D // 4):
            return _bf(w[a * (D // 4) + r:a * (D // 4) + r + n, _at(c * (D // 2) + j * LANE, LANE)])

        def prepare(w, sums, j, r, size):
            for n, i in enumerate(_STORED):
                sums.at[j][r:r + size, n * LANE:(n + 1) * LANE] = pltpu.bitcast(
                    _rhs(i, lambda a, c: quad(w, j, a, c, r, size)), U32)

        def store_lhs(ref, r, rows, size=UNIT):
            k = D // 2
            for q in range(0, size // 2, RC):
                top, bot = rows(q), rows(size // 2 + q)
                for n, v in enumerate(_lhs7(top[:, :k], top[:, k:], bot[:, :k], bot[:, k:])):
                    ref.at[n][(r + q) // 2:(r + q + RC) // 2, :] = _words(v)

        def norm1(r0, ref, size=UNIT):
            def rows(r):
                x = x_rows(r0 + r, RC)
                xc = x - jnp.sum(x, axis=-1, keepdims=True) * (1.0 / D)
                var = jnp.sum(xc * xc, axis=-1, keepdims=True) * (1.0 / D)
                inv = lax.rsqrt(var + _EPS)
                xn = xc * inv
                part_v[_at(r0 + r, RC), :] = xn
                return xn * lax.rsqrt(var * inv * inv + _EPS)
            store_lhs(ref, 0, rows, size)

        def shift(u, slot):
            def rows(r):
                r0 = u * UNIT + r
                parts = []
                for g, by in enumerate((-1, 1, -2, 2)):
                    c = slice(g * D // 4, (g + 1) * D // 4)
                    if by < 0:
                        parts.append(pltpu.roll(h_v[_at(r0, RC + 8, 8), c], -by, 0)[8:])
                    else:
                        parts.append(pltpu.roll(h_v[_at(r0 + 8, RC + 8, 8), c], RC + 8 - by, 0)[:RC])
                return jnp.concatenate(parts, axis=1)
            store_lhs(lhs_v.at[slot], 0, rows)

        def norm3(i, k):
            store_lhs(l3_v.at[i], k * half, lambda r: _ln(part_v[_at(i * TM + k * UNIT + r, RC), :]))

        def matmul(w, sums, lhs, emit, arriving=None):
            for j in range(pairs):
                if arriving:
                    for c in arriving(j):
                        c.wait()
                prods = [None] * 7
                for n in (1, 0, 2, 3, 4, 5, 6):
                    if n not in _STORED:
                        rhs = quad(w, j, n // 4, n // 4)
                    else:
                        lanes = _at(_STORED.index(n) * LANE, LANE)
                        if arriving:
                            rhs = _rhs(n, functools.partial(quad, w, j))
                            sums.at[j][:, lanes] = pltpu.bitcast(rhs, U32)
                        else:
                            rhs = _bf(sums.at[j][:, lanes])
                    prods[n] = _dot(_bf(lhs.at[n][...]), rhs)
                for q, v in enumerate(_combine(prods)):
                    emit((q // 2) * v.shape[0], cols(j, q % 2), v)

        def emit_h(r0, r, c, v):
            h_v[_at(8 + r0 + r, v.shape[0], 8), c] = _gelu(v)

        def h_body(i, _):
            @pl.when(i + 2 < n_blk)
            def _():
                x_copy(i + 2).start()

            for c in w_copies(1, w2_hbm, w2_v, i):
                c.start()
            w3_copy(i).start()
            x_copy(i).wait()
            for c in w_copies(1, w2_hbm, w2_v, i - 1):
                c.wait()
            norm1(i * TM, lhs_v.at[0])
            for k in range(units):
                r0 = i * TM + k * UNIT
                if k + 1 < units:
                    norm1(r0 + UNIT, lhs_v.at[(k + 1) % 2])
                matmul(w1_v, s1_v, lhs_v.at[k % 2], functools.partial(emit_h, r0))
                prepare(w2_v, s2_v, i - 1, k * (D // 4 // units), D // 4 // units)
            return 0

        def mix_body(i, _):
            copy(w4_hbm, w4_v, sem_w.at[2], _at(i * (FF // 2 // n_blk), FF // 2 // n_blk)).start()

            @pl.when(i == 1)
            def _():
                for c in attn_copies(0):
                    c.start()

            norm3(jnp.maximum(i - 1, 0), units - 1)
            for k in range(units):
                u = i * units + k
                shift(jnp.minimum(u + 1, n_unit - 1), (k + 1) % 2)

                def emit(r, c, v):
                    part_v[_at(u * UNIT + r, half), c] += v
                matmul(w2_v, s2_v, lhs_v.at[k % 2], emit)
                if k + 1 < units:
                    norm3(i, k)
            return 0

        def w3_copy(i):
            return copy(w3_hbm, w3_v, sem_w.at[1], _at(i * (D // 2 // n_blk), D // 2 // n_blk))

        with jax.named_scope("pro"):
            first = [copy(x_hbm, x_v, sem, _at(k * R // 2, R // 2)) for k, sem in enumerate((sem_w.at[0], sem_x.at[0]))]
            w1_copies = functools.partial(w_copies, 0, w1_hbm, w1_v)
            for c in ([first[0]] + w1_copies(0) + w1_copies(1) + [first[1]] + w1_copies(2) + w1_copies(3)
                      + [x_copy(1)] + w_copies(1, w2_hbm, w2_v, 0) + [x_copy(2), w3_copy(0)]):
                c.start()
            h_v[0:8, :] = jnp.zeros((8, D), F32)
            h_v[S + 8:S + 16, :] = jnp.zeros((8, D), F32)
            first[0].wait()
            norm1(0, tmp_v.at[0], R)
            matmul(w1_v, s1_v, tmp_v.at[0], functools.partial(emit_h, 0),
                   lambda j: w1_copies(j) + [first[1]] * (j == 2))
            norm1(R, tmp_v.at[1], R)
            matmul(w1_v, s1_v, tmp_v.at[1], functools.partial(emit_h, R))
        with jax.named_scope("b1"):
            lax.fori_loop(1, n_blk, h_body, 0)
            shift(0, 0)
            for c in w_copies(1, w2_hbm, w2_v, pairs - 1):
                c.wait()
            for r in range(0, D // 4, WC):
                prepare(w2_v, s2_v, pairs - 1, r, WC)
            lax.fori_loop(0, n_blk, mix_body, 0)
            norm3(n_blk - 1, units - 1)

    if SKIP_B1:
        for c in [half_copy(w3_hbm, w3_v, 1, 0), half_copy(w3_hbm, w3_v, 1, 1), half_copy(w4_hbm, w4_v, 2, 0),
                  half_copy(w4_hbm, w4_v, 2, 1)] + attn_copies(0):
            c.start()
    else:
        pl.run_scoped(
            mixing,
            pltpu.VMEM((S + 16, D), F32),
            pltpu.VMEM((D // 2, D), U32),
            pltpu.VMEM((D // 2, D), U32),
            pltpu.VMEM((D // 2 // LANE, D // 4, 5 * LANE), U32),
            pltpu.VMEM((D // 2 // LANE, D // 4, 5 * LANE), U32),
            pltpu.VMEM((2, 7, UNIT // 4, D // 2), U32),
            pltpu.VMEM((2, 7, R // 4, D // 2), U32),
        )
    mem0_copy.start()
    for k in range(2):
        half_copy(w3_hbm, w3_v, 1, k).wait()
        half_copy(w4_hbm, w4_v, 2, k).wait()

    def channel_mlp(sums_v, u_v, acc_v, lead_v):
        up_pairs, down_pairs = FF // 4 // LANE, D // 2 // LANE

        def acc(slot):
            if SEP:
                return [(acc_v.at[n], 0, 0) for n in range(7 * slot, 7 * slot + 7)]
            return [(raw_v.at[2 * slabs + n // 4], (n % 2) * R, (n // 2 % 2) * LANE) for n in range(7 * slot, 7 * slot + 7)]

        pending, ready = [], []

        def paced(it, words, ok):
            if pending or ready:
                hint = functools.reduce(jnp.bitwise_or, [ref[(it // n_grp,) + (slice(0, 8), slice(0, LANE))]
                                                         for ref in pending] + ready)
                words = jnp.concatenate([jnp.where(it < 0, hint, words[:8]), words[8:]], axis=0)
                pending.clear()
                ready.clear()
            return _bf(words)

        def attn_weight_tasks(g):
            def store(slab, r, block, direct=DIRECT):
                for n, v in enumerate(_hk_weights(block)):
                    sums_v.at[slab][r:r + AC, n * LANE:(n + 1) * LANE] = w = _words(v)
                    if n in REG and direct:
                        ready.append(w)
                if FEN and not direct:
                    pending.extend(ref for ref in ((), (wqkv_v,), (sums_v,), (sums_v, wqkv_v))[FEN] if not any(ref is q for q in pending))

            def qkv(m, r):
                blocks = {}
                for j in range(G):
                    src = raw_v.at[g % 2 * slabs + m * G + j]
                    for i in range(P):
                        rr = i * (D // 2 // P) + r
                        a, b = src[rr:rr + AC, :LANE], src[rr:rr + AC, LANE:]
                        for n, w in enumerate(((a & jnp.uint32(0xFFFF)) | (b << 16),
                                               (a >> 16) | (b & jnp.uint32(0xFFFF0000)))):
                            wqkv_v[m * H + g * P + 2 * j + n, rr:rr + AC, :] = w
                            blocks[i, 2 * j + n] = _bf(w)
                store(m * n_grp + g, r, lambda i, j: blocks[i, j])

            def out(r):
                def block(i, j):
                    r0, c0 = (j % 2) * grows + i * (Dh // 2) + r % (Dh // 2), r // (Dh // 2) * LANE
                    return _bf(raw_v.at[g % 2 * slabs + 3 * G + j // 2][r0:r0 + AC, c0:c0 + LANE])
                store(3 * n_grp + g, r, block, True)

            return ([functools.partial(qkv, m, r) for m in range(3) for r in range(0, D // 2 // P, AC)]
                    + [functools.partial(out, r) for r in range(0, D // 2 // P, AC)])

        def emit_up(j, r, quads):
            for n, v in enumerate(_lhs7(*[_gelu(q) for q in quads])):
                u_v.at[n][r // 2:(r + RC) // 2, j * LANE:(j + 1) * LANE] = w = _words(v)
                if n in PU and j + 1 < up_pairs:
                    ready.append(w)

        def emit_down(i, j, r, quads):
            for q, v in enumerate(quads):
                r0 = i * TM + r // (UNIT // 2) * UNIT + (q // 2) * (UNIT // 2) + r % (UNIT // 2)
                part_v[_at(r0, RC), cols(j, q % 2)] += v

        def last_epilogue(i):
            return _finish_tasks(acc(2), functools.partial(emit_down, i, down_pairs - 1))

        for ref, r0, c0 in acc(2):
            ref[r0:r0 + R, c0:c0 + LANE] = jnp.zeros((R, LANE), U32)

        def w3_quad(f, j, a, c):
            return w3_v[a * (D // 4):(a + 1) * (D // 4), _at(c * (FF // 2) + f * (FF // 4) + j * LANE, LANE)]

        for f in range(2 * LEAD):
            for k, n in enumerate(_STORED):
                lead_v.at[f][:, k * LANE:(k + 1) * LANE] = pltpu.bitcast(
                    _rhs(n, lambda a, c: _bf(w3_quad(f, 0, a, c))), U32)

        def body(it, _):
            i, f = it // 2, it % 2

            @pl.when(it + 1 < n_grp)
            def _():
                for c in attn_copies(it + 1):
                    c.start()

            for c in attn_copies(it):
                c.wait()
            slots = [n % 2 for n in range(up_pairs + down_pairs - 1)] + [2]
            next_acc = lambda: acc(slots.pop(0))

            def up_rhs(j, n):
                if LEAD and j == 0 and n in _STORED:
                    return paced(it, lead_v.at[f][:, _at(_STORED.index(n) * LANE, LANE)], True)
                return _rhs(n, lambda a, c: paced(it, w3_quad(f, j, a, c), True))

            up, tail = _matmul_tasks(
                lambda n: _bf(l3_v.at[i, n][...]),
                up_rhs,
                up_pairs, next_acc, emit_up, last_epilogue(jnp.maximum(it - 1, 0) // 2) if CARRY else [])
            down, end = _matmul_tasks(
                lambda n: _bf(u_v.at[n][...]),
                lambda j, n: _rhs(n, lambda a, c: paced(it,
                    w4_v[_at(a * (FF // 4) + f * (FF // 8), FF // 8, 64), cols(j, c)], n in _STORED)),
                down_pairs, next_acc, functools.partial(emit_down, i), [])
            side = attn_weight_tasks(it)
            cut = int(len(side) * CUT)
            _run(up[:HEAD] + _weave(up[HEAD:], side[:cut]) + tail + _weave(down[:len(down) - FOOT], side[cut:]) + down[len(down) - FOOT:] + ([] if CARRY else end))
            return 0

        with jax.named_scope("b2"):
            lax.fori_loop(0, n_grp, body, 0)
            if CARRY:
                _run(last_epilogue(n_blk - 1))

    def recurrence(sums_v, own_v, lhs_v, next_v, hq_v, ho_v):
        scale = float(Dh) ** -0.5
        own = seg - 8
        row = lax.broadcasted_iota(jnp.int32, (2 * L, LANE if WIDE else 2 * L), 0)
        col = lax.broadcasted_iota(jnp.int32, (2 * L, LANE if WIDE else 2 * L), 1)
        r_in = jnp.where(row >= L, row - L, row)
        c_in = jnp.where(col >= L, col - L, col)
        same_head = ((row >= L) == (col >= L)) & (col < 2 * L)
        keep = same_head & ((r_in < M) | (r_in >= c_in))
        fill = jnp.where(same_head, _NEG / scale, -jnp.inf).astype(F32)

        def load_own(s):
            own_v[...] = _ln(x_rows(s * seg, seg)[:own])

        def load_held(s, q):
            next_v[8 * q:8 * q + 8, :] = _ln(x_rows(s * seg + seg - 16, 16)[8:])

        def load_lhs(mem):
            for n, v in enumerate(_hk_left(jnp.concatenate([mem, own_v[...]], axis=0), next_v[...])):
                lhs_v[:, n * (D // P):(n + 1) * (D // P)] = _words(v)

        def by_head(split, dot, a, b):
            return jnp.concatenate([dot(a[:L], b), dot(a[L:], b)], axis=0) if split else dot(a, b)

        def scores(split, q, k):
            s = jnp.where(keep, by_head(split, _dot_nt, q, widen(k)), fill)
            e = jnp.exp2((s - jnp.max(s, axis=-1, keepdims=True)) * (scale * _LOG2E))
            total = jnp.sum(e, axis=-1, keepdims=True)
            return e, pl.reciprocal(total, full_range=False) if RCP else 1.0 / total

        def widen(x):
            return (jnp.concatenate([x, x[:LANE - 2 * L]], axis=0) if WIDE else x).astype(BF16)

        def step(s, r, mem):
            first = isinstance(r, int) and r == 0
            last = isinstance(r, int) and r == PERIOD - 1
            top = None if first else jnp.concatenate([mem, own_v[...]], axis=0)
            early = {} if first else {
                h: _dot(top[:, :D // 2].astype(BF16), _bf(wqkv_v[h, :D // 4, :])) for h in (0, 1, H, H + 1, 2 * H)[:SPLIT]}

            def plain(h):
                if h in early:
                    return early[h] + _dot(top[:, D // 2:].astype(BF16), _bf(wqkv_v[h, D // 4:, :]))
                return _dot(top.astype(BF16), _bf(wqkv_v[h]))

            def project(g):
                res = []
                for m in range(3):
                    h0, k = m * H + g * P, D // 2 // P
                    if first:
                        tops, bots = _hk_result(_hk_matmul(
                            lambda n: _bf(lhs_v[:, n * (D // P):(n + 1) * (D // P)]),
                            lambda i, j: _bf(wqkv_v[h0 + j, i * k:(i + 1) * k, :]),
                            lambda n: _bf(sums_v.at[m * n_grp + g][:, n * LANE:(n + 1) * LANE]),
                            range(len(_HK)), {}))
                        for j in range(P):
                            hq_v[h0 + j] = bots[j][8:]
                        held = [b[:8] for b in bots]
                    else:
                        tops = [plain(h0 + j) for j in range(P)]
                        held = [hq_v[h0 + j, 8 * (r - 1):8 * r, :] for j in range(P)]
                    res.append([jnp.concatenate([tops[j], held[j], tops[j + 1], held[j + 1]], axis=0)
                                for j in range(0, P, 2)])
                return list(zip(*res))

            def merge(g, heads, acc):
                tops = jnp.concatenate([o[:L - 8] for o in heads], axis=1)
                held = jnp.concatenate([o[L - 8:] for o in heads], axis=1)
                lanes = slice(g * P * Dh, (g + 1) * P * Dh)
                if last:
                    left = _hk_left(tops, jnp.concatenate([ho_v[:, lanes], held], axis=0))
                    k, n = Dh // 2, D // P
                    return _hk_matmul(
                        lambda q: left[q].astype(BF16),
                        lambda i, j: _bf(wo_v[g * grows + i * k:g * grows + (i + 1) * k, j * n:(j + 1) * n]),
                        lambda q: jnp.concatenate(
                            [_bf(sums_v.at[3 * n_grp + g][c * k:(c + 1) * k, q * LANE:(q + 1) * LANE])
                             for c in range(n // LANE)], axis=1),
                        sorted(range(len(_HK)), key=lambda q: all(f == 1 for _, f, _ in _HK[q][2])), acc or {})
                ho_v[8 * r:8 * r + 8, lanes] = held
                y = _dot(tops.astype(BF16), _bf(wo_v[g * grows:(g + 1) * grows, :]))
                return y if acc is None else acc + y

            qkv, prob, heads = {}, {}, {}
            acc, done = None, 0
            for t in range(n_grp + 3):
                if t < n_grp:
                    qkv[t] = project(t)
                upto = {n_grp: UP0, n_grp + 1: UP1, n_grp + 2: n_grp}.get(t, t - LAG + 1)
                while done < upto:
                    acc = merge(done, heads.pop(done), acc)
                    done += 1
                if 0 <= t - 2 < n_grp:
                    heads[t - 2] = []
                    for (e, inv), (_, _, v) in zip(prob.pop(t - 2), qkv.pop(t - 2)):
                        split = S1 and t - 2 in P1T or ALLSPLIT
                        if PRE:
                            o = by_head(split, _dot, e * inv, widen(v))
                        else:
                            o = by_head(split, _dot, e, widen(v)) * inv
                        heads[t - 2] += [o[:L], o[L:]]
                if 0 <= t - 1 < n_grp:
                    prob[t - 1] = [scores(S1 and t in S1T or ALLSPLIT, q, k) for q, k, _ in qkv[t - 1]]
                if last and 1 <= t <= PERIOD:
                    load_held(jnp.minimum(s + t, n_seg - 1), t - 1)
                if t == n_grp - 1:
                    load_own(jnp.minimum(s + 1, n_seg - 1))
            if last:
                y, y_held = [jnp.concatenate(half, axis=1) for half in _hk_result(acc)]
                load_lhs(y[:M])
            else:
                y = acc
            base = x_rows(s * seg, seg) + part.get(s * seg, seg)
            x_v[_at(s * (seg // 2), 8), :] = _words(base[:16] + y[M:M + 16])
            part.set(s * seg + 16, jnp.concatenate([base[16:24] + y[M + 16:], base[24:]], axis=0))
            if last:
                for q in range(PERIOD):
                    r0 = (s - (PERIOD - 1) + q) * seg + 16
                    rest = part.get(r0, 16)
                    x_v[_at(r0 // 2, 8), :] = _words(jnp.concatenate(
                        [rest[:8], rest[8:] + y_held[8 * q:8 * q + 8]], axis=0))
            return y[:M]

        def period(p, _):
            s = p * PERIOD
            mem = step(s, 0, None)
            if UNROLL:
                for r in range(1, PERIOD - 1):
                    mem = step(s + r, r, mem)
            else:
                mem = lax.fori_loop(1, PERIOD - 1, lambda r, mem: step(s + r, r, mem), mem)
            mem = step(s + PERIOD - 1, PERIOD - 1, mem)
            rows = _at(s * (seg // 2), PERIOD * seg // 2)
            pltpu.make_async_copy(x_v.at[rows], out_hbm.bitcast(U32).at[rows], sem_out).start()
            return 0

        load_own(0)
        for q in range(PERIOD):
            load_held(q, q)
        mem0_copy.wait()
        load_lhs(mem0_v[...].astype(F32))
        with jax.named_scope("aloop"):
            lax.fori_loop(0, n_seg // PERIOD, period, 0)

    def rest(sums_v):
        if not SKIP_B2:
            pl.run_scoped(functools.partial(channel_mlp, sums_v), pltpu.VMEM((7, R // 2, FF // 4), U32), pltpu.VMEM((21, R, LANE), U32),
                          pltpu.VMEM((2, D // 4, 5 * LANE), U32))
        if SKIP_A:
            x_v[0:8, :] = jnp.concatenate([sums_v[5, 0:8, 0:512]] * 2, axis=1) + l3_v[pl.semaphore_read(sem_out), 3, 0:8, 0:1] + wqkv_v[7, 0:8, 0:1]
            pltpu.make_async_copy(x_v, out_hbm.bitcast(U32), sem_out).start()
            return
        pl.run_scoped(
            functools.partial(recurrence, sums_v),
            pltpu.VMEM((seg - 8, D), F32),
            pltpu.VMEM(((L - 8) // 2, len(_HK) * D // P), U32),
            pltpu.VMEM((8 * PERIOD, D), F32),
            pltpu.VMEM((3 * H, 8 * (PERIOD - 1), Dh), F32),
            pltpu.VMEM((8 * (PERIOD - 1), H * Dh), F32),
        )

    pl.run_scoped(rest, pltpu.VMEM((4 * n_grp, D // 2 // P, len(_HK_STORED) * LANE), U32))
    pltpu.make_async_copy(x_v, out_hbm.bitcast(U32), sem_out).wait()


@functools.partial(jax.jit, static_argnames=("A_seg_len",))
def pallas_parallel_sum__memory_aug_recurrent_mem_tr__mixer_s_mlp__prompt_kernel(
    A_x: jax.Array,
    A_mem0: jax.Array,
    A_Wq: jax.Array,
    A_Wk: jax.Array,
    A_Wv: jax.Array,
    A_Wo: jax.Array,
    A_seg_len: int,
    B_x: jax.Array,
    B_w1: jax.Array,
    B_w2: jax.Array,
    B_w3: jax.Array,
    B_w4: jax.Array,
):
    del B_x
    B, S, D = A_x.shape
    H, Dh = A_Wq.shape[1], A_Wq.shape[2]
    M = A_mem0.shape[1]
    FF = B_w3.shape[1]
    assert (B, M, A_seg_len) == (1, 8, 32)
    n_blk = S // TM

    hbm = pl.BlockSpec(memory_space=pl.ANY)
    out = pl.pallas_call(
        functools.partial(_kernel, seg=A_seg_len),
        out_shape=jax.ShapeDtypeStruct((S, D), A_x.dtype),
        in_specs=[hbm] * 10,
        out_specs=hbm,
        scratch_shapes=[
            pltpu.VMEM((S // 2, D), U32), pltpu.VMEM((S, D), F32),
            pltpu.VMEM((3 * H, D // 2, Dh), U32),
            pltpu.VMEM((H * Dh // 2, D), U32),
            pltpu.VMEM((D // 2, FF), U32),
            pltpu.VMEM((FF // 2, D), U32),
            pltpu.VMEM((n_blk, 7, TM // 4, D // 2), U32),
            pltpu.VMEM((8 * G, D // 2, 2 * LANE), U32),
            pltpu.VMEM((M, D), A_mem0.dtype),
            pltpu.SemaphoreType.DMA((n_blk,)),
            pltpu.SemaphoreType.DMA((2, D // 2 // LANE)),
            pltpu.SemaphoreType.DMA((4,)),
            pltpu.SemaphoreType.DMA((2 * n_blk,)),
            pltpu.SemaphoreType.DMA,
        ],
        compiler_params=pltpu.CompilerParams(
            vmem_limit_bytes=126 * 1024 * 1024, disable_bounds_checks=True),
    )(A_x.reshape(S, D), A_mem0.reshape(M, D),
      A_Wq.reshape(D // 2, 2, H, Dh), A_Wk.reshape(D // 2, 2, H, Dh), A_Wv.reshape(D // 2, 2, H, Dh),
      A_Wo.reshape(H * Dh, D), B_w1, B_w2, B_w3, B_w4)
    return out.reshape(B, S, D)
```

```python
import functools

import jax
import jax.numpy as jnp
import numpy as np
from jax import lax
import jax.experimental.pallas as pl
import jax.experimental.pallas.tpu as pltpu

F32 = jnp.float32
BF16 = jnp.bfloat16
U32 = jnp.uint32

_EPS = 1e-5
_NEG = -1e9
_LOG2E = float(np.log2(np.e))
_GELU_C = float(np.sqrt(2.0 / np.pi))

LANE = 128
TM = 512
UNIT = 64
RC = 16
AC = 8
WC = 32
FEN = 1
SUMONLY = False
SEP = True
PU = ()
REG = (0,)
DIRECT = False
HKG = 8
MARK = 'mvVw'
P0 = 0
P1 = 28
Q0 = 5
Q1 = 28
HD = 6
FULL = True
ALL4 = 64
NL = 2
MIXP = True
FLAGS = None
HA = 0
SPREAD = 16
LL = (4, 5, 6)
LF = (5, 4, 6)
LEAD = False
CARRY = False
G = 2
PERIOD = 4
LAG = 5
CUT = 0.6
HEAD = 1
FOOT = 1
LHS_DT = BF16
KEEP = True
PIN1 = False
UNROLL = True
SPLIT = 4
S1 = True
UP0 = 4
UP1 = 5
WIDE = False
RCP = True
PRE = False
S1T = (1,)
P1T = (7,)
ALLSPLIT = False
LN2 = True
OPQ = True
OP3 = True
OPS = False
TWO = False
ORDER = 1
E1 = 24
PIN3 = False
EARLY = 1
SKIP_B1 = False
SKIP_B2 = False
SKIP_A = False


def _dot(a, b):
    return lax.dot_general(a, b, (((1,), (0,)), ((), ())), preferred_element_type=F32)


def _dot_nt(a, b):
    return lax.dot_general(a, b, (((1,), (1,)), ((), ())), preferred_element_type=F32)


def _bf(words):
    return pltpu.bitcast(words, BF16)


def _words(x):
    return pltpu.bitcast(x.astype(BF16), U32)


def _at(start, n, align=None):
    return pl.ds(start if isinstance(start, int) else pl.multiple_of(start, align or n), n)


def _ln(x):
    inv_n = 1.0 / x.shape[-1]
    xc = x - jnp.sum(x, axis=-1, keepdims=True) * inv_n
    var = jnp.sum(xc * xc, axis=-1, keepdims=True) * inv_n
    return xc * lax.rsqrt(var + _EPS)


def _gelu(x):
    inner = x * (_GELU_C + (_GELU_C * 0.044715) * (x * x))
    hx = 0.5 * x
    return hx + hx * jnp.tanh(inner)


def _lhs7(a11, a12, a21, a22):
    return (a11 + a22, a21 + a22, a11, a22, a11 + a12, a21 - a11, a12 - a22)


def _rhs(i, b):
    if i in (1, 4):
        return b(i // 4, i // 4)
    p, q, sign = {0: ((0, 0), (1, 1), 1), 2: ((0, 1), (1, 1), -1), 3: ((1, 0), (0, 0), -1),
                  5: ((0, 0), (0, 1), 1), 6: ((1, 0), (1, 1), 1)}[i]
    p, q = b(*p).astype(F32), b(*q).astype(F32)
    return (p + q if sign > 0 else p - q).astype(BF16)


_STORED = (0, 2, 3, 5, 6)


def _combine(m):
    return (m[0] + m[3] - m[4] + m[6], m[2] + m[4], m[1] + m[3], m[0] - m[1] + m[2] + m[5])


def _hopcroft_kerr(p):
    own = {0: ((1, 2, 1), (2, 0, 1)), 1: ((2, 1, -1), (0, 2, 1)), 2: ((1, 1, 1), (0, 0, 1))}
    cross = {(0, 1): ((1, 0, 1, 0, 1, -1), (0, -1, 0, -1, 0, 1, -1), (-1, 0, 1, 0, 1, 0, 1)),
             (0, 2): ((2, 0, 1, 2, 1, 1), (-1, 0, 0, -1, 0, 1, -1), (0, -1, -1, 0, -1, 0, 1)),
             (1, 2): ((2, 1, -1, 2, 0, 1), (0, -1, -1, 0, 1, 0, 1), (1, 0, 0, -1, 0, 1, -1))}
    prods, diag, entry = [], {}, {}

    def product(left, out):
        prods.append((left, out))
        return len(prods) - 1

    def diagonal(idx, kind):
        diag[idx] = [product([(i, f, 1) for i in idx], [(i, g, 1) for i in idx]) for f, g, _ in own[kind]]

    def pair(a, ka, b, kb):
        if ka > kb:
            return pair(b, kb, a, ka)[::-1]
        (f0, f1, s, g0, g1, t), ab, ba = cross[ka, kb]
        diagonal(a + b, 3 - ka - kb)
        used = diag[a] + diag[b] + diag[a + b] + [product(
            [(i, f0, 1) for i in a] + [(i, f1, s) for i in b], [(i, g0, 1) for i in a] + [(i, g1, t) for i in b])]
        return dict(zip(used, ab)), dict(zip(used, ba))

    for i in range(p):
        diagonal((i,), i % 3)
        entry[i, i] = {r: sign for r, (_, _, sign) in zip(diag[i,], own[i % 3])}
    for j in range(p):
        for i in range(j):
            if i % 3 != j % 3:
                entry[i, j], entry[j, i] = pair((i,), i % 3, (j,), j % 3)
    for j in range(p):
        for i in range(j % 3, j, 3):
            k = i + 1
            both = (i, k) if (i, k) in diag else (k, i)
            entry[i, j], entry[j, i] = pair(both, 3 - i % 3 - k % 3, (j,), j % 3)
            for ij, kj in (((i, j), (k, j)), ((j, i), (j, k))):
                for r, c in entry[kj].items():
                    entry[ij][r] = entry[ij].get(r, 0) - c
    return [(left, [(i, j, c[r]) for (i, j), c in sorted(entry.items()) if c.get(r)], out)
            for r, (left, out) in enumerate(prods)]

P = 2 * G
_HK = _hopcroft_kerr(P)
_HK_STORED = [r for r, (_, weight, _) in enumerate(_HK) if len(weight) > 1]


def _signed_sum(terms):
    terms = sorted(terms, key=lambda t: -t[0])
    assert terms[0][0] > 0
    total = terms[0][1]
    for sign, value in terms[1:]:
        total = total + value if sign > 0 else total - value
    return total


def _hk_left(top, bot):
    k = top.shape[1] // P
    forms = [(t, b, t - b) for t, b in ((top[:, i * k:(i + 1) * k], bot[:, i * k:(i + 1) * k]) for i in range(P))]
    return [_signed_sum([(sign, forms[i][f]) for i, f, sign in left]) for left, _, _ in _HK]


def _hk_weights(block):
    wide = {(i, j): block(i, j).astype(F32) for i in range(P) for j in range(P)}
    return [_signed_sum([(sign, wide[i, j]) for i, j, sign in _HK[r][1]]) for r in _HK_STORED]


def _hk_matmul(left, block, stored, order, acc):
    acc = dict(acc)
    for r in order:
        _, weight, out = _HK[r]
        if r in _HK_STORED:
            flip, w = 1, stored(_HK_STORED.index(r))
        else:
            flip, w = weight[0][2], block(*weight[0][:2])
        m = _dot(left(r), w)
        for j, f, sign in out:
            if (j, f) in acc:
                acc[j, f] = acc[j, f] + m if sign * flip > 0 else acc[j, f] - m
            else:
                acc[j, f] = m if sign * flip > 0 else -m
    return acc


def _hk_result(acc):
    return ([acc[j, 0] + acc[j, 2] for j in range(P)], [acc[j, 1] + acc[j, 2] for j in range(P)])


def _weave(main, side):
    out, k = [], 0
    for i, task in enumerate(main):
        out.append(task)
        while k < len(side) and (k + 1) * len(main) <= (i + 1) * len(side):
            out.append(side[k])
            k += 1
    return out


def _run(tasks):
    for task in tasks:
        task()


def _finish_tasks(acc, emit):
    def finish(r):
        emit(r, _combine([pltpu.bitcast(ref[r0 + r:r0 + r + RC, c0:c0 + LANE], F32) for ref, r0, c0 in acc]))
    return [functools.partial(finish, r) for r in range(0, TM // 2, RC)]


def _matmul_tasks(lhs, rhs, pairs, next_acc, emit, tail):
    def product(acc, j, i):
        ref, r0, c0 = acc[i]
        ref[r0:r0 + TM // 2, c0:c0 + LANE] = pltpu.bitcast(
            _dot(lhs(i), rhs(j, i)), U32)

    out = []
    for j in range(pairs):
        acc = next_acc()
        out += _weave([functools.partial(product, acc, j, i) for i in (1, 0, 2, 3, 4, 5, 6)], tail)
        tail = _finish_tasks(acc, functools.partial(emit, j))
    return out, tail


def _kernel(x_hbm, mem0_hbm, wq_hbm, wk_hbm, wv_hbm, wo_hbm, w1_hbm, w2_hbm, w3_hbm, w4_hbm,
            out_hbm,
            x_v, part_v, wqkv_v, wo_v, w3_v, w4_v, l3_v, raw_v, mem0_v,
            sem_x, sem_w1, sem_w, sem_a, sem_out, *, seg):
    S, D = x_hbm.shape
    H, Dh = wq_hbm.shape[2], wq_hbm.shape[3]
    M = mem0_hbm.shape[0]
    FF = w3_hbm.shape[1]
    HP = H // 2
    L = M + seg
    R = TM // 2
    n_blk = S // TM
    n_seg = S // seg
    n_grp = HP // G
    assert n_grp == 2 * n_blk
    grows = G * Dh

    class part:
        @staticmethod
        def get(r0, n, c=slice(None)):
            return part_v[_at(r0, n, 8), c]

        @staticmethod
        def set(r0, v, c=slice(None)):
            part_v[_at(r0, v.shape[0], 8), c] = v

    def copy(hbm, vmem, sem, *idx):
        return pltpu.make_async_copy(hbm.bitcast(U32).at[idx], vmem.at[idx], sem)

    slabs = 4 * G

    def attn_copies(g):
        rows = _at(g * grows, grows)
        copies = [copy(wo_hbm, wo_v, sem_a.at[g], rows)]
        base = g % 2 * slabs
        for m, hbm in enumerate((wq_hbm, wk_hbm, wv_hbm)):
            for j in range(G):
                for par in range(2):
                    copies.append(pltpu.make_async_copy(
                        hbm.bitcast(U32).at[:, par, g * G + j, :],
                        raw_v.at[base + m * G + j, :, par * LANE:(par + 1) * LANE], sem_a.at[g]))
        for n in range(4):
            copies.append(pltpu.make_async_copy(
                wo_hbm.bitcast(U32).at[rows, n * D // 4:(n + 1) * D // 4],
                raw_v.at[base + 3 * G + n // 2, (n % 2) * grows:(n % 2 + 1) * grows], sem_a.at[g]))
        return copies

    mem0_copy = pltpu.make_async_copy(mem0_hbm, mem0_v, sem_w.at[3])

    def half_copy(hbm, vmem, n, k):
        rows = vmem.shape[0] // 2
        return copy(hbm, vmem, sem_w.at[n], _at(k * rows, rows))

    def x_rows(r0, n):
        return _bf(x_v[_at(r0 // 2, n // 2), :]).astype(F32)

    def cols(j, c):
        return slice(c * (D // 2) + j * LANE, c * (D // 2) + (j + 1) * LANE)

    def mixing(h_v, w1_v, w2_v, s1_v, s2_v, lhs_v, tmp_v):
        pairs = D // 2 // LANE
        units = TM // UNIT
        n_unit = S // UNIT
        half = UNIT // 2

        def w_copies(n, hbm, vmem, j):
            return [copy(hbm, vmem, sem_w1.at[n, j], slice(None), _at(c * (D // 2) + j * LANE, LANE))
                    for c in range(2)]

        def x_copy(i):
            return copy(x_hbm, x_v, sem_x.at[i], _at(i * R, R))

        def quad(w, j, a, c, r=0, n=D // 4):
            return _bf(w[a * (D // 4) + r:a * (D // 4) + r + n, _at(c * (D // 2) + j * LANE, LANE)])

        def prepare(w, sums, j, r, size):
            for n, i in enumerate(_STORED):
                sums.at[j][r:r + size, n * LANE:(n + 1) * LANE] = pltpu.bitcast(
                    _rhs(i, lambda a, c: quad(w, j, a, c, r, size)), U32)

        marks = []

        def mark(kind, v):
            if kind in MARK:
                marks.append(pltpu.bitcast(jnp.broadcast_to(v, (v.shape[0], LANE))[-8:], U32))
            return v

        def store_lhs(ref, r, rows, size=UNIT):
            k = D // 2
            for q in range(0, size // 2, RC):
                top, bot = rows(q), rows(size // 2 + q)
                for n, v in enumerate(_lhs7(top[:, :k], top[:, k:], bot[:, :k], bot[:, k:])):
                    ref.at[n][(r + q) // 2:(r + q + RC) // 2, :] = w = _words(v)
                    if n in (1, 4):
                        u = pltpu.bitcast(v, U32)
                        u = u[:8] | u[8:] if FULL else u[8:]
                        mark('w', u[:, :LANE] | u[:, LANE:2 * LANE] | u[:, 2 * LANE:3 * LANE] | u[:, 3 * LANE:])

        def norm1(r0, ref, size=UNIT):
            def rows(r):
                x = x_rows(r0 + r, RC)
                xc = x - mark('m', jnp.sum(x, axis=-1, keepdims=True)) * (1.0 / D)
                var = mark('v', jnp.sum(xc * xc, axis=-1, keepdims=True)) * (1.0 / D)
                inv = lax.rsqrt(var + _EPS)
                xn = xc * inv
                part_v[_at(r0 + r, RC), :] = xn
                return xn * lax.rsqrt(var * inv * inv + _EPS)
            store_lhs(ref, 0, rows, size)

        def shift(u, slot):
            def rows(r):
                r0 = u * UNIT + r
                parts = []
                for g, by in enumerate((-1, 1, -2, 2)):
                    c = slice(g * D // 4, (g + 1) * D // 4)
                    if by < 0:
                        parts.append(pltpu.roll(h_v[_at(r0, RC + 8, 8), c], -by, 0)[8:])
                    else:
                        parts.append(pltpu.roll(h_v[_at(r0 + 8, RC + 8, 8), c], RC + 8 - by, 0)[:RC])
                return jnp.concatenate(parts, axis=1)
            store_lhs(lhs_v.at[slot], 0, rows)

        def ln(x):
            xc = x - mark('M', jnp.sum(x, axis=-1, keepdims=True)) * (1.0 / D)
            var = mark('V', jnp.sum(xc * xc, axis=-1, keepdims=True)) * (1.0 / D)
            return xc * lax.rsqrt(var + _EPS)

        def norm3(i, k):
            store_lhs(l3_v.at[i], k * half, lambda r: ln(part_v[_at(i * TM + k * UNIT + r, RC), :]))

        def matmul(w, sums, lhs, emit, arriving=None, never=None):
            todo = list(marks) if never is not None else []
            marks.clear()
            total, pos, late = len(todo), 0, []
            p0, p1 = (P0, P1) if w is w1_v else (Q0, Q1)
            for j in range(pairs):
                if arriving:
                    for c in arriving(j):
                        c.wait()
                prods = [None] * 7
                for n in (1, 0, 2, 3, 4, 5, 6):
                    if n not in _STORED:
                        rhs = quad(w, j, n // 4, n // 4)
                    else:
                        lanes = _at(_STORED.index(n) * LANE, LANE)
                        if arriving:
                            rhs = _rhs(n, functools.partial(quad, w, j))
                            sums.at[j][:, lanes] = pltpu.bitcast(rhs, U32)
                        else:
                            rhs = _bf(sums.at[j][:, lanes])
                    pos += 1
                    while todo and (total - len(todo) + 1) * (p1 - p0) <= (pos - p0) * total:
                        words = pltpu.bitcast(rhs, U32)
                        hint = todo.pop(0)
                        rhs = _bf(jnp.concatenate(sum(
                            ([jnp.where(never, hint, words[k:k + 8]), words[k + 8:k + ALL4]]
                             for k in range(0, D // 4, ALL4)), []), axis=0))
                    while late and late[0][0] <= pos:
                        words = pltpu.bitcast(rhs, U32)
                        rhs = _bf(jnp.concatenate([jnp.where(never, late.pop(0)[1], words[:8]), words[8:]], axis=0))
                    prods[n] = _dot(_bf(lhs.at[n][...]), rhs)
                for q, v in enumerate(_combine(prods)):
                    v = emit((q // 2) * v.shape[0], cols(j, q % 2), v)
                    if 'h' in MARK and never is not None and v is not None:
                        late.append((pos + HD + q, pltpu.bitcast(v[-8:], U32)))

        def emit_h(r0, r, c, v):
            h_v[_at(8 + r0 + r, v.shape[0], 8), c] = v = _gelu(v)
            return v

        def h_body(i, _):
            marks.clear()
            @pl.when(i + 2 < n_blk)
            def _():
                x_copy(i + 2).start()

            @pl.when(i + 1 < n_blk)
            def _():
                x_copy(i + 1).wait()

            for c in w_copies(1, w2_hbm, w2_v, i):
                c.start()
            w3_copy(i).start()
            for c in w_copies(1, w2_hbm, w2_v, i - 1):
                c.wait()
            for k in range(units):
                r0 = i * TM + k * UNIT
                norm1(r0 + UNIT, lhs_v.at[(k + 1) % 2])
                matmul(w1_v, s1_v, lhs_v.at[k % 2], functools.partial(emit_h, r0), never=i < 0)
                prepare(w2_v, s2_v, i - 1, k * (D // 4 // units), D // 4 // units)
            return 0

        def mix_body(i, _):
            marks.clear()
            copy(w4_hbm, w4_v, sem_w.at[2], _at(i * (FF // 2 // n_blk), FF // 2 // n_blk)).start()

            @pl.when(i == 1)
            def _():
                for c in attn_copies(0):
                    c.start()

            for k in range(units):
                u = i * units + k
                shift(jnp.minimum(u + 1, n_unit - 1), (k + 1) % 2)
                norm3(i if k >= NL else jnp.maximum(i - 1, 0), (k - NL) % units)

                def emit(r, c, v):
                    part_v[_at(u * UNIT + r, half), c] += v
                matmul(w2_v, s2_v, lhs_v.at[k % 2], emit, never=i < 0 if MIXP else None)
            return 0

        def w3_copy(i):
            return copy(w3_hbm, w3_v, sem_w.at[1], _at(i * (D // 2 // n_blk), D // 2 // n_blk))

        with jax.named_scope("pro"):
            first = [copy(x_hbm, x_v, sem, _at(k * R // 2, R // 2)) for k, sem in enumerate((sem_w.at[0], sem_x.at[0]))]
            w1_copies = functools.partial(w_copies, 0, w1_hbm, w1_v)
            for c in ([first[0]] + w1_copies(0) + w1_copies(1) + [first[1]] + w1_copies(2) + w1_copies(3)
                      + [x_copy(1)] + w_copies(1, w2_hbm, w2_v, 0) + [x_copy(2), w3_copy(0)]):
                c.start()
            h_v[0:8, :] = jnp.zeros((8, D), F32)
            h_v[S + 8:S + 16, :] = jnp.zeros((8, D), F32)
            x_v[S // 2:, :] = jnp.zeros((UNIT // 2, D), U32)
            first[0].wait()
            norm1(0, tmp_v.at[0], R)
            matmul(w1_v, s1_v, tmp_v.at[0], functools.partial(emit_h, 0),
                   lambda j: w1_copies(j) + [first[1]] * (j == 2))
            norm1(R, tmp_v.at[1], R)
            x_copy(1).wait()
            marks.clear()
            norm1(TM, lhs_v.at[0])
            matmul(w1_v, s1_v, tmp_v.at[1], functools.partial(emit_h, R))
        with jax.named_scope("b1"):
            lax.fori_loop(1, n_blk, h_body, 0)
            shift(0, 0)
            for c in w_copies(1, w2_hbm, w2_v, pairs - 1):
                c.wait()
            for r in range(0, D // 4, WC):
                prepare(w2_v, s2_v, pairs - 1, r, WC)
            lax.fori_loop(0, n_blk, mix_body, 0)
            for k in range(units - NL, units):
                norm3(n_blk - 1, k)

    if SKIP_B1:
        for c in [half_copy(w3_hbm, w3_v, 1, 0), half_copy(w3_hbm, w3_v, 1, 1), half_copy(w4_hbm, w4_v, 2, 0),
                  half_copy(w4_hbm, w4_v, 2, 1)] + attn_copies(0):
            c.start()
    else:
        pl.run_scoped(
            mixing,
            pltpu.VMEM((S + 16, D), F32),
            pltpu.VMEM((D // 2, D), U32),
            pltpu.VMEM((D // 2, D), U32),
            pltpu.VMEM((D // 2 // LANE, D // 4, 5 * LANE), U32),
            pltpu.VMEM((D // 2 // LANE, D // 4, 5 * LANE), U32),
            pltpu.VMEM((2, 7, UNIT // 4, D // 2), U32),
            pltpu.VMEM((2, 7, R // 4, D // 2), U32),
        )
    mem0_copy.start()
    for k in range(2):
        half_copy(w3_hbm, w3_v, 1, k).wait()
        half_copy(w4_hbm, w4_v, 2, k).wait()

    def channel_mlp(sums_v, u_v, acc_v, lead_v):
        up_pairs, down_pairs = FF // 4 // LANE, D // 2 // LANE

        def acc(slot):
            if SEP:
                return [(acc_v.at[n], 0, 0) for n in range(7 * slot, 7 * slot + 7)]
            return [(raw_v.at[2 * slabs + n // 4], (n % 2) * R, (n // 2 % 2) * LANE) for n in range(7 * slot, 7 * slot + 7)]

        pending, ready = [], []

        def paced(it, words, ok):
            if pending or ready:
                hint = functools.reduce(jnp.bitwise_or, [ref[(it // n_grp,) + (slice(0, 8), slice(0, LANE))]
                                                         for ref in pending] + ready)
                words = jnp.concatenate([jnp.where(it < 0, hint, words[:8]), words[8:]], axis=0)
                pending.clear()
                ready.clear()
            return _bf(words)

        def attn_weight_tasks(g):
            def store(slab, r, block, direct=DIRECT):
                for n, v in enumerate(_hk_weights(block)):
                    sums_v.at[slab][r:r + AC, n * LANE:(n + 1) * LANE] = w = _words(v)
                    if n in REG and direct:
                        ready.append(w)
                if FEN and not direct:
                    pending.extend(ref for ref in ((), (wqkv_v,), (sums_v,), (sums_v, wqkv_v))[FEN] if not any(ref is q for q in pending))

            def qkv(m, r):
                blocks = {}
                for j in range(G):
                    src = raw_v.at[g % 2 * slabs + m * G + j]
                    for i in range(P):
                        rr = i * (D // 2 // P) + r
                        a, b = src[rr:rr + AC, :LANE], src[rr:rr + AC, LANE:]
                        for n, w in enumerate(((a & jnp.uint32(0xFFFF)) | (b << 16),
                                               (a >> 16) | (b & jnp.uint32(0xFFFF0000)))):
                            wqkv_v[m * H + g * P + 2 * j + n, rr:rr + AC, :] = w
                            blocks[i, 2 * j + n] = _bf(w)
                store(m * n_grp + g, r, lambda i, j: blocks[i, j])

            def out(r):
                def block(i, j):
                    r0, c0 = (j % 2) * grows + i * (Dh // 2) + r % (Dh // 2), r // (Dh // 2) * LANE
                    return _bf(raw_v.at[g % 2 * slabs + 3 * G + j // 2][r0:r0 + AC, c0:c0 + LANE])
                store(3 * n_grp + g, r, block, True)

            return ([functools.partial(qkv, m, r) for m in range(3) for r in range(0, D // 2 // P, AC)]
                    + [functools.partial(out, r) for r in range(0, D // 2 // P, AC)])

        def emit_up(j, r, quads):
            for n, v in enumerate(_lhs7(*[_gelu(q) for q in quads])):
                u_v.at[n][r // 2:(r + RC) // 2, j * LANE:(j + 1) * LANE] = w = _words(v)
                if n in PU and j + 1 < up_pairs:
                    ready.append(w)

        def emit_down(i, j, r, quads):
            for q, v in enumerate(quads):
                r0 = i * TM + r // (UNIT // 2) * UNIT + (q // 2) * (UNIT // 2) + r % (UNIT // 2)
                part_v[_at(r0, RC), cols(j, q % 2)] += v

        def last_epilogue(i):
            return _finish_tasks(acc(2), functools.partial(emit_down, i, down_pairs - 1))

        for ref, r0, c0 in acc(2):
            ref[r0:r0 + R, c0:c0 + LANE] = jnp.zeros((R, LANE), U32)

        def w3_quad(f, j, a, c):
            return w3_v[a * (D // 4):(a + 1) * (D // 4), _at(c * (FF // 2) + f * (FF // 4) + j * LANE, LANE)]

        for f in range(2 * LEAD):
            for k, n in enumerate(_STORED):
                lead_v.at[f][:, k * LANE:(k + 1) * LANE] = pltpu.bitcast(
                    _rhs(n, lambda a, c: _bf(w3_quad(f, 0, a, c))), U32)

        def body(it, _):
            i, f = it // 2, it % 2

            @pl.when(it + 1 < n_grp)
            def _():
                for c in attn_copies(it + 1):
                    c.start()

            for c in attn_copies(it):
                c.wait()
            slots = [n % 2 for n in range(up_pairs + down_pairs - 1)] + [2]
            next_acc = lambda: acc(slots.pop(0))

            def up_rhs(j, n):
                if LEAD and j == 0 and n in _STORED:
                    return paced(it, lead_v.at[f][:, _at(_STORED.index(n) * LANE, LANE)], True)
                return _rhs(n, lambda a, c: paced(it, w3_quad(f, j, a, c), True))

            up, tail = _matmul_tasks(
                lambda n: _bf(l3_v.at[i, n][...]),
                up_rhs,
                up_pairs, next_acc, emit_up, last_epilogue(jnp.maximum(it - 1, 0) // 2) if CARRY else [])
            down, end = _matmul_tasks(
                lambda n: _bf(u_v.at[n][...]),
                lambda j, n: _rhs(n, lambda a, c: paced(it,
                    w4_v[_at(a * (FF // 4) + f * (FF // 8), FF // 8, 64), cols(j, c)], n in _STORED)),
                down_pairs, next_acc, functools.partial(emit_down, i), [])
            side = attn_weight_tasks(it)
            cut = int(len(side) * CUT)
            _run(up[:HEAD] + _weave(up[HEAD:], side[:cut]) + tail + _weave(down[:len(down) - FOOT], side[cut:]) + down[len(down) - FOOT:] + ([] if CARRY else end))
            return 0

        with jax.named_scope("b2"):
            lax.fori_loop(0, n_grp, body, 0)
            if CARRY:
                _run(last_epilogue(n_blk - 1))

    def recurrence(sums_v, own_v, lhs_v, next_v, hq_v, ho_v):
        scale = float(Dh) ** -0.5
        own = seg - 8
        row = lax.broadcasted_iota(jnp.int32, (2 * L, LANE if WIDE else 2 * L), 0)
        col = lax.broadcasted_iota(jnp.int32, (2 * L, LANE if WIDE else 2 * L), 1)
        r_in = jnp.where(row >= L, row - L, row)
        c_in = jnp.where(col >= L, col - L, col)
        same_head = ((row >= L) == (col >= L)) & (col < 2 * L)
        keep = same_head & ((r_in < M) | (r_in >= c_in))
        fill = jnp.where(same_head, _NEG / scale, -jnp.inf).astype(F32)

        def load_own(s):
            own_v[...] = _ln(x_rows(s * seg, seg)[:own])

        def load_held(s, q):
            next_v[8 * q:8 * q + 8, :] = _ln(x_rows(s * seg + seg - 16, 16)[8:])

        def load_lhs(mem):
            for n, v in enumerate(_hk_left(jnp.concatenate([mem, own_v[...]], axis=0), next_v[...])):
                lhs_v[:, n * (D // P):(n + 1) * (D // P)] = _words(v)

        def by_head(split, dot, a, b):
            return jnp.concatenate([dot(a[:L], b), dot(a[L:], b)], axis=0) if split else dot(a, b)

        def scores(split, q, k):
            s = jnp.where(keep, by_head(split, _dot_nt, q, widen(k)), fill)
            e = jnp.exp2((s - jnp.max(s, axis=-1, keepdims=True)) * (scale * _LOG2E))
            total = jnp.sum(e, axis=-1, keepdims=True)
            return e, pl.reciprocal(total, full_range=False) if RCP else 1.0 / total

        def widen(x):
            return (jnp.concatenate([x, x[:LANE - 2 * L]], axis=0) if WIDE else x).astype(BF16)

        def step(s, r, mem):
            first = isinstance(r, int) and r == 0
            last = isinstance(r, int) and r == PERIOD - 1
            top = None if first else jnp.concatenate([mem, own_v[...]], axis=0)
            early = {} if first else {
                h: _dot(top[:, :D // 2].astype(BF16), _bf(wqkv_v[h, :D // 4, :])) for h in (0, 1, H, H + 1, 2 * H)[:SPLIT]}

            ready = []

            def paced(words):
                if ready:
                    n = -(-len(ready) // SPREAD)
                    hint = functools.reduce(jnp.bitwise_or, ready[:n])
                    del ready[:n]
                    words = jnp.concatenate([jnp.where(s < 0, hint, words[:8]), words[8:]], axis=0)
                return _bf(words)

            def plain(h):
                if h in early:
                    return early[h] + _dot(top[:, D // 2:].astype(BF16), _bf(wqkv_v[h, D // 4:, :]))
                return _dot(top.astype(BF16), paced(wqkv_v[h]))

            def project(g):
                res = []
                for m in range(3):
                    h0, k = m * H + g * P, D // 2 // P
                    if first:
                        tops, bots = _hk_result(_hk_matmul(
                            lambda n: _bf(lhs_v[:, n * (D // P):(n + 1) * (D // P)]),
                            lambda i, j: _bf(wqkv_v[h0 + j, i * k:(i + 1) * k, :]),
                            lambda n: _bf(sums_v.at[m * n_grp + g][:, n * LANE:(n + 1) * LANE]),
                            range(len(_HK)), {}))
                        for j in range(P):
                            hq_v[h0 + j] = bots[j][8:]
                        held = [b[:8] for b in bots]
                    else:
                        tops = [plain(h0 + j) for j in range(P)]
                        held = [hq_v[h0 + j, 8 * (r - 1):8 * r, :] for j in range(P)]
                    res.append([jnp.concatenate([tops[j], held[j], tops[j + 1], held[j + 1]], axis=0)
                                for j in range(0, P, 2)])
                return list(zip(*res))

            def merge(g, heads, acc):
                tops = jnp.concatenate([o[:L - 8] for o in heads], axis=1)
                held = jnp.concatenate([o[L - 8:] for o in heads], axis=1)
                lanes = slice(g * P * Dh, (g + 1) * P * Dh)
                if last and g >= HKG:
                    both = jnp.concatenate([tops, jnp.concatenate([ho_v[:, lanes], held], axis=0)], axis=0)
                    y = _dot(both.astype(BF16), _bf(wo_v[g * grows:(g + 1) * grows, :]))
                    n = D // P
                    return {(j, f): v + y[32 * f:32 * f + 32, j * n:(j + 1) * n] if f < 2 else v
                            for (j, f), v in acc.items()}
                if last:
                    left = _hk_left(tops, jnp.concatenate([ho_v[:, lanes], held], axis=0))
                    k, n = Dh // 2, D // P
                    return _hk_matmul(
                        lambda q: left[q].astype(BF16),
                        lambda i, j: _bf(wo_v[g * grows + i * k:g * grows + (i + 1) * k, j * n:(j + 1) * n]),
                        lambda q: jnp.concatenate(
                            [paced(sums_v.at[3 * n_grp + g][c * k:(c + 1) * k, q * LANE:(q + 1) * LANE])
                             for c in range(n // LANE)], axis=1),
                        sorted(range(len(_HK)), key=lambda q: all(f == 1 for _, f, _ in _HK[q][2])), acc or {})
                ho_v[8 * r:8 * r + 8, lanes] = held
                y = _dot(tops.astype(BF16), _bf(wo_v[g * grows:(g + 1) * grows, :]))
                return y if acc is None else acc + y

            qkv, prob, heads = {}, {}, {}
            acc, done = None, 0
            for t in range(n_grp + 3):
                if t < n_grp:
                    qkv[t] = project(t)
                lag, up0, up1 = LL if last else LF if first else (LAG, UP0, UP1)
                upto = {n_grp: up0, n_grp + 1: up1, n_grp + 2: n_grp}.get(t, t - lag + 1)
                while done < upto:
                    acc = merge(done, heads.pop(done), acc)
                    done += 1
                    if last and HA and done < n_grp:
                        for v in acc.values():
                            v = pltpu.bitcast(v, U32)
                            ready.extend(v[i:i + 8, c:c + LANE] for i in range(0, 32, 32 // HA)
                                         for c in range(0, v.shape[1], LANE))
                if 0 <= t - 2 < n_grp:
                    heads[t - 2] = []
                    for (e, inv), (_, _, v) in zip(prob.pop(t - 2), qkv.pop(t - 2)):
                        split = S1 and t - 2 in P1T or ALLSPLIT
                        if PRE:
                            o = by_head(split, _dot, e * inv, widen(v))
                        else:
                            o = by_head(split, _dot, e, widen(v)) * inv
                        heads[t - 2] += [o[:L], o[L:]]
                if 0 <= t - 1 < n_grp:
                    prob[t - 1] = [scores(S1 and t in S1T or ALLSPLIT, q, k) for q, k, _ in qkv[t - 1]]
                if last and 1 <= t <= PERIOD:
                    load_held(jnp.minimum(s + t, n_seg - 1), t - 1)
                if t == n_grp - 1:
                    load_own(jnp.minimum(s + 1, n_seg - 1))
            if last:
                y, y_held = [jnp.concatenate(half, axis=1) for half in _hk_result(acc)]
                load_lhs(y[:M])
            else:
                y = acc
            base = x_rows(s * seg, seg) + part.get(s * seg, seg)
            x_v[_at(s * (seg // 2), 8), :] = _words(base[:16] + y[M:M + 16])
            part.set(s * seg + 16, jnp.concatenate([base[16:24] + y[M + 16:], base[24:]], axis=0))
            if last:
                for q in range(PERIOD):
                    r0 = (s - (PERIOD - 1) + q) * seg + 16
                    rest = part.get(r0, 16)
                    x_v[_at(r0 // 2, 8), :] = _words(jnp.concatenate(
                        [rest[:8], rest[8:] + y_held[8 * q:8 * q + 8]], axis=0))
            return y[:M]

        def period(p, _):
            s = p * PERIOD
            mem = step(s, 0, None)
            if UNROLL:
                for r in range(1, PERIOD - 1):
                    mem = step(s + r, r, mem)
            else:
                mem = lax.fori_loop(1, PERIOD - 1, lambda r, mem: step(s + r, r, mem), mem)
            mem = step(s + PERIOD - 1, PERIOD - 1, mem)
            rows = _at(s * (seg // 2), PERIOD * seg // 2)
            pltpu.make_async_copy(x_v.at[rows], out_hbm.bitcast(U32).at[rows], sem_out).start()
            return 0

        load_own(0)
        for q in range(PERIOD):
            load_held(q, q)
        mem0_copy.wait()
        load_lhs(mem0_v[...].astype(F32))
        with jax.named_scope("aloop"):
            lax.fori_loop(0, n_seg // PERIOD, period, 0)

    def rest(sums_v):
        if not SKIP_B2:
            pl.run_scoped(functools.partial(channel_mlp, sums_v), pltpu.VMEM((7, R // 2, FF // 4), U32), pltpu.VMEM((21, R, LANE), U32),
                          pltpu.VMEM((2, D // 4, 5 * LANE), U32))
        if SKIP_A:
            x_v[0:8, :] = jnp.concatenate([sums_v[5, 0:8, 0:512]] * 2, axis=1) + l3_v[pl.semaphore_read(sem_out), 3, 0:8, 0:1] + wqkv_v[7, 0:8, 0:1]
            pltpu.make_async_copy(x_v.at[0:S // 2], out_hbm.bitcast(U32), sem_out).start()
            return
        pl.run_scoped(
            functools.partial(recurrence, sums_v),
            pltpu.VMEM((seg - 8, D), F32),
            pltpu.VMEM(((L - 8) // 2, len(_HK) * D // P), U32),
            pltpu.VMEM((8 * PERIOD, D), F32),
            pltpu.VMEM((3 * H, 8 * (PERIOD - 1), Dh), F32),
            pltpu.VMEM((8 * (PERIOD - 1), H * Dh), F32),
        )

    pl.run_scoped(rest, pltpu.VMEM((4 * n_grp, D // 2 // P, len(_HK_STORED) * LANE), U32))
    pltpu.make_async_copy(x_v.at[0:S // 2], out_hbm.bitcast(U32), sem_out).wait()


@functools.partial(jax.jit, static_argnames=("A_seg_len",))
def pallas_parallel_sum__memory_aug_recurrent_mem_tr__mixer_s_mlp__prompt_kernel(
    A_x: jax.Array,
    A_mem0: jax.Array,
    A_Wq: jax.Array,
    A_Wk: jax.Array,
    A_Wv: jax.Array,
    A_Wo: jax.Array,
    A_seg_len: int,
    B_x: jax.Array,
    B_w1: jax.Array,
    B_w2: jax.Array,
    B_w3: jax.Array,
    B_w4: jax.Array,
):
    del B_x
    B, S, D = A_x.shape
    H, Dh = A_Wq.shape[1], A_Wq.shape[2]
    M = A_mem0.shape[1]
    FF = B_w3.shape[1]
    assert (B, M, A_seg_len) == (1, 8, 32)
    n_blk = S // TM

    hbm = pl.BlockSpec(memory_space=pl.ANY)
    out = pl.pallas_call(
        functools.partial(_kernel, seg=A_seg_len),
        out_shape=jax.ShapeDtypeStruct((S, D), A_x.dtype),
        in_specs=[hbm] * 10,
        out_specs=hbm,
        scratch_shapes=[
            pltpu.VMEM(((S + UNIT) // 2, D), U32), pltpu.VMEM((S + UNIT, D), F32),
            pltpu.VMEM((3 * H, D // 2, Dh), U32),
            pltpu.VMEM((H * Dh // 2, D), U32),
            pltpu.VMEM((D // 2, FF), U32),
            pltpu.VMEM((FF // 2, D), U32),
            pltpu.VMEM((n_blk, 7, TM // 4, D // 2), U32),
            pltpu.VMEM((8 * G, D // 2, 2 * LANE), U32),
            pltpu.VMEM((M, D), A_mem0.dtype),
            pltpu.SemaphoreType.DMA((n_blk,)),
            pltpu.SemaphoreType.DMA((2, D // 2 // LANE)),
            pltpu.SemaphoreType.DMA((4,)),
            pltpu.SemaphoreType.DMA((2 * n_blk,)),
            pltpu.SemaphoreType.DMA,
        ],
        compiler_params=pltpu.CompilerParams(
            vmem_limit_bytes=126 * 1024 * 1024, disable_bounds_checks=True, flags=FLAGS),
    )(A_x.reshape(S, D), A_mem0.reshape(M, D),
      A_Wq.reshape(D // 2, 2, H, Dh), A_Wk.reshape(D // 2, 2, H, Dh), A_Wv.reshape(D // 2, 2, H, Dh),
      A_Wo.reshape(H * Dh, D), B_w1, B_w2, B_w3, B_w4)
    return out.reshape(B, S, D)
```

```python
import functools

import jax
import jax.numpy as jnp
import numpy as np
from jax import lax
import jax.experimental.pallas as pl
import jax.experimental.pallas.tpu as pltpu

F32 = jnp.float32
BF16 = jnp.bfloat16
U32 = jnp.uint32

_EPS = 1e-5
_NEG = -1e9
_LOG2E = float(np.log2(np.e))
_GELU_C = float(np.sqrt(2.0 / np.pi))

LANE = 128
TM = 512
UNIT = 64
UNIT2 = 128
RC = 16
P = 4
PERIOD = 4
SKIP_B1 = False
SKIP_B2 = False
SKIP_A = False
P0, P1, Q0, Q1, R0, R1 = 0, 1.0, 0.18, 1.0, 0.02, 1.0
O4 = (18, 15, 9, 1, 16, 7, 19, 3, 10, 5, 24, 6, 14, 21, 2, 12, 0, 22, 25, 4, 13, 8, 20, 23, 11, 17)
O5 = (5, 18, 16, 9, 3, 15, 1, 24, 7, 19, 10, 0, 13, 14, 2, 22, 21, 12, 6, 20, 25, 23, 17, 4, 11, 8)
ORD = O5
LO = True
GM = ()
OPQ = False
TIGHT = False
G0, G1 = 20, 40
NSEL = 4


def _dot(a, b):
    return lax.dot_general(a, b, (((1,), (0,)), ((), ())), preferred_element_type=F32)


def _dot_nt(a, b):
    return lax.dot_general(a, b, (((1,), (1,)), ((), ())), preferred_element_type=F32)


def _bf(words):
    return pltpu.bitcast(words, BF16)


def _words(x):
    return pltpu.bitcast(x.astype(BF16), U32)


def _at(start, n, align=None):
    return pl.ds(start if isinstance(start, int) else pl.multiple_of(start, align or n), n)


def _tile(j):
    return _at(j * LANE, LANE)


def _moments(x, note=lambda v: v):
    inv_n = 1.0 / x.shape[-1]
    xc = x - note(jnp.sum(x, axis=-1, keepdims=True)) * inv_n
    return xc, note(jnp.sum(xc * xc, axis=-1, keepdims=True)) * inv_n


def _ln(x, note=lambda v: v):
    xc, var = _moments(x, note)
    return xc * lax.rsqrt(var + _EPS)


def _gelu(x):
    inner = x * (_GELU_C + (_GELU_C * 0.044715) * (x * x))
    hx = 0.5 * x
    return hx + hx * jnp.tanh(inner)


def _signed_sum(terms):
    terms = sorted(terms, key=lambda t: -t[0])
    assert terms[0][0] > 0
    total = terms[0][1]
    for sign, value in terms[1:]:
        total = total + value if sign > 0 else total - value
    return total


class _HopcroftKerr:
    def __init__(self, p):
        own = {0: ((1, 2, 1), (2, 0, 1)), 1: ((2, 1, -1), (0, 2, 1)), 2: ((1, 1, 1), (0, 0, 1))}
        cross = {(0, 1): ((1, 0, 1, 0, 1, -1), (0, -1, 0, -1, 0, 1, -1), (-1, 0, 1, 0, 1, 0, 1)),
                 (0, 2): ((2, 0, 1, 2, 1, 1), (-1, 0, 0, -1, 0, 1, -1), (0, -1, -1, 0, -1, 0, 1)),
                 (1, 2): ((2, 1, -1, 2, 0, 1), (0, -1, -1, 0, 1, 0, 1), (1, 0, 0, -1, 0, 1, -1))}
        products, diag, uses = [], {}, {}

        def product(left, out):
            products.append((left, out))
            return len(products) - 1

        def diagonal(idx, kind):
            diag[idx] = [product([(i, f, 1) for i in idx], [(i, g, 1) for i in idx]) for f, g, _ in own[kind]]

        def pair(a, ka, b, kb):
            if ka > kb:
                return pair(b, kb, a, ka)[::-1]
            (f0, f1, s, g0, g1, t), ab, ba = cross[ka, kb]
            diagonal(a + b, 3 - ka - kb)
            used = diag[a] + diag[b] + diag[a + b] + [product(
                [(i, f0, 1) for i in a] + [(i, f1, s) for i in b],
                [(i, g0, 1) for i in a] + [(i, g1, t) for i in b])]
            return dict(zip(used, ab)), dict(zip(used, ba))

        for i in range(p):
            diagonal((i,), i % 3)
            uses[i, i] = {r: sign for r, (_, _, sign) in zip(diag[i,], own[i % 3])}
        for j in range(p):
            for i in range(j):
                if i % 3 != j % 3:
                    uses[i, j], uses[j, i] = pair((i,), i % 3, (j,), j % 3)
        for j in range(p):
            for i in range(j % 3, j, 3):
                k = i + 1
                both = (i, k) if (i, k) in diag else (k, i)
                uses[i, j], uses[j, i] = pair(both, 3 - i % 3 - k % 3, (j,), j % 3)
                for ij, kj in (((i, j), (k, j)), ((j, i), (j, k))):
                    for r, c in uses[kj].items():
                        uses[ij][r] = uses[ij].get(r, 0) - c
        self.p = p
        self.products = [(left, [(i, j, c[r]) for (i, j), c in sorted(uses.items()) if c.get(r)], out)
                         for r, (left, out) in enumerate(products)]
        self.summed = [r for r, (_, weight, _) in enumerate(self.products) if len(weight) > 1]

    def left(self, upper, lower):
        forms = [(u, l, u - l) for u, l in zip(upper, lower)]
        return [_signed_sum([(sign, forms[i][f]) for i, f, sign in left]) for left, _, _ in self.products]

    def right(self, n, block):
        return _signed_sum([(sign, block(i, j).astype(F32)) for i, j, sign in self.products[self.summed[n]][1]])

    def accumulate(self, left, block, summed, acc=(), order=None):
        acc = dict(acc)
        for r in order or (ORD if self.p == 4 and ORD else range(len(self.products))):
            _, weight, out = self.products[r]
            if r in self.summed:
                flip, w = 1, summed(self.summed.index(r))
            else:
                flip, w = weight[0][2], block(*weight[0][:2])
            m = _dot(left(r), w)
            for j, f, sign in out:
                if (j, f) in acc:
                    acc[j, f] = acc[j, f] + m if sign * flip > 0 else acc[j, f] - m
                else:
                    acc[j, f] = m if sign * flip > 0 else -m
        return acc

    def result(self, acc):
        return [[functools.reduce(jnp.add, [acc[j, g] for g in (f, 2) if (j, g) in acc])
                 for j in range(self.p)] for f in range(2)]


_HK = _HopcroftKerr(P)
_HK2 = _HopcroftKerr(2)


def _split(x, n):
    k = x.shape[1] // n
    return [x[:, i * k:(i + 1) * k] for i in range(n)]


class _Pace:
    def __init__(self, never):
        self.never, self.noted, self.due, self.pos = never, [], [], 0

    def note(self, v):
        u = pltpu.bitcast(jnp.broadcast_to(v, (v.shape[0], max(v.shape[1], LANE))), U32)
        self.noted.append(functools.reduce(jnp.bitwise_or, [
            u[r:r + 8, c:c + LANE] for r in range(0, u.shape[0], 8) for c in range(0, u.shape[1], LANE)]))
        return v

    def spread(self, first, last):
        n = len(self.noted)
        self.due += [(self.pos + first + (k + 1) * (last - first) / n, v) for k, v in enumerate(self.noted)]
        self.due.sort(key=lambda t: t[0])
        self.noted = []

    def load(self, words):
        self.pos += 1
        hints = []
        while self.due and self.due[0][0] <= self.pos:
            hints.append(self.due.pop(0)[1])
        if hints:
            hint, parts = functools.reduce(jnp.bitwise_or, hints), []
            step = 64 if NSEL > 1 else words.shape[0]
            for k in range(0, words.shape[0], step):
                parts += [jnp.where(self.never, hint, words[k:k + 8]), words[k + 8:k + step]]
            words = jnp.concatenate(parts, axis=0)
        return _bf(words)


def _kernel(x_hbm, mem0_hbm, wq_hbm, wk_hbm, wv_hbm, wo_hbm, w1_hbm, w2_hbm, w3_hbm, w4_hbm,
            out_hbm,
            x_v, part_v, mem0_v, wqkv_v, wo_v, raw_v, w3_v, w4_v, s3_v, s4_v,
            sem_x, sem_mix, sem_mlp, sem_attn, sem_mem, sem_out, *, seg):
    S, D = x_hbm.shape
    H, Dh = wq_hbm.shape[2], wq_hbm.shape[3]
    M = mem0_hbm.shape[0]
    FF = w3_hbm.shape[1]
    L = M + seg
    n_blk = S // TM
    n_seg = S // seg
    n_grp = H // P
    kw = D // 2 // P
    fw = FF // 2 // P
    ft = FF // P // LANE
    dt = D // P // LANE
    grows = P * Dh // 2

    def copy(hbm, vmem, sem, *idx):
        return pltpu.make_async_copy(hbm.bitcast(U32).at[idx], vmem.at[idx], sem)

    def attn_copies(g):
        rows = _at(g * grows, grows)
        copies = [copy(wo_hbm, wo_v, sem_attn.at[g], rows)]
        for m, hbm in enumerate((wq_hbm, wk_hbm, wv_hbm)):
            for j in range(P // 2):
                for par in range(2):
                    copies.append(pltpu.make_async_copy(
                        hbm.bitcast(U32).at[:, par, g * (P // 2) + j, :],
                        raw_v.at[g % 2, m * (P // 2) + j, :, _tile(par)], sem_attn.at[g]))
        return copies

    def mlp_copies(q):
        return [copy(hbm, vmem, sem_mlp.at[q], _at(i * n + q * (n // n_blk), n // n_blk, 8))
                for hbm, vmem, n in ((w3_hbm, w3_v, kw), (w4_hbm, w4_v, fw)) for i in range(P)]

    mem0_copy = pltpu.make_async_copy(mem0_hbm, mem0_v, sem_mem)

    def x_rows(r0, n):
        return _bf(x_v[_at(r0 // 2, n // 2), :]).astype(F32)

    def store_left(hk, ref, rows, size, note):
        for q in range(0, size // 2, RC):
            for n, v in enumerate(hk.left(_split(rows(q), hk.p), _split(rows(size // 2 + q), hk.p))):
                ref.at[n][q // 2:(q + RC) // 2, :] = _words(v)
                if n in (len(hk.products) - 1, len(hk.products) - 2):
                    note(v)

    def store_right(hk, ref, rows, block):
        for n in range(len(hk.summed)):
            v = hk.right(n, block)
            ref[rows, _tile(n)] = _words(v)
            if n == 0:
                first = v
        return first

    def mixing(h_v, w_v, sums_v, left_v, first_v):
        pairs = D // 2 // LANE
        units = TM // UNIT
        loads = pairs * len(_HK2.products)

        def w_copies(n, j):
            return [copy((w1_hbm, w2_hbm)[n], w_v.at[n], sem_mix.at[n, j], slice(None), _tile(c * pairs + j))
                    for c in range(2)]

        def x_copy(i):
            return copy(x_hbm, x_v, sem_x.at[i + 1], _at(i * (TM // 2), TM // 2))

        def block(n, j, r=0, size=D // 4):
            return lambda a, c: w_v.at[n][a * (D // 4) + r:a * (D // 4) + r + size, _tile(c * pairs + j)]

        def prepare(j, r, size):
            store_right(_HK2, sums_v.at[1, j], slice(r, r + size), lambda a, c: _bf(block(1, j, r, size)(a, c)))

        def norm(r0, ref, size, note=lambda v: v):
            def rows(r):
                xc, var = _moments(x_rows(r0 + r, RC), note)
                inv = lax.rsqrt(var + _EPS)
                xn = xc * inv
                part_v[_at(r0 + r, RC), :] = xn
                return xn * lax.rsqrt(var * inv * inv + _EPS)
            store_left(_HK2, ref, rows, size, note)

        def shift(r0, ref, note=lambda v: v):
            def rows(r):
                parts = []
                for g, by in enumerate((-1, 1, -2, 2)):
                    c = slice(g * D // 4, (g + 1) * D // 4)
                    if by < 0:
                        parts.append(pltpu.roll(h_v[_at(r0 + r, RC + 8, 8), c], -by, 0)[8:])
                    else:
                        parts.append(pltpu.roll(h_v[_at(r0 + r + 8, RC + 8, 8), c], RC + 8 - by, 0)[:RC])
                return jnp.concatenate(parts, axis=1)
            store_left(_HK2, ref, rows, UNIT, note)

        def matmul(n, left, r0, load=_bf, arriving=None):
            for j in range(pairs):
                def summed(k):
                    if not arriving:
                        return load(sums_v.at[n, j][:, _tile(k)])
                    w = _HK2.right(k, lambda a, c: _bf(block(n, j)(a, c))).astype(BF16)
                    sums_v.at[n, j][:, _tile(k)] = pltpu.bitcast(w, U32)
                    return w

                for c in arriving(j) if arriving else ():
                    c.wait()
                halves = _HK2.result(_HK2.accumulate(
                    lambda r: _bf(left.at[r][...]), lambda a, c: load(block(n, j)(a, c)), summed))
                for f, half in enumerate(halves):
                    for c, v in enumerate(half):
                        size, lanes = v.shape[0], _tile(c * pairs + j)
                        if n == 0:
                            h_v[_at(8 + r0 + f * size, size, 8), lanes] = _gelu(v)
                        else:
                            part_v[_at(r0 + f * size, size), lanes] += v

        def h_body(i, _):
            @pl.when(i + 2 < n_blk)
            def _():
                x_copy(i + 2).start()

            @pl.when(i + 1 < n_blk)
            def _():
                x_copy(i + 1).wait()

            for c in w_copies(1, i) + mlp_copies(i - 1):
                c.start()
            for c in w_copies(1, i - 1):
                c.wait()
            pace = _Pace(i < 0)
            for k in range(units):
                r0 = i * TM + k * UNIT
                norm(r0 + UNIT, left_v.at[(k + 1) % 2], UNIT, pace.note)
                pace.spread(P0 * loads, P1 * loads)
                matmul(0, left_v.at[k % 2], r0, pace.load)
                prepare(i - 1, k * (D // 4 // units), D // 4 // units)
            return 0

        def mix_body(i, _):
            @pl.when(i == 0)
            def _():
                for c in mlp_copies(n_blk - 1):
                    c.start()

            @pl.when(i == 1)
            def _():
                for c in attn_copies(0):
                    c.start()

            for c in mlp_copies(i):
                c.wait()

            def up(n, r):
                rows = _at(i * (kw // n_blk) + r, 8)
                return store_right(_HK, s3_v.at[n], rows, lambda a, c: _bf(
                    w3_v[_at(a * kw + i * (kw // n_blk) + r, 8), _tile(c * ft + n)]))

            def down(n, r):
                rows = _at(i * (fw // n_blk) + r, 8)
                return store_right(_HK, s4_v.at[n], rows, lambda a, c: _bf(
                    w4_v[_at(a * fw + i * (fw // n_blk) + r, 8), _tile(c * dt + n)]))

            side = ([functools.partial(up, n, r) for n in range(ft) for r in range(0, kw // n_blk, 8)]
                    + [functools.partial(down, n, r) for n in range(dt) for r in range(0, fw // n_blk, 8)])
            pace = _Pace(i < 0)
            for k in range(units):
                r0 = i * TM + k * UNIT
                for task in side[k * len(side) // units:(k + 1) * len(side) // units]:
                    pace.note(task())
                pace.spread(Q0 * loads, Q1 * loads)
                shift(jnp.minimum(r0 + UNIT, S - UNIT), left_v.at[(k + 1) % 2], pace.note)
                pace.spread(Q0 * loads, Q1 * loads)
                matmul(1, left_v.at[k % 2], r0, pace.load)
            return 0

        with jax.named_scope("pro"):
            first = [copy(x_hbm, x_v, sem_x.at[k], _at(k * TM // 4, TM // 4)) for k in range(2)]
            for c in ([first[0]] + w_copies(0, 0) + w_copies(0, 1) + [first[1]] + w_copies(0, 2) + w_copies(0, 3)
                      + [x_copy(1)] + w_copies(1, 0) + [x_copy(2), mem0_copy]):
                c.start()
            h_v[0:8, :] = jnp.zeros((8, D), F32)
            h_v[S + 8:S + 16, :] = jnp.zeros((8, D), F32)
            x_v[S // 2:, :] = jnp.zeros((UNIT // 2, D), U32)
            first[0].wait()
            norm(0, first_v.at[0], TM // 2)
            matmul(0, first_v.at[0], 0, arriving=lambda j: w_copies(0, j) + [first[1]] * (j == 2))
            norm(TM // 2, first_v.at[1], TM // 2)
            x_copy(1).wait()
            norm(TM, left_v.at[0], UNIT)
            matmul(0, first_v.at[1], TM // 2)
        with jax.named_scope("b1"):
            lax.fori_loop(1, n_blk, h_body, 0)
            shift(0, left_v.at[0])
            for c in w_copies(1, pairs - 1):
                c.wait()
            for r in range(0, D // 4, 32):
                prepare(pairs - 1, r, 32)
            lax.fori_loop(0, n_blk, mix_body, 0)

    if SKIP_B1:
        for c in sum([mlp_copies(q) for q in range(4)], []) + attn_copies(0) + [mem0_copy]:
            c.start()
        for c in sum([mlp_copies(q) for q in range(4)], []):
            c.wait()
    else:
        pl.run_scoped(
            mixing,
            pltpu.VMEM((S + 16, D), F32),
            pltpu.VMEM((2, D // 2, D), U32),
            pltpu.VMEM((2, D // 2 // LANE, D // 4, len(_HK2.summed) * LANE), U32),
            pltpu.VMEM((2, len(_HK2.products), UNIT // 4, D // 2), U32),
            pltpu.VMEM((2, len(_HK2.products), TM // 8, D // 2), U32),
        )

    def channel_mlp(sums_v, *buffers):
        left_v, hidden_v = buffers[:2], buffers[2:]
        units = S // UNIT2 // n_grp
        n_prod = len(_HK.products)

        def norm(r0, slot, note=lambda v: v):
            store_left(_HK, left_v[slot], lambda r: _ln(part_v[_at(r0 + r, RC), :], note), UNIT2, note)

        def body(g, _):
            @pl.when(g + 1 < n_grp)
            def _():
                for c in attn_copies(g + 1):
                    c.start()

            for c in attn_copies(g):
                c.wait()
            pace = _Pace(g < 0)
            zero = g // n_grp if OPQ else 0

            def qkv(m, r):
                blocks = {}
                for j in range(P // 2):
                    src = raw_v.at[g % 2, m * (P // 2) + j]
                    for i in range(P):
                        rows = slice(i * kw + r, i * kw + r + 8)
                        a, b = src[rows, :LANE], src[rows, LANE:]
                        for n, w in enumerate(((a & jnp.uint32(0xFFFF)) | (b << 16),
                                               (a >> 16) | (b & jnp.uint32(0xFFFF0000)))):
                            wqkv_v[m * H + g * P + 2 * j + n, rows, :] = w
                            blocks[i, 2 * j + n] = _bf(w)
                return store_right(_HK, sums_v.at[m * n_grp + g], slice(r, r + 8), lambda i, j: blocks[i, j])

            def out(r):
                return store_right(_HK, sums_v.at[3 * n_grp + g], slice(r, r + 8), lambda i, j: _bf(
                    wo_v[_at(g * grows + i * (Dh // 2) + r % (Dh // 2), 8), _tile(j * dt + r // (Dh // 2))]))

            def up(k):
                for n in range(ft):
                    upper, lower = _HK.result(_HK.accumulate(
                        lambda r: _bf(left_v[k % 2].at[r + zero][...]),
                        lambda i, j: pace.load(w3_v[i * kw:(i + 1) * kw, _tile(j * ft + n)]),
                        lambda r: pace.load(s3_v.at[n][:, _tile(r)])))
                    for r, v in enumerate(_HK.left([_gelu(v) for v in upper], [_gelu(v) for v in lower])):
                        hidden_v[k % 2].at[r][:, _tile(n)] = _words(v)
                        if r in GM:
                            pace.note(v)
                    pace.spread(G0, G1)

            def down(k):
                for n in range(dt):
                    halves = _HK.result(_HK.accumulate(
                        lambda r: _bf(hidden_v[k % 2].at[r + zero][...]),
                        lambda i, j: pace.load(w4_v[i * fw:(i + 1) * fw, _tile(j * dt + n)]),
                        lambda r: pace.load(s4_v.at[n][:, _tile(r)])))
                    for f, half in enumerate(halves):
                        for j, v in enumerate(half):
                            part_v[_at((g * units + k) * UNIT2 + f * v.shape[0], v.shape[0]), _tile(j * dt + n)] += v

            for task in ([functools.partial(qkv, m, r) for m in range(3) for r in range(0, kw, 8)]
                         + [functools.partial(out, r) for r in range(0, kw, 8)]):
                pace.note(task())
            total = units * (ft + dt) * n_prod
            pace.spread(R0 * total, R1 * total)
            for k in range(units):
                norm((g * units + k + 1) * UNIT2, (k + 1) % 2, pace.note)
                pace.spread(8, ft * n_prod)
                up(k)
                if TIGHT:
                    down(k)
                elif k > 0:
                    down(k - 1)
            if not TIGHT:
                down(units - 1)
            return 0

        with jax.named_scope("b2"):
            norm(0, 0)
            lax.fori_loop(0, n_grp, body, 0)

    def recurrence(sums_v, own_v, left_v, next_v, hq_v, ho_v):
        scale = float(Dh) ** -0.5
        row = lax.broadcasted_iota(jnp.int32, (2 * L, 2 * L), 0)
        col = lax.broadcasted_iota(jnp.int32, (2 * L, 2 * L), 1)
        r_in = jnp.where(row >= L, row - L, row)
        c_in = jnp.where(col >= L, col - L, col)
        same_head = (row >= L) == (col >= L)
        keep = same_head & ((r_in < M) | (r_in >= c_in))
        fill = jnp.where(same_head, _NEG / scale, -jnp.inf).astype(F32)

        def load_own(s):
            own_v[...] = _ln(x_rows(s * seg, seg)[:seg - 8])

        def load_next(s, q):
            next_v[8 * q:8 * q + 8, :] = _ln(x_rows(s * seg + seg - 16, 16)[8:])

        def load_left(mem):
            upper = jnp.concatenate([mem, own_v[...]], axis=0)
            for n, v in enumerate(_HK.left(_split(upper, P), _split(next_v[...], P))):
                left_v.at[n][...] = _words(v)

        def by_head(apart, dot, a, b):
            return jnp.concatenate([dot(a[:L], b), dot(a[L:], b)], axis=0) if apart else dot(a, b)

        def softmax(apart, q, k):
            s = jnp.where(keep, by_head(apart, _dot_nt, q, k.astype(BF16)), fill)
            e = jnp.exp2((s - jnp.max(s, axis=-1, keepdims=True)) * (scale * _LOG2E))
            return e, pl.reciprocal(jnp.sum(e, axis=-1, keepdims=True), full_range=False)

        def step(s, r, mem):
            first, last = r == 0, r == PERIOD - 1
            if not first:
                upper = jnp.concatenate([mem, own_v[...]], axis=0)
                early = {h: _dot(upper[:, :D // 2].astype(BF16), _bf(wqkv_v[h, :D // 4, :]))
                         for h in (0, 1, H, H + 1)}

            def plain(h):
                if h in early:
                    return early[h] + _dot(upper[:, D // 2:].astype(BF16), _bf(wqkv_v[h, D // 4:, :]))
                return _dot(upper.astype(BF16), _bf(wqkv_v[h]))

            def project(g):
                res = []
                for m in range(3):
                    h0 = m * H + g * P
                    if first:
                        tops, rest = _HK.result(_HK.accumulate(
                            lambda n: _bf(left_v.at[n][...]),
                            lambda i, j: _bf(wqkv_v[h0 + j, i * kw:(i + 1) * kw, :]),
                            lambda n: _bf(sums_v.at[m * n_grp + g][:, _tile(n)])))
                        for j in range(P):
                            hq_v[h0 + j] = rest[j][8:]
                        held = [v[:8] for v in rest]
                    else:
                        tops = [plain(h0 + j) for j in range(P)]
                        held = [hq_v[h0 + j, 8 * (r - 1):8 * r, :] for j in range(P)]
                    res.append([jnp.concatenate([tops[j], held[j], tops[j + 1], held[j + 1]], axis=0)
                                for j in range(0, P, 2)])
                return list(zip(*res))

            def merge(g, heads, acc):
                tops, held = [o[:L - 8] for o in heads], [o[L - 8:] for o in heads]
                if last:
                    left = _HK.left(tops, [jnp.concatenate([ho_v[:, _tile(g * P + j)], held[j]], axis=0)
                                           for j in range(P)])
                    k = Dh // 2
                    return _HK.accumulate(
                        lambda n: left[n].astype(BF16),
                        lambda i, j: _bf(wo_v[g * grows + i * k:g * grows + (i + 1) * k,
                                              j * dt * LANE:(j + 1) * dt * LANE]),
                        lambda n: jnp.concatenate([_bf(sums_v.at[3 * n_grp + g][c * k:(c + 1) * k, _tile(n)])
                                                   for c in range(dt)], axis=1),
                        acc or (),
                        ORD if LO else sorted(range(len(left)), key=lambda n: all(f == 1 for _, f, _ in _HK.products[n][2])))
                for j in range(P):
                    ho_v[8 * r:8 * r + 8, _tile(g * P + j)] = held[j]
                y = _dot(jnp.concatenate(tops, axis=1).astype(BF16), _bf(wo_v[g * grows:(g + 1) * grows, :]))
                return y if acc is None else acc + y

            lag, late = (4, (5, 6)) if last else (5, (4, 6)) if first else (5, (4, 5))
            qkv, prob, heads = {}, {}, {}
            acc, done = None, 0
            for t in range(n_grp + 3):
                if t < n_grp:
                    qkv[t] = project(t)
                while done < (t - lag + 1 if t < n_grp else (late + (n_grp,))[t - n_grp]):
                    acc = merge(done, heads.pop(done), acc)
                    done += 1
                if 0 <= t - 2 < n_grp:
                    heads[t - 2] = []
                    for (e, inv), (_, _, v) in zip(prob.pop(t - 2), qkv.pop(t - 2)):
                        o = by_head(t - 2 == n_grp - 1, _dot, e, v.astype(BF16)) * inv
                        heads[t - 2] += [o[:L], o[L:]]
                if 0 <= t - 1 < n_grp:
                    prob[t - 1] = [softmax(t == 1, q, k) for q, k, _ in qkv[t - 1]]
                if last and 1 <= t <= PERIOD:
                    load_next(jnp.minimum(s + t, n_seg - 1), t - 1)
                if t == n_grp - 1:
                    load_own(jnp.minimum(s + 1, n_seg - 1))
            if last:
                y, y_held = [jnp.concatenate(half, axis=1) for half in _HK.result(acc)]
                load_left(y[:M])
            else:
                y = acc
            base = x_rows(s * seg, seg) + part_v[_at(s * seg, seg), :]
            x_v[_at(s * (seg // 2), 8), :] = _words(base[:16] + y[M:M + 16])
            part_v[_at(s * seg + 16, 16), :] = jnp.concatenate([base[16:24] + y[M + 16:], base[24:]], axis=0)
            if last:
                for q in range(PERIOD):
                    r0 = (s - (PERIOD - 1) + q) * seg + 16
                    rest = part_v[_at(r0, 16), :]
                    x_v[_at(r0 // 2, 8), :] = _words(jnp.concatenate(
                        [rest[:8], rest[8:] + y_held[8 * q:8 * q + 8]], axis=0))
            return y[:M]

        def period(p, _):
            mem = None
            for r in range(PERIOD):
                mem = step(p * PERIOD + r, r, mem)
            rows = _at(p * (PERIOD * seg // 2), PERIOD * seg // 2)
            pltpu.make_async_copy(x_v.at[rows], out_hbm.bitcast(U32).at[rows], sem_out).start()
            return 0

        load_own(0)
        for q in range(PERIOD):
            load_next(q, q)
        mem0_copy.wait()
        load_left(mem0_v[...].astype(F32))
        with jax.named_scope("aloop"):
            lax.fori_loop(0, n_seg // PERIOD, period, 0)

    def rest(sums_v):
        if not SKIP_B2:
            pl.run_scoped(
                functools.partial(channel_mlp, sums_v),
                *[pltpu.VMEM((len(_HK.products), UNIT2 // 4, k // P), U32) for k in (D, D, FF, FF)]
            )
        if SKIP_A:
            z = pl.semaphore_read(sem_out)
            x_v[0:8, :] = (sums_v[z, 0:8, 0:D] + s3_v[z, 0:8, 0:D] + s4_v[z, 0:8, 0:D] + wqkv_v[z, 0:8, 0:1]
                           + pltpu.bitcast(part_v[_at(z, 8), :], U32))
            pltpu.make_async_copy(x_v.at[0:S // 2], out_hbm.bitcast(U32), sem_out).start()
            mem0_copy.wait()
            return
        pl.run_scoped(
            functools.partial(recurrence, sums_v),
            pltpu.VMEM((seg - 8, D), F32),
            pltpu.VMEM((len(_HK.products), (L - 8) // 2, D // P), U32),
            pltpu.VMEM((8 * PERIOD, D), F32),
            pltpu.VMEM((3 * H, 8 * (PERIOD - 1), Dh), F32),
            pltpu.VMEM((8 * (PERIOD - 1), H * Dh), F32),
        )

    pl.run_scoped(rest, pltpu.VMEM((4 * n_grp, kw, len(_HK.summed) * LANE), U32))
    pltpu.make_async_copy(x_v.at[0:S // 2], out_hbm.bitcast(U32), sem_out).wait()


@functools.partial(jax.jit, static_argnames=("A_seg_len",))
def pallas_parallel_sum__memory_aug_recurrent_mem_tr__mixer_s_mlp__prompt_kernel(
    A_x: jax.Array,
    A_mem0: jax.Array,
    A_Wq: jax.Array,
    A_Wk: jax.Array,
    A_Wv: jax.Array,
    A_Wo: jax.Array,
    A_seg_len: int,
    B_x: jax.Array,
    B_w1: jax.Array,
    B_w2: jax.Array,
    B_w3: jax.Array,
    B_w4: jax.Array,
):
    del B_x
    B, S, D = A_x.shape
    H, Dh = A_Wq.shape[1], A_Wq.shape[2]
    M = A_mem0.shape[1]
    FF = B_w3.shape[1]
    assert (B, M, A_seg_len) == (1, 8, 32)
    n_blk = S // TM
    sums = len(_HK.summed) * LANE
    pad = max(UNIT, UNIT2)

    hbm = pl.BlockSpec(memory_space=pl.ANY)
    out = pl.pallas_call(
        functools.partial(_kernel, seg=A_seg_len),
        out_shape=jax.ShapeDtypeStruct((S, D), A_x.dtype),
        in_specs=[hbm] * 10,
        out_specs=hbm,
        scratch_shapes=[
            pltpu.VMEM(((S + UNIT) // 2, D), U32),
            pltpu.VMEM((S + pad, D), F32),
            pltpu.VMEM((M, D), A_mem0.dtype),
            pltpu.VMEM((3 * H, D // 2, Dh), U32),
            pltpu.VMEM((H * Dh // 2, D), U32),
            pltpu.VMEM((2, 3 * P // 2, D // 2, 2 * LANE), U32),
            pltpu.VMEM((D // 2, FF), U32),
            pltpu.VMEM((FF // 2, D), U32),
            pltpu.VMEM((FF // P // LANE, D // 2 // P, sums), U32),
            pltpu.VMEM((D // P // LANE, FF // 2 // P, sums), U32),
            pltpu.SemaphoreType.DMA((n_blk + 1,)),
            pltpu.SemaphoreType.DMA((2, D // 2 // LANE)),
            pltpu.SemaphoreType.DMA((n_blk,)),
            pltpu.SemaphoreType.DMA((H // P,)),
            pltpu.SemaphoreType.DMA,
            pltpu.SemaphoreType.DMA,
        ],
        compiler_params=pltpu.CompilerParams(
            vmem_limit_bytes=126 * 1024 * 1024, disable_bounds_checks=True),
    )(A_x.reshape(S, D), A_mem0.reshape(M, D),
      A_Wq.reshape(D // 2, 2, H, Dh), A_Wk.reshape(D // 2, 2, H, Dh), A_Wv.reshape(D // 2, 2, H, Dh),
      A_Wo.reshape(H * Dh, D), B_w1, B_w2, B_w3, B_w4)
    return out.reshape(B, S, D)
```

```python
import functools

import jax
import jax.numpy as jnp
import numpy as np
from jax import lax
import jax.experimental.pallas as pl
import jax.experimental.pallas.tpu as pltpu

F32 = jnp.float32
BF16 = jnp.bfloat16
U32 = jnp.uint32

_EPS = 1e-5
_NEG = -1e9
_LOG2E = float(np.log2(np.e))
_GELU_C = float(np.sqrt(2.0 / np.pi))

LANE = 128
TM = 512
UNIT = 128
UNIT2 = 128
RC = 16
P = 4
PERIOD = 4
SKIP_B1 = False
SKIP_B2 = False
SKIP_A = False
P0, P1, Q0, Q1, R0, R1 = 0.1, 1.0, 0.05, 1.0, 0.3, 0.9
O4 = (18, 15, 9, 1, 16, 7, 19, 3, 10, 5, 24, 6, 14, 21, 2, 12, 0, 22, 25, 4, 13, 8, 20, 23, 11, 17)
O5 = (5, 18, 16, 9, 3, 15, 1, 24, 7, 19, 10, 0, 13, 14, 2, 22, 21, 12, 6, 20, 25, 23, 17, 4, 11, 8)
ORD = O5
LO = True
NA = range(18)
NB = (0,)
ALL = tuple(range(26))
PH, PM = 2, 4
GM = ()
OPQ = False
TIGHT = False
G0, G1 = 20, 40
NSEL = 4


def _dot(a, b):
    return lax.dot_general(a, b, (((1,), (0,)), ((), ())), preferred_element_type=F32)


def _dot_nt(a, b):
    return lax.dot_general(a, b, (((1,), (1,)), ((), ())), preferred_element_type=F32)


def _bf(words):
    return pltpu.bitcast(words, BF16)


def _words(x):
    return pltpu.bitcast(x.astype(BF16), U32)


def _at(start, n, align=None):
    return pl.ds(start if isinstance(start, int) else pl.multiple_of(start, align or n), n)


def _tile(j):
    return _at(j * LANE, LANE)


def _moments(x, note=lambda v: v):
    inv_n = 1.0 / x.shape[-1]
    xc = x - note(jnp.sum(x, axis=-1, keepdims=True)) * inv_n
    return xc, note(jnp.sum(xc * xc, axis=-1, keepdims=True)) * inv_n


def _ln(x, note=lambda v: v):
    xc, var = _moments(x, note)
    return xc * lax.rsqrt(var + _EPS)


def _gelu(x):
    inner = x * (_GELU_C + (_GELU_C * 0.044715) * (x * x))
    hx = 0.5 * x
    return hx + hx * jnp.tanh(inner)


def _signed_sum(terms):
    terms = sorted(terms, key=lambda t: -t[0])
    assert terms[0][0] > 0
    total = terms[0][1]
    for sign, value in terms[1:]:
        total = total + value if sign > 0 else total - value
    return total


class _HopcroftKerr:
    def __init__(self, p):
        own = {0: ((1, 2, 1), (2, 0, 1)), 1: ((2, 1, -1), (0, 2, 1)), 2: ((1, 1, 1), (0, 0, 1))}
        cross = {(0, 1): ((1, 0, 1, 0, 1, -1), (0, -1, 0, -1, 0, 1, -1), (-1, 0, 1, 0, 1, 0, 1)),
                 (0, 2): ((2, 0, 1, 2, 1, 1), (-1, 0, 0, -1, 0, 1, -1), (0, -1, -1, 0, -1, 0, 1)),
                 (1, 2): ((2, 1, -1, 2, 0, 1), (0, -1, -1, 0, 1, 0, 1), (1, 0, 0, -1, 0, 1, -1))}
        products, diag, uses = [], {}, {}

        def product(left, out):
            products.append((left, out))
            return len(products) - 1

        def diagonal(idx, kind):
            diag[idx] = [product([(i, f, 1) for i in idx], [(i, g, 1) for i in idx]) for f, g, _ in own[kind]]

        def pair(a, ka, b, kb):
            if ka > kb:
                return pair(b, kb, a, ka)[::-1]
            (f0, f1, s, g0, g1, t), ab, ba = cross[ka, kb]
            diagonal(a + b, 3 - ka - kb)
            used = diag[a] + diag[b] + diag[a + b] + [product(
                [(i, f0, 1) for i in a] + [(i, f1, s) for i in b],
                [(i, g0, 1) for i in a] + [(i, g1, t) for i in b])]
            return dict(zip(used, ab)), dict(zip(used, ba))

        for i in range(p):
            diagonal((i,), i % 3)
            uses[i, i] = {r: sign for r, (_, _, sign) in zip(diag[i,], own[i % 3])}
        for j in range(p):
            for i in range(j):
                if i % 3 != j % 3:
                    uses[i, j], uses[j, i] = pair((i,), i % 3, (j,), j % 3)
        for j in range(p):
            for i in range(j % 3, j, 3):
                k = i + 1
                both = (i, k) if (i, k) in diag else (k, i)
                uses[i, j], uses[j, i] = pair(both, 3 - i % 3 - k % 3, (j,), j % 3)
                for ij, kj in (((i, j), (k, j)), ((j, i), (j, k))):
                    for r, c in uses[kj].items():
                        uses[ij][r] = uses[ij].get(r, 0) - c
        self.p = p
        self.products = [(left, [(i, j, c[r]) for (i, j), c in sorted(uses.items()) if c.get(r)], out)
                         for r, (left, out) in enumerate(products)]
        self.summed = [r for r, (_, weight, _) in enumerate(self.products) if len(weight) > 1]

    def left(self, upper, lower):
        forms = [(u, l, u - l) for u, l in zip(upper, lower)]
        return [_signed_sum([(sign, forms[i][f]) for i, f, sign in left]) for left, _, _ in self.products]

    def right(self, n, block):
        return _signed_sum([(sign, block(i, j).astype(F32)) for i, j, sign in self.products[self.summed[n]][1]])

    def accumulate(self, left, block, summed, acc=(), order=None):
        acc = dict(acc)
        for r in order or (ORD if self.p == 4 and ORD else range(len(self.products))):
            _, weight, out = self.products[r]
            if r in self.summed:
                flip, w = 1, summed(self.summed.index(r))
            else:
                flip, w = weight[0][2], block(*weight[0][:2])
            m = _dot(left(r), w)
            for j, f, sign in out:
                if (j, f) in acc:
                    acc[j, f] = acc[j, f] + m if sign * flip > 0 else acc[j, f] - m
                else:
                    acc[j, f] = m if sign * flip > 0 else -m
        return acc

    def result(self, acc):
        return [[functools.reduce(jnp.add, [acc[j, g] for g in (f, 2) if (j, g) in acc])
                 for j in range(self.p)] for f in range(2)]


_HK = _HopcroftKerr(P)
_HK2 = _HopcroftKerr(2)


def _split(x, n):
    k = x.shape[1] // n
    return [x[:, i * k:(i + 1) * k] for i in range(n)]


class _Pace:
    def __init__(self, never):
        self.never, self.noted, self.due, self.pos = never, [], [], 0

    def note(self, v):
        u = pltpu.bitcast(jnp.broadcast_to(v, (v.shape[0], max(v.shape[1], LANE))), U32)
        self.noted.append(functools.reduce(jnp.bitwise_or, [
            u[r:r + 8, c:c + LANE] for r in range(0, u.shape[0], 8) for c in range(0, u.shape[1], LANE)]))
        return v

    def spread(self, first, last):
        n = len(self.noted)
        self.due += [(self.pos + first + (k + 1) * (last - first) / n, v) for k, v in enumerate(self.noted)]
        self.due.sort(key=lambda t: t[0])
        self.noted = []

    def load(self, words):
        self.pos += 1
        hints = []
        while self.due and self.due[0][0] <= self.pos:
            hints.append(self.due.pop(0)[1])
        if hints:
            hint, parts = functools.reduce(jnp.bitwise_or, hints), []
            step = 64 if NSEL > 1 else words.shape[0]
            for k in range(0, words.shape[0], step):
                parts += [jnp.where(self.never, hint, words[k:k + 8]), words[k + 8:k + step]]
            words = jnp.concatenate(parts, axis=0)
        return _bf(words)


def _kernel(x_hbm, mem0_hbm, wq_hbm, wk_hbm, wv_hbm, wo_hbm, w1_hbm, w2_hbm, w3_hbm, w4_hbm,
            out_hbm,
            x_v, part_v, mem0_v, wqkv_v, wo_v, raw_v, w3_v, w4_v, s3_v, s4_v,
            sem_x, sem_mix, sem_mlp, sem_attn, sem_mem, sem_out, *, seg):
    S, D = x_hbm.shape
    H, Dh = wq_hbm.shape[2], wq_hbm.shape[3]
    M = mem0_hbm.shape[0]
    FF = w3_hbm.shape[1]
    L = M + seg
    n_blk = S // TM
    n_seg = S // seg
    n_grp = H // P
    kw = D // 2 // P
    fw = FF // 2 // P
    ft = FF // P // LANE
    dt = D // P // LANE
    grows = P * Dh // 2

    def copy(hbm, vmem, sem, *idx):
        return pltpu.make_async_copy(hbm.bitcast(U32).at[idx], vmem.at[idx], sem)

    def attn_copies(g):
        rows = _at(g * grows, grows)
        copies = [copy(wo_hbm, wo_v, sem_attn.at[g], rows)]
        for m, hbm in enumerate((wq_hbm, wk_hbm, wv_hbm)):
            for j in range(P // 2):
                for par in range(2):
                    copies.append(pltpu.make_async_copy(
                        hbm.bitcast(U32).at[:, par, g * (P // 2) + j, :],
                        raw_v.at[g % 2, m * (P // 2) + j, :, _tile(par)], sem_attn.at[g]))
        return copies

    def mlp_copies(q):
        return [copy(hbm, vmem, sem_mlp.at[q], _at(i * n + q * (n // n_blk), n // n_blk, 8))
                for hbm, vmem, n in ((w3_hbm, w3_v, kw), (w4_hbm, w4_v, fw)) for i in range(P)]

    mem0_copy = pltpu.make_async_copy(mem0_hbm, mem0_v, sem_mem)

    def x_rows(r0, n):
        return _bf(x_v[_at(r0 // 2, n // 2), :]).astype(F32)

    def store_left(hk, ref, rows, size, note):
        for q in range(0, size // 2, RC):
            for n, v in enumerate(hk.left(_split(rows(q), hk.p), _split(rows(size // 2 + q), hk.p))):
                ref.at[n][q // 2:(q + RC) // 2, :] = _words(v)
                if n in (len(hk.products) - 1, len(hk.products) - 2):
                    note(v)

    def store_right(hk, ref, rows, block, noted=0):
        out = []
        for n in range(len(hk.summed)):
            v = hk.right(n, block)
            ref[rows, _tile(n)] = _words(v)
            if n < noted:
                out.append(v[:8])
        return jnp.concatenate(out, axis=0) if out else None

    def mixing(h_v, w_v, sums_v, left_v, first_v):
        pairs = D // 2 // LANE
        units = TM // UNIT
        loads = pairs * len(_HK2.products)

        def w_copies(n, j):
            return [copy((w1_hbm, w2_hbm)[n], w_v.at[n], sem_mix.at[n, j], slice(None), _tile(c * pairs + j))
                    for c in range(2)]

        def x_copy(i):
            return copy(x_hbm, x_v, sem_x.at[i + 1], _at(i * (TM // 2), TM // 2))

        def block(n, j, r=0, size=D // 4):
            return lambda a, c: w_v.at[n][a * (D // 4) + r:a * (D // 4) + r + size, _tile(c * pairs + j)]

        def prepare(j, r, size):
            store_right(_HK2, sums_v.at[1, j], slice(r, r + size), lambda a, c: _bf(block(1, j, r, size)(a, c)))

        def norm(r0, ref, size, note=lambda v: v):
            def rows(r):
                xc, var = _moments(x_rows(r0 + r, RC), note)
                inv = lax.rsqrt(var + _EPS)
                xn = xc * inv
                part_v[_at(r0 + r, RC), :] = xn
                return xn * lax.rsqrt(var * inv * inv + _EPS)
            store_left(_HK2, ref, rows, size, note)

        def shift(r0, ref, note=lambda v: v):
            def rows(r):
                parts = []
                for g, by in enumerate((-1, 1, -2, 2)):
                    c = slice(g * D // 4, (g + 1) * D // 4)
                    if by < 0:
                        parts.append(pltpu.roll(h_v[_at(r0 + r, RC + 8, 8), c], -by, 0)[8:])
                    else:
                        parts.append(pltpu.roll(h_v[_at(r0 + r + 8, RC + 8, 8), c], RC + 8 - by, 0)[:RC])
                return jnp.concatenate(parts, axis=1)
            store_left(_HK2, ref, rows, UNIT, note)

        def matmul(n, left, r0, load=_bf, arriving=None):
            for j in range(pairs):
                def summed(k):
                    if not arriving:
                        return load(sums_v.at[n, j][:, _tile(k)])
                    w = _HK2.right(k, lambda a, c: _bf(block(n, j)(a, c))).astype(BF16)
                    sums_v.at[n, j][:, _tile(k)] = pltpu.bitcast(w, U32)
                    return w

                for c in arriving(j) if arriving else ():
                    c.wait()
                halves = _HK2.result(_HK2.accumulate(
                    lambda r: _bf(left.at[r][...]), lambda a, c: load(block(n, j)(a, c)), summed))
                for f, half in enumerate(halves):
                    for c, v in enumerate(half):
                        size, lanes = v.shape[0], _tile(c * pairs + j)
                        if n == 0:
                            h_v[_at(8 + r0 + f * size, size, 8), lanes] = _gelu(v)
                        else:
                            part_v[_at(r0 + f * size, size), lanes] += v

        def h_unit(r0, k, pace):
            norm(r0 + UNIT, left_v.at[(k + 1) % 2], UNIT, pace.note)
            pace.spread(P0 * loads, loads)
            matmul(0, left_v.at[k % 2], r0, pace.load)

        def h_body(i, _):
            @pl.when(i + 2 < n_blk)
            def _():
                x_copy(i + 2).start()

            @pl.when(i + 1 < n_blk)
            def _():
                x_copy(i + 1).wait()

            for c in w_copies(1, i) + mlp_copies(i - 1):
                c.start()
            for c in w_copies(1, i - 1):
                c.wait()
            pace = _Pace(i < 0)
            for k in range(units):
                h_unit(i * TM + k * UNIT, k, pace)
                prepare(i - 1, k * (D // 4 // units), D // 4 // units)
            return 0

        def mix_body(i, _):
            @pl.when(i == 0)
            def _():
                for c in mlp_copies(n_blk - 1):
                    c.start()

            @pl.when(i == 1)
            def _():
                for c in attn_copies(0):
                    c.start()

            for c in mlp_copies(i):
                c.wait()

            def sums(w, ref, k, tiles, n, r):
                r += i * (k // n_blk)
                return store_right(_HK, ref.at[n], _at(r, 8), lambda a, c: _bf(
                    w[_at(a * k + r, 8), _tile(c * tiles + n)]), len(_HK.summed))

            side = [functools.partial(sums, w, ref, k, tiles, n, r)
                    for w, ref, k, tiles in ((w3_v, s3_v, kw, ft), (w4_v, s4_v, fw, dt))
                    for n in range(tiles) for r in range(0, k // n_blk, 8)]
            pace = _Pace(i < 0)
            for k in range(units):
                r0 = i * TM + k * UNIT
                for task in side[k * len(side) // units:(k + 1) * len(side) // units]:
                    pace.note(task())
                pace.spread(Q0 * loads, loads)
                shift(jnp.minimum(r0 + UNIT, S - UNIT), left_v.at[(k + 1) % 2], pace.note)
                pace.spread(Q0 * loads, loads)
                matmul(1, left_v.at[k % 2], r0, pace.load)
            return 0

        with jax.named_scope("pro"):
            first = [copy(x_hbm, x_v, sem_x.at[k], _at(k * TM // 4, TM // 4)) for k in range(2)]
            for c in ([first[0]] + sum((w_copies(0, j) for j in range(pairs)), [])
                      + [first[1], x_copy(1)] + w_copies(1, 0) + [x_copy(2), mem0_copy]):
                c.start()
            h_v[0:8, :] = jnp.zeros((8, D), F32)
            h_v[S + 8:S + 16, :] = jnp.zeros((8, D), F32)
            x_v[S // 2:, :] = jnp.zeros((UNIT // 2, D), U32)
            first[0].wait()
            norm(0, first_v, TM // 2)
            matmul(0, first_v, 0, arriving=functools.partial(w_copies, 0))
            first[1].wait()
            pace = _Pace(pl.semaphore_read(sem_out) < 0)
            norm(TM // 2, left_v.at[units // 2 % 2], UNIT)
            for k in range(units // 2, units):
                if k == units - 1:
                    x_copy(1).wait()
                h_unit(k * UNIT, k, pace)
        with jax.named_scope("b1"):
            lax.fori_loop(1, n_blk, h_body, 0)
            shift(0, left_v.at[0])
            for c in w_copies(1, pairs - 1):
                c.wait()
            for r in range(0, D // 4, 32):
                prepare(pairs - 1, r, 32)
            lax.fori_loop(0, n_blk, mix_body, 0)

    if SKIP_B1:
        for c in sum([mlp_copies(q) for q in range(4)], []) + attn_copies(0) + [mem0_copy]:
            c.start()
        for c in sum([mlp_copies(q) for q in range(4)], []):
            c.wait()
    else:
        pl.run_scoped(
            mixing,
            pltpu.VMEM((S + 16, D), F32),
            pltpu.VMEM((2, D // 2, D), U32),
            pltpu.VMEM((2, D // 2 // LANE, D // 4, len(_HK2.summed) * LANE), U32),
            pltpu.VMEM((2, len(_HK2.products), UNIT // 4, D // 2), U32),
            pltpu.VMEM((len(_HK2.products), TM // 8, D // 2), U32),
        )

    def channel_mlp(sums_v, *buffers):
        left_v, hidden_v = buffers[:2], buffers[2:]
        units = S // UNIT2 // n_grp
        n_prod = len(_HK.products)

        def norm(r0, slot, note=lambda v: v):
            store_left(_HK, left_v[slot], lambda r: _ln(part_v[_at(r0 + r, RC), :], note), UNIT2, note)

        def body(g, _):
            @pl.when(g + 1 < n_grp)
            def _():
                for c in attn_copies(g + 1):
                    c.start()

            for c in attn_copies(g):
                c.wait()
            pace = _Pace(g < 0)
            zero = g // n_grp if OPQ else 0

            def qkv(m, r):
                blocks = {}
                for j in range(P // 2):
                    src = raw_v.at[g % 2, m * (P // 2) + j]
                    for i in range(P):
                        rows = slice(i * kw + r, i * kw + r + 8)
                        a, b = src[rows, :LANE], src[rows, LANE:]
                        for n, w in enumerate(((a & jnp.uint32(0xFFFF)) | (b << 16),
                                               (a >> 16) | (b & jnp.uint32(0xFFFF0000)))):
                            wqkv_v[m * H + g * P + 2 * j + n, rows, :] = w
                            blocks[i, 2 * j + n] = _bf(w)
                return store_right(_HK, sums_v.at[m * n_grp + g], slice(r, r + 8), lambda i, j: blocks[i, j], 1)

            def out(r):
                return store_right(_HK, sums_v.at[3 * n_grp + g], slice(r, r + 8), lambda i, j: _bf(
                    wo_v[_at(g * grows + i * (Dh // 2) + r % (Dh // 2), 8), _tile(j * dt + r // (Dh // 2))]), 1)

            def up(k):
                for n in range(ft):
                    upper, lower = _HK.result(_HK.accumulate(
                        lambda r: _bf(left_v[k % 2].at[r + zero][...]),
                        lambda i, j: pace.load(w3_v[i * kw:(i + 1) * kw, _tile(j * ft + n)]),
                        lambda r: pace.load(s3_v.at[n][:, _tile(r)])))
                    for r, v in enumerate(_HK.left([_gelu(v) for v in upper], [_gelu(v) for v in lower])):
                        hidden_v[k % 2].at[r][:, _tile(n)] = _words(v)
                        if r in GM:
                            pace.note(v)
                    if GM:
                        pace.spread(G0, G1)

            def down(k):
                for n in range(dt):
                    halves = _HK.result(_HK.accumulate(
                        lambda r: _bf(hidden_v[k % 2].at[r + zero][...]),
                        lambda i, j: pace.load(w4_v[i * fw:(i + 1) * fw, _tile(j * dt + n)]),
                        lambda r: pace.load(s4_v.at[n][:, _tile(r)])))
                    for f, half in enumerate(halves):
                        for j, v in enumerate(half):
                            part_v[_at((g * units + k) * UNIT2 + f * v.shape[0], v.shape[0]), _tile(j * dt + n)] += v

            for task in ([functools.partial(qkv, m, r) for m in range(3) for r in range(0, kw, 8)]
                         + [functools.partial(out, r) for r in range(0, kw, 8)]):
                pace.note(task())
            total = units * (ft + dt) * n_prod
            pace.spread(R0 * total, R1 * total)
            for k in range(units):
                norm((g * units + k + 1) * UNIT2, (k + 1) % 2, pace.note)
                pace.spread(8, ft * n_prod)
                up(k)
                if TIGHT:
                    down(k)
                elif k > 0:
                    down(k - 1)
            if not TIGHT:
                down(units - 1)
            return 0

        with jax.named_scope("b2"):
            norm(0, 0)
            lax.fori_loop(0, n_grp, body, 0)

    def recurrence(sums_v, own_v, left_v, next_v, hq_v, ho_v):
        scale = float(Dh) ** -0.5
        row = lax.broadcasted_iota(jnp.int32, (2 * L, 2 * L), 0)
        col = lax.broadcasted_iota(jnp.int32, (2 * L, 2 * L), 1)
        r_in = jnp.where(row >= L, row - L, row)
        c_in = jnp.where(col >= L, col - L, col)
        same_head = (row >= L) == (col >= L)
        keep = same_head & ((r_in < M) | (r_in >= c_in))
        fill = jnp.where(same_head, _NEG / scale, -jnp.inf).astype(F32)

        def load_own(s):
            own_v[...] = _ln(x_rows(s * seg, seg)[:seg - 8])

        def load_next(s, q):
            next_v[8 * q:8 * q + 8, :] = _ln(x_rows(s * seg + seg - 16, 16)[8:])

        def load_left(mem):
            upper = jnp.concatenate([mem, own_v[...]], axis=0)
            for n, v in enumerate(_HK.left(_split(upper, P), _split(next_v[...], P))):
                left_v.at[n][...] = _words(v)

        def by_head(apart, dot, a, b):
            return jnp.concatenate([dot(a[:L], b), dot(a[L:], b)], axis=0) if apart else dot(a, b)

        def softmax(apart, q, k):
            s = jnp.where(keep, by_head(apart, _dot_nt, q, k.astype(BF16)), fill)
            e = jnp.exp2((s - jnp.max(s, axis=-1, keepdims=True)) * (scale * _LOG2E))
            return e, pl.reciprocal(jnp.sum(e, axis=-1, keepdims=True), full_range=False)

        def step(s, r, mem):
            first, last = r == 0, r == PERIOD - 1
            if not first:
                upper = jnp.concatenate([mem, own_v[...]], axis=0)
                early = {h: _dot(upper[:, :D // 2].astype(BF16), _bf(wqkv_v[h, :D // 4, :]))
                         for h in (0, 1, H, H + 1)}

            def plain(h):
                if h in early:
                    return early[h] + _dot(upper[:, D // 2:].astype(BF16), _bf(wqkv_v[h, D // 4:, :]))
                return _dot(upper.astype(BF16), _bf(wqkv_v[h]))

            def project(g):
                res = []
                for m in range(3):
                    h0 = m * H + g * P
                    if first:
                        tops, rest = _HK.result(_HK.accumulate(
                            lambda n: _bf(left_v.at[n][...]),
                            lambda i, j: _bf(wqkv_v[h0 + j, i * kw:(i + 1) * kw, :]),
                            lambda n: _bf(sums_v.at[m * n_grp + g][:, _tile(n)])))
                        for j in range(P):
                            hq_v[h0 + j] = rest[j][8:]
                        held = [v[:8] for v in rest]
                    else:
                        tops = [plain(h0 + j) for j in range(P)]
                        held = [hq_v[h0 + j, 8 * (r - 1):8 * r, :] for j in range(P)]
                    res.append([jnp.concatenate([tops[j], held[j], tops[j + 1], held[j + 1]], axis=0)
                                for j in range(0, P, 2)])
                return list(zip(*res))

            def merge(g, heads, acc):
                tops, held = [o[:L - 8] for o in heads], [o[L - 8:] for o in heads]
                if last:
                    left = _HK.left(tops, [jnp.concatenate([ho_v[:, _tile(g * P + j)], held[j]], axis=0)
                                           for j in range(P)])
                    k = Dh // 2
                    return _HK.accumulate(
                        lambda n: left[n].astype(BF16),
                        lambda i, j: _bf(wo_v[g * grows + i * k:g * grows + (i + 1) * k,
                                              j * dt * LANE:(j + 1) * dt * LANE]),
                        lambda n: jnp.concatenate([_bf(sums_v.at[3 * n_grp + g][c * k:(c + 1) * k, _tile(n)])
                                                   for c in range(dt)], axis=1),
                        acc or (),
                        ORD if LO else sorted(range(len(left)), key=lambda n: all(f == 1 for _, f, _ in _HK.products[n][2])))
                for j in range(P):
                    ho_v[8 * r:8 * r + 8, _tile(g * P + j)] = held[j]
                y = _dot(jnp.concatenate(tops, axis=1).astype(BF16), _bf(wo_v[g * grows:(g + 1) * grows, :]))
                return y if acc is None else acc + y

            lag, late = (4, (5, 6)) if last else (5, (4, 6)) if first else (5, (4, 5))
            qkv, prob, heads = {}, {}, {}
            acc, done = None, 0
            for t in range(n_grp + 3):
                if t < n_grp:
                    qkv[t] = project(t)
                while done < (t - lag + 1 if t < n_grp else (late + (n_grp,))[t - n_grp]):
                    acc = merge(done, heads.pop(done), acc)
                    done += 1
                if 0 <= t - 2 < n_grp:
                    heads[t - 2] = []
                    for (e, inv), (_, _, v) in zip(prob.pop(t - 2), qkv.pop(t - 2)):
                        o = by_head(t - 2 == n_grp - 1, _dot, e, v.astype(BF16)) * inv
                        heads[t - 2] += [o[:L], o[L:]]
                if 0 <= t - 1 < n_grp:
                    prob[t - 1] = [softmax(t == 1, q, k) for q, k, _ in qkv[t - 1]]
                if last and 1 <= t <= PERIOD:
                    load_next(jnp.minimum(s + t, n_seg - 1), t - 1)
                if t == n_grp - 1:
                    load_own(jnp.minimum(s + 1, n_seg - 1))
            if last:
                y, y_held = [jnp.concatenate(half, axis=1) for half in _HK.result(acc)]
                load_left(y[:M])
            else:
                y = acc
            base = x_rows(s * seg, seg) + part_v[_at(s * seg, seg), :]
            x_v[_at(s * (seg // 2), 8), :] = _words(base[:16] + y[M:M + 16])
            part_v[_at(s * seg + 16, 16), :] = jnp.concatenate([base[16:24] + y[M + 16:], base[24:]], axis=0)
            if last:
                for q in range(PERIOD):
                    r0 = (s - (PERIOD - 1) + q) * seg + 16
                    rest = part_v[_at(r0, 16), :]
                    x_v[_at(r0 // 2, 8), :] = _words(jnp.concatenate(
                        [rest[:8], rest[8:] + y_held[8 * q:8 * q + 8]], axis=0))
            return y[:M]

        def period(p, _):
            mem = None
            for r in range(PERIOD):
                mem = step(p * PERIOD + r, r, mem)
            rows = _at(p * (PERIOD * seg // 2), PERIOD * seg // 2)
            pltpu.make_async_copy(x_v.at[rows], out_hbm.bitcast(U32).at[rows], sem_out).start()
            return 0

        load_own(0)
        for q in range(PERIOD):
            load_next(q, q)
        mem0_copy.wait()
        load_left(mem0_v[...].astype(F32))
        with jax.named_scope("aloop"):
            lax.fori_loop(0, n_seg // PERIOD, period, 0)

    def rest(sums_v):
        if not SKIP_B2:
            pl.run_scoped(
                functools.partial(channel_mlp, sums_v),
                *[pltpu.VMEM((len(_HK.products), UNIT2 // 4, k // P), U32) for k in (D, D, FF, FF)]
            )
        if SKIP_A:
            z = pl.semaphore_read(sem_out)
            x_v[0:8, :] = (sums_v[z, 0:8, 0:D] + s3_v[z, 0:8, 0:D] + s4_v[z, 0:8, 0:D] + wqkv_v[z, 0:8, 0:1]
                           + pltpu.bitcast(part_v[_at(z, 8), :], U32))
            pltpu.make_async_copy(x_v.at[0:S // 2], out_hbm.bitcast(U32), sem_out).start()
            mem0_copy.wait()
            return
        pl.run_scoped(
            functools.partial(recurrence, sums_v),
            pltpu.VMEM((seg - 8, D), F32),
            pltpu.VMEM((len(_HK.products), (L - 8) // 2, D // P), U32),
            pltpu.VMEM((8 * PERIOD, D), F32),
            pltpu.VMEM((3 * H, 8 * (PERIOD - 1), Dh), F32),
            pltpu.VMEM((8 * (PERIOD - 1), H * Dh), F32),
        )

    pl.run_scoped(rest, pltpu.VMEM((4 * n_grp, kw, len(_HK.summed) * LANE), U32))
    pltpu.make_async_copy(x_v.at[0:S // 2], out_hbm.bitcast(U32), sem_out).wait()


@functools.partial(jax.jit, static_argnames=("A_seg_len",))
def pallas_parallel_sum__memory_aug_recurrent_mem_tr__mixer_s_mlp__prompt_kernel(
    A_x: jax.Array,
    A_mem0: jax.Array,
    A_Wq: jax.Array,
    A_Wk: jax.Array,
    A_Wv: jax.Array,
    A_Wo: jax.Array,
    A_seg_len: int,
    B_x: jax.Array,
    B_w1: jax.Array,
    B_w2: jax.Array,
    B_w3: jax.Array,
    B_w4: jax.Array,
):
    del B_x
    B, S, D = A_x.shape
    H, Dh = A_Wq.shape[1], A_Wq.shape[2]
    M = A_mem0.shape[1]
    FF = B_w3.shape[1]
    assert (B, M, A_seg_len) == (1, 8, 32)
    n_blk = S // TM
    sums = len(_HK.summed) * LANE
    pad = max(UNIT, UNIT2)

    hbm = pl.BlockSpec(memory_space=pl.ANY)
    out = pl.pallas_call(
        functools.partial(_kernel, seg=A_seg_len),
        out_shape=jax.ShapeDtypeStruct((S, D), A_x.dtype),
        in_specs=[hbm] * 10,
        out_specs=hbm,
        scratch_shapes=[
            pltpu.VMEM(((S + UNIT) // 2, D), U32),
            pltpu.VMEM((S + pad, D), F32),
            pltpu.VMEM((M, D), A_mem0.dtype),
            pltpu.VMEM((3 * H, D // 2, Dh), U32),
            pltpu.VMEM((H * Dh // 2, D), U32),
            pltpu.VMEM((2, 3 * P // 2, D // 2, 2 * LANE), U32),
            pltpu.VMEM((D // 2, FF), U32),
            pltpu.VMEM((FF // 2, D), U32),
            pltpu.VMEM((FF // P // LANE, D // 2 // P, sums), U32),
            pltpu.VMEM((D // P // LANE, FF // 2 // P, sums), U32),
            pltpu.SemaphoreType.DMA((n_blk + 1,)),
            pltpu.SemaphoreType.DMA((2, D // 2 // LANE)),
            pltpu.SemaphoreType.DMA((n_blk,)),
            pltpu.SemaphoreType.DMA((H // P,)),
            pltpu.SemaphoreType.DMA,
            pltpu.SemaphoreType.DMA,
        ],
        compiler_params=pltpu.CompilerParams(
            vmem_limit_bytes=126 * 1024 * 1024, disable_bounds_checks=True),
    )(A_x.reshape(S, D), A_mem0.reshape(M, D),
      A_Wq.reshape(D // 2, 2, H, Dh), A_Wk.reshape(D // 2, 2, H, Dh), A_Wv.reshape(D // 2, 2, H, Dh),
      A_Wo.reshape(H * Dh, D), B_w1, B_w2, B_w3, B_w4)
    return out.reshape(B, S, D)
```

```python
import functools

import jax
import jax.numpy as jnp
import numpy as np
from jax import lax
import jax.experimental.pallas as pl
import jax.experimental.pallas.tpu as pltpu

F32 = jnp.float32
BF16 = jnp.bfloat16
U32 = jnp.uint32

_EPS = 1e-5
_NEG = -1e9
_LOG2E = float(np.log2(np.e))
_GELU_C = float(np.sqrt(2.0 / np.pi))

LANE = 128
TM = 512
UNIT = 128
UNIT2 = 128
RC = 16
P = 4
PERIOD = 4
SKIP_B1 = SKIP_B2 = SKIP_A = False
P0, Q0, R0, R1, N0 = 0.1, 0.05, 0.3, 0.9, 8


def _dot(a, b):
    return lax.dot_general(a, b, (((1,), (0,)), ((), ())), preferred_element_type=F32)


def _dot_nt(a, b):
    return lax.dot_general(a, b, (((1,), (1,)), ((), ())), preferred_element_type=F32)


def _bf(words):
    return pltpu.bitcast(words, BF16)


def _words(x):
    return pltpu.bitcast(x.astype(BF16), U32)


def _at(start, n, align=None):
    return pl.ds(start if isinstance(start, int) else pl.multiple_of(start, align or n), n)


def _tile(j):
    return _at(j * LANE, LANE)


def _moments(x, note=lambda v: v):
    inv_n = 1.0 / x.shape[-1]
    xc = x - note(jnp.sum(x, axis=-1, keepdims=True)) * inv_n
    return xc, note(jnp.sum(xc * xc, axis=-1, keepdims=True)) * inv_n


def _ln(x, note=lambda v: v):
    xc, var = _moments(x, note)
    return xc * lax.rsqrt(var + _EPS)


def _gelu2(x):
    return x * (1.0 + jnp.tanh(x * (_GELU_C + (_GELU_C * 0.044715) * (x * x))))


def _signed_sum(terms):
    terms = sorted(terms, key=lambda t: -t[0])
    assert terms[0][0] > 0
    total = terms[0][1]
    for sign, value in terms[1:]:
        total = total + value if sign > 0 else total - value
    return total


class _HopcroftKerr:
    def __init__(self, p, order=None):
        own = {0: ((1, 2, 1), (2, 0, 1)), 1: ((2, 1, -1), (0, 2, 1)), 2: ((1, 1, 1), (0, 0, 1))}
        cross = {(0, 1): ((1, 0, 1, 0, 1, -1), (0, -1, 0, -1, 0, 1, -1), (-1, 0, 1, 0, 1, 0, 1)),
                 (0, 2): ((2, 0, 1, 2, 1, 1), (-1, 0, 0, -1, 0, 1, -1), (0, -1, -1, 0, -1, 0, 1)),
                 (1, 2): ((2, 1, -1, 2, 0, 1), (0, -1, -1, 0, 1, 0, 1), (1, 0, 0, -1, 0, 1, -1))}
        products, diag, uses = [], {}, {}

        def product(left, out):
            products.append((left, out))
            return len(products) - 1

        def diagonal(idx, kind):
            diag[idx] = [product([(i, f, 1) for i in idx], [(i, g, 1) for i in idx]) for f, g, _ in own[kind]]

        def pair(a, ka, b, kb):
            if ka > kb:
                return pair(b, kb, a, ka)[::-1]
            (f0, f1, s, g0, g1, t), ab, ba = cross[ka, kb]
            diagonal(a + b, 3 - ka - kb)
            used = diag[a] + diag[b] + diag[a + b] + [product(
                [(i, f0, 1) for i in a] + [(i, f1, s) for i in b],
                [(i, g0, 1) for i in a] + [(i, g1, t) for i in b])]
            return dict(zip(used, ab)), dict(zip(used, ba))

        for i in range(p):
            diagonal((i,), i % 3)
            uses[i, i] = {r: sign for r, (_, _, sign) in zip(diag[i,], own[i % 3])}
        for j in range(p):
            for i in range(j):
                if i % 3 != j % 3:
                    uses[i, j], uses[j, i] = pair((i,), i % 3, (j,), j % 3)
        for j in range(p):
            for i in range(j % 3, j, 3):
                k = i + 1
                both = (i, k) if (i, k) in diag else (k, i)
                uses[i, j], uses[j, i] = pair(both, 3 - i % 3 - k % 3, (j,), j % 3)
                for ij, kj in (((i, j), (k, j)), ((j, i), (j, k))):
                    for r, c in uses[kj].items():
                        uses[ij][r] = uses[ij].get(r, 0) - c
        self.p = p
        self.order = order or range(len(products))
        self.products = [(left, [(i, j, c[r]) for (i, j), c in sorted(uses.items()) if c.get(r)], out)
                         for r, (left, out) in enumerate(products)]
        self.summed = [r for r, (_, weight, _) in enumerate(self.products) if len(weight) > 1]

    def left(self, upper, lower):
        forms = [(u, l, u - l) for u, l in zip(upper, lower)]
        return [_signed_sum([(sign, forms[i][f]) for i, f, sign in left]) for left, _, _ in self.products]

    def right(self, n, block):
        return _signed_sum([(sign, block(i, j).astype(F32)) for i, j, sign in self.products[self.summed[n]][1]])

    def accumulate(self, left, block, summed, acc=()):
        acc = dict(acc)
        for r in self.order:
            _, weight, out = self.products[r]
            if r in self.summed:
                flip, w = 1, summed(self.summed.index(r))
            else:
                flip, w = weight[0][2], block(*weight[0][:2])
            m = _dot(left(r), w)
            for j, f, sign in out:
                if (j, f) in acc:
                    acc[j, f] = acc[j, f] + m if sign * flip > 0 else acc[j, f] - m
                else:
                    acc[j, f] = m if sign * flip > 0 else -m
        return acc

    def result(self, acc):
        return [[functools.reduce(jnp.add, [acc[j, g] for g in (f, 2) if (j, g) in acc])
                 for j in range(self.p)] for f in range(2)]


_HK = _HopcroftKerr(P, (5, 18, 16, 9, 3, 15, 1, 24, 7, 19, 10, 0, 13, 14, 2, 22, 21, 12, 6, 20, 25, 23, 17, 4, 11, 8))
_HK2 = _HopcroftKerr(2)


def _split(x, n):
    k = x.shape[1] // n
    return [x[:, i * k:(i + 1) * k] for i in range(n)]


class _Pace:
    def __init__(self, never):
        self.never, self.noted, self.due, self.pos = never, [], [], 0

    def note(self, v):
        u = pltpu.bitcast(jnp.broadcast_to(v, (v.shape[0], max(v.shape[1], LANE))), U32)
        self.noted.append(functools.reduce(jnp.bitwise_or, [
            u[r:r + 8, c:c + LANE] for r in range(0, u.shape[0], 8) for c in range(0, u.shape[1], LANE)]))
        return v

    def spread(self, first, last):
        n = len(self.noted)
        self.due += [(self.pos + first + (k + 1) * (last - first) / n, v) for k, v in enumerate(self.noted)]
        self.due.sort(key=lambda t: t[0])
        self.noted = []

    def load(self, words):
        self.pos += 1
        hints = []
        while self.due and self.due[0][0] <= self.pos:
            hints.append(self.due.pop(0)[1])
        if hints:
            hint, parts = functools.reduce(jnp.bitwise_or, hints), []
            for k in range(0, words.shape[0], LANE // 2):
                parts += [jnp.where(self.never, hint, words[k:k + 8]), words[k + 8:k + LANE // 2]]
            words = jnp.concatenate(parts, axis=0)
        return _bf(words)


def _kernel(x_hbm, mem0_hbm, wq_hbm, wk_hbm, wv_hbm, wo_hbm, w1_hbm, w2_hbm, w3_hbm, w4_hbm,
            out_hbm,
            x_v, part_v, mem0_v, wqkv_v, wo_v, raw_v, w3_v, w4_v, s3_v, s4_v,
            sem_x, sem_mix, sem_mlp, sem_attn, sem_mem, sem_out, *, seg):
    S, D = x_hbm.shape
    H, Dh = wq_hbm.shape[2], wq_hbm.shape[3]
    M = mem0_hbm.shape[0]
    FF = w3_hbm.shape[1]
    L = M + seg
    n_blk = S // TM
    n_seg = S // seg
    n_grp = H // P
    kw = D // 2 // P
    fw = FF // 2 // P
    ft = FF // P // LANE
    dt = D // P // LANE
    grows = P * Dh // 2

    def copy(hbm, vmem, sem, *idx):
        return pltpu.make_async_copy(hbm.bitcast(U32).at[idx], vmem.at[idx], sem)

    def attn_copies(g):
        rows = _at(g * grows, grows)
        copies = [copy(wo_hbm, wo_v, sem_attn.at[g], rows)]
        for m, hbm in enumerate((wq_hbm, wk_hbm, wv_hbm)):
            for j in range(P // 2):
                for par in range(2):
                    copies.append(pltpu.make_async_copy(
                        hbm.bitcast(U32).at[:, par, g * (P // 2) + j, :],
                        raw_v.at[g % 2, m * (P // 2) + j, :, _tile(par)], sem_attn.at[g]))
        return copies

    def mlp_copies(q):
        return [copy(hbm, vmem, sem_mlp.at[q], _at(i * n + q * (n // n_blk), n // n_blk, 8))
                for hbm, vmem, n in ((w3_hbm, w3_v, kw), (w4_hbm, w4_v, fw)) for i in range(P)]

    mem0_copy = pltpu.make_async_copy(mem0_hbm, mem0_v, sem_mem)

    def x_rows(r0, n):
        return _bf(x_v[_at(r0 // 2, n // 2), :]).astype(F32)

    def store_left(hk, ref, rows, size, note):
        for q in range(0, size // 2, RC):
            for n, v in enumerate(hk.left(_split(rows(q), hk.p), _split(rows(size // 2 + q), hk.p))):
                ref.at[n][q // 2:(q + RC) // 2, :] = _words(v)
                if n in (len(hk.products) - 1, len(hk.products) - 2):
                    note(v)

    def store_right(hk, ref, rows, block, noted=0):
        out = []
        for n in range(len(hk.summed)):
            v = hk.right(n, block)
            ref[rows, _tile(n)] = _words(v)
            if n < noted:
                out.append(v[:8])
        return jnp.concatenate(out, axis=0) if out else None

    def mixing(h_v, w_v, sums_v, left_v, first_v):
        pairs = D // 2 // LANE
        units = TM // UNIT
        loads = pairs * len(_HK2.products)

        def w_copies(n, j):
            return [copy((w1_hbm, w2_hbm)[n], w_v.at[n], sem_mix.at[n, j], slice(None), _tile(c * pairs + j))
                    for c in range(2)]

        def x_copy(i):
            return copy(x_hbm, x_v, sem_x.at[i + 1], _at(i * (TM // 2), TM // 2))

        def block(n, j, r=0, size=D // 4):
            return lambda a, c: w_v.at[n][a * (D // 4) + r:a * (D // 4) + r + size, _tile(c * pairs + j)]

        def prepare(j, r, size):
            store_right(_HK2, sums_v.at[1, j], slice(r, r + size), lambda a, c: _bf(block(1, j, r, size)(a, c)))

        def norm(r0, ref, size, note=lambda v: v):
            def rows(r):
                xc, var = _moments(x_rows(r0 + r, RC), note)
                inv = lax.rsqrt(var + _EPS)
                xn = xc * inv
                part_v[_at(r0 + r, RC), :] = xn
                return xn * lax.rsqrt(var * inv * inv + _EPS)
            store_left(_HK2, ref, rows, size, note)

        def shift(r0, ref, note=lambda v: v):
            def rows(r):
                parts = []
                for g, by in enumerate((-1, 1, -2, 2)):
                    c = slice(g * D // 4, (g + 1) * D // 4)
                    if by < 0:
                        parts.append(pltpu.roll(h_v[_at(r0 + r, RC + 8, 8), c], -by, 0)[8:])
                    else:
                        parts.append(pltpu.roll(h_v[_at(r0 + r + 8, RC + 8, 8), c], RC + 8 - by, 0)[:RC])
                return jnp.concatenate(parts, axis=1)
            store_left(_HK2, ref, rows, UNIT, note)

        def matmul(n, left, r0, load=_bf, arriving=None):
            for j in range(pairs):
                def summed(k):
                    if not arriving:
                        return load(sums_v.at[n, j][:, _tile(k)])
                    w = _HK2.right(k, lambda a, c: _bf(block(n, j)(a, c))).astype(BF16)
                    sums_v.at[n, j][:, _tile(k)] = pltpu.bitcast(w, U32)
                    return w

                for c in arriving(j) if arriving else ():
                    c.wait()
                halves = _HK2.result(_HK2.accumulate(
                    lambda r: _bf(left.at[r][...]), lambda a, c: load(block(n, j)(a, c)), summed))
                for f, half in enumerate(halves):
                    for c, v in enumerate(half):
                        size, lanes = v.shape[0], _tile(c * pairs + j)
                        if n == 0:
                            h_v[_at(8 + r0 + f * size, size, 8), lanes] = _gelu2(v)
                        else:
                            part_v[_at(r0 + f * size, size), lanes] += 0.5 * v

        def h_unit(r0, k, pace):
            norm(r0 + UNIT, left_v.at[(k + 1) % 2], UNIT, pace.note)
            pace.spread(P0 * loads, loads)
            matmul(0, left_v.at[k % 2], r0, pace.load)

        def h_body(i, _):
            @pl.when(i + 2 < n_blk)
            def _():
                x_copy(i + 2).start()

            @pl.when(i + 1 < n_blk)
            def _():
                x_copy(i + 1).wait()

            for c in w_copies(1, i) + mlp_copies(i - 1):
                c.start()
            for c in w_copies(1, i - 1):
                c.wait()
            pace = _Pace(i < 0)
            for k in range(units):
                h_unit(i * TM + k * UNIT, k, pace)
                prepare(i - 1, k * (D // 4 // units), D // 4 // units)
            return 0

        def mix_body(i, _):
            @pl.when(i == 0)
            def _():
                for c in mlp_copies(n_blk - 1):
                    c.start()

            @pl.when(i == 1)
            def _():
                for c in attn_copies(0):
                    c.start()

            for c in mlp_copies(i):
                c.wait()

            def sums(w, ref, k, tiles, n, r):
                r += i * (k // n_blk)
                return store_right(_HK, ref.at[n], _at(r, 8), lambda a, c: _bf(
                    w[_at(a * k + r, 8), _tile(c * tiles + n)]), len(_HK.summed))

            side = [functools.partial(sums, w, ref, k, tiles, n, r)
                    for w, ref, k, tiles in ((w3_v, s3_v, kw, ft), (w4_v, s4_v, fw, dt))
                    for n in range(tiles) for r in range(0, k // n_blk, 8)]
            pace = _Pace(i < 0)
            for k in range(units):
                r0 = i * TM + k * UNIT
                for task in side[k * len(side) // units:(k + 1) * len(side) // units]:
                    pace.note(task())
                pace.spread(Q0 * loads, loads)
                shift(jnp.minimum(r0 + UNIT, S - UNIT), left_v.at[(k + 1) % 2], pace.note)
                pace.spread(Q0 * loads, loads)
                matmul(1, left_v.at[k % 2], r0, pace.load)
            return 0

        with jax.named_scope("pro"):
            first = [copy(x_hbm, x_v, sem_x.at[k], _at(k * TM // 4, TM // 4)) for k in range(2)]
            for c in ([first[0]] + sum((w_copies(0, j) for j in range(pairs)), [])
                      + [first[1], x_copy(1)] + w_copies(1, 0) + [x_copy(2), mem0_copy]):
                c.start()
            h_v[0:8, :] = jnp.zeros((8, D), F32)
            h_v[S + 8:S + 16, :] = jnp.zeros((8, D), F32)
            x_v[S // 2:, :] = jnp.zeros((UNIT // 2, D), U32)
            first[0].wait()
            norm(0, first_v, TM // 2)
            matmul(0, first_v, 0, arriving=functools.partial(w_copies, 0))
            first[1].wait()
            pace = _Pace(jnp.square(part_v[0:8, 0:LANE]) < 0)
            norm(TM // 2, left_v.at[units // 2 % 2], UNIT)
            for k in range(units // 2, units):
                if k == units - 1:
                    x_copy(1).wait()
                h_unit(k * UNIT, k, pace)
        with jax.named_scope("b1"):
            lax.fori_loop(1, n_blk, h_body, 0)
            shift(0, left_v.at[0])
            for c in w_copies(1, pairs - 1):
                c.wait()
            for r in range(0, D // 4, 32):
                prepare(pairs - 1, r, 32)
            lax.fori_loop(0, n_blk, mix_body, 0)

    if SKIP_B1:
        for c in sum([mlp_copies(q) for q in range(4)], []) + attn_copies(0) + [mem0_copy]:
            c.start()
        for c in sum([mlp_copies(q) for q in range(4)], []):
            c.wait()
    else:
        pl.run_scoped(
            mixing,
            pltpu.VMEM((S + 16, D), F32),
            pltpu.VMEM((2, D // 2, D), U32),
            pltpu.VMEM((2, D // 2 // LANE, D // 4, len(_HK2.summed) * LANE), U32),
            pltpu.VMEM((2, len(_HK2.products), UNIT // 4, D // 2), U32),
            pltpu.VMEM((len(_HK2.products), TM // 8, D // 2), U32),
        )

    def channel_mlp(sums_v, *buffers):
        left_v, hidden_v = buffers[:2], buffers[2:]
        units = S // UNIT2 // n_grp
        n_prod = len(_HK.products)

        def norm(r0, slot, note=lambda v: v):
            store_left(_HK, left_v[slot], lambda r: _ln(part_v[_at(r0 + r, RC), :], note), UNIT2, note)

        def body(g, _):
            @pl.when(g + 1 < n_grp)
            def _():
                for c in attn_copies(g + 1):
                    c.start()

            for c in attn_copies(g):
                c.wait()
            pace = _Pace(g < 0)

            def qkv(m, r):
                blocks = {}
                for j in range(P // 2):
                    src = raw_v.at[g % 2, m * (P // 2) + j]
                    for i in range(P):
                        rows = slice(i * kw + r, i * kw + r + 8)
                        a, b = src[rows, :LANE], src[rows, LANE:]
                        for n, w in enumerate(((a & jnp.uint32(0xFFFF)) | (b << 16),
                                               (a >> 16) | (b & jnp.uint32(0xFFFF0000)))):
                            wqkv_v[m * H + g * P + 2 * j + n, rows, :] = w
                            blocks[i, 2 * j + n] = _bf(w)
                return store_right(_HK, sums_v.at[m * n_grp + g], slice(r, r + 8), lambda i, j: blocks[i, j], 1)

            def out(r):
                return store_right(_HK, sums_v.at[3 * n_grp + g], slice(r, r + 8), lambda i, j: _bf(
                    wo_v[_at(g * grows + i * (Dh // 2) + r % (Dh // 2), 8), _tile(j * dt + r // (Dh // 2))]), 1)

            def up(k):
                for n in range(ft):
                    upper, lower = _HK.result(_HK.accumulate(
                        lambda r: _bf(left_v[k % 2].at[r][...]),
                        lambda i, j: pace.load(w3_v[i * kw:(i + 1) * kw, _tile(j * ft + n)]),
                        lambda r: pace.load(s3_v.at[n][:, _tile(r)])))
                    for r, v in enumerate(_HK.left([_gelu2(v) for v in upper], [_gelu2(v) for v in lower])):
                        hidden_v[k % 2].at[r][:, _tile(n)] = _words(v)

            def down(k):
                for n in range(dt):
                    halves = _HK.result(_HK.accumulate(
                        lambda r: _bf(hidden_v[k % 2].at[r][...]),
                        lambda i, j: pace.load(w4_v[i * fw:(i + 1) * fw, _tile(j * dt + n)]),
                        lambda r: pace.load(s4_v.at[n][:, _tile(r)])))
                    for f, half in enumerate(halves):
                        for j, v in enumerate(half):
                            part_v[_at((g * units + k) * UNIT2 + f * v.shape[0], v.shape[0]), _tile(j * dt + n)] += 0.5 * v

            for task in ([functools.partial(qkv, m, r) for m in range(3) for r in range(0, kw, 8)]
                         + [functools.partial(out, r) for r in range(0, kw, 8)]):
                pace.note(task())
            total = units * (ft + dt) * n_prod
            pace.spread(R0 * total, R1 * total)
            for k in range(units):
                norm((g * units + k + 1) * UNIT2, (k + 1) % 2, pace.note)
                pace.spread(N0, ft * n_prod)
                up(k)
                if k > 0:
                    down(k - 1)
            down(units - 1)
            return 0

        with jax.named_scope("b2"):
            norm(0, 0)
            lax.fori_loop(0, n_grp, body, 0)

    def recurrence(sums_v, own_v, left_v, next_v, hq_v, ho_v):
        scale = float(Dh) ** -0.5
        row = lax.broadcasted_iota(jnp.int32, (2 * L, 2 * L), 0)
        col = lax.broadcasted_iota(jnp.int32, (2 * L, 2 * L), 1)
        r_in = jnp.where(row >= L, row - L, row)
        c_in = jnp.where(col >= L, col - L, col)
        same_head = (row >= L) == (col >= L)
        keep = same_head & ((r_in < M) | (r_in >= c_in))
        fill = jnp.where(same_head, _NEG / scale, -jnp.inf).astype(F32)

        def load_own(s):
            own_v[...] = _ln(x_rows(s * seg, seg)[:seg - 8])

        def load_next(s, q):
            next_v[8 * q:8 * q + 8, :] = _ln(x_rows(s * seg + seg - 16, 16)[8:])

        def load_left(mem):
            upper = jnp.concatenate([mem, own_v[...]], axis=0)
            for n, v in enumerate(_HK.left(_split(upper, P), _split(next_v[...], P))):
                left_v.at[n][...] = _words(v)

        def by_head(apart, dot, a, b):
            return jnp.concatenate([dot(a[:L], b), dot(a[L:], b)], axis=0) if apart else dot(a, b)

        def softmax(apart, q, k):
            s = jnp.where(keep, by_head(apart, _dot_nt, q, k.astype(BF16)), fill)
            e = jnp.exp2((s - jnp.max(s, axis=-1, keepdims=True)) * (scale * _LOG2E))
            return e, pl.reciprocal(jnp.sum(e, axis=-1, keepdims=True), full_range=False)

        def step(s, r, mem):
            first, last = r == 0, r == PERIOD - 1
            if not first:
                upper = jnp.concatenate([mem, own_v[...]], axis=0)
                early = {h: _dot(upper[:, :D // 2].astype(BF16), _bf(wqkv_v[h, :D // 4, :]))
                         for h in (0, 1, H, H + 1)}

            def plain(h):
                if h in early:
                    return early[h] + _dot(upper[:, D // 2:].astype(BF16), _bf(wqkv_v[h, D // 4:, :]))
                return _dot(upper.astype(BF16), _bf(wqkv_v[h]))

            def project(g):
                res = []
                for m in range(3):
                    h0 = m * H + g * P
                    if first:
                        tops, rest = _HK.result(_HK.accumulate(
                            lambda n: _bf(left_v.at[n][...]),
                            lambda i, j: _bf(wqkv_v[h0 + j, i * kw:(i + 1) * kw, :]),
                            lambda n: _bf(sums_v.at[m * n_grp + g][:, _tile(n)])))
                        for j in range(P):
                            hq_v[h0 + j] = rest[j][8:]
                        held = [v[:8] for v in rest]
                    else:
                        tops = [plain(h0 + j) for j in range(P)]
                        held = [hq_v[h0 + j, 8 * (r - 1):8 * r, :] for j in range(P)]
                    res.append([jnp.concatenate([tops[j], held[j], tops[j + 1], held[j + 1]], axis=0)
                                for j in range(0, P, 2)])
                return list(zip(*res))

            def merge(g, heads, acc):
                tops, held = [o[:L - 8] for o in heads], [o[L - 8:] for o in heads]
                if last:
                    left = _HK.left(tops, [jnp.concatenate([ho_v[:, _tile(g * P + j)], held[j]], axis=0)
                                           for j in range(P)])
                    k = Dh // 2
                    return _HK.accumulate(
                        lambda n: left[n].astype(BF16),
                        lambda i, j: _bf(wo_v[g * grows + i * k:g * grows + (i + 1) * k,
                                              j * dt * LANE:(j + 1) * dt * LANE]),
                        lambda n: jnp.concatenate([_bf(sums_v.at[3 * n_grp + g][c * k:(c + 1) * k, _tile(n)])
                                                   for c in range(dt)], axis=1),
                        acc or ())
                for j in range(P):
                    ho_v[8 * r:8 * r + 8, _tile(g * P + j)] = held[j]
                y = _dot(jnp.concatenate(tops, axis=1).astype(BF16), _bf(wo_v[g * grows:(g + 1) * grows, :]))
                return y if acc is None else acc + y

            lag, late = (4, (5, 6)) if last else (5, (4, 6)) if first else (5, (4, 5))
            qkv, prob, heads = {}, {}, {}
            acc, done = None, 0
            for t in range(n_grp + 3):
                if t < n_grp:
                    qkv[t] = project(t)
                while done < (t - lag + 1 if t < n_grp else (late + (n_grp,))[t - n_grp]):
                    acc = merge(done, heads.pop(done), acc)
                    done += 1
                if 0 <= t - 2 < n_grp:
                    heads[t - 2] = []
                    for (e, inv), (_, _, v) in zip(prob.pop(t - 2), qkv.pop(t - 2)):
                        o = by_head(t - 2 == n_grp - 1, _dot, e, v.astype(BF16)) * inv
                        heads[t - 2] += [o[:L], o[L:]]
                if 0 <= t - 1 < n_grp:
                    prob[t - 1] = [softmax(t == 1, q, k) for q, k, _ in qkv[t - 1]]
                if last and 1 <= t <= PERIOD:
                    load_next(jnp.minimum(s + t, n_seg - 1), t - 1)
                if t == n_grp - 1:
                    load_own(jnp.minimum(s + 1, n_seg - 1))
            if last:
                y, y_held = [jnp.concatenate(half, axis=1) for half in _HK.result(acc)]
                load_left(y[:M])
            else:
                y = acc
            base = x_rows(s * seg, seg) + part_v[_at(s * seg, seg), :]
            x_v[_at(s * (seg // 2), 8), :] = _words(base[:16] + y[M:M + 16])
            part_v[_at(s * seg + 16, 16), :] = jnp.concatenate([base[16:24] + y[M + 16:], base[24:]], axis=0)
            if last:
                for q in range(PERIOD):
                    r0 = (s - (PERIOD - 1) + q) * seg + 16
                    rest = part_v[_at(r0, 16), :]
                    x_v[_at(r0 // 2, 8), :] = _words(jnp.concatenate(
                        [rest[:8], rest[8:] + y_held[8 * q:8 * q + 8]], axis=0))
            return y[:M]

        def period(p, _):
            mem = None
            for r in range(PERIOD):
                mem = step(p * PERIOD + r, r, mem)
            rows = _at(p * (PERIOD * seg // 2), PERIOD * seg // 2)
            pltpu.make_async_copy(x_v.at[rows], out_hbm.bitcast(U32).at[rows], sem_out).start()
            return 0

        load_own(0)
        for q in range(PERIOD):
            load_next(q, q)
        mem0_copy.wait()
        load_left(mem0_v[...].astype(F32))
        with jax.named_scope("aloop"):
            lax.fori_loop(0, n_seg // PERIOD, period, 0)

    def rest(sums_v):
        if not SKIP_B2:
            pl.run_scoped(
                functools.partial(channel_mlp, sums_v),
                *[pltpu.VMEM((len(_HK.products), UNIT2 // 4, k // P), U32) for k in (D, D, FF, FF)]
            )
        if SKIP_A:
            z = pl.semaphore_read(sem_out)
            x_v[0:8, :] = (sums_v[z, 0:8, 0:D] + s3_v[z, 0:8, 0:D] + s4_v[z, 0:8, 0:D] + wqkv_v[z, 0:8, 0:1]
                           + pltpu.bitcast(part_v[_at(z, 8), :], U32))
            pltpu.make_async_copy(x_v.at[0:S // 2], out_hbm.bitcast(U32), sem_out).start()
            mem0_copy.wait()
            return
        pl.run_scoped(
            functools.partial(recurrence, sums_v),
            pltpu.VMEM((seg - 8, D), F32),
            pltpu.VMEM((len(_HK.products), (L - 8) // 2, D // P), U32),
            pltpu.VMEM((8 * PERIOD, D), F32),
            pltpu.VMEM((3 * H, 8 * (PERIOD - 1), Dh), F32),
            pltpu.VMEM((8 * (PERIOD - 1), H * Dh), F32),
        )

    pl.run_scoped(rest, pltpu.VMEM((4 * n_grp, kw, len(_HK.summed) * LANE), U32))
    pltpu.make_async_copy(x_v.at[0:S // 2], out_hbm.bitcast(U32), sem_out).wait()


@functools.partial(jax.jit, static_argnames=("A_seg_len",))
def pallas_parallel_sum__memory_aug_recurrent_mem_tr__mixer_s_mlp__prompt_kernel(
    A_x: jax.Array,
    A_mem0: jax.Array,
    A_Wq: jax.Array,
    A_Wk: jax.Array,
    A_Wv: jax.Array,
    A_Wo: jax.Array,
    A_seg_len: int,
    B_x: jax.Array,
    B_w1: jax.Array,
    B_w2: jax.Array,
    B_w3: jax.Array,
    B_w4: jax.Array,
):
    del B_x
    B, S, D = A_x.shape
    H, Dh = A_Wq.shape[1], A_Wq.shape[2]
    M = A_mem0.shape[1]
    FF = B_w3.shape[1]
    assert (B, M, A_seg_len) == (1, 8, 32)
    n_blk = S // TM
    sums = len(_HK.summed) * LANE
    pad = max(UNIT, UNIT2)

    hbm = pl.BlockSpec(memory_space=pl.ANY)
    out = pl.pallas_call(
        functools.partial(_kernel, seg=A_seg_len),
        out_shape=jax.ShapeDtypeStruct((S, D), A_x.dtype),
        in_specs=[hbm] * 10,
        out_specs=hbm,
        scratch_shapes=[
            pltpu.VMEM(((S + UNIT) // 2, D), U32),
            pltpu.VMEM((S + pad, D), F32),
            pltpu.VMEM((M, D), A_mem0.dtype),
            pltpu.VMEM((3 * H, D // 2, Dh), U32),
            pltpu.VMEM((H * Dh // 2, D), U32),
            pltpu.VMEM((2, 3 * P // 2, D // 2, 2 * LANE), U32),
            pltpu.VMEM((D // 2, FF), U32),
            pltpu.VMEM((FF // 2, D), U32),
            pltpu.VMEM((FF // P // LANE, D // 2 // P, sums), U32),
            pltpu.VMEM((D // P // LANE, FF // 2 // P, sums), U32),
            pltpu.SemaphoreType.DMA((n_blk + 1,)),
            pltpu.SemaphoreType.DMA((2, D // 2 // LANE)),
            pltpu.SemaphoreType.DMA((n_blk,)),
            pltpu.SemaphoreType.DMA((H // P,)),
            pltpu.SemaphoreType.DMA,
            pltpu.SemaphoreType.DMA,
        ],
        compiler_params=pltpu.CompilerParams(
            vmem_limit_bytes=126 * 1024 * 1024, disable_bounds_checks=True),
    )(A_x.reshape(S, D), A_mem0.reshape(M, D),
      A_Wq.reshape(D // 2, 2, H, Dh), A_Wk.reshape(D // 2, 2, H, Dh), A_Wv.reshape(D // 2, 2, H, Dh),
      A_Wo.reshape(H * Dh, D), B_w1, B_w2, B_w3, B_w4)
    return out.reshape(B, S, D)
```

```python
import functools

import jax
import jax.numpy as jnp
import numpy as np
from jax import lax
import jax.experimental.pallas as pl
import jax.experimental.pallas.tpu as pltpu

F32 = jnp.float32
BF16 = jnp.bfloat16
U32 = jnp.uint32

_EPS = 1e-5
_NEG = -1e9
_LOG2E = float(np.log2(np.e))
_GELU_C = float(np.sqrt(2.0 / np.pi))

LANE = 128
TM = 512
UNIT = 128
UNIT2 = 128
RC = 16
P = 4
PERIOD = 4
ALL = tuple(range(26))
GM = (0, 2, 4, 6)
NB = 1
G0, G1 = 20, 50
SKIP_B1 = SKIP_B2 = SKIP_A = False
P0, Q0, R0, R1, N0 = 0.1, 0.05, 0.64, 0.99, 16


def _dot(a, b):
    return lax.dot_general(a, b, (((1,), (0,)), ((), ())), preferred_element_type=F32)


def _dot_nt(a, b):
    return lax.dot_general(a, b, (((1,), (1,)), ((), ())), preferred_element_type=F32)


def _bf(words):
    return pltpu.bitcast(words, BF16)


def _words(x):
    return pltpu.bitcast(x.astype(BF16), U32)


def _at(start, n, align=None):
    return pl.ds(start if isinstance(start, int) else pl.multiple_of(start, align or n), n)


def _tile(j):
    return _at(j * LANE, LANE)


def _moments(x, note=lambda v: v):
    inv_n = 1.0 / x.shape[-1]
    xc = x - note(jnp.sum(x, axis=-1, keepdims=True)) * inv_n
    return xc, note(jnp.sum(xc * xc, axis=-1, keepdims=True)) * inv_n


def _ln(x, note=lambda v: v):
    xc, var = _moments(x, note)
    return xc * lax.rsqrt(var + _EPS)


def _gelu2(x):
    return x * (1.0 + jnp.tanh(x * (_GELU_C + (_GELU_C * 0.044715) * (x * x))))


def _signed_sum(terms):
    terms = sorted(terms, key=lambda t: -t[0])
    assert terms[0][0] > 0
    total = terms[0][1]
    for sign, value in terms[1:]:
        total = total + value if sign > 0 else total - value
    return total


class _HopcroftKerr:
    def __init__(self, p, order=None):
        own = {0: ((1, 2, 1), (2, 0, 1)), 1: ((2, 1, -1), (0, 2, 1)), 2: ((1, 1, 1), (0, 0, 1))}
        cross = {(0, 1): ((1, 0, 1, 0, 1, -1), (0, -1, 0, -1, 0, 1, -1), (-1, 0, 1, 0, 1, 0, 1)),
                 (0, 2): ((2, 0, 1, 2, 1, 1), (-1, 0, 0, -1, 0, 1, -1), (0, -1, -1, 0, -1, 0, 1)),
                 (1, 2): ((2, 1, -1, 2, 0, 1), (0, -1, -1, 0, 1, 0, 1), (1, 0, 0, -1, 0, 1, -1))}
        products, diag, uses = [], {}, {}

        def product(left, out):
            products.append((left, out))
            return len(products) - 1

        def diagonal(idx, kind):
            diag[idx] = [product([(i, f, 1) for i in idx], [(i, g, 1) for i in idx]) for f, g, _ in own[kind]]

        def pair(a, ka, b, kb):
            if ka > kb:
                return pair(b, kb, a, ka)[::-1]
            (f0, f1, s, g0, g1, t), ab, ba = cross[ka, kb]
            diagonal(a + b, 3 - ka - kb)
            used = diag[a] + diag[b] + diag[a + b] + [product(
                [(i, f0, 1) for i in a] + [(i, f1, s) for i in b],
                [(i, g0, 1) for i in a] + [(i, g1, t) for i in b])]
            return dict(zip(used, ab)), dict(zip(used, ba))

        for i in range(p):
            diagonal((i,), i % 3)
            uses[i, i] = {r: sign for r, (_, _, sign) in zip(diag[i,], own[i % 3])}
        for j in range(p):
            for i in range(j):
                if i % 3 != j % 3:
                    uses[i, j], uses[j, i] = pair((i,), i % 3, (j,), j % 3)
        for j in range(p):
            for i in range(j % 3, j, 3):
                k = i + 1
                both = (i, k) if (i, k) in diag else (k, i)
                uses[i, j], uses[j, i] = pair(both, 3 - i % 3 - k % 3, (j,), j % 3)
                for ij, kj in (((i, j), (k, j)), ((j, i), (j, k))):
                    for r, c in uses[kj].items():
                        uses[ij][r] = uses[ij].get(r, 0) - c
        self.p = p
        self.order = order or range(len(products))
        self.products = [(left, [(i, j, c[r]) for (i, j), c in sorted(uses.items()) if c.get(r)], out)
                         for r, (left, out) in enumerate(products)]
        self.summed = [r for r, (_, weight, _) in enumerate(self.products) if len(weight) > 1]

    def left(self, upper, lower):
        forms = [(u, l, u - l) for u, l in zip(upper, lower)]
        return [_signed_sum([(sign, forms[i][f]) for i, f, sign in left]) for left, _, _ in self.products]

    def right(self, n, block):
        return _signed_sum([(sign, block(i, j).astype(F32)) for i, j, sign in self.products[self.summed[n]][1]])

    def accumulate(self, left, block, summed, acc=()):
        acc = dict(acc)
        for r in self.order:
            _, weight, out = self.products[r]
            if r in self.summed:
                flip, w = 1, summed(self.summed.index(r))
            else:
                flip, w = weight[0][2], block(*weight[0][:2])
            m = _dot(left(r), w)
            for j, f, sign in out:
                if (j, f) in acc:
                    acc[j, f] = acc[j, f] + m if sign * flip > 0 else acc[j, f] - m
                else:
                    acc[j, f] = m if sign * flip > 0 else -m
        return acc

    def result(self, acc):
        return [[functools.reduce(jnp.add, [acc[j, g] for g in (f, 2) if (j, g) in acc])
                 for j in range(self.p)] for f in range(2)]


_HK = _HopcroftKerr(P, (5, 18, 16, 9, 3, 15, 1, 24, 7, 19, 10, 0, 13, 14, 2, 22, 21, 12, 6, 20, 25, 23, 17, 4, 11, 8))
_HK2 = _HopcroftKerr(2)


def _split(x, n):
    k = x.shape[1] // n
    return [x[:, i * k:(i + 1) * k] for i in range(n)]


class _Pace:
    def __init__(self, never):
        self.never, self.noted, self.due, self.pos = never, [], [], 0

    def note(self, v):
        u = pltpu.bitcast(jnp.broadcast_to(v, (v.shape[0], max(v.shape[1], LANE))), U32)
        self.noted.append(functools.reduce(jnp.bitwise_or, [
            u[r:r + 8, c:c + LANE] for r in range(0, u.shape[0], 8) for c in range(0, u.shape[1], LANE)]))
        return v

    def spread(self, first, last):
        n = len(self.noted)
        self.due += [(self.pos + first + (k + 1) * (last - first) / n, v) for k, v in enumerate(self.noted)]
        self.due.sort(key=lambda t: t[0])
        self.noted = []

    def load(self, words):
        self.pos += words.shape[0] // (LANE // 2)
        hints = []
        while self.due and self.due[0][0] <= self.pos:
            hints.append(self.due.pop(0)[1])
        if hints:
            hint, parts = functools.reduce(jnp.bitwise_or, hints), []
            for k in range(0, words.shape[0], LANE // 2):
                parts += [jnp.where(self.never, hint, words[k:k + 8]), words[k + 8:k + LANE // 2]]
            words = jnp.concatenate(parts, axis=0)
        return _bf(words)


def _kernel(x_hbm, mem0_hbm, wq_hbm, wk_hbm, wv_hbm, wo_hbm, w1_hbm, w2_hbm, w3_hbm, w4_hbm,
            out_hbm,
            x_v, part_v, mem0_v, wqkv_v, wo_v, raw_v, w3_v, w4_v, s3_v, s4_v,
            sem_x, sem_mix, sem_mlp, sem_attn, sem_mem, sem_out, *, seg):
    S, D = x_hbm.shape
    H, Dh = wq_hbm.shape[2], wq_hbm.shape[3]
    M = mem0_hbm.shape[0]
    FF = w3_hbm.shape[1]
    L = M + seg
    n_blk = S // TM
    n_seg = S // seg
    n_grp = H // P
    kw = D // 2 // P
    fw = FF // 2 // P
    ft = FF // P // LANE
    dt = D // P // LANE
    grows = P * Dh // 2

    def copy(hbm, vmem, sem, *idx):
        return pltpu.make_async_copy(hbm.bitcast(U32).at[idx], vmem.at[idx], sem)

    def attn_copies(g):
        rows = _at(g * grows, grows)
        copies = [copy(wo_hbm, wo_v, sem_attn.at[g], rows)]
        for m, hbm in enumerate((wq_hbm, wk_hbm, wv_hbm)):
            for j in range(P // 2):
                for par in range(2):
                    copies.append(pltpu.make_async_copy(
                        hbm.bitcast(U32).at[:, par, g * (P // 2) + j, :],
                        raw_v.at[g % 2, m * (P // 2) + j, :, _tile(par)], sem_attn.at[g]))
        return copies

    def mlp_copies(q):
        return [copy(hbm, vmem, sem_mlp.at[q], _at(i * n + q * (n // n_blk), n // n_blk, 8))
                for hbm, vmem, n in ((w3_hbm, w3_v, kw), (w4_hbm, w4_v, fw)) for i in range(P)]

    mem0_copy = pltpu.make_async_copy(mem0_hbm, mem0_v, sem_mem)

    def x_rows(r0, n):
        return _bf(x_v[_at(r0 // 2, n // 2), :]).astype(F32)

    def store_left(hk, ref, rows, size, note):
        for q in range(0, size // 2, RC):
            for n, v in enumerate(hk.left(_split(rows(q), hk.p), _split(rows(size // 2 + q), hk.p))):
                ref.at[n][q // 2:(q + RC) // 2, :] = _words(v)
                if n in (len(hk.products) - 1, len(hk.products) - 2):
                    note(v)

    def store_right(hk, ref, rows, block, noted=0):
        out = []
        for n in range(len(hk.summed)):
            v = hk.right(n, block)
            ref[rows, _tile(n)] = _words(v)
            if n < noted:
                out.append(v[:8])
        return jnp.concatenate(out, axis=0) if out else None

    def mixing(h_v, w_v, sums_v, left_v, first_v):
        pairs = D // 2 // LANE
        units = TM // UNIT
        loads = pairs * len(_HK2.products) * (D // 2 // LANE)

        def w_copies(n, j):
            return [copy((w1_hbm, w2_hbm)[n], w_v.at[n], sem_mix.at[n, j], slice(None), _tile(c * pairs + j))
                    for c in range(2)]

        def x_copy(i):
            return copy(x_hbm, x_v, sem_x.at[i + 1], _at(i * (TM // 2), TM // 2))

        def block(n, j, r=0, size=D // 4):
            return lambda a, c: w_v.at[n][a * (D // 4) + r:a * (D // 4) + r + size, _tile(c * pairs + j)]

        def prepare(j, r, size):
            store_right(_HK2, sums_v.at[1, j], slice(r, r + size), lambda a, c: _bf(block(1, j, r, size)(a, c)))

        def norm(r0, ref, size, note=lambda v: v):
            def rows(r):
                xc, var = _moments(x_rows(r0 + r, RC), note)
                inv = lax.rsqrt(var + _EPS)
                xn = xc * inv
                part_v[_at(r0 + r, RC), :] = xn
                return xn * lax.rsqrt(var * inv * inv + _EPS)
            store_left(_HK2, ref, rows, size, note)

        def shift(r0, ref, note=lambda v: v):
            def rows(r):
                parts = []
                for g, by in enumerate((-1, 1, -2, 2)):
                    c = slice(g * D // 4, (g + 1) * D // 4)
                    if by < 0:
                        parts.append(pltpu.roll(h_v[_at(r0 + r, RC + 8, 8), c], -by, 0)[8:])
                    else:
                        parts.append(pltpu.roll(h_v[_at(r0 + r + 8, RC + 8, 8), c], RC + 8 - by, 0)[:RC])
                return jnp.concatenate(parts, axis=1)
            store_left(_HK2, ref, rows, UNIT, note)

        def matmul(n, left, r0, load=_bf, arriving=None):
            for j in range(pairs):
                def summed(k):
                    if not arriving:
                        return load(sums_v.at[n, j][:, _tile(k)])
                    w = _HK2.right(k, lambda a, c: _bf(block(n, j)(a, c))).astype(BF16)
                    sums_v.at[n, j][:, _tile(k)] = pltpu.bitcast(w, U32)
                    return w

                for c in arriving(j) if arriving else ():
                    c.wait()
                halves = _HK2.result(_HK2.accumulate(
                    lambda r: _bf(left.at[r][...]), lambda a, c: load(block(n, j)(a, c)), summed))
                for f, half in enumerate(halves):
                    for c, v in enumerate(half):
                        size, lanes = v.shape[0], _tile(c * pairs + j)
                        if n == 0:
                            h_v[_at(8 + r0 + f * size, size, 8), lanes] = _gelu2(v)
                        else:
                            part_v[_at(r0 + f * size, size), lanes] += 0.5 * v

        def h_unit(r0, k, pace):
            norm(r0 + UNIT, left_v.at[(k + 1) % 2], UNIT, pace.note)
            pace.spread(P0 * loads, loads)
            matmul(0, left_v.at[k % 2], r0, pace.load)

        def h_body(i, _):
            @pl.when(i + 2 < n_blk)
            def _():
                x_copy(i + 2).start()

            @pl.when(i + 1 < n_blk)
            def _():
                x_copy(i + 1).wait()

            for c in w_copies(1, i) + mlp_copies(i - 1):
                c.start()
            for c in w_copies(1, i - 1):
                c.wait()
            pace = _Pace(i < 0)
            for k in range(units):
                h_unit(i * TM + k * UNIT, k, pace)
                prepare(i - 1, k * (D // 4 // units), D // 4 // units)
            return 0

        def mix_body(i, _):
            @pl.when(i == 0)
            def _():
                for c in mlp_copies(n_blk - 1):
                    c.start()

            @pl.when(i == 1)
            def _():
                for c in attn_copies(0):
                    c.start()

            for c in mlp_copies(i):
                c.wait()

            def sums(w, ref, k, tiles, n, r):
                r += i * (k // n_blk)
                return store_right(_HK, ref.at[n], _at(r, 8), lambda a, c: _bf(
                    w[_at(a * k + r, 8), _tile(c * tiles + n)]), len(_HK.summed))

            side = [functools.partial(sums, w, ref, k, tiles, n, r)
                    for w, ref, k, tiles in ((w3_v, s3_v, kw, ft), (w4_v, s4_v, fw, dt))
                    for n in range(tiles) for r in range(0, k // n_blk, 8)]
            pace = _Pace(i < 0)
            for k in range(units):
                r0 = i * TM + k * UNIT
                for task in side[k * len(side) // units:(k + 1) * len(side) // units]:
                    pace.note(task())
                pace.spread(Q0 * loads, loads)
                shift(jnp.minimum(r0 + UNIT, S - UNIT), left_v.at[(k + 1) % 2], pace.note)
                pace.spread(Q0 * loads, loads)
                matmul(1, left_v.at[k % 2], r0, pace.load)
            return 0

        with jax.named_scope("pro"):
            first = [copy(x_hbm, x_v, sem_x.at[k], _at(k * TM // 4, TM // 4)) for k in range(2)]
            for c in ([first[0]] + sum((w_copies(0, j) for j in range(pairs)), [])
                      + [first[1], x_copy(1)] + w_copies(1, 0) + [x_copy(2), mem0_copy]):
                c.start()
            h_v[0:8, :] = jnp.zeros((8, D), F32)
            h_v[S + 8:S + 16, :] = jnp.zeros((8, D), F32)
            x_v[S // 2:, :] = jnp.zeros((UNIT // 2, D), U32)
            first[0].wait()
            norm(0, first_v, TM // 2)
            matmul(0, first_v, 0, arriving=functools.partial(w_copies, 0))
            first[1].wait()
            pace = _Pace(jnp.square(part_v[0:8, 0:LANE]) < 0)
            norm(TM // 2, left_v.at[units // 2 % 2], UNIT)
            for k in range(units // 2, units):
                if k == units - 1:
                    x_copy(1).wait()
                h_unit(k * UNIT, k, pace)
        with jax.named_scope("b1"):
            lax.fori_loop(1, n_blk, h_body, 0)
            shift(0, left_v.at[0])
            for c in w_copies(1, pairs - 1):
                c.wait()
            for r in range(0, D // 4, 32):
                prepare(pairs - 1, r, 32)
            lax.fori_loop(0, n_blk, mix_body, 0)

    if SKIP_B1:
        for c in sum([mlp_copies(q) for q in range(4)], []) + attn_copies(0) + [mem0_copy]:
            c.start()
        for c in sum([mlp_copies(q) for q in range(4)], []):
            c.wait()
    else:
        pl.run_scoped(
            mixing,
            pltpu.VMEM((S + 16, D), F32),
            pltpu.VMEM((2, D // 2, D), U32),
            pltpu.VMEM((2, D // 2 // LANE, D // 4, len(_HK2.summed) * LANE), U32),
            pltpu.VMEM((2, len(_HK2.products), UNIT // 4, D // 2), U32),
            pltpu.VMEM((len(_HK2.products), TM // 8, D // 2), U32),
        )

    def channel_mlp(sums_v, *buffers):
        left_v, hidden_v = buffers[:2], buffers[2:]
        units = S // UNIT2 // n_grp
        n_prod = len(_HK.products)

        def norm(r0, slot, note=lambda v: v):
            store_left(_HK, left_v[slot], lambda r: _ln(part_v[_at(r0 + r, RC), :], note), UNIT2, note)

        def body(g, _):
            @pl.when(g + 1 < n_grp)
            def _():
                for c in attn_copies(g + 1):
                    c.start()

            for c in attn_copies(g):
                c.wait()
            pace = _Pace(g < 0)

            def qkv(m, r):
                blocks = {}
                for j in range(P // 2):
                    src = raw_v.at[g % 2, m * (P // 2) + j]
                    for i in range(P):
                        rows = slice(i * kw + r, i * kw + r + 8)
                        a, b = src[rows, :LANE], src[rows, LANE:]
                        for n, w in enumerate(((a & jnp.uint32(0xFFFF)) | (b << 16),
                                               (a >> 16) | (b & jnp.uint32(0xFFFF0000)))):
                            wqkv_v[m * H + g * P + 2 * j + n, rows, :] = w
                            blocks[i, 2 * j + n] = _bf(w)
                return store_right(_HK, sums_v.at[m * n_grp + g], slice(r, r + 8), lambda i, j: blocks[i, j], NB)

            def out(r):
                return store_right(_HK, sums_v.at[3 * n_grp + g], slice(r, r + 8), lambda i, j: _bf(
                    wo_v[_at(g * grows + i * (Dh // 2) + r % (Dh // 2), 8), _tile(j * dt + r // (Dh // 2))]), NB)

            def up(k):
                for n in range(ft):
                    upper, lower = _HK.result(_HK.accumulate(
                        lambda r: _bf(left_v[k % 2].at[r][...]),
                        lambda i, j: pace.load(w3_v[i * kw:(i + 1) * kw, _tile(j * ft + n)]),
                        lambda r: pace.load(s3_v.at[n][:, _tile(r)])))
                    for r, v in enumerate(_HK.left([_gelu2(v) for v in upper], [_gelu2(v) for v in lower])):
                        hidden_v[k % 2].at[r][:, _tile(n)] = _words(v)
                        if r in GM:
                            pace.note(v)
                    if GM and (n + 1 < ft or k):
                        pace.spread(G0, G1)
                    pace.noted = []

            def down(k):
                for n in range(dt):
                    halves = _HK.result(_HK.accumulate(
                        lambda r: _bf(hidden_v[k % 2].at[r][...]),
                        lambda i, j: pace.load(w4_v[i * fw:(i + 1) * fw, _tile(j * dt + n)]),
                        lambda r: pace.load(s4_v.at[n][:, _tile(r)])))
                    for f, half in enumerate(halves):
                        for j, v in enumerate(half):
                            part_v[_at((g * units + k) * UNIT2 + f * v.shape[0], v.shape[0]), _tile(j * dt + n)] += 0.5 * v

            for task in ([functools.partial(qkv, m, r) for m in range(3) for r in range(0, kw, 8)]
                         + [functools.partial(out, r) for r in range(0, kw, 8)]):
                pace.note(task())
            total = units * 2 * ft * dt * n_prod
            pace.spread(R0 * total, R1 * total)
            for k in range(units):
                norm((g * units + k + 1) * UNIT2, (k + 1) % 2, pace.note)
                pace.spread(N0, ft * dt * n_prod)
                up(k)
                if k > 0:
                    down(k - 1)
            down(units - 1)
            return 0

        with jax.named_scope("b2"):
            norm(0, 0)
            lax.fori_loop(0, n_grp, body, 0)

    def recurrence(sums_v, own_v, left_v, next_v, hq_v, ho_v):
        scale = float(Dh) ** -0.5
        row = lax.broadcasted_iota(jnp.int32, (2 * L, 2 * L), 0)
        col = lax.broadcasted_iota(jnp.int32, (2 * L, 2 * L), 1)
        r_in = jnp.where(row >= L, row - L, row)
        c_in = jnp.where(col >= L, col - L, col)
        same_head = (row >= L) == (col >= L)
        keep = same_head & ((r_in < M) | (r_in >= c_in))
        fill = jnp.where(same_head, _NEG / scale, -jnp.inf).astype(F32)

        def load_own(s):
            own_v[...] = _ln(x_rows(s * seg, seg)[:seg - 8])

        def load_next(s, q):
            next_v[8 * q:8 * q + 8, :] = _ln(x_rows(s * seg + seg - 16, 16)[8:])

        def load_left(mem):
            upper = jnp.concatenate([mem, own_v[...]], axis=0)
            for n, v in enumerate(_HK.left(_split(upper, P), _split(next_v[...], P))):
                left_v.at[n][...] = _words(v)

        def by_head(apart, dot, a, b):
            return jnp.concatenate([dot(a[:L], b), dot(a[L:], b)], axis=0) if apart else dot(a, b)

        def softmax(apart, q, k):
            s = jnp.where(keep, by_head(apart, _dot_nt, q, k.astype(BF16)), fill)
            e = jnp.exp2((s - jnp.max(s, axis=-1, keepdims=True)) * (scale * _LOG2E))
            return e, pl.reciprocal(jnp.sum(e, axis=-1, keepdims=True), full_range=False)

        def step(s, r, mem):
            first, last = r == 0, r == PERIOD - 1
            if not first:
                upper = jnp.concatenate([mem, own_v[...]], axis=0)
                early = {h: _dot(upper[:, :D // 2].astype(BF16), _bf(wqkv_v[h, :D // 4, :]))
                         for h in (0, 1, H, H + 1)}

            def plain(h):
                if h in early:
                    return early[h] + _dot(upper[:, D // 2:].astype(BF16), _bf(wqkv_v[h, D // 4:, :]))
                return _dot(upper.astype(BF16), _bf(wqkv_v[h]))

            def project(g):
                res = []
                for m in range(3):
                    h0 = m * H + g * P
                    if first:
                        tops, rest = _HK.result(_HK.accumulate(
                            lambda n: _bf(left_v.at[n][...]),
                            lambda i, j: _bf(wqkv_v[h0 + j, i * kw:(i + 1) * kw, :]),
                            lambda n: _bf(sums_v.at[m * n_grp + g][:, _tile(n)])))
                        for j in range(P):
                            hq_v[h0 + j] = rest[j][8:]
                        held = [v[:8] for v in rest]
                    else:
                        tops = [plain(h0 + j) for j in range(P)]
                        held = [hq_v[h0 + j, 8 * (r - 1):8 * r, :] for j in range(P)]
                    res.append([jnp.concatenate([tops[j], held[j], tops[j + 1], held[j + 1]], axis=0)
                                for j in range(0, P, 2)])
                return list(zip(*res))

            def merge(g, heads, acc):
                tops, held = [o[:L - 8] for o in heads], [o[L - 8:] for o in heads]
                if last:
                    left = _HK.left(tops, [jnp.concatenate([ho_v[:, _tile(g * P + j)], held[j]], axis=0)
                                           for j in range(P)])
                    k = Dh // 2
                    return _HK.accumulate(
                        lambda n: left[n].astype(BF16),
                        lambda i, j: _bf(wo_v[g * grows + i * k:g * grows + (i + 1) * k,
                                              j * dt * LANE:(j + 1) * dt * LANE]),
                        lambda n: jnp.concatenate([_bf(sums_v.at[3 * n_grp + g][c * k:(c + 1) * k, _tile(n)])
                                                   for c in range(dt)], axis=1),
                        acc or ())
                for j in range(P):
                    ho_v[8 * r:8 * r + 8, _tile(g * P + j)] = held[j]
                y = _dot(jnp.concatenate(tops, axis=1).astype(BF16), _bf(wo_v[g * grows:(g + 1) * grows, :]))
                return y if acc is None else acc + y

            lag, late = (4, (5, 6)) if last else (5, (4, 6)) if first else (5, (4, 5))
            qkv, prob, heads = {}, {}, {}
            acc, done = None, 0
            for t in range(n_grp + 3):
                if t < n_grp:
                    qkv[t] = project(t)
                while done < (t - lag + 1 if t < n_grp else (late + (n_grp,))[t - n_grp]):
                    acc = merge(done, heads.pop(done), acc)
                    done += 1
                if 0 <= t - 2 < n_grp:
                    heads[t - 2] = []
                    for (e, inv), (_, _, v) in zip(prob.pop(t - 2), qkv.pop(t - 2)):
                        o = by_head(t - 2 == n_grp - 1, _dot, e, v.astype(BF16)) * inv
                        heads[t - 2] += [o[:L], o[L:]]
                if 0 <= t - 1 < n_grp:
                    prob[t - 1] = [softmax(t == 1, q, k) for q, k, _ in qkv[t - 1]]
                if last and 1 <= t <= PERIOD:
                    load_next(jnp.minimum(s + t, n_seg - 1), t - 1)
                if t == n_grp - 1:
                    load_own(jnp.minimum(s + 1, n_seg - 1))
            if last:
                y, y_held = [jnp.concatenate(half, axis=1) for half in _HK.result(acc)]
                load_left(y[:M])
            else:
                y = acc
            base = x_rows(s * seg, seg) + part_v[_at(s * seg, seg), :]
            x_v[_at(s * (seg // 2), 8), :] = _words(base[:16] + y[M:M + 16])
            part_v[_at(s * seg + 16, 16), :] = jnp.concatenate([base[16:24] + y[M + 16:], base[24:]], axis=0)
            if last:
                for q in range(PERIOD):
                    r0 = (s - (PERIOD - 1) + q) * seg + 16
                    rest = part_v[_at(r0, 16), :]
                    x_v[_at(r0 // 2, 8), :] = _words(jnp.concatenate(
                        [rest[:8], rest[8:] + y_held[8 * q:8 * q + 8]], axis=0))
            return y[:M]

        def period(p, _):
            mem = None
            for r in range(PERIOD):
                mem = step(p * PERIOD + r, r, mem)
            rows = _at(p * (PERIOD * seg // 2), PERIOD * seg // 2)
            pltpu.make_async_copy(x_v.at[rows], out_hbm.bitcast(U32).at[rows], sem_out).start()
            return 0

        load_own(0)
        for q in range(PERIOD):
            load_next(q, q)
        mem0_copy.wait()
        load_left(mem0_v[...].astype(F32))
        with jax.named_scope("aloop"):
            lax.fori_loop(0, n_seg // PERIOD, period, 0)

    def rest(sums_v):
        if not SKIP_B2:
            pl.run_scoped(
                functools.partial(channel_mlp, sums_v),
                *[pltpu.VMEM((len(_HK.products), UNIT2 // 4, k // P), U32) for k in (D, D, FF, FF)]
            )
        if SKIP_A:
            z = pl.semaphore_read(sem_out)
            x_v[0:8, :] = (sums_v[z, 0:8, 0:D] + s3_v[z, 0:8, 0:D] + s4_v[z, 0:8, 0:D] + wqkv_v[z, 0:8, 0:1]
                           + pltpu.bitcast(part_v[_at(z, 8), :], U32))
            pltpu.make_async_copy(x_v.at[0:S // 2], out_hbm.bitcast(U32), sem_out).start()
            mem0_copy.wait()
            return
        pl.run_scoped(
            functools.partial(recurrence, sums_v),
            pltpu.VMEM((seg - 8, D), F32),
            pltpu.VMEM((len(_HK.products), (L - 8) // 2, D // P), U32),
            pltpu.VMEM((8 * PERIOD, D), F32),
            pltpu.VMEM((3 * H, 8 * (PERIOD - 1), Dh), F32),
            pltpu.VMEM((8 * (PERIOD - 1), H * Dh), F32),
        )

    pl.run_scoped(rest, pltpu.VMEM((4 * n_grp, kw, len(_HK.summed) * LANE), U32))
    pltpu.make_async_copy(x_v.at[0:S // 2], out_hbm.bitcast(U32), sem_out).wait()


@functools.partial(jax.jit, static_argnames=("A_seg_len",))
def pallas_parallel_sum__memory_aug_recurrent_mem_tr__mixer_s_mlp__prompt_kernel(
    A_x: jax.Array,
    A_mem0: jax.Array,
    A_Wq: jax.Array,
    A_Wk: jax.Array,
    A_Wv: jax.Array,
    A_Wo: jax.Array,
    A_seg_len: int,
    B_x: jax.Array,
    B_w1: jax.Array,
    B_w2: jax.Array,
    B_w3: jax.Array,
    B_w4: jax.Array,
):
    del B_x
    B, S, D = A_x.shape
    H, Dh = A_Wq.shape[1], A_Wq.shape[2]
    M = A_mem0.shape[1]
    FF = B_w3.shape[1]
    assert (B, M, A_seg_len) == (1, 8, 32)
    n_blk = S // TM
    sums = len(_HK.summed) * LANE
    pad = max(UNIT, UNIT2)

    hbm = pl.BlockSpec(memory_space=pl.ANY)
    out = pl.pallas_call(
        functools.partial(_kernel, seg=A_seg_len),
        out_shape=jax.ShapeDtypeStruct((S, D), A_x.dtype),
        in_specs=[hbm] * 10,
        out_specs=hbm,
        scratch_shapes=[
            pltpu.VMEM(((S + UNIT) // 2, D), U32),
            pltpu.VMEM((S + pad, D), F32),
            pltpu.VMEM((M, D), A_mem0.dtype),
            pltpu.VMEM((3 * H, D // 2, Dh), U32),
            pltpu.VMEM((H * Dh // 2, D), U32),
            pltpu.VMEM((2, 3 * P // 2, D // 2, 2 * LANE), U32),
            pltpu.VMEM((D // 2, FF), U32),
            pltpu.VMEM((FF // 2, D), U32),
            pltpu.VMEM((FF // P // LANE, D // 2 // P, sums), U32),
            pltpu.VMEM((D // P // LANE, FF // 2 // P, sums), U32),
            pltpu.SemaphoreType.DMA((n_blk + 1,)),
            pltpu.SemaphoreType.DMA((2, D // 2 // LANE)),
            pltpu.SemaphoreType.DMA((n_blk,)),
            pltpu.SemaphoreType.DMA((H // P,)),
            pltpu.SemaphoreType.DMA,
            pltpu.SemaphoreType.DMA,
        ],
        compiler_params=pltpu.CompilerParams(
            vmem_limit_bytes=255 * 512 * 1024, disable_bounds_checks=True),
    )(A_x.reshape(S, D), A_mem0.reshape(M, D),
      A_Wq.reshape(D // 2, 2, H, Dh), A_Wk.reshape(D // 2, 2, H, Dh), A_Wv.reshape(D // 2, 2, H, Dh),
      A_Wo.reshape(H * Dh, D), B_w1, B_w2, B_w3, B_w4)
    return out.reshape(B, S, D)
```

```python
import functools

import jax
import jax.numpy as jnp
import numpy as np
from jax import lax
import jax.experimental.pallas as pl
import jax.experimental.pallas.tpu as pltpu

F32 = jnp.float32
BF16 = jnp.bfloat16
U32 = jnp.uint32

_EPS = 1e-5
_MASKED = -1e9
_LOG2E = float(np.log2(np.e))
_GELU_C = float(np.sqrt(2.0 / np.pi))

LANE = 128
TM = 512
UNIT = 128
RC = 16
P = 4
PERIOD = 4


def _dot(a, b):
    return lax.dot_general(a, b, (((1,), (0,)), ((), ())), preferred_element_type=F32)


def _dot_nt(a, b):
    return lax.dot_general(a, b, (((1,), (1,)), ((), ())), preferred_element_type=F32)


def _bf(words):
    return pltpu.bitcast(words, BF16)


def _words(x):
    return pltpu.bitcast(x.astype(BF16), U32)


def _at(start, n, align=None):
    return pl.ds(start if isinstance(start, int) else pl.multiple_of(start, align or n), n)


def _tile(j):
    return _at(j * LANE, LANE)


def _split(x, n):
    k = x.shape[1] // n
    return [x[:, i * k:(i + 1) * k] for i in range(n)]


def _same(v):
    return v


def _moments(x, note=_same):
    inv_n = 1.0 / x.shape[-1]
    xc = x - note(jnp.sum(x, axis=-1, keepdims=True)) * inv_n
    return xc, note(jnp.sum(xc * xc, axis=-1, keepdims=True)) * inv_n


def _ln(x, note=_same):
    xc, var = _moments(x, note)
    return xc * lax.rsqrt(var + _EPS)


def _gelu2(x):
    return x * (1.0 + jnp.tanh(x * (_GELU_C + (_GELU_C * 0.044715) * (x * x))))


def _signed_sum(terms):
    terms = sorted(terms, key=lambda t: -t[0])
    assert terms[0][0] > 0
    total = terms[0][1]
    for sign, value in terms[1:]:
        total = total + value if sign > 0 else total - value
    return total


class _HopcroftKerr:
    def __init__(self, p, order=None):
        own = {0: ((1, 2, 1), (2, 0, 1)), 1: ((2, 1, -1), (0, 2, 1)), 2: ((1, 1, 1), (0, 0, 1))}
        cross = {(0, 1): ((1, 0, 1, 0, 1, -1), (0, -1, 0, -1, 0, 1, -1), (-1, 0, 1, 0, 1, 0, 1)),
                 (0, 2): ((2, 0, 1, 2, 1, 1), (-1, 0, 0, -1, 0, 1, -1), (0, -1, -1, 0, -1, 0, 1)),
                 (1, 2): ((2, 1, -1, 2, 0, 1), (0, -1, -1, 0, 1, 0, 1), (1, 0, 0, -1, 0, 1, -1))}
        products, diag, uses = [], {}, {}

        def product(left, out):
            products.append((left, out))
            return len(products) - 1

        def diagonal(idx, kind):
            diag[idx] = [product([(i, f, 1) for i in idx], [(i, g, 1) for i in idx]) for f, g, _ in own[kind]]

        def pair(a, ka, b, kb):
            if ka > kb:
                return pair(b, kb, a, ka)[::-1]
            (f0, f1, s, g0, g1, t), ab, ba = cross[ka, kb]
            diagonal(a + b, 3 - ka - kb)
            used = diag[a] + diag[b] + diag[a + b] + [product(
                [(i, f0, 1) for i in a] + [(i, f1, s) for i in b],
                [(i, g0, 1) for i in a] + [(i, g1, t) for i in b])]
            return dict(zip(used, ab)), dict(zip(used, ba))

        for i in range(p):
            diagonal((i,), i % 3)
            uses[i, i] = {r: sign for r, (_, _, sign) in zip(diag[i,], own[i % 3])}
        for j in range(p):
            for i in range(j):
                if i % 3 != j % 3:
                    uses[i, j], uses[j, i] = pair((i,), i % 3, (j,), j % 3)
        for j in range(p):
            for i in range(j % 3, j, 3):
                k = i + 1
                both = (i, k) if (i, k) in diag else (k, i)
                uses[i, j], uses[j, i] = pair(both, 3 - i % 3 - k % 3, (j,), j % 3)
                for ij, kj in (((i, j), (k, j)), ((j, i), (j, k))):
                    for r, c in uses[kj].items():
                        uses[ij][r] = uses[ij].get(r, 0) - c
        self.p = p
        self.order = order or range(len(products))
        self.products = [(left, [(i, j, c[r]) for (i, j), c in sorted(uses.items()) if c.get(r)], out)
                         for r, (left, out) in enumerate(products)]
        self.summed = [r for r, (_, weight, _) in enumerate(self.products) if len(weight) > 1]

    def left(self, upper, lower):
        forms = [(u, l, u - l) for u, l in zip(upper, lower)]
        return [_signed_sum([(sign, forms[i][f]) for i, f, sign in left]) for left, _, _ in self.products]

    def right(self, n, block):
        return _signed_sum([(sign, block(i, j).astype(F32)) for i, j, sign in self.products[self.summed[n]][1]])

    def accumulate(self, left, block, summed, acc=()):
        acc = dict(acc)
        for r in self.order:
            _, weight, out = self.products[r]
            if r in self.summed:
                flip, w = 1, summed(self.summed.index(r))
            else:
                flip, w = weight[0][2], block(*weight[0][:2])
            m = _dot(left(r), w)
            for j, f, sign in out:
                if (j, f) in acc:
                    acc[j, f] = acc[j, f] + m if sign * flip > 0 else acc[j, f] - m
                else:
                    acc[j, f] = m if sign * flip > 0 else -m
        return acc

    def result(self, acc):
        return [[functools.reduce(jnp.add, [acc[j, g] for g in (f, 2) if (j, g) in acc])
                 for j in range(self.p)] for f in range(2)]


_HK = _HopcroftKerr(P, (5, 18, 16, 9, 3, 15, 1, 24, 7, 19, 10, 0, 13, 14, 2, 22, 21, 12, 6, 20, 25, 23, 17, 4, 11, 8))
_HKQ = _HopcroftKerr(P, (10, 19, 18, 7, 16, 1, 2, 9, 5, 15, 23, 20, 11, 4, 17, 8, 22, 25, 0, 13, 21, 24, 14, 3, 12, 6))
_HK2 = _HopcroftKerr(2)


class _Pace:
    def __init__(self, never):
        self.never, self.noted, self.due, self.pos = never, [], [], 0

    def note(self, v):
        u = pltpu.bitcast(jnp.broadcast_to(v, (v.shape[0], max(v.shape[1], LANE))), U32)
        self.noted.append(functools.reduce(jnp.bitwise_or, [
            u[r:r + 8, c:c + LANE] for r in range(0, u.shape[0], 8) for c in range(0, u.shape[1], LANE)]))
        return v

    def spread(self, first, last):
        n = len(self.noted)
        self.due += [(self.pos + first + (k + 1) * (last - first) / n, v) for k, v in enumerate(self.noted)]
        self.due.sort(key=lambda t: t[0])
        self.noted = []

    def load(self, words):
        self.pos += words.shape[0] // (LANE // 2)
        hints = []
        while self.due and self.due[0][0] <= self.pos:
            hints.append(self.due.pop(0)[1])
        if hints:
            hint, parts = functools.reduce(jnp.bitwise_or, hints), []
            for k in range(0, words.shape[0], LANE // 2):
                parts += [jnp.where(self.never, hint, words[k:k + 8]), words[k + 8:k + LANE // 2]]
            words = jnp.concatenate(parts, axis=0)
        return _bf(words)


def _kernel(x_hbm, mem0_hbm, wq_hbm, wk_hbm, wv_hbm, wo_hbm, w1_hbm, w2_hbm, w3_hbm, w4_hbm,
            out_hbm,
            x_v, part_v, mem0_v, wqkv_v, wo_v, raw_v, w3_v, w4_v, s3_v, s4_v,
            sem_x, sem_mix, sem_mlp, sem_attn, sem_mem, sem_out, *, seg):
    S, D = x_hbm.shape
    H, Dh = wq_hbm.shape[-2:]
    M = mem0_hbm.shape[0]
    FF = w3_hbm.shape[1]
    L = M + seg
    n_blk = S // TM
    n_seg = S // seg
    n_grp = H // P
    n_prod = len(_HK.products)
    kw = D // 2 // P
    fw = FF // 2 // P
    ft = FF // P // LANE
    dt = D // P // LANE
    grows = P * Dh // 2

    def copy(hbm, vmem, sem, *idx):
        return pltpu.make_async_copy(hbm.bitcast(U32).at[idx], vmem.at[idx], sem)

    def attn_copies(g):
        copies = [copy(wo_hbm, wo_v, sem_attn.at[g], _at(g * grows, grows))]
        for m, hbm in enumerate((wq_hbm, wk_hbm, wv_hbm)):
            for j in range(P // 2):
                for par in range(2):
                    copies.append(pltpu.make_async_copy(
                        hbm.bitcast(U32).at[:, par, g * (P // 2) + j, :],
                        raw_v.at[g % 2, m * P + 2 * j + par], sem_attn.at[g]))
        return copies

    def mlp_copies(q):
        return [copy(hbm, vmem, sem_mlp.at[q], _at(i * n + q * (n // n_blk), n // n_blk, 8))
                for hbm, vmem, n in ((w3_hbm, w3_v, kw), (w4_hbm, w4_v, fw)) for i in range(P)]

    def out_copy(rows):
        return pltpu.make_async_copy(x_v.at[rows], out_hbm.bitcast(U32).at[rows], sem_out)

    mem0_copy = pltpu.make_async_copy(mem0_hbm, mem0_v, sem_mem)

    def x_rows(r0, n):
        return _bf(x_v[_at(r0 // 2, n // 2), :]).astype(F32)

    def store_left(hk, ref, rows, size, note):
        for q in range(0, size // 2, RC):
            for n, v in enumerate(hk.left(_split(rows(q), hk.p), _split(rows(size // 2 + q), hk.p))):
                ref.at[n][q // 2:(q + RC) // 2, :] = _words(v)
                if n >= len(hk.products) - 2:
                    note(v)

    def store_right(hk, ref, rows, block):
        out = []
        for n in range(len(hk.summed)):
            v = hk.right(n, block)
            ref[rows, _tile(n)] = _words(v)
            out.append(v[:8])
        return out

    def token_mixing(h_v, w_v, sums_v, left_v, first_v):
        pairs = D // 2 // LANE
        units = TM // UNIT
        loads = pairs * len(_HK2.products) * (D // 2 // LANE)

        def w_copies(n, j):
            return [copy((w1_hbm, w2_hbm)[n], w_v.at[n], sem_mix.at[n, j], slice(None), _tile(c * pairs + j))
                    for c in range(2)]

        def x_copy(i):
            return copy(x_hbm, x_v, sem_x.at[i + 1], _at(i * (TM // 2), TM // 2))

        def block(n, j, r=0, size=D // 4):
            return lambda a, c: w_v.at[n][a * (D // 4) + r:a * (D // 4) + r + size, _tile(c * pairs + j)]

        def prepare(j, r, size):
            store_right(_HK2, sums_v.at[1, j], slice(r, r + size), lambda a, c: _bf(block(1, j, r, size)(a, c)))

        def norm(r0, ref, size, note=_same):
            def rows(r):
                xc, var = _moments(x_rows(r0 + r, RC), note)
                inv = lax.rsqrt(var + _EPS)
                xn = xc * inv
                part_v[_at(r0 + r, RC), :] = xn
                return xn * lax.rsqrt(var * inv * inv + _EPS)
            store_left(_HK2, ref, rows, size, note)

        def shift(r0, ref, note=_same):
            def rows(r):
                parts = []
                for g, by in enumerate((-1, 1, -2, 2)):
                    c = slice(g * D // 4, (g + 1) * D // 4)
                    if by < 0:
                        parts.append(pltpu.roll(h_v[_at(r0 + r, RC + 8, 8), c], -by, 0)[8:])
                    else:
                        parts.append(pltpu.roll(h_v[_at(r0 + r + 8, RC + 8, 8), c], RC + 8 - by, 0)[:RC])
                return jnp.concatenate(parts, axis=1)
            store_left(_HK2, ref, rows, UNIT, note)

        def matmul(n, left, r0, load=_bf, arriving=False):
            for j in range(pairs):
                def summed(k):
                    if not arriving:
                        return load(sums_v.at[n, j][:, _tile(k)])
                    w = _HK2.right(k, lambda a, c: _bf(block(n, j)(a, c))).astype(BF16)
                    sums_v.at[n, j][:, _tile(k)] = pltpu.bitcast(w, U32)
                    return w

                if arriving:
                    for c in w_copies(n, j):
                        c.wait()
                halves = _HK2.result(_HK2.accumulate(
                    lambda r: _bf(left.at[r][...]), lambda a, c: load(block(n, j)(a, c)), summed))
                for f, half in enumerate(halves):
                    for c, v in enumerate(half):
                        size, lanes = v.shape[0], _tile(c * pairs + j)
                        if n == 0:
                            h_v[_at(8 + r0 + f * size, size, 8), lanes] = _gelu2(v)
                        else:
                            part_v[_at(r0 + f * size, size), lanes] += 0.5 * v

        def h_unit(r0, k, pace):
            norm(r0 + UNIT, left_v.at[(k + 1) % 2], UNIT, pace.note)
            pace.spread(0.1 * loads, loads)
            matmul(0, left_v.at[k % 2], r0, pace.load)

        def h_body(i, _):
            @pl.when(i + 2 < n_blk)
            def _():
                x_copy(i + 2).start()

            @pl.when(i + 1 < n_blk)
            def _():
                x_copy(i + 1).wait()

            for c in w_copies(1, i) + mlp_copies(i - 1):
                c.start()
            for c in w_copies(1, i - 1):
                c.wait()
            pace = _Pace(i < 0)
            for k in range(units):
                h_unit(i * TM + k * UNIT, k, pace)
                prepare(i - 1, k * (D // 4 // units), D // 4 // units)
            return 0

        def mix_body(i, _):
            @pl.when(i == 0)
            def _():
                for c in mlp_copies(n_blk - 1):
                    c.start()

            @pl.when(i == 1)
            def _():
                for c in attn_copies(0):
                    c.start()

            for c in mlp_copies(i):
                c.wait()

            def sums(w, ref, k, tiles, n, r):
                r += i * (k // n_blk)
                return jnp.concatenate(store_right(_HK, ref.at[n], _at(r, 8), lambda a, c: _bf(
                    w[_at(a * k + r, 8), _tile(c * tiles + n)])), axis=0)

            side = [functools.partial(sums, w, ref, k, tiles, n, r)
                    for w, ref, k, tiles in ((w3_v, s3_v, kw, ft), (w4_v, s4_v, fw, dt))
                    for n in range(tiles) for r in range(0, k // n_blk, 8)]
            pace = _Pace(i < 0)
            for k in range(units):
                r0 = i * TM + k * UNIT
                for task in side[k * len(side) // units:(k + 1) * len(side) // units]:
                    pace.note(task())
                pace.spread(0.05 * loads, loads)
                shift(jnp.minimum(r0 + UNIT, S - UNIT), left_v.at[(k + 1) % 2], pace.note)
                pace.spread(0.05 * loads, loads)
                matmul(1, left_v.at[k % 2], r0, pace.load)
            return 0

        first = [copy(x_hbm, x_v, sem_x.at[k], _at(k * TM // 4, TM // 4)) for k in range(2)]
        for c in ([first[0]] + sum((w_copies(0, j) for j in range(pairs)), [])
                  + [first[1], x_copy(1)] + w_copies(1, 0) + [x_copy(2), mem0_copy]):
            c.start()
        h_v[0:8, :] = jnp.zeros((8, D), F32)
        h_v[S + 8:S + 16, :] = jnp.zeros((8, D), F32)
        x_v[S // 2:, :] = jnp.zeros((UNIT // 2, D), U32)
        first[0].wait()
        norm(0, first_v, TM // 2)
        matmul(0, first_v, 0, arriving=True)
        first[1].wait()
        pace = _Pace(jnp.square(part_v[0:8, 0:LANE]) < 0)
        norm(TM // 2, left_v.at[units // 2 % 2], UNIT)
        for k in range(units // 2, units):
            if k == units - 1:
                x_copy(1).wait()
            h_unit(k * UNIT, k, pace)
        lax.fori_loop(1, n_blk, h_body, 0)
        shift(0, left_v.at[0])
        for c in w_copies(1, pairs - 1):
            c.wait()
        for r in range(0, D // 4, 32):
            prepare(pairs - 1, r, 32)
        lax.fori_loop(0, n_blk, mix_body, 0)

    def channel_mlp(sums_v, *buffers):
        left_v, hidden_v = buffers[:2], buffers[2:]
        units = S // UNIT // n_grp

        def norm(r0, slot, note=_same):
            store_left(_HK, left_v[slot], lambda r: _ln(part_v[_at(r0 + r, RC), :], note), UNIT, note)

        def body(g, _):
            @pl.when(g + 1 < n_grp)
            def _():
                for c in attn_copies(g + 1):
                    c.start()

            for c in attn_copies(g):
                c.wait()
            pace = _Pace(g < 0)

            def prepare_qkv(m, r):
                blocks = {}
                for j in range(0, P, 2):
                    for i in range(P):
                        rows = slice(i * kw + r, i * kw + r + 8)
                        even, odd = raw_v.at[g % 2, m * P + j][rows, :], raw_v.at[g % 2, m * P + j + 1][rows, :]
                        for n, w in enumerate(((even & jnp.uint32(0xFFFF)) | (odd << 16),
                                               (even >> 16) | (odd & jnp.uint32(0xFFFF0000)))):
                            wqkv_v[m * H + g * P + j + n, rows, :] = w
                            blocks[i, j + n] = _bf(w)
                return store_right(_HK, sums_v.at[m * n_grp + g], slice(r, r + 8), lambda i, j: blocks[i, j])

            def prepare_out(r):
                return store_right(_HK, sums_v.at[3 * n_grp + g], slice(r, r + 8), lambda i, j: _bf(
                    wo_v[_at(g * grows + i * (Dh // 2) + r % (Dh // 2), 8), _tile(j * dt + r // (Dh // 2))]))

            def up(k):
                for n in range(ft):
                    upper, lower = _HK.result(_HK.accumulate(
                        lambda r: _bf(left_v[k % 2].at[r][...]),
                        lambda i, j: pace.load(w3_v[i * kw:(i + 1) * kw, _tile(j * ft + n)]),
                        lambda r: pace.load(s3_v.at[n][:, _tile(r)])))
                    for r, v in enumerate(_HK.left([_gelu2(v) for v in upper], [_gelu2(v) for v in lower])):
                        hidden_v[k % 2].at[r][:, _tile(n)] = _words(v)
                        if r < 2 * P and r % 2 == 0 and (n + 1 < ft or k):
                            pace.note(v)
                    pace.spread(20, 50)

            def down(k):
                for n in range(dt):
                    halves = _HK.result(_HK.accumulate(
                        lambda r: _bf(hidden_v[k % 2].at[r][...]),
                        lambda i, j: pace.load(w4_v[i * fw:(i + 1) * fw, _tile(j * dt + n)]),
                        lambda r: pace.load(s4_v.at[n][:, _tile(r)])))
                    for f, half in enumerate(halves):
                        for j, v in enumerate(half):
                            rows = _at((g * units + k) * UNIT + f * (UNIT // 2), UNIT // 2)
                            part_v[rows, _tile(j * dt + n)] += 0.5 * v

            for m in range(3):
                for r in range(0, kw, 8):
                    pace.note(prepare_qkv(m, r)[0])
            for r in range(0, kw, 8):
                pace.note(prepare_out(r)[0])
            loads = units * 2 * ft * dt * n_prod
            pace.spread(0.64 * loads, 0.99 * loads)
            for k in range(units):
                norm((g * units + k + 1) * UNIT, (k + 1) % 2, pace.note)
                pace.spread(40, ft * dt * n_prod)
                up(k)
                if k > 0:
                    down(k - 1)
            down(units - 1)
            return 0

        norm(0, 0)
        lax.fori_loop(0, n_grp, body, 0)

    def recurrence(sums_v, own_v, left_v, next_v, hq_v, ho_v):
        scale = float(Dh) ** -0.5
        row = lax.broadcasted_iota(jnp.int32, (2 * L, 2 * L), 0)
        col = lax.broadcasted_iota(jnp.int32, (2 * L, 2 * L), 1)
        r_in = jnp.where(row >= L, row - L, row)
        c_in = jnp.where(col >= L, col - L, col)
        same_head = (row >= L) == (col >= L)
        keep = same_head & ((r_in < M) | (r_in >= c_in))
        fill = jnp.where(same_head, _MASKED / scale, -jnp.inf).astype(F32)

        def load_own(s):
            own_v[...] = _ln(x_rows(s * seg, seg)[:seg - 8])

        def load_next(s, q):
            next_v[8 * q:8 * q + 8, :] = _ln(x_rows(s * seg + seg - 16, 16)[8:])

        def load_left(mem):
            upper = jnp.concatenate([mem, own_v[...]], axis=0)
            for n, v in enumerate(_HK.left(_split(upper, P), _split(next_v[...], P))):
                left_v.at[n][...] = _words(v)

        def by_head(apart, dot, a, b):
            return jnp.concatenate([dot(a[:L], b), dot(a[L:], b)], axis=0) if apart else dot(a, b)

        def softmax(apart, q, k):
            s = jnp.where(keep, by_head(apart, _dot_nt, q, k.astype(BF16)), fill)
            e = jnp.exp2((s - jnp.max(s, axis=-1, keepdims=True)) * (scale * _LOG2E))
            return e, pl.reciprocal(jnp.sum(e, axis=-1, keepdims=True), full_range=False)

        def step(s, r, mem):
            first, last = r == 0, r == PERIOD - 1
            if not first:
                upper = jnp.concatenate([mem, own_v[...]], axis=0)
                early = {h: _dot(upper[:, :D // 2].astype(BF16), _bf(wqkv_v[h, :D // 4, :]))
                         for h in (0, 1, H, H + 1)}

            def plain(h):
                if h in early:
                    return early[h] + _dot(upper[:, D // 2:].astype(BF16), _bf(wqkv_v[h, D // 4:, :]))
                return _dot(upper.astype(BF16), _bf(wqkv_v[h]))

            def project(g):
                res = []
                for m in range(3):
                    h0 = m * H + g * P
                    if first:
                        tops, rest = _HKQ.result(_HKQ.accumulate(
                            lambda n: _bf(left_v.at[n][...]),
                            lambda i, j: _bf(wqkv_v[h0 + j, i * kw:(i + 1) * kw, :]),
                            lambda n: _bf(sums_v.at[m * n_grp + g][:, _tile(n)])))
                        for j in range(P):
                            hq_v[h0 + j] = rest[j][8:]
                        held = [v[:8] for v in rest]
                    else:
                        tops = [plain(h0 + j) for j in range(P)]
                        held = [hq_v[h0 + j, 8 * (r - 1):8 * r, :] for j in range(P)]
                    res.append([jnp.concatenate([tops[j], held[j], tops[j + 1], held[j + 1]], axis=0)
                                for j in range(0, P, 2)])
                return list(zip(*res))

            def merge(g, heads, acc):
                tops, held = [o[:L - 8] for o in heads], [o[L - 8:] for o in heads]
                if last:
                    left = _HK.left(tops, [jnp.concatenate([ho_v[:, _tile(g * P + j)], held[j]], axis=0)
                                           for j in range(P)])
                    k = Dh // 2
                    return _HK.accumulate(
                        lambda n: left[n].astype(BF16),
                        lambda i, j: _bf(wo_v[g * grows + i * k:g * grows + (i + 1) * k,
                                              j * dt * LANE:(j + 1) * dt * LANE]),
                        lambda n: jnp.concatenate([_bf(sums_v.at[3 * n_grp + g][c * k:(c + 1) * k, _tile(n)])
                                                   for c in range(dt)], axis=1),
                        acc or ())
                for j in range(P):
                    ho_v[8 * r:8 * r + 8, _tile(g * P + j)] = held[j]
                y = _dot(jnp.concatenate(tops, axis=1).astype(BF16), _bf(wo_v[g * grows:(g + 1) * grows, :]))
                return y if acc is None else acc + y

            lag, late = (4, (5, 6)) if last else (5, (4, 6)) if first else (5, (4, 5))
            qkv, prob, heads = {}, {}, {}
            acc, done = None, 0
            for t in range(n_grp + 3):
                if t < n_grp:
                    qkv[t] = project(t)
                while done < (t - lag + 1 if t < n_grp else (late + (n_grp,))[t - n_grp]):
                    acc = merge(done, heads.pop(done), acc)
                    done += 1
                if 0 <= t - 2 < n_grp:
                    heads[t - 2] = []
                    for (e, inv), (_, _, v) in zip(prob.pop(t - 2), qkv.pop(t - 2)):
                        o = by_head(t - 2 == n_grp - 1, _dot, e, v.astype(BF16)) * inv
                        heads[t - 2] += [o[:L], o[L:]]
                if 0 <= t - 1 < n_grp:
                    prob[t - 1] = [softmax(t == 1, q, k) for q, k, _ in qkv[t - 1]]
                if last and 1 <= t <= PERIOD:
                    load_next(jnp.minimum(s + t, n_seg - 1), t - 1)
                if t == n_grp - 1:
                    load_own(jnp.minimum(s + 1, n_seg - 1))
            if last:
                y, y_held = [jnp.concatenate(half, axis=1) for half in _HK.result(acc)]
                load_left(y[:M])
            else:
                y = acc
            base = x_rows(s * seg, seg) + part_v[_at(s * seg, seg), :]
            x_v[_at(s * (seg // 2), 8), :] = _words(base[:16] + y[M:M + 16])
            part_v[_at(s * seg + 16, 16), :] = jnp.concatenate([base[16:24] + y[M + 16:], base[24:]], axis=0)
            if last:
                for q in range(PERIOD):
                    r0 = (s - (PERIOD - 1) + q) * seg + 16
                    rest = part_v[_at(r0, 16), :]
                    x_v[_at(r0 // 2, 8), :] = _words(jnp.concatenate(
                        [rest[:8], rest[8:] + y_held[8 * q:8 * q + 8]], axis=0))
            return y[:M]

        def period(p, _):
            mem = None
            for r in range(PERIOD):
                mem = step(p * PERIOD + r, r, mem)
            out_copy(_at(p * (PERIOD * seg // 2), PERIOD * seg // 2)).start()
            return 0

        load_own(0)
        for q in range(PERIOD):
            load_next(q, q)
        mem0_copy.wait()
        load_left(mem0_v[...].astype(F32))
        lax.fori_loop(0, n_seg // PERIOD, period, 0)

    def with_attention_sums(sums_v):
        pl.run_scoped(
            functools.partial(channel_mlp, sums_v),
            *[pltpu.VMEM((n_prod, UNIT // 4, k // P), U32) for k in (D, D, FF, FF)])
        pl.run_scoped(
            functools.partial(recurrence, sums_v),
            pltpu.VMEM((seg - 8, D), F32),
            pltpu.VMEM((n_prod, (L - 8) // 2, D // P), U32),
            pltpu.VMEM((8 * PERIOD, D), F32),
            pltpu.VMEM((3 * H, 8 * (PERIOD - 1), Dh), F32),
            pltpu.VMEM((8 * (PERIOD - 1), H * Dh), F32))

    pl.run_scoped(
        token_mixing,
        pltpu.VMEM((S + 16, D), F32),
        pltpu.VMEM((2, D // 2, D), U32),
        pltpu.VMEM((2, D // 2 // LANE, D // 4, len(_HK2.summed) * LANE), U32),
        pltpu.VMEM((2, len(_HK2.products), UNIT // 4, D // 2), U32),
        pltpu.VMEM((len(_HK2.products), TM // 8, D // 2), U32))
    pl.run_scoped(with_attention_sums, pltpu.VMEM((4 * n_grp, kw, len(_HK.summed) * LANE), U32))
    out_copy(slice(0, S // 2)).wait()


@functools.partial(jax.jit, static_argnames=("A_seg_len",))
def pallas_parallel_sum__memory_aug_recurrent_mem_tr__mixer_s_mlp__prompt_kernel(
    A_x: jax.Array,
    A_mem0: jax.Array,
    A_Wq: jax.Array,
    A_Wk: jax.Array,
    A_Wv: jax.Array,
    A_Wo: jax.Array,
    A_seg_len: int,
    B_x: jax.Array,
    B_w1: jax.Array,
    B_w2: jax.Array,
    B_w3: jax.Array,
    B_w4: jax.Array,
):
    del B_x
    B, S, D = A_x.shape
    H, Dh = A_Wq.shape[1:]
    M = A_mem0.shape[1]
    FF = B_w3.shape[1]
    assert (B, S, D, H, Dh, M, A_seg_len) == (1, 2048, 1024, 32, 128, 8, 32)
    sums = len(_HK.summed) * LANE

    hbm = pl.BlockSpec(memory_space=pl.ANY)
    out = pl.pallas_call(
        functools.partial(_kernel, seg=A_seg_len),
        out_shape=jax.ShapeDtypeStruct((S, D), A_x.dtype),
        in_specs=[hbm] * 10,
        out_specs=hbm,
        scratch_shapes=[
            pltpu.VMEM(((S + UNIT) // 2, D), U32),
            pltpu.VMEM((S + UNIT, D), F32),
            pltpu.VMEM((M, D), A_mem0.dtype),
            pltpu.VMEM((3 * H, D // 2, Dh), U32),
            pltpu.VMEM((H * Dh // 2, D), U32),
            pltpu.VMEM((2, 3 * P, D // 2, Dh), U32),
            pltpu.VMEM((D // 2, FF), U32),
            pltpu.VMEM((FF // 2, D), U32),
            pltpu.VMEM((FF // P // LANE, D // 2 // P, sums), U32),
            pltpu.VMEM((D // P // LANE, FF // 2 // P, sums), U32),
            pltpu.SemaphoreType.DMA((S // TM + 1,)),
            pltpu.SemaphoreType.DMA((2, D // 2 // LANE)),
            pltpu.SemaphoreType.DMA((S // TM,)),
            pltpu.SemaphoreType.DMA((H // P,)),
            pltpu.SemaphoreType.DMA,
            pltpu.SemaphoreType.DMA,
        ],
        compiler_params=pltpu.CompilerParams(
            vmem_limit_bytes=127 * 1024 * 1024, disable_bounds_checks=True),
    )(A_x.reshape(S, D), A_mem0.reshape(M, D),
      *[w.reshape(D // 2, 2, H, Dh) for w in (A_Wq, A_Wk, A_Wv)],
      A_Wo.reshape(H * Dh, D), B_w1, B_w2, B_w3, B_w4)
    return out.reshape(B, S, D)
```

```python
import functools

import jax
import jax.numpy as jnp
import numpy as np
from jax import lax
import jax.experimental.pallas as pl
import jax.experimental.pallas.tpu as pltpu

F32 = jnp.float32
BF16 = jnp.bfloat16
U32 = jnp.uint32

_EPS = 1e-5
_MASKED = -1e9
_LOG2E = float(np.log2(np.e))
_GELU_C = float(np.sqrt(2.0 / np.pi))

LANE = 128
TM = 512
UNIT = 128
RC = 16
P = 4
PERIOD = 4


def _dot(a, b):
    return lax.dot_general(a, b, (((1,), (0,)), ((), ())), preferred_element_type=F32)


def _dot_nt(a, b):
    return lax.dot_general(a, b, (((1,), (1,)), ((), ())), preferred_element_type=F32)


def _bf(words):
    return pltpu.bitcast(words, BF16)


def _words(x):
    return pltpu.bitcast(x.astype(BF16), U32)


def _at(start, n, align=None):
    return pl.ds(start if isinstance(start, int) else pl.multiple_of(start, align or n), n)


def _tile(j):
    return _at(j * LANE, LANE)


def _split(x, n):
    k = x.shape[1] // n
    return [x[:, i * k:(i + 1) * k] for i in range(n)]


def _same(v):
    return v


def _moments(x, note=_same):
    inv_n = 1.0 / x.shape[-1]
    xc = x - note(jnp.sum(x, axis=-1, keepdims=True)) * inv_n
    return xc, note(jnp.sum(xc * xc, axis=-1, keepdims=True)) * inv_n


def _ln(x, note=_same):
    xc, var = _moments(x, note)
    return xc * lax.rsqrt(var + _EPS)


def _gelu2(x):
    return x * (1.0 + jnp.tanh(x * (_GELU_C + (_GELU_C * 0.044715) * (x * x))))


def _signed_sum(terms):
    terms = sorted(terms, key=lambda t: -t[0])
    assert terms[0][0] > 0
    total = terms[0][1]
    for sign, value in terms[1:]:
        total = total + value if sign > 0 else total - value
    return total


class _HopcroftKerr:
    def __init__(self, p, order=None):
        own = {0: ((1, 2, 1), (2, 0, 1)), 1: ((2, 1, -1), (0, 2, 1)), 2: ((1, 1, 1), (0, 0, 1))}
        cross = {(0, 1): ((1, 0, 1, 0, 1, -1), (0, -1, 0, -1, 0, 1, -1), (-1, 0, 1, 0, 1, 0, 1)),
                 (0, 2): ((2, 0, 1, 2, 1, 1), (-1, 0, 0, -1, 0, 1, -1), (0, -1, -1, 0, -1, 0, 1)),
                 (1, 2): ((2, 1, -1, 2, 0, 1), (0, -1, -1, 0, 1, 0, 1), (1, 0, 0, -1, 0, 1, -1))}
        products, diag, uses = [], {}, {}

        def product(left, out):
            products.append((left, out))
            return len(products) - 1

        def diagonal(idx, kind):
            diag[idx] = [product([(i, f, 1) for i in idx], [(i, g, 1) for i in idx]) for f, g, _ in own[kind]]

        def pair(a, ka, b, kb):
            if ka > kb:
                return pair(b, kb, a, ka)[::-1]
            (f0, f1, s, g0, g1, t), ab, ba = cross[ka, kb]
            diagonal(a + b, 3 - ka - kb)
            used = diag[a] + diag[b] + diag[a + b] + [product(
                [(i, f0, 1) for i in a] + [(i, f1, s) for i in b],
                [(i, g0, 1) for i in a] + [(i, g1, t) for i in b])]
            return dict(zip(used, ab)), dict(zip(used, ba))

        for i in range(p):
            diagonal((i,), i % 3)
            uses[i, i] = {r: sign for r, (_, _, sign) in zip(diag[i,], own[i % 3])}
        for j in range(p):
            for i in range(j):
                if i % 3 != j % 3:
                    uses[i, j], uses[j, i] = pair((i,), i % 3, (j,), j % 3)
        for j in range(p):
            for i in range(j % 3, j, 3):
                k = i + 1
                both = (i, k) if (i, k) in diag else (k, i)
                uses[i, j], uses[j, i] = pair(both, 3 - i % 3 - k % 3, (j,), j % 3)
                for ij, kj in (((i, j), (k, j)), ((j, i), (j, k))):
                    for r, c in uses[kj].items():
                        uses[ij][r] = uses[ij].get(r, 0) - c
        self.p = p
        self.order = order or range(len(products))
        self.products = [(left, [(i, j, c[r]) for (i, j), c in sorted(uses.items()) if c.get(r)], out)
                         for r, (left, out) in enumerate(products)]
        self.summed = [r for r, (_, weight, _) in enumerate(self.products) if len(weight) > 1]

    def left(self, upper, lower):
        forms = [(u, l, u - l) for u, l in zip(upper, lower)]
        return [_signed_sum([(sign, forms[i][f]) for i, f, sign in left]) for left, _, _ in self.products]

    def right(self, n, block):
        return _signed_sum([(sign, block(i, j).astype(F32)) for i, j, sign in self.products[self.summed[n]][1]])

    def accumulate(self, left, block, summed, acc=()):
        acc = dict(acc)
        for r in self.order:
            _, weight, out = self.products[r]
            if r in self.summed:
                flip, w = 1, summed(self.summed.index(r))
            else:
                flip, w = weight[0][2], block(*weight[0][:2])
            m = _dot(left(r), w)
            for j, f, sign in out:
                if (j, f) in acc:
                    acc[j, f] = acc[j, f] + m if sign * flip > 0 else acc[j, f] - m
                else:
                    acc[j, f] = m if sign * flip > 0 else -m
        return acc

    def result(self, acc):
        return [[functools.reduce(jnp.add, [acc[j, g] for g in (f, 2) if (j, g) in acc])
                 for j in range(self.p)] for f in range(2)]


_HK = _HopcroftKerr(P, (5, 18, 16, 9, 3, 15, 1, 24, 7, 19, 10, 0, 13, 14, 2, 22, 21, 12, 6, 20, 25, 23, 17, 4, 11, 8))
_HKQ = _HopcroftKerr(P, (10, 19, 18, 7, 16, 1, 2, 9, 5, 15, 23, 20, 11, 4, 17, 8, 22, 25, 0, 13, 21, 24, 14, 3, 12, 6))
_HK2 = _HopcroftKerr(2)


class _Pace:
    def __init__(self, never):
        self.never, self.noted, self.due, self.pos = never, [], [], 0

    def note(self, v):
        u = pltpu.bitcast(jnp.broadcast_to(v, (v.shape[0], max(v.shape[1], LANE))), U32)
        self.noted.append(functools.reduce(jnp.bitwise_or, [
            u[r:r + 8, c:c + LANE] for r in range(0, u.shape[0], 8) for c in range(0, u.shape[1], LANE)]))
        return v

    def spread(self, first, last):
        n = len(self.noted)
        self.due += [(self.pos + first + (k + 1) * (last - first) / n, v) for k, v in enumerate(self.noted)]
        self.due.sort(key=lambda t: t[0])
        self.noted = []

    def load(self, words):
        self.pos += words.shape[0] // (LANE // 2)
        hints = []
        while self.due and self.due[0][0] <= self.pos:
            hints.append(self.due.pop(0)[1])
        if hints:
            hint, parts = functools.reduce(jnp.bitwise_or, hints), []
            for k in range(0, words.shape[0], LANE // 2):
                parts += [jnp.where(self.never, hint, words[k:k + 8]), words[k + 8:k + LANE // 2]]
            words = jnp.concatenate(parts, axis=0)
        return _bf(words)


def _kernel(x_hbm, mem0_hbm, wq_hbm, wk_hbm, wv_hbm, wo_hbm, w1_hbm, w2_hbm, w3_hbm, w4_hbm,
            out_hbm,
            x_v, part_v, mem0_v, wqkv_v, wo_v, raw_v, w3_v, w4_v, s3_v, s4_v,
            sem_x, sem_mix, sem_mlp, sem_attn, sem_mem, sem_out, *, seg):
    S, D = x_hbm.shape
    H, Dh = wq_hbm.shape[-2:]
    M = mem0_hbm.shape[0]
    FF = w3_hbm.shape[1]
    L = M + seg
    n_blk = S // TM
    n_seg = S // seg
    n_grp = H // P
    n_prod = len(_HK.products)
    kw = D // 2 // P
    fw = FF // 2 // P
    ft = FF // P // LANE
    dt = D // P // LANE
    grows = P * Dh // 2

    def copy(hbm, vmem, sem, *idx):
        return pltpu.make_async_copy(hbm.bitcast(U32).at[idx], vmem.at[idx], sem)

    def attn_copies(g):
        copies = [copy(wo_hbm, wo_v, sem_attn.at[g], _at(g * grows, grows))]
        for m, hbm in enumerate((wq_hbm, wk_hbm, wv_hbm)):
            for j in range(P // 2):
                for par in range(2):
                    copies.append(pltpu.make_async_copy(
                        hbm.bitcast(U32).at[:, par, g * (P // 2) + j, :],
                        raw_v.at[g % 2, m * P + 2 * j + par], sem_attn.at[g]))
        return copies

    def mlp_copies(q):
        return [copy(hbm, vmem, sem_mlp.at[q], _at(i * n + q * (n // n_blk), n // n_blk, 8))
                for hbm, vmem, n in ((w3_hbm, w3_v, kw), (w4_hbm, w4_v, fw)) for i in range(P)]

    def out_copy(rows):
        return pltpu.make_async_copy(x_v.at[rows], out_hbm.bitcast(U32).at[rows], sem_out)

    mem0_copy = pltpu.make_async_copy(mem0_hbm, mem0_v, sem_mem)

    def x_rows(r0, n):
        return _bf(x_v[_at(r0 // 2, n // 2), :]).astype(F32)

    def store_left(hk, ref, rows, size, note):
        for q in range(0, size // 2, RC):
            for n, v in enumerate(hk.left(_split(rows(q), hk.p), _split(rows(size // 2 + q), hk.p))):
                ref.at[n][q // 2:(q + RC) // 2, :] = _words(v)
                if n >= len(hk.products) - 2:
                    note(v)

    def store_right(hk, ref, rows, block):
        out = []
        for n in range(len(hk.summed)):
            v = hk.right(n, block)
            ref[rows, _tile(n)] = _words(v)
            out.append(v[:8])
        return out

    def token_mixing(h_v, w_v, sums_v, left_v, first_v):
        pairs = D // 2 // LANE
        units = TM // UNIT
        loads = pairs * len(_HK2.products) * (D // 2 // LANE)

        def w_copies(n, j):
            return [copy((w1_hbm, w2_hbm)[n], w_v.at[n], sem_mix.at[n, j], slice(None), _tile(c * pairs + j))
                    for c in range(2)]

        def x_copy(i):
            return copy(x_hbm, x_v, sem_x.at[i + 1], slice((i * TM + UNIT) // 2, min(S, (i + 1) * TM + UNIT) // 2))

        def block(n, j, r=0, size=D // 4):
            return lambda a, c: w_v.at[n][a * (D // 4) + r:a * (D // 4) + r + size, _tile(c * pairs + j)]

        def prepare(j, r, size):
            store_right(_HK2, sums_v.at[1, j], slice(r, r + size), lambda a, c: _bf(block(1, j, r, size)(a, c)))

        def norm(r0, ref, size, note=_same):
            def rows(r):
                xc, var = _moments(x_rows(r0 + r, RC), note)
                inv = lax.rsqrt(var + _EPS)
                xn = xc * inv
                part_v[_at(r0 + r, RC), :] = xn
                return xn * lax.rsqrt(var * inv * inv + _EPS)
            store_left(_HK2, ref, rows, size, note)

        def shift(r0, ref, note=_same):
            def rows(r):
                return jnp.concatenate(
                    [h_v.at[c][pl.ds(r0 + r + 8 + (-1, 1, -2, 2)[4 * c * LANE // D], RC), :]
                     for c in range(D // LANE)], axis=1)
            store_left(_HK2, ref, rows, UNIT, note)

        def matmul(n, left, r0, load=_bf, arriving=False):
            for j in range(pairs):
                def summed(k):
                    if not arriving:
                        return load(sums_v.at[n, j][:, _tile(k)])
                    w = _HK2.right(k, lambda a, c: _bf(block(n, j)(a, c))).astype(BF16)
                    sums_v.at[n, j][:, _tile(k)] = pltpu.bitcast(w, U32)
                    return w

                if arriving:
                    for c in w_copies(n, j):
                        c.wait()
                halves = _HK2.result(_HK2.accumulate(
                    lambda r: _bf(left.at[r][...]), lambda a, c: load(block(n, j)(a, c)), summed))
                for f, half in enumerate(halves):
                    for c, v in enumerate(half):
                        size = v.shape[0]
                        if n == 0:
                            h_v.at[c * pairs + j][_at(8 + r0 + f * size, size, 8), :] = _gelu2(v)
                        else:
                            part_v[_at(r0 + f * size, size), _tile(c * pairs + j)] += 0.5 * v

        def h_unit(r0, k, pace):
            norm(r0 + UNIT, left_v.at[(k + 1) % 2], UNIT, pace.note)
            pace.spread(0.1 * loads, loads)
            matmul(0, left_v.at[k % 2], r0, pace.load)

        def h_body(i, _):
            for n in range(1, n_blk):
                @pl.when(i == n)
                def _():
                    for later in range(2, n_blk) if n == 1 else ():
                        for c in [x_copy(later)] + w_copies(1, later - 1):
                            c.start()
                    for c in w_copies(1, pairs - 1) if n == 2 else ():
                        c.start()
                    x_copy(n).wait()

            for c in mlp_copies(i - 1):
                c.start()
            for c in w_copies(1, i - 1):
                c.wait()
            pace = _Pace(i < 0)
            for k in range(units):
                h_unit(i * TM + k * UNIT, k, pace)
                prepare(i - 1, k * (D // 4 // units), D // 4 // units)
            return 0

        def mix_body(i, _):
            @pl.when(i == 0)
            def _():
                for c in mlp_copies(n_blk - 1):
                    c.start()

            @pl.when(i == 1)
            def _():
                for c in attn_copies(0):
                    c.start()

            for c in mlp_copies(i):
                c.wait()

            def sums(w, ref, k, tiles, n, r):
                r += i * (k // n_blk)
                return jnp.concatenate(store_right(_HK, ref.at[n], _at(r, 8), lambda a, c: _bf(
                    w[_at(a * k + r, 8), _tile(c * tiles + n)])), axis=0)

            side = [functools.partial(sums, w, ref, k, tiles, n, r)
                    for w, ref, k, tiles in ((w3_v, s3_v, kw, ft), (w4_v, s4_v, fw, dt))
                    for n in range(tiles) for r in range(0, k // n_blk, 8)]
            pace = _Pace(i < 0)
            for k in range(units):
                r0 = i * TM + k * UNIT
                for task in side[k * len(side) // units:(k + 1) * len(side) // units]:
                    pace.note(task())
                pace.spread(0.05 * loads, loads)
                shift(jnp.minimum(r0 + UNIT, S - UNIT), left_v.at[(k + 1) % 2], pace.note)
                pace.spread(0.05 * loads, loads)
                matmul(1, left_v.at[k % 2], r0, pace.load)
            return 0

        first = [copy(x_hbm, x_v, sem_x.at[k], rows)
                 for k, rows in enumerate((slice(0, TM // 4), slice(TM // 4, (TM + UNIT) // 2)))]
        for c in ([first[0]] + sum((w_copies(0, j) for j in range(pairs)), [])
                  + [first[1], x_copy(1)] + w_copies(1, 0) + [mem0_copy]):
            c.start()
        h_v[:, 0:8, :] = jnp.zeros((D // LANE, 8, LANE), F32)
        h_v[:, S + 8:S + 16, :] = jnp.zeros((D // LANE, 8, LANE), F32)
        x_v[S // 2:, :] = jnp.zeros((UNIT // 2, D), U32)
        first[0].wait()
        norm(0, first_v, TM // 2)
        matmul(0, first_v, 0, arriving=True)
        first[1].wait()
        pace = _Pace(jnp.square(part_v[0:8, 0:LANE]) < 0)
        norm(TM // 2, left_v.at[units // 2 % 2], UNIT)
        for k in range(units // 2, units):
            h_unit(k * UNIT, k, pace)
        lax.fori_loop(1, n_blk, h_body, 0)
        shift(0, left_v.at[0])
        for c in w_copies(1, pairs - 1):
            c.wait()
        for r in range(0, D // 4, 32):
            prepare(pairs - 1, r, 32)
        lax.fori_loop(0, n_blk, mix_body, 0)

    def channel_mlp(sums_v, *buffers):
        left_v, hidden_v = buffers[:2], buffers[2:]
        units = S // UNIT // n_grp

        def norm(r0, slot, note=_same):
            store_left(_HK, left_v[slot], lambda r: _ln(part_v[_at(r0 + r, RC), :], note), UNIT, note)

        def body(g, _):
            @pl.when(g + 1 < n_grp)
            def _():
                for c in attn_copies(g + 1):
                    c.start()

            for c in attn_copies(g):
                c.wait()
            pace = _Pace(g < 0)

            def prepare_qkv(m, r):
                blocks = {}
                for j in range(0, P, 2):
                    for i in range(P):
                        rows = slice(i * kw + r, i * kw + r + 8)
                        even, odd = raw_v.at[g % 2, m * P + j][rows, :], raw_v.at[g % 2, m * P + j + 1][rows, :]
                        for n, w in enumerate(((even & jnp.uint32(0xFFFF)) | (odd << 16),
                                               (even >> 16) | (odd & jnp.uint32(0xFFFF0000)))):
                            wqkv_v[m * H + g * P + j + n, rows, :] = w
                            blocks[i, j + n] = _bf(w)
                return store_right(_HK, sums_v.at[m * n_grp + g], slice(r, r + 8), lambda i, j: blocks[i, j])

            def prepare_out(r):
                return store_right(_HK, sums_v.at[3 * n_grp + g], slice(r, r + 8), lambda i, j: _bf(
                    wo_v[_at(g * grows + i * (Dh // 2) + r % (Dh // 2), 8), _tile(j * dt + r // (Dh // 2))]))

            def up(k):
                for n in range(ft):
                    upper, lower = _HK.result(_HK.accumulate(
                        lambda r: _bf(left_v[k % 2].at[r][...]),
                        lambda i, j: pace.load(w3_v[i * kw:(i + 1) * kw, _tile(j * ft + n)]),
                        lambda r: pace.load(s3_v.at[n][:, _tile(r)])))
                    for r, v in enumerate(_HK.left([_gelu2(v) for v in upper], [_gelu2(v) for v in lower])):
                        hidden_v[k % 2].at[r][:, _tile(n)] = _words(v)
                        if r < 2 * P and r % 2 == 0 and (n + 1 < ft or k):
                            pace.note(v)
                    pace.spread(20, 50)

            def down(k):
                for n in range(dt):
                    halves = _HK.result(_HK.accumulate(
                        lambda r: _bf(hidden_v[k % 2].at[r][...]),
                        lambda i, j: pace.load(w4_v[i * fw:(i + 1) * fw, _tile(j * dt + n)]),
                        lambda r: pace.load(s4_v.at[n][:, _tile(r)])))
                    for f, half in enumerate(halves):
                        for j, v in enumerate(half):
                            rows = _at((g * units + k) * UNIT + f * (UNIT // 2), UNIT // 2)
                            part_v[rows, _tile(j * dt + n)] += 0.5 * v

            for m in range(3):
                for r in range(0, kw, 8):
                    pace.note(prepare_qkv(m, r)[0])
            for r in range(0, kw, 8):
                pace.note(prepare_out(r)[0])
            loads = units * 2 * ft * dt * n_prod
            pace.spread(0.64 * loads, 0.99 * loads)
            for k in range(units):
                norm((g * units + k + 1) * UNIT, (k + 1) % 2, pace.note)
                pace.spread(40, ft * dt * n_prod)
                up(k)
                if k > 0:
                    down(k - 1)
            down(units - 1)
            return 0

        norm(0, 0)
        lax.fori_loop(0, n_grp, body, 0)

    def recurrence(sums_v, own_v, left_v, next_v, hq_v, ho_v):
        scale = float(Dh) ** -0.5
        row = lax.broadcasted_iota(jnp.int32, (2 * L, 2 * L), 0)
        col = lax.broadcasted_iota(jnp.int32, (2 * L, 2 * L), 1)
        r_in = jnp.where(row >= L, row - L, row)
        c_in = jnp.where(col >= L, col - L, col)
        same_head = (row >= L) == (col >= L)
        keep = same_head & ((r_in < M) | (r_in >= c_in))
        fill = jnp.where(same_head, _MASKED / scale, -jnp.inf).astype(F32)

        def load_own(s):
            own_v[...] = _ln(x_rows(s * seg, seg)[:seg - 8])

        def load_next(s, q):
            next_v[8 * q:8 * q + 8, :] = _ln(x_rows(s * seg + seg - 16, 16)[8:])

        def load_left(mem):
            upper = jnp.concatenate([mem, own_v[...]], axis=0)
            for n, v in enumerate(_HK.left(_split(upper, P), _split(next_v[...], P))):
                left_v.at[n][...] = _words(v)

        def by_head(apart, dot, a, b):
            return jnp.concatenate([dot(a[:L], b), dot(a[L:], b)], axis=0) if apart else dot(a, b)

        def softmax(apart, q, k):
            s = jnp.where(keep, by_head(apart, _dot_nt, q, k.astype(BF16)), fill)
            e = jnp.exp2((s - jnp.max(s, axis=-1, keepdims=True)) * (scale * _LOG2E))
            return e, pl.reciprocal(jnp.sum(e, axis=-1, keepdims=True), full_range=False)

        def step(s, r, mem):
            first, last = r == 0, r == PERIOD - 1
            if not first:
                upper = jnp.concatenate([mem, own_v[...]], axis=0)
                early = {h: _dot(upper[:, :D // 2].astype(BF16), _bf(wqkv_v[h, :D // 4, :]))
                         for h in (0, 1, H, H + 1)}

            def plain(h):
                if h in early:
                    return early[h] + _dot(upper[:, D // 2:].astype(BF16), _bf(wqkv_v[h, D // 4:, :]))
                return _dot(upper.astype(BF16), _bf(wqkv_v[h]))

            def project(g):
                res = []
                for m in range(3):
                    h0 = m * H + g * P
                    if first:
                        tops, rest = _HKQ.result(_HKQ.accumulate(
                            lambda n: _bf(left_v.at[n][...]),
                            lambda i, j: _bf(wqkv_v[h0 + j, i * kw:(i + 1) * kw, :]),
                            lambda n: _bf(sums_v.at[m * n_grp + g][:, _tile(n)])))
                        for j in range(P):
                            hq_v[h0 + j] = rest[j][8:]
                        held = [v[:8] for v in rest]
                    else:
                        tops = [plain(h0 + j) for j in range(P)]
                        held = [hq_v[h0 + j, 8 * (r - 1):8 * r, :] for j in range(P)]
                    res.append([jnp.concatenate([tops[j], held[j], tops[j + 1], held[j + 1]], axis=0)
                                for j in range(0, P, 2)])
                return list(zip(*res))

            def merge(g, heads, acc):
                tops, held = [o[:L - 8] for o in heads], [o[L - 8:] for o in heads]
                if last:
                    left = _HK.left(tops, [jnp.concatenate([ho_v[:, _tile(g * P + j)], held[j]], axis=0)
                                           for j in range(P)])
                    k = Dh // 2
                    return _HK.accumulate(
                        lambda n: left[n].astype(BF16),
                        lambda i, j: _bf(wo_v[g * grows + i * k:g * grows + (i + 1) * k,
                                              j * dt * LANE:(j + 1) * dt * LANE]),
                        lambda n: jnp.concatenate([_bf(sums_v.at[3 * n_grp + g][c * k:(c + 1) * k, _tile(n)])
                                                   for c in range(dt)], axis=1),
                        acc or ())
                for j in range(P):
                    ho_v[8 * r:8 * r + 8, _tile(g * P + j)] = held[j]
                y = _dot(jnp.concatenate(tops, axis=1).astype(BF16), _bf(wo_v[g * grows:(g + 1) * grows, :]))
                return y if acc is None else acc + y

            lag, late = (4, (5, 6)) if last else (5, (4, 6)) if first else (5, (4, 5))
            qkv, prob, heads = {}, {}, {}
            acc, done = None, 0
            for t in range(n_grp + 3):
                if t < n_grp:
                    qkv[t] = project(t)
                while done < (t - lag + 1 if t < n_grp else (late + (n_grp,))[t - n_grp]):
                    acc = merge(done, heads.pop(done), acc)
                    done += 1
                if 0 <= t - 2 < n_grp:
                    heads[t - 2] = []
                    for (e, inv), (_, _, v) in zip(prob.pop(t - 2), qkv.pop(t - 2)):
                        o = by_head(t - 2 == n_grp - 1, _dot, e, v.astype(BF16)) * inv
                        heads[t - 2] += [o[:L], o[L:]]
                if 0 <= t - 1 < n_grp:
                    prob[t - 1] = [softmax(t == 1, q, k) for q, k, _ in qkv[t - 1]]
                if last and 1 <= t <= PERIOD:
                    load_next(jnp.minimum(s + t, n_seg - 1), t - 1)
                if t == n_grp - 1:
                    load_own(jnp.minimum(s + 1, n_seg - 1))
            if last:
                y, y_held = [jnp.concatenate(half, axis=1) for half in _HK.result(acc)]
                load_left(y[:M])
            else:
                y = acc
            base = x_rows(s * seg, seg) + part_v[_at(s * seg, seg), :]
            x_v[_at(s * (seg // 2), 8), :] = _words(base[:16] + y[M:M + 16])
            part_v[_at(s * seg + 16, 16), :] = jnp.concatenate([base[16:24] + y[M + 16:], base[24:]], axis=0)
            if last:
                for q in range(PERIOD):
                    r0 = (s - (PERIOD - 1) + q) * seg + 16
                    rest = part_v[_at(r0, 16), :]
                    x_v[_at(r0 // 2, 8), :] = _words(jnp.concatenate(
                        [rest[:8], rest[8:] + y_held[8 * q:8 * q + 8]], axis=0))
            return y[:M]

        def period(p, _):
            mem = None
            for r in range(PERIOD):
                mem = step(p * PERIOD + r, r, mem)
            out_copy(_at(p * (PERIOD * seg // 2), PERIOD * seg // 2)).start()
            return 0

        load_own(0)
        for q in range(PERIOD):
            load_next(q, q)
        mem0_copy.wait()
        load_left(mem0_v[...].astype(F32))
        lax.fori_loop(0, n_seg // PERIOD, period, 0)

    def with_attention_sums(sums_v):
        pl.run_scoped(
            functools.partial(channel_mlp, sums_v),
            *[pltpu.VMEM((n_prod, UNIT // 4, k // P), U32) for k in (D, D, FF, FF)])
        pl.run_scoped(
            functools.partial(recurrence, sums_v),
            pltpu.VMEM((seg - 8, D), F32),
            pltpu.VMEM((n_prod, (L - 8) // 2, D // P), U32),
            pltpu.VMEM((8 * PERIOD, D), F32),
            pltpu.VMEM((3 * H, 8 * (PERIOD - 1), Dh), F32),
            pltpu.VMEM((8 * (PERIOD - 1), H * Dh), F32))

    pl.run_scoped(
        token_mixing,
        pltpu.VMEM((D // LANE, S + 16, LANE), F32),
        pltpu.VMEM((2, D // 2, D), U32),
        pltpu.VMEM((2, D // 2 // LANE, D // 4, len(_HK2.summed) * LANE), U32),
        pltpu.VMEM((2, len(_HK2.products), UNIT // 4, D // 2), U32),
        pltpu.VMEM((len(_HK2.products), TM // 8, D // 2), U32))
    pl.run_scoped(with_attention_sums, pltpu.VMEM((4 * n_grp, kw, len(_HK.summed) * LANE), U32))
    out_copy(slice(0, S // 2)).wait()


@functools.partial(jax.jit, static_argnames=("A_seg_len",))
def pallas_parallel_sum__memory_aug_recurrent_mem_tr__mixer_s_mlp__prompt_kernel(
    A_x: jax.Array,
    A_mem0: jax.Array,
    A_Wq: jax.Array,
    A_Wk: jax.Array,
    A_Wv: jax.Array,
    A_Wo: jax.Array,
    A_seg_len: int,
    B_x: jax.Array,
    B_w1: jax.Array,
    B_w2: jax.Array,
    B_w3: jax.Array,
    B_w4: jax.Array,
):
    del B_x
    B, S, D = A_x.shape
    H, Dh = A_Wq.shape[1:]
    M = A_mem0.shape[1]
    FF = B_w3.shape[1]
    assert (B, S, D, H, Dh, M, A_seg_len) == (1, 2048, 1024, 32, 128, 8, 32)
    sums = len(_HK.summed) * LANE

    hbm = pl.BlockSpec(memory_space=pl.ANY)
    out = pl.pallas_call(
        functools.partial(_kernel, seg=A_seg_len),
        out_shape=jax.ShapeDtypeStruct((S, D), A_x.dtype),
        in_specs=[hbm] * 10,
        out_specs=hbm,
        scratch_shapes=[
            pltpu.VMEM(((S + UNIT) // 2, D), U32),
            pltpu.VMEM((S + UNIT, D), F32),
            pltpu.VMEM((M, D), A_mem0.dtype),
            pltpu.VMEM((3 * H, D // 2, Dh), U32),
            pltpu.VMEM((H * Dh // 2, D), U32),
            pltpu.VMEM((2, 3 * P, D // 2, Dh), U32),
            pltpu.VMEM((D // 2, FF), U32),
            pltpu.VMEM((FF // 2, D), U32),
            pltpu.VMEM((FF // P // LANE, D // 2 // P, sums), U32),
            pltpu.VMEM((D // P // LANE, FF // 2 // P, sums), U32),
            pltpu.SemaphoreType.DMA((S // TM + 1,)),
            pltpu.SemaphoreType.DMA((2, D // 2 // LANE)),
            pltpu.SemaphoreType.DMA((S // TM,)),
            pltpu.SemaphoreType.DMA((H // P,)),
            pltpu.SemaphoreType.DMA,
            pltpu.SemaphoreType.DMA,
        ],
        compiler_params=pltpu.CompilerParams(
            vmem_limit_bytes=127 * 1024 * 1024, disable_bounds_checks=True),
    )(A_x.reshape(S, D), A_mem0.reshape(M, D),
      *[w.reshape(D // 2, 2, H, Dh) for w in (A_Wq, A_Wk, A_Wv)],
      A_Wo.reshape(H * Dh, D), B_w1, B_w2, B_w3, B_w4)
    return out.reshape(B, S, D)
```

```python
import functools

import jax
import jax.numpy as jnp
import numpy as np
from jax import lax
import jax.experimental.pallas as pl
import jax.experimental.pallas.tpu as pltpu

F32 = jnp.float32
BF16 = jnp.bfloat16
U32 = jnp.uint32

_EPS = 1e-5
_MASKED = -1e9
_LOG2E = float(np.log2(np.e))
_GELU_C = float(np.sqrt(2.0 / np.pi))

LANE = 128
TM = 512
UNIT = 128
RC = 16
P = 4
PERIOD = 4
AHEAD = {(0, 8): 12, (1, 8): 8, (2, 8): 8, (3, 5): 2, (3, 6): 10, (3, 7): 8, (3, 8): 12}
FIRST_AHEAD = 8
ENDS = (1, 4, 5, 7)
LAGS = ((5, (4, 6)), (5, (4, 5)), (4, (5, 6)))


def _dot(a, b):
    return lax.dot_general(a, b, (((1,), (0,)), ((), ())), preferred_element_type=F32)


def _dot_nt(a, b):
    return lax.dot_general(a, b, (((1,), (1,)), ((), ())), preferred_element_type=F32)


def _bf(words):
    return pltpu.bitcast(words, BF16)


def _words(x):
    return pltpu.bitcast(x.astype(BF16), U32)


def _at(start, n, align=None):
    return pl.ds(start if isinstance(start, int) else pl.multiple_of(start, align or n), n)


def _tile(j):
    return _at(j * LANE, LANE)


def _split(x, n):
    k = x.shape[1] // n
    return [x[:, i * k:(i + 1) * k] for i in range(n)]


def _same(v):
    return v


def _moments(x, note=_same):
    inv_n = 1.0 / x.shape[-1]
    xc = x - note(jnp.sum(x, axis=-1, keepdims=True)) * inv_n
    return xc, note(jnp.sum(xc * xc, axis=-1, keepdims=True)) * inv_n


def _ln(x, note=_same):
    xc, var = _moments(x, note)
    return xc * lax.rsqrt(var + _EPS)


def _gelu2(x):
    return x * (1.0 + jnp.tanh(x * (_GELU_C + (_GELU_C * 0.044715) * (x * x))))


def _signed_sum(terms):
    terms = sorted(terms, key=lambda t: -t[0])
    assert terms[0][0] > 0
    total = terms[0][1]
    for sign, value in terms[1:]:
        total = total + value if sign > 0 else total - value
    return total


class _HopcroftKerr:
    def __init__(self, p, order=None):
        own = {0: ((1, 2, 1), (2, 0, 1)), 1: ((2, 1, -1), (0, 2, 1)), 2: ((1, 1, 1), (0, 0, 1))}
        cross = {(0, 1): ((1, 0, 1, 0, 1, -1), (0, -1, 0, -1, 0, 1, -1), (-1, 0, 1, 0, 1, 0, 1)),
                 (0, 2): ((2, 0, 1, 2, 1, 1), (-1, 0, 0, -1, 0, 1, -1), (0, -1, -1, 0, -1, 0, 1)),
                 (1, 2): ((2, 1, -1, 2, 0, 1), (0, -1, -1, 0, 1, 0, 1), (1, 0, 0, -1, 0, 1, -1))}
        products, diag, uses = [], {}, {}

        def product(left, out):
            products.append((left, out))
            return len(products) - 1

        def diagonal(idx, kind):
            diag[idx] = [product([(i, f, 1) for i in idx], [(i, g, 1) for i in idx]) for f, g, _ in own[kind]]

        def pair(a, ka, b, kb):
            if ka > kb:
                return pair(b, kb, a, ka)[::-1]
            (f0, f1, s, g0, g1, t), ab, ba = cross[ka, kb]
            diagonal(a + b, 3 - ka - kb)
            used = diag[a] + diag[b] + diag[a + b] + [product(
                [(i, f0, 1) for i in a] + [(i, f1, s) for i in b],
                [(i, g0, 1) for i in a] + [(i, g1, t) for i in b])]
            return dict(zip(used, ab)), dict(zip(used, ba))

        for i in range(p):
            diagonal((i,), i % 3)
            uses[i, i] = {r: sign for r, (_, _, sign) in zip(diag[i,], own[i % 3])}
        for j in range(p):
            for i in range(j):
                if i % 3 != j % 3:
                    uses[i, j], uses[j, i] = pair((i,), i % 3, (j,), j % 3)
        for j in range(p):
            for i in range(j % 3, j, 3):
                k = i + 1
                both = (i, k) if (i, k) in diag else (k, i)
                uses[i, j], uses[j, i] = pair(both, 3 - i % 3 - k % 3, (j,), j % 3)
                for ij, kj in (((i, j), (k, j)), ((j, i), (j, k))):
                    for r, c in uses[kj].items():
                        uses[ij][r] = uses[ij].get(r, 0) - c
        self.p = p
        self.order = order or range(len(products))
        self.products = [(left, [(i, j, c[r]) for (i, j), c in sorted(uses.items()) if c.get(r)], out)
                         for r, (left, out) in enumerate(products)]
        self.summed = [r for r, (_, weight, _) in enumerate(self.products) if len(weight) > 1]
        self.lower = [r for r in self.order if all(f == 1 for _, f, _ in self.products[r][0])]

    def left(self, upper, lower):
        forms = [(u, l, u - l) for u, l in zip(upper, lower)]
        return [_signed_sum([(sign, forms[i][f]) for i, f, sign in left]) for left, _, _ in self.products]

    def right(self, n, block):
        return _signed_sum([(sign, block(i, j).astype(F32)) for i, j, sign in self.products[self.summed[n]][1]])

    def product(self, r, left, block, summed):
        w = summed(self.summed.index(r)) if r in self.summed else block(*self.products[r][1][0][:2])
        return _dot(left(r), w)

    def accumulate(self, left, block, summed, acc=(), known=()):
        acc = dict(acc)
        for r in self.order:
            _, weight, out = self.products[r]
            flip = 1 if r in self.summed else weight[0][2]
            m = known[r][...] if r in known else self.product(r, left, block, summed)
            for j, f, sign in out:
                if (j, f) in acc:
                    acc[j, f] = acc[j, f] + m if sign * flip > 0 else acc[j, f] - m
                else:
                    acc[j, f] = m if sign * flip > 0 else -m
        return acc

    def result(self, acc):
        return [[functools.reduce(jnp.add, [acc[j, g] for g in (f, 2) if (j, g) in acc])
                 for j in range(self.p)] for f in range(2)]


_HK = _HopcroftKerr(P, (5, 18, 16, 9, 3, 15, 1, 24, 7, 19, 10, 0, 13, 14, 2, 22, 21, 12, 6, 20, 25, 23, 17, 4, 11, 8))
_HKQ = _HopcroftKerr(P, (10, 19, 18, 7, 16, 1, 2, 9, 5, 15, 23, 20, 11, 4, 17, 8, 22, 25, 0, 13, 21, 24, 14, 3, 12, 6))
_HK2 = _HopcroftKerr(2)


class _Pace:
    def __init__(self, never):
        self.never, self.noted, self.due, self.pos = never, [], [], 0

    def note(self, v):
        u = pltpu.bitcast(jnp.broadcast_to(v, (v.shape[0], max(v.shape[1], LANE))), U32)
        self.noted.append(functools.reduce(jnp.bitwise_or, [
            u[r:r + 8, c:c + LANE] for r in range(0, u.shape[0], 8) for c in range(0, u.shape[1], LANE)]))
        return v

    def spread(self, first, last):
        n = len(self.noted)
        self.due += [(self.pos + first + (k + 1) * (last - first) / n, v) for k, v in enumerate(self.noted)]
        self.due.sort(key=lambda t: t[0])
        self.noted = []

    def load(self, words):
        self.pos += words.shape[0] // (LANE // 2)
        hints = []
        while self.due and self.due[0][0] <= self.pos:
            hints.append(self.due.pop(0)[1])
        if hints:
            hint, parts = functools.reduce(jnp.bitwise_or, hints), []
            for k in range(0, words.shape[0], LANE // 2):
                parts += [jnp.where(self.never, hint, words[k:k + 8]), words[k + 8:k + LANE // 2]]
            words = jnp.concatenate(parts, axis=0)
        return _bf(words)


def _kernel(x_hbm, mem0_hbm, wq_hbm, wk_hbm, wv_hbm, wo_hbm, w1_hbm, w2_hbm, w3_hbm, w4_hbm,
            out_hbm,
            x_v, part_v, mem0_v, wqkv_v, wo_v, raw_v, w3_v, w4_v, s3_v, s4_v,
            sem_x, sem_mix, sem_mlp, sem_attn, sem_mem, sem_out, *, seg):
    S, D = x_hbm.shape
    H, Dh = wq_hbm.shape[-2:]
    M = mem0_hbm.shape[0]
    FF = w3_hbm.shape[1]
    L = M + seg
    n_blk = S // TM
    n_seg = S // seg
    n_grp = H // P
    n_prod = len(_HK.products)
    kw = D // 2 // P
    fw = FF // 2 // P
    ft = FF // P // LANE
    dt = D // P // LANE
    grows = P * Dh // 2

    def copy(hbm, vmem, sem, *idx):
        return pltpu.make_async_copy(hbm.bitcast(U32).at[idx], vmem.at[idx], sem)

    def attn_copies(g):
        copies = [copy(wo_hbm, wo_v, sem_attn.at[g], _at(g * grows, grows))]
        for m, hbm in enumerate((wq_hbm, wk_hbm, wv_hbm)):
            for j in range(P // 2):
                for par in range(2):
                    copies.append(pltpu.make_async_copy(
                        hbm.bitcast(U32).at[:, par, g * (P // 2) + j, :],
                        raw_v.at[g % 2, m * P + 2 * j + par], sem_attn.at[g]))
        return copies

    def mlp_copies(q):
        return [copy(hbm, vmem, sem_mlp.at[q], _at(i * n + q * (n // n_blk), n // n_blk, 8))
                for hbm, vmem, n in ((w3_hbm, w3_v, kw), (w4_hbm, w4_v, fw)) for i in range(P)]

    def out_copy(rows):
        return pltpu.make_async_copy(x_v.at[rows], out_hbm.bitcast(U32).at[rows], sem_out)

    mem0_copy = pltpu.make_async_copy(mem0_hbm, mem0_v, sem_mem)

    def x_rows(r0, n):
        return _bf(x_v[_at(r0 // 2, n // 2), :]).astype(F32)

    def store_left(hk, ref, rows, size, note):
        for q in range(0, size // 2, RC):
            for n, v in enumerate(hk.left(_split(rows(q), hk.p), _split(rows(size // 2 + q), hk.p))):
                ref.at[n][q // 2:(q + RC) // 2, :] = _words(v)
                if n >= len(hk.products) - 2:
                    note(v)

    def store_right(hk, ref, rows, block):
        out = []
        for n in range(len(hk.summed)):
            v = hk.right(n, block)
            ref[rows, _tile(n)] = _words(v)
            out.append(v[:8])
        return out

    def token_mixing(h_v, w_v, sums_v, left_v, first_v):
        pairs = D // 2 // LANE
        units = TM // UNIT
        loads = pairs * len(_HK2.products) * (D // 2 // LANE)

        def w_copies(n, j):
            return [copy((w1_hbm, w2_hbm)[n], w_v.at[n], sem_mix.at[n, j], slice(None), _tile(c * pairs + j))
                    for c in range(2)]

        def x_copy(i):
            return copy(x_hbm, x_v, sem_x.at[i + 1], slice((i * TM + UNIT) // 2, min(S, (i + 1) * TM + UNIT) // 2))

        def block(n, j, r=0, size=D // 4):
            return lambda a, c: w_v.at[n][a * (D // 4) + r:a * (D // 4) + r + size, _tile(c * pairs + j)]

        def prepare(j, r, size):
            store_right(_HK2, sums_v.at[1, j], slice(r, r + size), lambda a, c: _bf(block(1, j, r, size)(a, c)))

        def norm(r0, ref, size, note=_same):
            def rows(r):
                xc, var = _moments(x_rows(r0 + r, RC), note)
                inv = lax.rsqrt(var + _EPS)
                xn = xc * inv
                part_v[_at(r0 + r, RC), :] = xn
                return xn * lax.rsqrt(var * inv * inv + _EPS)
            store_left(_HK2, ref, rows, size, note)

        def shift(r0, ref, note=_same):
            def rows(r):
                return jnp.concatenate(
                    [h_v.at[c][pl.ds(r0 + r + 8 + (-1, 1, -2, 2)[4 * c * LANE // D], RC), :]
                     for c in range(D // LANE)], axis=1)
            store_left(_HK2, ref, rows, UNIT, note)

        def matmul(n, left, r0, load=_bf, arriving=False):
            for j in range(pairs):
                def summed(k):
                    if not arriving:
                        return load(sums_v.at[n, j][:, _tile(k)])
                    w = _HK2.right(k, lambda a, c: _bf(block(n, j)(a, c))).astype(BF16)
                    sums_v.at[n, j][:, _tile(k)] = pltpu.bitcast(w, U32)
                    return w

                if arriving:
                    for c in w_copies(n, j):
                        c.wait()
                halves = _HK2.result(_HK2.accumulate(
                    lambda r: _bf(left.at[r][...]), lambda a, c: load(block(n, j)(a, c)), summed))
                for f, half in enumerate(halves):
                    for c, v in enumerate(half):
                        size = v.shape[0]
                        if n == 0:
                            h_v.at[c * pairs + j][_at(8 + r0 + f * size, size, 8), :] = _gelu2(v)
                        else:
                            part_v[_at(r0 + f * size, size), _tile(c * pairs + j)] += 0.5 * v

        def h_unit(r0, k, pace):
            norm(r0 + UNIT, left_v.at[(k + 1) % 2], UNIT, pace.note)
            pace.spread(0.1 * loads, loads)
            matmul(0, left_v.at[k % 2], r0, pace.load)

        def h_body(i, _):
            for n in range(1, n_blk):
                @pl.when(i == n)
                def _():
                    for later in range(2, n_blk) if n == 1 else ():
                        for c in [x_copy(later)] + w_copies(1, later - 1):
                            c.start()
                    for c in w_copies(1, pairs - 1) if n == 2 else ():
                        c.start()
                    x_copy(n).wait()

            for c in mlp_copies(i - 1):
                c.start()
            for c in w_copies(1, i - 1):
                c.wait()
            pace = _Pace(i < 0)
            for k in range(units):
                h_unit(i * TM + k * UNIT, k, pace)
                prepare(i - 1, k * (D // 4 // units), D // 4 // units)
            return 0

        def mix_body(i, _):
            @pl.when(i == 0)
            def _():
                for c in mlp_copies(n_blk - 1):
                    c.start()

            @pl.when(i == 1)
            def _():
                for c in attn_copies(0):
                    c.start()

            for c in mlp_copies(i):
                c.wait()

            def sums(w, ref, k, tiles, n, r):
                r += i * (k // n_blk)
                return jnp.concatenate(store_right(_HK, ref.at[n], _at(r, 8), lambda a, c: _bf(
                    w[_at(a * k + r, 8), _tile(c * tiles + n)])), axis=0)

            side = [functools.partial(sums, w, ref, k, tiles, n, r)
                    for w, ref, k, tiles in ((w3_v, s3_v, kw, ft), (w4_v, s4_v, fw, dt))
                    for n in range(tiles) for r in range(0, k // n_blk, 8)]
            pace = _Pace(i < 0)
            for k in range(units):
                r0 = i * TM + k * UNIT
                for task in side[k * len(side) // units:(k + 1) * len(side) // units]:
                    pace.note(task())
                pace.spread(0.05 * loads, loads)
                shift(jnp.minimum(r0 + UNIT, S - UNIT), left_v.at[(k + 1) % 2], pace.note)
                pace.spread(0.05 * loads, loads)
                matmul(1, left_v.at[k % 2], r0, pace.load)
            return 0

        first = [copy(x_hbm, x_v, sem_x.at[k], rows)
                 for k, rows in enumerate((slice(0, TM // 4), slice(TM // 4, (TM + UNIT) // 2)))]
        for c in ([first[0]] + sum((w_copies(0, j) for j in range(pairs)), [])
                  + [first[1], x_copy(1)] + w_copies(1, 0) + [mem0_copy]):
            c.start()
        h_v[:, 0:8, :] = jnp.zeros((D // LANE, 8, LANE), F32)
        h_v[:, S + 8:S + 16, :] = jnp.zeros((D // LANE, 8, LANE), F32)
        x_v[S // 2:, :] = jnp.zeros((UNIT // 2, D), U32)
        first[0].wait()
        norm(0, first_v, TM // 2)
        matmul(0, first_v, 0, arriving=True)
        first[1].wait()
        pace = _Pace(jnp.square(part_v[0:8, 0:LANE]) < 0)
        norm(TM // 2, left_v.at[units // 2 % 2], UNIT)
        for k in range(units // 2, units):
            h_unit(k * UNIT, k, pace)
        lax.fori_loop(1, n_blk, h_body, 0)
        shift(0, left_v.at[0])
        for c in w_copies(1, pairs - 1):
            c.wait()
        for r in range(0, D // 4, 32):
            prepare(pairs - 1, r, 32)
        lax.fori_loop(0, n_blk, mix_body, 0)

    def channel_mlp(sums_v, *buffers):
        left_v, hidden_v = buffers[:2], buffers[2:]
        units = S // UNIT // n_grp

        def norm(r0, slot, note=_same):
            store_left(_HK, left_v[slot], lambda r: _ln(part_v[_at(r0 + r, RC), :], note), UNIT, note)

        def body(g, _):
            @pl.when(g + 1 < n_grp)
            def _():
                for c in attn_copies(g + 1):
                    c.start()

            for c in attn_copies(g):
                c.wait()
            pace = _Pace(g < 0)

            def prepare_qkv(m, r):
                blocks = {}
                for j in range(0, P, 2):
                    for i in range(P):
                        rows = slice(i * kw + r, i * kw + r + 8)
                        even, odd = raw_v.at[g % 2, m * P + j][rows, :], raw_v.at[g % 2, m * P + j + 1][rows, :]
                        for n, w in enumerate(((even & jnp.uint32(0xFFFF)) | (odd << 16),
                                               (even >> 16) | (odd & jnp.uint32(0xFFFF0000)))):
                            wqkv_v[m * H + g * P + j + n, rows, :] = w
                            blocks[i, j + n] = _bf(w)
                return store_right(_HK, sums_v.at[m * n_grp + g], slice(r, r + 8), lambda i, j: blocks[i, j])

            def prepare_out(r):
                return store_right(_HK, sums_v.at[3 * n_grp + g], slice(r, r + 8), lambda i, j: _bf(
                    wo_v[_at(g * grows + i * (Dh // 2) + r % (Dh // 2), 8), _tile(j * dt + r // (Dh // 2))]))

            def up(k):
                for n in range(ft):
                    upper, lower = _HK.result(_HK.accumulate(
                        lambda r: _bf(left_v[k % 2].at[r][...]),
                        lambda i, j: pace.load(w3_v[i * kw:(i + 1) * kw, _tile(j * ft + n)]),
                        lambda r: pace.load(s3_v.at[n][:, _tile(r)])))
                    for r, v in enumerate(_HK.left([_gelu2(v) for v in upper], [_gelu2(v) for v in lower])):
                        hidden_v[k % 2].at[r][:, _tile(n)] = _words(v)
                        if r < 2 * P and r % 2 == 0 and (n + 1 < ft or k):
                            pace.note(v)
                    pace.spread(20, 50)

            def down(k):
                for n in range(dt):
                    halves = _HK.result(_HK.accumulate(
                        lambda r: _bf(hidden_v[k % 2].at[r][...]),
                        lambda i, j: pace.load(w4_v[i * fw:(i + 1) * fw, _tile(j * dt + n)]),
                        lambda r: pace.load(s4_v.at[n][:, _tile(r)])))
                    for f, half in enumerate(halves):
                        for j, v in enumerate(half):
                            rows = _at((g * units + k) * UNIT + f * (UNIT // 2), UNIT // 2)
                            part_v[rows, _tile(j * dt + n)] += 0.5 * v

            for m in range(3):
                for r in range(0, kw, 8):
                    pace.note(prepare_qkv(m, r)[0])
            for r in range(0, kw, 8):
                pace.note(prepare_out(r)[0])
            loads = units * 2 * ft * dt * n_prod
            pace.spread(0.64 * loads, 0.99 * loads)
            for k in range(units):
                norm((g * units + k + 1) * UNIT, (k + 1) % 2, pace.note)
                pace.spread(40, ft * dt * n_prod)
                up(k)
                if k > 0:
                    down(k - 1)
            down(units - 1)
            return 0

        norm(0, 0)
        lax.fori_loop(0, n_grp, body, 0)

    def recurrence(sums_v, own_v, left_v, next_v, hq_v, ho_v, ahead_v):
        scale = float(Dh) ** -0.5
        row = lax.broadcasted_iota(jnp.int32, (2 * L, 2 * L), 0)
        col = lax.broadcasted_iota(jnp.int32, (2 * L, 2 * L), 1)
        r_in = jnp.where(row >= L, row - L, row)
        c_in = jnp.where(col >= L, col - L, col)
        same_head = (row >= L) == (col >= L)
        keep = same_head & ((r_in < M) | (r_in >= c_in))
        fill = jnp.where(same_head, _MASKED / scale, -jnp.inf).astype(F32)

        def load_own(s):
            own_v[...] = _ln(x_rows(s * seg, seg)[:seg - 8])

        def load_next(s, q):
            next_v[8 * q:8 * q + 8, :] = _ln(x_rows(s * seg + seg - 16, 16)[8:])

        def load_left(mem=None):
            lower = next_v[...]
            upper = lower if mem is None else jnp.concatenate([mem, own_v[...]], axis=0)
            for n, v in enumerate(_HK.left(_split(upper, P), _split(lower, P))):
                if (n in _HKQ.lower) == (mem is None):
                    left_v.at[n][...] = _words(v)

        def operands(g, m):
            return (lambda n: _bf(left_v.at[n][...]),
                    lambda i, j: _bf(wqkv_v.at[m * H + g * P + j][i * kw:(i + 1) * kw, :]),
                    lambda n: _bf(sums_v.at[m * n_grp + g][:, _tile(n)]))

        ahead = list(zip([when for when, n in AHEAD.items() for _ in range(n)],
                         [(k // 3, k % 3, n) for k in range(FIRST_AHEAD, 3 * n_grp) for n in _HKQ.lower]))

        def run_ahead(*now):
            for k, (when, (g, m, n)) in enumerate(ahead):
                if when in now:
                    ahead_v[k] = _HKQ.product(n, *operands(g, m))

        def by_head(apart, dot, a, b):
            return jnp.concatenate([dot(a[:L], b), dot(a[L:], b)], axis=0) if apart else dot(a, b)

        def softmax(apart, q, k):
            s = jnp.where(keep, by_head(apart, _dot_nt, q, k.astype(BF16)), fill)
            e = jnp.exp2((s - jnp.max(s, axis=-1, keepdims=True)) * (scale * _LOG2E))
            return e, pl.reciprocal(jnp.sum(e, axis=-1, keepdims=True), full_range=False)

        def step(s, r, mem):
            first, last = r == 0, r == PERIOD - 1
            if not first:
                upper = jnp.concatenate([mem, own_v[...]], axis=0)

            def project(g):
                res = []
                for m in range(3):
                    h0 = m * H + g * P
                    if first:
                        tops, rest = _HKQ.result(_HKQ.accumulate(*operands(g, m), known={
                            which[2]: ahead_v.at[k] for k, (_, which) in enumerate(ahead) if which[:2] == (g, m)}))
                        for j in range(P):
                            hq_v[h0 + j] = rest[j][8:]
                        held = [v[:8] for v in rest]
                    else:
                        tops = [_dot(upper.astype(BF16), _bf(wqkv_v[h0 + j])) for j in range(P)]
                        held = [hq_v[h0 + j, 8 * (r - 1):8 * r, :] for j in range(P)]
                    res.append([jnp.concatenate([tops[j], held[j], tops[j + 1], held[j + 1]], axis=0)
                                for j in range(0, P, 2)])
                return list(zip(*res))

            def merge(g, heads, acc):
                tops, held = [o[:L - 8] for o in heads], [o[L - 8:] for o in heads]
                if last:
                    waiting[g] = _HK.left(tops, [jnp.concatenate([ho_v[:, _tile(g * P + j)], held[j]], axis=0)
                                                 for j in range(P)])
                    if g not in ENDS:
                        return acc
                    left = {a: waiting.pop(a) for a in sorted(waiting)}
                    k = Dh // 2
                    return _HK.accumulate(
                        lambda n: jnp.concatenate([v[n].astype(BF16) for v in left.values()], axis=1),
                        lambda i, j: jnp.concatenate([
                            _bf(wo_v[a * grows + i * k:a * grows + (i + 1) * k, j * dt * LANE:(j + 1) * dt * LANE])
                            for a in left], axis=0),
                        lambda n: jnp.concatenate([
                            jnp.concatenate([_bf(sums_v.at[3 * n_grp + a][c * k:(c + 1) * k, _tile(n)])
                                             for c in range(dt)], axis=1) for a in left], axis=0),
                        acc or ())
                for j in range(P):
                    ho_v[8 * r:8 * r + 8, _tile(g * P + j)] = held[j]
                y = _dot(jnp.concatenate(tops, axis=1).astype(BF16), _bf(wo_v[g * grows:(g + 1) * grows, :]))
                return y if acc is None else acc + y

            lag, late = LAGS[2 if last else 0 if first else 1]
            qkv, prob, heads, waiting = {}, {}, {}, {}
            acc, done = None, 0
            for t in range(n_grp + 3):
                if t < n_grp:
                    qkv[t] = project(t)
                while done < (t - lag + 1 if t < n_grp else (late + (n_grp,))[t - n_grp]):
                    run_ahead((r, done))
                    acc = merge(done, heads.pop(done), acc)
                    done += 1
                if 0 <= t - 2 < n_grp:
                    heads[t - 2] = []
                    for (e, inv), (_, _, v) in zip(prob.pop(t - 2), qkv.pop(t - 2)):
                        o = by_head(t - 2 == n_grp - 1, _dot, e, v.astype(BF16)) * inv
                        heads[t - 2] += [o[:L], o[L:]]
                if 0 <= t - 1 < n_grp:
                    prob[t - 1] = [softmax(t == 1, q, k) for q, k, _ in qkv[t - 1]]
                if first and 1 <= t <= PERIOD:
                    load_next(jnp.minimum(s + PERIOD - 1 + t, n_seg - 1), t - 1)
                if first and t == n_grp:
                    load_left()
                if t == n_grp - 1:
                    load_own(jnp.minimum(s + 1, n_seg - 1))
            run_ahead((r, n_grp))
            if last:
                y, y_held = [jnp.concatenate(half, axis=1) for half in _HK.result(acc)]
                load_left(y[:M])
            else:
                y = acc
            base = x_rows(s * seg, seg) + part_v[_at(s * seg, seg), :]
            x_v[_at(s * (seg // 2), 8), :] = _words(base[:16] + y[M:M + 16])
            tail = jnp.concatenate([base[16:24] + y[M + 16:], base[24:]], axis=0)
            if not last:
                part_v[_at(s * seg + 16, 16), :] = tail
            else:
                for q in range(PERIOD):
                    r0 = (s - r + q) * seg + 16
                    rest = part_v[_at(r0, 16), :] if q < r else tail
                    x_v[_at(r0 // 2, 8), :] = _words(jnp.concatenate(
                        [rest[:8], rest[8:] + y_held[8 * q:8 * q + 8]], axis=0))
            return y[:M]

        def period(p, _):
            mem = None
            for r in range(PERIOD):
                mem = step(p * PERIOD + r, r, mem)
            out_copy(_at(p * (PERIOD * seg // 2), PERIOD * seg // 2)).start()
            return 0

        mem0_copy.wait()
        for q in range(PERIOD):
            load_next(q, q)
        load_left()
        run_ahead(*AHEAD)
        load_own(0)
        load_left(mem0_v[...].astype(F32))
        lax.fori_loop(0, n_seg // PERIOD, period, 0)

    def with_attention_sums(sums_v):
        pl.run_scoped(
            functools.partial(channel_mlp, sums_v),
            *[pltpu.VMEM((n_prod, UNIT // 4, k // P), U32) for k in (D, D, FF, FF)])
        pl.run_scoped(
            functools.partial(recurrence, sums_v),
            pltpu.VMEM((seg - 8, D), F32),
            pltpu.VMEM((n_prod, (L - 8) // 2, D // P), U32),
            pltpu.VMEM((8 * PERIOD, D), F32),
            pltpu.VMEM((3 * H, 8 * (PERIOD - 1), Dh), F32),
            pltpu.VMEM((8 * (PERIOD - 1), H * Dh), F32),
            pltpu.VMEM((sum(AHEAD.values()), L - 8, Dh), F32))

    pl.run_scoped(
        token_mixing,
        pltpu.VMEM((D // LANE, S + 16, LANE), F32),
        pltpu.VMEM((2, D // 2, D), U32),
        pltpu.VMEM((2, D // 2 // LANE, D // 4, len(_HK2.summed) * LANE), U32),
        pltpu.VMEM((2, len(_HK2.products), UNIT // 4, D // 2), U32),
        pltpu.VMEM((len(_HK2.products), TM // 8, D // 2), U32))
    pl.run_scoped(with_attention_sums, pltpu.VMEM((4 * n_grp, kw, len(_HK.summed) * LANE), U32))
    out_copy(slice(0, S // 2)).wait()


@functools.partial(jax.jit, static_argnames=("A_seg_len",))
def pallas_parallel_sum__memory_aug_recurrent_mem_tr__mixer_s_mlp__prompt_kernel(
    A_x: jax.Array,
    A_mem0: jax.Array,
    A_Wq: jax.Array,
    A_Wk: jax.Array,
    A_Wv: jax.Array,
    A_Wo: jax.Array,
    A_seg_len: int,
    B_x: jax.Array,
    B_w1: jax.Array,
    B_w2: jax.Array,
    B_w3: jax.Array,
    B_w4: jax.Array,
):
    del B_x
    B, S, D = A_x.shape
    H, Dh = A_Wq.shape[1:]
    M = A_mem0.shape[1]
    FF = B_w3.shape[1]
    assert (B, S, D, H, Dh, M, A_seg_len) == (1, 2048, 1024, 32, 128, 8, 32)
    sums = len(_HK.summed) * LANE

    hbm = pl.BlockSpec(memory_space=pl.ANY)
    out = pl.pallas_call(
        functools.partial(_kernel, seg=A_seg_len),
        out_shape=jax.ShapeDtypeStruct((S, D), A_x.dtype),
        in_specs=[hbm] * 10,
        out_specs=hbm,
        scratch_shapes=[
            pltpu.VMEM(((S + UNIT) // 2, D), U32),
            pltpu.VMEM((S + UNIT, D), F32),
            pltpu.VMEM((M, D), A_mem0.dtype),
            pltpu.VMEM((3 * H, D // 2, Dh), U32),
            pltpu.VMEM((H * Dh // 2, D), U32),
            pltpu.VMEM((2, 3 * P, D // 2, Dh), U32),
            pltpu.VMEM((D // 2, FF), U32),
            pltpu.VMEM((FF // 2, D), U32),
            pltpu.VMEM((FF // P // LANE, D // 2 // P, sums), U32),
            pltpu.VMEM((D // P // LANE, FF // 2 // P, sums), U32),
            pltpu.SemaphoreType.DMA((S // TM + 1,)),
            pltpu.SemaphoreType.DMA((2, D // 2 // LANE)),
            pltpu.SemaphoreType.DMA((S // TM,)),
            pltpu.SemaphoreType.DMA((H // P,)),
            pltpu.SemaphoreType.DMA,
            pltpu.SemaphoreType.DMA,
        ],
        compiler_params=pltpu.CompilerParams(
            vmem_limit_bytes=127 * 1024 * 1024, disable_bounds_checks=True),
    )(A_x.reshape(S, D), A_mem0.reshape(M, D),
      *[w.reshape(D // 2, 2, H, Dh) for w in (A_Wq, A_Wk, A_Wv)],
      A_Wo.reshape(H * Dh, D), B_w1, B_w2, B_w3, B_w4)
    return out.reshape(B, S, D)
```

```python
import functools

import jax
import jax.numpy as jnp
import numpy as np
from jax import lax
import jax.experimental.pallas as pl
import jax.experimental.pallas.tpu as pltpu

F32 = jnp.float32
BF16 = jnp.bfloat16
U32 = jnp.uint32

_EPS = 1e-5
_MASKED = -1e9
_LOG2E = float(np.log2(np.e))
_GELU_C = float(np.sqrt(2.0 / np.pi))

LANE = 128
TM = 512
UNIT = 128
RC = 16
P = 4
PERIOD = 4
AHEAD = {(0, 8): 12, (1, 8): 10, (2, 8): 8, (3, 5): 2, (3, 6): 8, (3, 7): 8, (3, 8): 12}


def _dot(a, b):
    return lax.dot_general(a, b, (((1,), (0,)), ((), ())), preferred_element_type=F32)


def _dot_nt(a, b):
    return lax.dot_general(a, b, (((1,), (1,)), ((), ())), preferred_element_type=F32)


def _bf(words):
    return pltpu.bitcast(words, BF16)


def _words(x):
    return pltpu.bitcast(x.astype(BF16), U32)


def _at(start, n, align=None):
    return pl.ds(start if isinstance(start, int) else pl.multiple_of(start, align or n), n)


def _tile(j):
    return _at(j * LANE, LANE)


def _split(x, n):
    k = x.shape[1] // n
    return [x[:, i * k:(i + 1) * k] for i in range(n)]


def _same(v):
    return v


def _moments(x, note=_same):
    inv_n = 1.0 / x.shape[-1]
    xc = x - note(jnp.sum(x, axis=-1, keepdims=True)) * inv_n
    return xc, note(jnp.sum(xc * xc, axis=-1, keepdims=True)) * inv_n


def _ln(x, note=_same):
    xc, var = _moments(x, note)
    return xc * lax.rsqrt(var + _EPS)


def _gelu2(x):
    return x * (1.0 + jnp.tanh(x * (_GELU_C + (_GELU_C * 0.044715) * (x * x))))


def _signed_sum(terms):
    terms = sorted(terms, key=lambda t: -t[0])
    assert terms[0][0] > 0
    total = terms[0][1]
    for sign, value in terms[1:]:
        total = total + value if sign > 0 else total - value
    return total


class _HopcroftKerr:
    def __init__(self, p, order=None):
        own = {0: ((1, 2, 1), (2, 0, 1)), 1: ((2, 1, -1), (0, 2, 1)), 2: ((1, 1, 1), (0, 0, 1))}
        cross = {(0, 1): ((1, 0, 1, 0, 1, -1), (0, -1, 0, -1, 0, 1, -1), (-1, 0, 1, 0, 1, 0, 1)),
                 (0, 2): ((2, 0, 1, 2, 1, 1), (-1, 0, 0, -1, 0, 1, -1), (0, -1, -1, 0, -1, 0, 1)),
                 (1, 2): ((2, 1, -1, 2, 0, 1), (0, -1, -1, 0, 1, 0, 1), (1, 0, 0, -1, 0, 1, -1))}
        products, diag, uses = [], {}, {}

        def product(left, out):
            products.append((left, out))
            return len(products) - 1

        def diagonal(idx, kind):
            diag[idx] = [product([(i, f, 1) for i in idx], [(i, g, 1) for i in idx]) for f, g, _ in own[kind]]

        def pair(a, ka, b, kb):
            if ka > kb:
                return pair(b, kb, a, ka)[::-1]
            (f0, f1, s, g0, g1, t), ab, ba = cross[ka, kb]
            diagonal(a + b, 3 - ka - kb)
            used = diag[a] + diag[b] + diag[a + b] + [product(
                [(i, f0, 1) for i in a] + [(i, f1, s) for i in b],
                [(i, g0, 1) for i in a] + [(i, g1, t) for i in b])]
            return dict(zip(used, ab)), dict(zip(used, ba))

        for i in range(p):
            diagonal((i,), i % 3)
            uses[i, i] = {r: sign for r, (_, _, sign) in zip(diag[i,], own[i % 3])}
        for j in range(p):
            for i in range(j):
                if i % 3 != j % 3:
                    uses[i, j], uses[j, i] = pair((i,), i % 3, (j,), j % 3)
        for j in range(p):
            for i in range(j % 3, j, 3):
                k = i + 1
                both = (i, k) if (i, k) in diag else (k, i)
                uses[i, j], uses[j, i] = pair(both, 3 - i % 3 - k % 3, (j,), j % 3)
                for ij, kj in (((i, j), (k, j)), ((j, i), (j, k))):
                    for r, c in uses[kj].items():
                        uses[ij][r] = uses[ij].get(r, 0) - c
        self.p = p
        self.order = order or range(len(products))
        self.products = [(left, [(i, j, c[r]) for (i, j), c in sorted(uses.items()) if c.get(r)], out)
                         for r, (left, out) in enumerate(products)]
        self.summed = [r for r, (_, weight, _) in enumerate(self.products) if len(weight) > 1]
        self.lower = [r for r in self.order if all(f == 1 for _, f, _ in self.products[r][0])]

    def left(self, upper, lower):
        forms = [(u, l, u - l) for u, l in zip(upper, lower)]
        return [_signed_sum([(sign, forms[i][f]) for i, f, sign in left]) for left, _, _ in self.products]

    def right(self, n, block):
        return _signed_sum([(sign, block(i, j).astype(F32)) for i, j, sign in self.products[self.summed[n]][1]])

    def product(self, r, left, block, summed):
        w = summed(self.summed.index(r)) if r in self.summed else block(*self.products[r][1][0][:2])
        return _dot(left(r), w)

    def accumulate(self, left, block, summed, acc=(), known=()):
        acc = dict(acc)
        for r in self.order:
            _, weight, out = self.products[r]
            flip = 1 if r in self.summed else weight[0][2]
            m = known[r][...] if r in known else self.product(r, left, block, summed)
            for j, f, sign in out:
                if (j, f) in acc:
                    acc[j, f] = acc[j, f] + m if sign * flip > 0 else acc[j, f] - m
                else:
                    acc[j, f] = m if sign * flip > 0 else -m
        return acc

    def result(self, acc):
        return [[functools.reduce(jnp.add, [acc[j, g] for g in (f, 2) if (j, g) in acc])
                 for j in range(self.p)] for f in range(2)]


_HK = _HopcroftKerr(P, (5, 18, 16, 9, 3, 15, 1, 24, 7, 19, 10, 0, 13, 14, 2, 22, 21, 12, 6, 20, 25, 23, 17, 4, 11, 8))
_HKQ = _HopcroftKerr(P, (10, 19, 18, 7, 16, 1, 2, 9, 5, 15, 23, 20, 11, 17, 4, 8, 22, 25, 0, 13, 21, 14, 24, 3, 12, 6))
_HKO = _HopcroftKerr(P, (5, 18, 16, 9, 15, 1, 3, 24, 7, 19, 10, 0, 22, 13, 14, 2, 20, 21, 12, 6, 4, 25, 23, 17, 11, 8))
_HK2 = _HopcroftKerr(2)


class _Pace:
    def __init__(self, never):
        self.never, self.noted, self.due, self.pos = never, [], [], 0

    def note(self, v):
        u = pltpu.bitcast(jnp.broadcast_to(v, (v.shape[0], max(v.shape[1], LANE))), U32)
        self.noted.append(functools.reduce(jnp.bitwise_or, [
            u[r:r + 8, c:c + LANE] for r in range(0, u.shape[0], 8) for c in range(0, u.shape[1], LANE)]))
        return v

    def spread(self, first, last):
        n = len(self.noted)
        self.due += [(self.pos + first + (k + 1) * (last - first) / n, v) for k, v in enumerate(self.noted)]
        self.due.sort(key=lambda t: t[0])
        self.noted = []

    def load(self, words):
        self.pos += words.shape[0] // (LANE // 2)
        hints = []
        while self.due and self.due[0][0] <= self.pos:
            hints.append(self.due.pop(0)[1])
        if hints:
            hint, parts = functools.reduce(jnp.bitwise_or, hints), []
            for k in range(0, words.shape[0], LANE // 2):
                parts += [jnp.where(self.never, hint, words[k:k + 8]), words[k + 8:k + LANE // 2]]
            words = jnp.concatenate(parts, axis=0)
        return _bf(words)


def _kernel(x_hbm, mem0_hbm, wq_hbm, wk_hbm, wv_hbm, wo_hbm, w1_hbm, w2_hbm, w3_hbm, w4_hbm,
            out_hbm,
            x_v, part_v, mem0_v, wqkv_v, wo_v, raw_v, w3_v, w4_v, s3_v, s4_v,
            sem_x, sem_mix, sem_mlp, sem_attn, sem_mem, sem_out, *, seg):
    S, D = x_hbm.shape
    H, Dh = wq_hbm.shape[-2:]
    M = mem0_hbm.shape[0]
    FF = w3_hbm.shape[1]
    L = M + seg
    n_blk = S // TM
    n_seg = S // seg
    n_grp = H // P
    n_prod = len(_HK.products)
    kw = D // 2 // P
    fw = FF // 2 // P
    ft = FF // P // LANE
    dt = D // P // LANE
    grows = P * Dh // 2

    def copy(hbm, vmem, sem, *idx):
        return pltpu.make_async_copy(hbm.bitcast(U32).at[idx], vmem.at[idx], sem)

    def attn_copies(g):
        copies = [copy(wo_hbm, wo_v, sem_attn.at[g], _at(g * grows, grows))]
        for m, hbm in enumerate((wq_hbm, wk_hbm, wv_hbm)):
            for j in range(P // 2):
                for par in range(2):
                    copies.append(pltpu.make_async_copy(
                        hbm.bitcast(U32).at[:, par, g * (P // 2) + j, :],
                        raw_v.at[g % 2, m * P + 2 * j + par], sem_attn.at[g]))
        return copies

    def mlp_copies(q):
        return [copy(hbm, vmem, sem_mlp.at[q], _at(i * n + q * (n // n_blk), n // n_blk, 8))
                for hbm, vmem, n in ((w3_hbm, w3_v, kw), (w4_hbm, w4_v, fw)) for i in range(P)]

    def out_copy(rows):
        return pltpu.make_async_copy(x_v.at[rows], out_hbm.bitcast(U32).at[rows], sem_out)

    mem0_copy = pltpu.make_async_copy(mem0_hbm, mem0_v, sem_mem)

    def x_rows(r0, n):
        return _bf(x_v[_at(r0 // 2, n // 2), :]).astype(F32)

    def store_left(hk, ref, rows, size, note):
        for q in range(0, size // 2, RC):
            for n, v in enumerate(hk.left(_split(rows(q), hk.p), _split(rows(size // 2 + q), hk.p))):
                ref.at[n][q // 2:(q + RC) // 2, :] = _words(v)
                if n >= len(hk.products) - 2:
                    note(v)

    def store_right(hk, ref, rows, block):
        out = []
        for n in range(len(hk.summed)):
            v = hk.right(n, block)
            ref[rows, _tile(n)] = _words(v)
            out.append(v[:8])
        return out

    def token_mixing(h_v, w_v, sums_v, left_v, first_v):
        pairs = D // 2 // LANE
        units = TM // UNIT
        loads = pairs * len(_HK2.products) * (D // 2 // LANE)

        def w_copies(n, j):
            return [copy((w1_hbm, w2_hbm)[n], w_v.at[n], sem_mix.at[n, j], slice(None), _tile(c * pairs + j))
                    for c in range(2)]

        def x_copy(i):
            return copy(x_hbm, x_v, sem_x.at[i + 1], slice((i * TM + UNIT) // 2, min(S, (i + 1) * TM + UNIT) // 2))

        def block(n, j, r=0, size=D // 4):
            return lambda a, c: w_v.at[n][a * (D // 4) + r:a * (D // 4) + r + size, _tile(c * pairs + j)]

        def prepare(j, r, size):
            store_right(_HK2, sums_v.at[1, j], slice(r, r + size), lambda a, c: _bf(block(1, j, r, size)(a, c)))

        def norm(r0, ref, size, note=_same):
            def rows(r):
                xc, var = _moments(x_rows(r0 + r, RC), note)
                inv = lax.rsqrt(var + _EPS)
                xn = xc * inv
                part_v[_at(r0 + r, RC), :] = xn
                return xn * lax.rsqrt(var * inv * inv + _EPS)
            store_left(_HK2, ref, rows, size, note)

        def shift(r0, ref, note=_same):
            def rows(r):
                return jnp.concatenate(
                    [h_v.at[c][pl.ds(r0 + r + 8 + (-1, 1, -2, 2)[4 * c * LANE // D], RC), :]
                     for c in range(D // LANE)], axis=1)
            store_left(_HK2, ref, rows, UNIT, note)

        def matmul(n, left, r0, load=_bf, arriving=False):
            for j in range(pairs):
                def summed(k):
                    if not arriving:
                        return load(sums_v.at[n, j][:, _tile(k)])
                    w = _HK2.right(k, lambda a, c: _bf(block(n, j)(a, c))).astype(BF16)
                    sums_v.at[n, j][:, _tile(k)] = pltpu.bitcast(w, U32)
                    return w

                if arriving:
                    for c in w_copies(n, j):
                        c.wait()
                halves = _HK2.result(_HK2.accumulate(
                    lambda r: _bf(left.at[r][...]), lambda a, c: load(block(n, j)(a, c)), summed))
                for f, half in enumerate(halves):
                    for c, v in enumerate(half):
                        size = v.shape[0]
                        if n == 0:
                            h_v.at[c * pairs + j][_at(8 + r0 + f * size, size, 8), :] = _gelu2(v)
                        else:
                            part_v[_at(r0 + f * size, size), _tile(c * pairs + j)] += 0.5 * v

        def h_unit(r0, k, pace):
            norm(r0 + UNIT, left_v.at[(k + 1) % 2], UNIT, pace.note)
            pace.spread(0.1 * loads, loads)
            matmul(0, left_v.at[k % 2], r0, pace.load)

        def h_body(i, _):
            for n in range(1, n_blk):
                @pl.when(i == n)
                def _():
                    for later in range(2, n_blk) if n == 1 else ():
                        for c in [x_copy(later)] + w_copies(1, later - 1):
                            c.start()
                    for c in w_copies(1, pairs - 1) if n == 2 else ():
                        c.start()
                    x_copy(n).wait()

            for c in mlp_copies(i - 1):
                c.start()
            for c in w_copies(1, i - 1):
                c.wait()
            pace = _Pace(i < 0)
            for k in range(units):
                h_unit(i * TM + k * UNIT, k, pace)
                prepare(i - 1, k * (D // 4 // units), D // 4 // units)
            return 0

        def mix_body(i, _):
            @pl.when(i == 0)
            def _():
                for c in mlp_copies(n_blk - 1):
                    c.start()

            @pl.when(i == 1)
            def _():
                for c in attn_copies(0):
                    c.start()

            for c in mlp_copies(i):
                c.wait()

            def sums(w, ref, k, tiles, n, r):
                r += i * (k // n_blk)
                return jnp.concatenate(store_right(_HK, ref.at[n], _at(r, 8), lambda a, c: _bf(
                    w[_at(a * k + r, 8), _tile(c * tiles + n)])), axis=0)

            side = [functools.partial(sums, w, ref, k, tiles, n, r)
                    for w, ref, k, tiles in ((w3_v, s3_v, kw, ft), (w4_v, s4_v, fw, dt))
                    for n in range(tiles) for r in range(0, k // n_blk, 8)]
            pace = _Pace(i < 0)
            for k in range(units):
                r0 = i * TM + k * UNIT
                for task in side[k * len(side) // units:(k + 1) * len(side) // units]:
                    pace.note(task())
                pace.spread(0.05 * loads, loads)
                shift(jnp.minimum(r0 + UNIT, S - UNIT), left_v.at[(k + 1) % 2], pace.note)
                pace.spread(0.05 * loads, loads)
                matmul(1, left_v.at[k % 2], r0, pace.load)
            return 0

        first = [copy(x_hbm, x_v, sem_x.at[k], rows)
                 for k, rows in enumerate((slice(0, TM // 4), slice(TM // 4, (TM + UNIT) // 2)))]
        for c in ([first[0]] + sum((w_copies(0, j) for j in range(pairs)), [])
                  + [first[1], x_copy(1)] + w_copies(1, 0) + [mem0_copy]):
            c.start()
        h_v[:, 0:8, :] = jnp.zeros((D // LANE, 8, LANE), F32)
        h_v[:, S + 8:S + 16, :] = jnp.zeros((D // LANE, 8, LANE), F32)
        x_v[S // 2:, :] = jnp.zeros((UNIT // 2, D), U32)
        first[0].wait()
        norm(0, first_v, TM // 2)
        matmul(0, first_v, 0, arriving=True)
        first[1].wait()
        pace = _Pace(jnp.square(part_v[0:8, 0:LANE]) < 0)
        norm(TM // 2, left_v.at[units // 2 % 2], UNIT)
        for k in range(units // 2, units):
            h_unit(k * UNIT, k, pace)
        lax.fori_loop(1, n_blk, h_body, 0)
        shift(0, left_v.at[0])
        for c in w_copies(1, pairs - 1):
            c.wait()
        for r in range(0, D // 4, 32):
            prepare(pairs - 1, r, 32)
        lax.fori_loop(0, n_blk, mix_body, 0)

    def channel_mlp(sums_v, *buffers):
        left_v, hidden_v = buffers[:2], buffers[2:]
        units = S // UNIT // n_grp

        def norm(r0, slot, note=_same):
            store_left(_HK, left_v[slot], lambda r: _ln(part_v[_at(r0 + r, RC), :], note), UNIT, note)

        def body(g, _):
            @pl.when(g + 1 < n_grp)
            def _():
                for c in attn_copies(g + 1):
                    c.start()

            for c in attn_copies(g):
                c.wait()
            pace = _Pace(g < 0)

            def prepare_qkv(m, r):
                blocks = {}
                for j in range(0, P, 2):
                    for i in range(P):
                        rows = slice(i * kw + r, i * kw + r + 8)
                        even, odd = raw_v.at[g % 2, m * P + j][rows, :], raw_v.at[g % 2, m * P + j + 1][rows, :]
                        for n, w in enumerate(((even & jnp.uint32(0xFFFF)) | (odd << 16),
                                               (even >> 16) | (odd & jnp.uint32(0xFFFF0000)))):
                            wqkv_v[m * H + g * P + j + n, rows, :] = w
                            blocks[i, j + n] = _bf(w)
                return store_right(_HK, sums_v.at[m * n_grp + g], slice(r, r + 8), lambda i, j: blocks[i, j])

            def prepare_out(r):
                return store_right(_HK, sums_v.at[3 * n_grp + g], slice(r, r + 8), lambda i, j: _bf(
                    wo_v[_at(g * grows + i * (Dh // 2) + r % (Dh // 2), 8), _tile(j * dt + r // (Dh // 2))]))

            def up(k):
                for n in range(ft):
                    upper, lower = _HK.result(_HK.accumulate(
                        lambda r: _bf(left_v[k % 2].at[r][...]),
                        lambda i, j: pace.load(w3_v[i * kw:(i + 1) * kw, _tile(j * ft + n)]),
                        lambda r: pace.load(s3_v.at[n][:, _tile(r)])))
                    for r, v in enumerate(_HK.left([_gelu2(v) for v in upper], [_gelu2(v) for v in lower])):
                        hidden_v[k % 2].at[r][:, _tile(n)] = _words(v)
                        if r < 2 * P and r % 2 == 0 and (n + 1 < ft or k):
                            pace.note(v)
                    pace.spread(20, 50)

            def down(k):
                for n in range(dt):
                    halves = _HK.result(_HK.accumulate(
                        lambda r: _bf(hidden_v[k % 2].at[r][...]),
                        lambda i, j: pace.load(w4_v[i * fw:(i + 1) * fw, _tile(j * dt + n)]),
                        lambda r: pace.load(s4_v.at[n][:, _tile(r)])))
                    for f, half in enumerate(halves):
                        for j, v in enumerate(half):
                            rows = _at((g * units + k) * UNIT + f * (UNIT // 2), UNIT // 2)
                            part_v[rows, _tile(j * dt + n)] += 0.5 * v

            for m in range(3):
                for r in range(0, kw, 8):
                    pace.note(prepare_qkv(m, r)[0])
            for r in range(0, kw, 8):
                pace.note(prepare_out(r)[0])
            loads = units * 2 * ft * dt * n_prod
            pace.spread(0.64 * loads, 0.99 * loads)
            for k in range(units):
                norm((g * units + k + 1) * UNIT, (k + 1) % 2, pace.note)
                pace.spread(40, ft * dt * n_prod)
                up(k)
                if k > 0:
                    down(k - 1)
            down(units - 1)
            return 0

        norm(0, 0)
        lax.fori_loop(0, n_grp, body, 0)

    def recurrence(sums_v, own_v, left_v, next_v, hq_v, ho_v, ahead_v):
        scale = float(Dh) ** -0.5
        row = lax.broadcasted_iota(jnp.int32, (2 * L, 2 * L), 0)
        col = lax.broadcasted_iota(jnp.int32, (2 * L, 2 * L), 1)
        r_in = jnp.where(row >= L, row - L, row)
        c_in = jnp.where(col >= L, col - L, col)
        same_head = (row >= L) == (col >= L)
        keep = same_head & ((r_in < M) | (r_in >= c_in))
        fill = jnp.where(same_head, _MASKED / scale, -jnp.inf).astype(F32)

        def load_own(s):
            own_v[...] = _ln(x_rows(s * seg, seg)[:seg - 8])

        def load_next(s, q):
            next_v[8 * q:8 * q + 8, :] = _ln(x_rows(s * seg + seg - 16, 16)[8:])

        def load_left(mem=None):
            lower = next_v[...]
            upper = lower if mem is None else jnp.concatenate([mem, own_v[...]], axis=0)
            for n, v in enumerate(_HK.left(_split(upper, P), _split(lower, P))):
                if (n in _HKQ.lower) == (mem is None):
                    left_v.at[n][...] = _words(v)

        def operands(g, m):
            return (lambda n: _bf(left_v.at[n][...]),
                    lambda i, j: _bf(wqkv_v.at[m * H + g * P + j][i * kw:(i + 1) * kw, :]),
                    lambda n: _bf(sums_v.at[m * n_grp + g][:, _tile(n)]))

        ahead = list(zip([when for when, n in AHEAD.items() for _ in range(n)],
                         [(k // 3, k % 3, n) for k in range(n_grp, 3 * n_grp) for n in _HKQ.lower]))

        def run_ahead(*now):
            for k, (when, (g, m, n)) in enumerate(ahead):
                if when in now:
                    ahead_v[k] = _HKQ.product(n, *operands(g, m))

        def by_head(apart, dot, a, b):
            return jnp.concatenate([dot(a[:L], b), dot(a[L:], b)], axis=0) if apart else dot(a, b)

        def softmax(apart, q, k):
            s = jnp.where(keep, by_head(apart, _dot_nt, q, k.astype(BF16)), fill)
            e = jnp.exp2((s - jnp.max(s, axis=-1, keepdims=True)) * (scale * _LOG2E))
            return e, pl.reciprocal(jnp.sum(e, axis=-1, keepdims=True), full_range=False)

        def step(s, r, mem):
            first, last = r == 0, r == PERIOD - 1
            if not first:
                upper = jnp.concatenate([mem, own_v[...]], axis=0)

            def project(g):
                res = []
                for m in range(3):
                    h0 = m * H + g * P
                    if first:
                        tops, rest = _HKQ.result(_HKQ.accumulate(*operands(g, m), known={
                            which[2]: ahead_v.at[k] for k, (_, which) in enumerate(ahead) if which[:2] == (g, m)}))
                        for j in range(P):
                            hq_v[h0 + j] = rest[j][8:]
                        held = [v[:8] for v in rest]
                    else:
                        tops = [_dot(upper.astype(BF16), _bf(wqkv_v[h0 + j])) for j in range(P)]
                        held = [hq_v[h0 + j, 8 * (r - 1):8 * r, :] for j in range(P)]
                    res.append([jnp.concatenate([tops[j], held[j], tops[j + 1], held[j + 1]], axis=0)
                                for j in range(0, P, 2)])
                return list(zip(*res))

            def merge(g, heads, acc):
                tops, held = [o[:L - 8] for o in heads], [o[L - 8:] for o in heads]
                if last:
                    waiting[g] = _HK.left(tops, [jnp.concatenate([ho_v[:, _tile(g * P + j)], held[j]], axis=0)
                                                 for j in range(P)])
                    if g not in (1, 4, 5, n_grp - 1):
                        return acc
                    left = {a: waiting.pop(a) for a in sorted(waiting)}
                    k = Dh // 2
                    return _HKO.accumulate(
                        lambda n: jnp.concatenate([v[n].astype(BF16) for v in left.values()], axis=1),
                        lambda i, j: jnp.concatenate([
                            _bf(wo_v[a * grows + i * k:a * grows + (i + 1) * k, j * dt * LANE:(j + 1) * dt * LANE])
                            for a in left], axis=0),
                        lambda n: jnp.concatenate([
                            jnp.concatenate([_bf(sums_v.at[3 * n_grp + a][c * k:(c + 1) * k, _tile(n)])
                                             for c in range(dt)], axis=1) for a in left], axis=0),
                        acc or ())
                for j in range(P):
                    ho_v[8 * r:8 * r + 8, _tile(g * P + j)] = held[j]
                y = _dot(jnp.concatenate(tops, axis=1).astype(BF16), _bf(wo_v[g * grows:(g + 1) * grows, :]))
                return y if acc is None else acc + y

            lag, late = (4, (5, 6)) if last else (5, (4, 6)) if first else (5, (4, 5))
            qkv, prob, heads, waiting = {}, {}, {}, {}
            acc, done = None, 0
            for t in range(n_grp + 3):
                if t < n_grp:
                    qkv[t] = project(t)
                while done < (t - lag + 1 if t < n_grp else (late + (n_grp,))[t - n_grp]):
                    run_ahead((r, done))
                    acc = merge(done, heads.pop(done), acc)
                    done += 1
                if 0 <= t - 2 < n_grp:
                    heads[t - 2] = []
                    for (e, inv), (_, _, v) in zip(prob.pop(t - 2), qkv.pop(t - 2)):
                        o = by_head(t - 2 == n_grp - 1, _dot, e, v.astype(BF16)) * inv
                        heads[t - 2] += [o[:L], o[L:]]
                if 0 <= t - 1 < n_grp:
                    prob[t - 1] = [softmax(t == 1, q, k) for q, k, _ in qkv[t - 1]]
                if first and 1 <= t <= PERIOD:
                    load_next(jnp.minimum(s + PERIOD - 1 + t, n_seg - 1), t - 1)
                if first and t == n_grp:
                    load_left()
                if t == n_grp - 1:
                    load_own(jnp.minimum(s + 1, n_seg - 1))
            run_ahead((r, n_grp))
            if last:
                y, y_held = [jnp.concatenate(half, axis=1) for half in _HK.result(acc)]
                load_left(y[:M])
            else:
                y = acc
            base = x_rows(s * seg, seg) + part_v[_at(s * seg, seg), :]
            x_v[_at(s * (seg // 2), 8), :] = _words(base[:16] + y[M:M + 16])
            tail = jnp.concatenate([base[16:24] + y[M + 16:], base[24:]], axis=0)
            if not last:
                part_v[_at(s * seg + 16, 16), :] = tail
            else:
                for q in range(PERIOD):
                    r0 = (s - r + q) * seg + 16
                    rest = part_v[_at(r0, 16), :] if q < r else tail
                    x_v[_at(r0 // 2, 8), :] = _words(jnp.concatenate(
                        [rest[:8], rest[8:] + y_held[8 * q:8 * q + 8]], axis=0))
            return y[:M]

        def period(p, _):
            mem = None
            for r in range(PERIOD):
                mem = step(p * PERIOD + r, r, mem)
            out_copy(_at(p * (PERIOD * seg // 2), PERIOD * seg // 2)).start()
            return 0

        mem0_copy.wait()
        for q in range(PERIOD):
            load_next(q, q)
        load_left()
        run_ahead(*AHEAD)
        load_own(0)
        load_left(mem0_v[...].astype(F32))
        lax.fori_loop(0, n_seg // PERIOD, period, 0)

    def with_attention_sums(sums_v):
        pl.run_scoped(
            functools.partial(channel_mlp, sums_v),
            *[pltpu.VMEM((n_prod, UNIT // 4, k // P), U32) for k in (D, D, FF, FF)])
        pl.run_scoped(
            functools.partial(recurrence, sums_v),
            pltpu.VMEM((seg - 8, D), F32),
            pltpu.VMEM((n_prod, (L - 8) // 2, D // P), U32),
            pltpu.VMEM((8 * PERIOD, D), F32),
            pltpu.VMEM((3 * H, 8 * (PERIOD - 1), Dh), F32),
            pltpu.VMEM((8 * (PERIOD - 1), H * Dh), F32),
            pltpu.VMEM((sum(AHEAD.values()), L - 8, Dh), F32))

    pl.run_scoped(
        token_mixing,
        pltpu.VMEM((D // LANE, S + 16, LANE), F32),
        pltpu.VMEM((2, D // 2, D), U32),
        pltpu.VMEM((2, D // 2 // LANE, D // 4, len(_HK2.summed) * LANE), U32),
        pltpu.VMEM((2, len(_HK2.products), UNIT // 4, D // 2), U32),
        pltpu.VMEM((len(_HK2.products), TM // 8, D // 2), U32))
    pl.run_scoped(with_attention_sums, pltpu.VMEM((4 * n_grp, kw, len(_HK.summed) * LANE), U32))
    out_copy(slice(0, S // 2)).wait()


@functools.partial(jax.jit, static_argnames=("A_seg_len",))
def pallas_parallel_sum__memory_aug_recurrent_mem_tr__mixer_s_mlp__prompt_kernel(
    A_x: jax.Array,
    A_mem0: jax.Array,
    A_Wq: jax.Array,
    A_Wk: jax.Array,
    A_Wv: jax.Array,
    A_Wo: jax.Array,
    A_seg_len: int,
    B_x: jax.Array,
    B_w1: jax.Array,
    B_w2: jax.Array,
    B_w3: jax.Array,
    B_w4: jax.Array,
):
    del B_x
    B, S, D = A_x.shape
    H, Dh = A_Wq.shape[1:]
    M = A_mem0.shape[1]
    FF = B_w3.shape[1]
    assert (B, S, D, H, Dh, M, A_seg_len) == (1, 2048, 1024, 32, 128, 8, 32)
    sums = len(_HK.summed) * LANE

    hbm = pl.BlockSpec(memory_space=pl.ANY)
    out = pl.pallas_call(
        functools.partial(_kernel, seg=A_seg_len),
        out_shape=jax.ShapeDtypeStruct((S, D), A_x.dtype),
        in_specs=[hbm] * 10,
        out_specs=hbm,
        scratch_shapes=[
            pltpu.VMEM(((S + UNIT) // 2, D), U32),
            pltpu.VMEM((S + UNIT, D), F32),
            pltpu.VMEM((M, D), A_mem0.dtype),
            pltpu.VMEM((3 * H, D // 2, Dh), U32),
            pltpu.VMEM((H * Dh // 2, D), U32),
            pltpu.VMEM((2, 3 * P, D // 2, Dh), U32),
            pltpu.VMEM((D // 2, FF), U32),
            pltpu.VMEM((FF // 2, D), U32),
            pltpu.VMEM((FF // P // LANE, D // 2 // P, sums), U32),
            pltpu.VMEM((D // P // LANE, FF // 2 // P, sums), U32),
            pltpu.SemaphoreType.DMA((S // TM + 1,)),
            pltpu.SemaphoreType.DMA((2, D // 2 // LANE)),
            pltpu.SemaphoreType.DMA((S // TM,)),
            pltpu.SemaphoreType.DMA((H // P,)),
            pltpu.SemaphoreType.DMA,
            pltpu.SemaphoreType.DMA,
        ],
        compiler_params=pltpu.CompilerParams(
            vmem_limit_bytes=127 * 1024 * 1024, disable_bounds_checks=True),
    )(A_x.reshape(S, D), A_mem0.reshape(M, D),
      *[w.reshape(D // 2, 2, H, Dh) for w in (A_Wq, A_Wk, A_Wv)],
      A_Wo.reshape(H * Dh, D), B_w1, B_w2, B_w3, B_w4)
    return out.reshape(B, S, D)
```

```python
import functools

import jax
import jax.numpy as jnp
import numpy as np
from jax import lax
import jax.experimental.pallas as pl
import jax.experimental.pallas.tpu as pltpu

F32 = jnp.float32
BF16 = jnp.bfloat16
U32 = jnp.uint32

_EPS = 1e-5
_MASKED = -1e9
_LOG2E = float(np.log2(np.e))
_GELU_C = float(np.sqrt(2.0 / np.pi))
_GELU_IN = float(np.cbrt(_GELU_C * 0.044715))
_GELU_OUT = 0.5 / _GELU_IN

LANE = 128
TM = 512
UNIT = 128
RC = 16
P = 4
PERIOD = 4
AHEAD = {(0, 8): 12, (1, 8): 10, (2, 8): 8, (3, 5): 2, (3, 6): 8, (3, 7): 8, (3, 8): 12}


def _dot(a, b):
    return lax.dot_general(a, b, (((1,), (0,)), ((), ())), preferred_element_type=F32)


def _dot_nt(a, b):
    return lax.dot_general(a, b, (((1,), (1,)), ((), ())), preferred_element_type=F32)


def _bf(words):
    return pltpu.bitcast(words, BF16)


def _words(x):
    return pltpu.bitcast(x.astype(BF16), U32)


def _at(start, n, align=None):
    return pl.ds(start if isinstance(start, int) else pl.multiple_of(start, align or n), n)


def _tile(j):
    return _at(j * LANE, LANE)


def _split(x, n):
    k = x.shape[1] // n
    return [x[:, i * k:(i + 1) * k] for i in range(n)]


def _same(v):
    return v


def _moments(x, note=_same):
    inv_n = 1.0 / x.shape[-1]
    xc = x - note(jnp.sum(x, axis=-1, keepdims=True)) * inv_n
    return xc, note(jnp.sum(xc * xc, axis=-1, keepdims=True)) * inv_n


def _ln(x):
    xc, var = _moments(x)
    return xc * lax.rsqrt(var + _EPS)


def _gelu(y):
    return y * (1.0 + jnp.tanh(y * (_GELU_C / _GELU_IN + y * y)))


def _signed_sum(terms):
    terms = sorted(terms, key=lambda t: -t[0])
    assert terms[0][0] > 0
    total = terms[0][1]
    for sign, value in terms[1:]:
        total = total + value if sign > 0 else total - value
    return total


class _HopcroftKerr:
    def __init__(self, p, order=None):
        own = {0: ((1, 2, 1), (2, 0, 1)), 1: ((2, 1, -1), (0, 2, 1)), 2: ((1, 1, 1), (0, 0, 1))}
        cross = {(0, 1): ((1, 0, 1, 0, 1, -1), (0, -1, 0, -1, 0, 1, -1), (-1, 0, 1, 0, 1, 0, 1)),
                 (0, 2): ((2, 0, 1, 2, 1, 1), (-1, 0, 0, -1, 0, 1, -1), (0, -1, -1, 0, -1, 0, 1)),
                 (1, 2): ((2, 1, -1, 2, 0, 1), (0, -1, -1, 0, 1, 0, 1), (1, 0, 0, -1, 0, 1, -1))}
        products, diag, uses = [], {}, {}

        def product(left, out):
            products.append((left, out))
            return len(products) - 1

        def diagonal(idx, kind):
            diag[idx] = [product([(i, f, 1) for i in idx], [(i, g, 1) for i in idx]) for f, g, _ in own[kind]]

        def pair(a, ka, b, kb):
            if ka > kb:
                return pair(b, kb, a, ka)[::-1]
            (f0, f1, s, g0, g1, t), ab, ba = cross[ka, kb]
            diagonal(a + b, 3 - ka - kb)
            used = diag[a] + diag[b] + diag[a + b] + [product(
                [(i, f0, 1) for i in a] + [(i, f1, s) for i in b],
                [(i, g0, 1) for i in a] + [(i, g1, t) for i in b])]
            return dict(zip(used, ab)), dict(zip(used, ba))

        for i in range(p):
            diagonal((i,), i % 3)
            uses[i, i] = {r: sign for r, (_, _, sign) in zip(diag[i,], own[i % 3])}
        for j in range(p):
            for i in range(j):
                if i % 3 != j % 3:
                    uses[i, j], uses[j, i] = pair((i,), i % 3, (j,), j % 3)
        for j in range(p):
            for i in range(j % 3, j, 3):
                k = i + 1
                both = (i, k) if (i, k) in diag else (k, i)
                uses[i, j], uses[j, i] = pair(both, 3 - i % 3 - k % 3, (j,), j % 3)
                for ij, kj in (((i, j), (k, j)), ((j, i), (j, k))):
                    for r, c in uses[kj].items():
                        uses[ij][r] = uses[ij].get(r, 0) - c
        self.p = p
        self.order = order or range(len(products))
        self.products = [(left, [(i, j, c[r]) for (i, j), c in sorted(uses.items()) if c.get(r)], out)
                         for r, (left, out) in enumerate(products)]
        self.summed = [r for r, (_, weight, _) in enumerate(self.products) if len(weight) > 1]
        self.lower = [r for r in self.order if all(f == 1 for _, f, _ in self.products[r][0])]

    def left(self, upper, lower):
        forms = [(u, l, u - l) for u, l in zip(upper, lower)]
        return [_signed_sum([(sign, forms[i][f]) for i, f, sign in left]) for left, _, _ in self.products]

    def right(self, n, block):
        def value(key):
            return block(*key).astype(F32) if isinstance(key[0], int) else value(key[0]) - value(key[1])

        terms = {(i, j): sign for i, j, sign in self.products[self.summed[n]][1]}
        for a, b in (((0, 3), (3, 0)), ((1, 0), (0, 3)), ((0, 1), (3, 0)), ((1, 3), ((0, 3), (3, 0)))):
            if terms.get(a, 0) * terms.get(b, 0) < 0:
                terms[a, b] = terms.pop(a)
                del terms[b]
        return _signed_sum([(sign, value(key)) for key, sign in terms.items()])

    def product(self, r, left, block, summed):
        w = summed(self.summed.index(r)) if r in self.summed else block(*self.products[r][1][0][:2])
        return _dot(left(r), w)

    def accumulate(self, left, block, summed, acc=(), known=()):
        acc = dict(acc)
        for r in self.order:
            _, weight, out = self.products[r]
            flip = 1 if r in self.summed else weight[0][2]
            m = known[r][...] if r in known else self.product(r, left, block, summed)
            for j, f, sign in out:
                if (j, f) in acc:
                    acc[j, f] = acc[j, f] + m if sign * flip > 0 else acc[j, f] - m
                else:
                    acc[j, f] = m if sign * flip > 0 else -m
        return acc

    def result(self, acc):
        return [[functools.reduce(jnp.add, [acc[j, g] for g in (f, 2) if (j, g) in acc])
                 for j in range(self.p)] for f in range(2)]


_HK = _HopcroftKerr(P, (9, 5, 18, 16, 3, 15, 1, 24, 7, 19, 10, 0, 13, 14, 2, 22, 21, 12, 6, 20, 25, 23, 17, 4, 11, 8))
_HKQ = _HopcroftKerr(P, (10, 19, 18, 7, 16, 1, 2, 9, 5, 15, 23, 20, 11, 17, 4, 8, 22, 25, 0, 13, 21, 14, 24, 3, 12, 6))
_HKO = _HopcroftKerr(P, (5, 18, 16, 9, 15, 1, 3, 24, 7, 19, 10, 0, 22, 13, 14, 2, 20, 21, 12, 6, 4, 25, 23, 17, 11, 8))
_HK2 = _HopcroftKerr(2, (4, 0, 1, 2, 3, 6, 5))


class _Pace:
    def __init__(self, never):
        self.never, self.noted, self.due, self.pos = never, [], [], 0

    def note(self, v):
        u = pltpu.bitcast(jnp.broadcast_to(v, (v.shape[0], max(v.shape[1], LANE))), U32)
        self.noted.append(functools.reduce(jnp.bitwise_or, [
            u[r:r + 8, c:c + LANE] for r in range(0, u.shape[0], 8) for c in range(0, u.shape[1], LANE)]))
        return v

    def spread(self, first, last):
        n = len(self.noted)
        self.due += [(self.pos + first + (k + 1) * (last - first) / n, v) for k, v in enumerate(self.noted)]
        self.due.sort(key=lambda t: t[0])
        self.noted = []

    def load(self, words):
        self.pos += words.shape[0] // (LANE // 2)
        hints = []
        while self.due and self.due[0][0] <= self.pos:
            hints.append(self.due.pop(0)[1])
        if hints:
            hint, parts = functools.reduce(jnp.bitwise_or, hints), []
            for k in range(0, words.shape[0], LANE // 2):
                parts += [jnp.where(self.never, hint, words[k:k + 8]), words[k + 8:k + LANE // 2]]
            words = jnp.concatenate(parts, axis=0)
        return _bf(words)


def _kernel(x_hbm, mem0_hbm, wq_hbm, wk_hbm, wv_hbm, wo_hbm, w1_hbm, w2_hbm, w3_hbm, w4_hbm,
            out_hbm,
            x_v, part_v, mem0_v, wqkv_v, wo_v, raw_v, w3_v, w4_v, s3_v, s4_v,
            sem_x, sem_mix, sem_mlp, sem_attn, sem_mem, sem_out, *, seg):
    S, D = x_hbm.shape
    H, Dh = wq_hbm.shape[-2:]
    M = mem0_hbm.shape[0]
    FF = w3_hbm.shape[1]
    L = M + seg
    n_blk = S // TM
    n_seg = S // seg
    n_grp = H // P
    n_prod = len(_HK.products)
    kw = D // 2 // P
    fw = FF // 2 // P
    ft = FF // P // LANE
    dt = D // P // LANE
    grows = P * Dh // 2

    def copy(hbm, vmem, sem, *idx):
        return pltpu.make_async_copy(hbm.bitcast(U32).at[idx], vmem.at[idx], sem)

    def attn_copies(g):
        copies = [copy(wo_hbm, wo_v, sem_attn.at[g], _at(g * grows, grows))]
        for m, hbm in enumerate((wq_hbm, wk_hbm, wv_hbm)):
            for j in range(P // 2):
                for par in range(2):
                    copies.append(pltpu.make_async_copy(
                        hbm.bitcast(U32).at[:, par, g * (P // 2) + j, :],
                        raw_v.at[g % 2, m * P + 2 * j + par], sem_attn.at[g]))
        return copies

    def mlp_copies(q):
        return [copy(hbm, vmem, sem_mlp.at[q], _at(i * n + q * (n // n_blk), n // n_blk, 8))
                for hbm, vmem, n in ((w3_hbm, w3_v, kw), (w4_hbm, w4_v, fw)) for i in range(P)]

    def out_copy(rows):
        return pltpu.make_async_copy(x_v.at[rows], out_hbm.bitcast(U32).at[rows], sem_out)

    mem0_copy = pltpu.make_async_copy(mem0_hbm, mem0_v, sem_mem)

    def x_rows(r0, n):
        return _bf(x_v[_at(r0 // 2, n // 2), :]).astype(F32)

    def store_left(hk, ref, rows, size, note):
        for q in range(0, size // 2, RC):
            for n, v in enumerate(hk.left(_split(rows(q), hk.p), _split(rows(size // 2 + q), hk.p))):
                ref.at[n][q // 2:(q + RC) // 2, :] = _words(v)
                if n >= len(hk.products) - 2:
                    note(v)

    def store_right(hk, ref, rows, block):
        out, block = [], functools.cache(block)
        for n in range(len(hk.summed)):
            v = hk.right(n, block)
            ref[rows, _tile(n)] = _words(v)
            out.append(v[:8])
        return out

    def token_mixing(h_v, w_v, sums_v, left_v, first_v):
        pairs = D // 2 // LANE
        units = TM // UNIT
        loads = pairs * len(_HK2.products) * (D // 2 // LANE)

        def w_copies(n, j):
            return [copy((w1_hbm, w2_hbm)[n], w_v.at[n], sem_mix.at[n, j], slice(None), _tile(c * pairs + j))
                    for c in range(2)]

        def x_copy(i):
            return copy(x_hbm, x_v, sem_x.at[i + 1], slice((i * TM + UNIT) // 2, min(S, (i + 1) * TM + UNIT) // 2))

        def block(n, j, r=0, size=D // 4):
            return lambda a, c: w_v.at[n][a * (D // 4) + r:a * (D // 4) + r + size, _tile(c * pairs + j)]

        def prepare(j, r, size):
            store_right(_HK2, sums_v.at[1, j], slice(r, r + size), lambda a, c: _bf(block(1, j, r, size)(a, c)))

        def norm(r0, ref, size, note=_same):
            def rows(r):
                xc, var = _moments(x_rows(r0 + r, RC), note)
                inv = lax.rsqrt(var + _EPS)
                part_v[_at(r0 + r, RC), :] = xc * (inv * (1.0 / _GELU_OUT))
                return xc * (inv * lax.rsqrt(var * inv * inv + _EPS) * _GELU_IN)
            store_left(_HK2, ref, rows, size, note)

        def shift(r0, ref, note=_same):
            def rows(r):
                return jnp.concatenate(
                    [h_v.at[c][pl.ds(r0 + r + 8 + (-1, 1, -2, 2)[4 * c * LANE // D], RC), :]
                     for c in range(D // LANE)], axis=1)
            store_left(_HK2, ref, rows, UNIT, note)

        def matmul(n, left, r0, load=_bf, arriving=False):
            for j in range(pairs):
                def summed(k):
                    if not arriving:
                        return load(sums_v.at[n, j][:, _tile(k)])
                    w = _HK2.right(k, lambda a, c: _bf(block(n, j)(a, c))).astype(BF16)
                    sums_v.at[n, j][:, _tile(k)] = pltpu.bitcast(w, U32)
                    return w

                if arriving:
                    for c in w_copies(n, j):
                        c.wait()
                halves = _HK2.result(_HK2.accumulate(
                    lambda r: _bf(left.at[r][...]), lambda a, c: load(block(n, j)(a, c)), summed))
                for f, half in enumerate(halves):
                    for c, v in enumerate(half):
                        size = v.shape[0]
                        if n == 0:
                            h_v.at[c * pairs + j][_at(8 + r0 + f * size, size, 8), :] = _gelu(v)
                        else:
                            part_v[_at(r0 + f * size, size), _tile(c * pairs + j)] += v

        def h_unit(r0, k, pace):
            norm(r0 + UNIT, left_v.at[(k + 1) % 2], UNIT, pace.note)
            pace.spread(0.15 * loads, loads)
            matmul(0, left_v.at[k % 2], r0, pace.load)

        def h_body(i, _):
            for n in range(1, n_blk):
                @pl.when(i == n)
                def _():
                    for later in range(2, n_blk) if n == 1 else ():
                        for c in [x_copy(later)] + w_copies(1, later - 1):
                            c.start()
                    for c in w_copies(1, pairs - 1) if n == 2 else ():
                        c.start()
                    x_copy(n).wait()

            for c in mlp_copies(i - 1):
                c.start()
            for c in w_copies(1, i - 1):
                c.wait()
            pace = _Pace(i < 0)
            for k in range(units):
                h_unit(i * TM + k * UNIT, k, pace)
                prepare(i - 1, k * (D // 4 // units), D // 4 // units)
            return 0

        def mix_body(i, _):
            @pl.when(i == 0)
            def _():
                for c in mlp_copies(n_blk - 1):
                    c.start()

            @pl.when(i == 1)
            def _():
                for c in attn_copies(0):
                    c.start()

            for c in mlp_copies(i):
                c.wait()

            def sums(w, ref, k, tiles, n, r):
                r += i * (k // n_blk)
                return jnp.concatenate(store_right(_HK, ref.at[n], _at(r, 8), lambda a, c: _bf(
                    w[_at(a * k + r, 8), _tile(c * tiles + n)])), axis=0)

            side = [functools.partial(sums, w, ref, k, tiles, n, r)
                    for w, ref, k, tiles in ((w3_v, s3_v, kw, ft), (w4_v, s4_v, fw, dt))
                    for n in range(tiles) for r in range(0, k // n_blk, 8)]
            pace = _Pace(i < 0)
            for k in range(units):
                r0 = i * TM + k * UNIT
                for task in side[k * len(side) // units:(k + 1) * len(side) // units]:
                    pace.note(task())
                pace.spread(0.05 * loads, 0.95 * loads)
                shift(jnp.minimum(r0 + UNIT, S - UNIT), left_v.at[(k + 1) % 2], pace.note)
                pace.spread(0.05 * loads, 0.9 * loads)
                matmul(1, left_v.at[k % 2], r0, pace.load)
            return 0

        first = [copy(x_hbm, x_v, sem_x.at[k], rows)
                 for k, rows in enumerate((slice(0, TM // 4), slice(TM // 4, (TM + UNIT) // 2)))]
        for c in ([first[0]] + sum((w_copies(0, j) for j in range(pairs)), [])
                  + [first[1], x_copy(1)] + w_copies(1, 0) + [mem0_copy]):
            c.start()
        h_v[:, 0:8, :] = jnp.zeros((D // LANE, 8, LANE), F32)
        h_v[:, S + 8:S + 16, :] = jnp.zeros((D // LANE, 8, LANE), F32)
        x_v[S // 2:, :] = jnp.zeros((UNIT // 2, D), U32)
        first[0].wait()
        norm(0, first_v, TM // 2)
        matmul(0, first_v, 0, arriving=True)
        first[1].wait()
        pace = _Pace(jnp.square(part_v[0:8, 0:LANE]) < 0)
        norm(TM // 2, left_v.at[units // 2 % 2], UNIT)
        for k in range(units // 2, units):
            h_unit(k * UNIT, k, pace)
        lax.fori_loop(1, n_blk, h_body, 0)
        shift(0, left_v.at[0])
        for c in w_copies(1, pairs - 1):
            c.wait()
        for r in range(0, D // 4, 32):
            prepare(pairs - 1, r, 32)
        lax.fori_loop(0, n_blk, mix_body, 0)

    def channel_mlp(sums_v, *buffers):
        left_v, hidden_v = buffers[:2], buffers[2:]
        units = S // UNIT // n_grp

        def norm(r0, slot, note=_same):
            def rows(r):
                xc, var = _moments(part_v[_at(r0 + r, RC), :], note)
                return xc * (lax.rsqrt(var + _EPS / _GELU_OUT ** 2) * _GELU_IN)
            store_left(_HK, left_v[slot], rows, UNIT, note)

        def body(g, _):
            @pl.when(g + 1 < n_grp)
            def _():
                for c in attn_copies(g + 1):
                    c.start()

            for c in attn_copies(g):
                c.wait()
            pace = _Pace(g < 0)

            def prepare_qkv(m, r):
                blocks = {}
                for j in range(0, P, 2):
                    for i in range(P):
                        rows = slice(i * kw + r, i * kw + r + 8)
                        raw = [raw_v.at[g % 2, m * P + j + par][rows, :] for par in range(2)]
                        for n in range(2):
                            blocks[i, j + n] = [pltpu.unpack_elementwise(
                                w, index=n, packed_dtype=BF16, unpacked_dtype=F32) for w in raw]
                            wqkv_v[m * H + g * P + j + n, rows, :] = pltpu.pack_elementwise(
                                blocks[i, j + n], packed_dtype=BF16)
                out = []
                for n in range(len(_HK.summed)):
                    v = [_HK.right(n, lambda i, j: blocks[i, j][par]) for par in range(2)]
                    sums_v.at[m * n_grp + g][r:r + 8, _tile(n)] = pltpu.pack_elementwise(v, packed_dtype=BF16)
                    out.append(v[0])
                return out

            def prepare_out(r):
                return store_right(_HK, sums_v.at[3 * n_grp + g], slice(r, r + 8), lambda i, j: _bf(
                    wo_v[_at(g * grows + i * (Dh // 2) + r % (Dh // 2), 8), _tile(j * dt + r // (Dh // 2))]))

            def up(k):
                for n in range(ft):
                    upper, lower = _HK.result(_HK.accumulate(
                        lambda r: _bf(left_v[k % 2].at[r][...]),
                        lambda i, j: pace.load(w3_v[i * kw:(i + 1) * kw, _tile(j * ft + n)]),
                        lambda r: pace.load(s3_v.at[n][:, _tile(r)])))
                    for r, v in enumerate(_HK.left([_gelu(v) for v in upper], [_gelu(v) for v in lower])):
                        hidden_v[k % 2].at[r][:, _tile(n)] = _words(v)
                        if r < 2 * P and (n + 1 < ft or k):
                            pace.note(v)
                    pace.spread(20, 47)

            def down(k):
                for n in range(dt):
                    halves = _HK.result(_HK.accumulate(
                        lambda r: _bf(hidden_v[k % 2].at[r][...]),
                        lambda i, j: pace.load(w4_v[i * fw:(i + 1) * fw, _tile(j * dt + n)]),
                        lambda r: pace.load(s4_v.at[n][:, _tile(r)])))
                    for f, half in enumerate(halves):
                        for j, v in enumerate(half):
                            rows = _at((g * units + k) * UNIT + f * (UNIT // 2), UNIT // 2)
                            part_v[rows, _tile(j * dt + n)] += v

            for m in range(3):
                for r in range(0, kw, 8):
                    pace.note(prepare_qkv(m, r)[0])
            for r in range(0, kw, 8):
                pace.note(prepare_out(r)[0])
            loads = units * 2 * ft * dt * n_prod
            pace.spread(0.64 * loads, 0.99 * loads)
            for k in range(units):
                norm((g * units + k + 1) * UNIT, (k + 1) % 2, pace.note)
                pace.spread(0, 324)
                up(k)
                if k > 0:
                    down(k - 1)
            down(units - 1)
            return 0

        norm(0, 0)
        lax.fori_loop(0, n_grp, body, 0)

    def recurrence(sums_v, own_v, left_v, next_v, hq_v, ho_v, ahead_v):
        scale = float(Dh) ** -0.5
        row = lax.broadcasted_iota(jnp.int32, (2 * L, 2 * L), 0)
        col = lax.broadcasted_iota(jnp.int32, (2 * L, 2 * L), 1)
        r_in = jnp.where(row >= L, row - L, row)
        c_in = jnp.where(col >= L, col - L, col)
        same_head = (row >= L) == (col >= L)
        keep = same_head & ((r_in < M) | (r_in >= c_in))
        fill = jnp.where(same_head, _MASKED / scale, -jnp.inf).astype(F32)

        def load_own(s):
            own_v[...] = _ln(x_rows(s * seg, seg)[:seg - 8])

        def load_next(s, q):
            next_v[8 * q:8 * q + 8, :] = _ln(x_rows(s * seg + seg - 16, 16)[8:])

        def load_left(mem=None):
            lower = next_v[...]
            upper = lower if mem is None else jnp.concatenate([mem, own_v[...]], axis=0)
            for n, v in enumerate(_HK.left(_split(upper, P), _split(lower, P))):
                if (n in _HKQ.lower) == (mem is None):
                    left_v.at[n][...] = _words(v)

        def operands(g, m):
            return (lambda n: _bf(left_v.at[n][...]),
                    lambda i, j: _bf(wqkv_v.at[m * H + g * P + j][i * kw:(i + 1) * kw, :]),
                    lambda n: _bf(sums_v.at[m * n_grp + g][:, _tile(n)]))

        ahead = list(zip([when for when, n in AHEAD.items() for _ in range(n)],
                         [(k // 3, k % 3, n) for k in range(n_grp, 3 * n_grp) for n in _HKQ.lower]))

        def run_ahead(*now):
            for k, (when, (g, m, n)) in enumerate(ahead):
                if when in now:
                    ahead_v[k] = _HKQ.product(n, *operands(g, m))

        def by_head(apart, dot, a, b):
            return jnp.concatenate([dot(a[:L], b), dot(a[L:], b)], axis=0) if apart else dot(a, b)

        def softmax(apart, q, k):
            s = jnp.where(keep, by_head(apart, _dot_nt, q, k.astype(BF16)), fill)
            e = jnp.exp2((s - jnp.max(s, axis=-1, keepdims=True)) * (scale * _LOG2E))
            return e, pl.reciprocal(jnp.sum(e, axis=-1, keepdims=True), full_range=False)

        def step(s, r, mem):
            first, last = r == 0, r == PERIOD - 1
            if not first:
                upper = jnp.concatenate([mem, own_v[...]], axis=0)

            def project(g):
                res = []
                for m in range(3):
                    h0 = m * H + g * P
                    if first:
                        tops, rest = _HKQ.result(_HKQ.accumulate(*operands(g, m), known={
                            which[2]: ahead_v.at[k] for k, (_, which) in enumerate(ahead) if which[:2] == (g, m)}))
                        for j in range(P):
                            hq_v[h0 + j] = rest[j][8:]
                        held = [v[:8] for v in rest]
                    else:
                        tops = [_dot(upper.astype(BF16), _bf(wqkv_v[h0 + j])) for j in range(P)]
                        held = [hq_v[h0 + j, 8 * (r - 1):8 * r, :] for j in range(P)]
                    res.append([jnp.concatenate([tops[j], held[j], tops[j + 1], held[j + 1]], axis=0)
                                for j in range(0, P, 2)])
                return list(zip(*res))

            def merge(g, heads, acc):
                tops, held = [o[:L - 8] for o in heads], [o[L - 8:] for o in heads]
                if last:
                    waiting[g] = _HK.left(tops, [jnp.concatenate([ho_v[:, _tile(g * P + j)], held[j]], axis=0)
                                                 for j in range(P)])
                    if g not in (1, 4, 5, n_grp - 1):
                        return acc
                    left = {a: waiting.pop(a) for a in sorted(waiting)}
                    k = Dh // 2
                    return _HKO.accumulate(
                        lambda n: jnp.concatenate([v[n].astype(BF16) for v in left.values()], axis=1),
                        lambda i, j: jnp.concatenate([
                            _bf(wo_v[a * grows + i * k:a * grows + (i + 1) * k, j * dt * LANE:(j + 1) * dt * LANE])
                            for a in left], axis=0),
                        lambda n: jnp.concatenate([
                            jnp.concatenate([_bf(sums_v.at[3 * n_grp + a][c * k:(c + 1) * k, _tile(n)])
                                             for c in range(dt)], axis=1) for a in left], axis=0),
                        acc or ())
                for j in range(P):
                    ho_v[8 * r:8 * r + 8, _tile(g * P + j)] = held[j]
                y = _dot(jnp.concatenate(tops, axis=1).astype(BF16), _bf(wo_v[g * grows:(g + 1) * grows, :]))
                return y if acc is None else acc + y

            lag, late = (4, (5, 6)) if last else (5, (4, 6)) if first else (5, (4, 5))
            qkv, prob, heads, waiting = {}, {}, {}, {}
            acc, done = None, 0
            for t in range(n_grp + 3):
                if t < n_grp:
                    qkv[t] = project(t)
                while done < (t - lag + 1 if t < n_grp else (late + (n_grp,))[t - n_grp]):
                    run_ahead((r, done))
                    acc = merge(done, heads.pop(done), acc)
                    done += 1
                if 0 <= t - 2 < n_grp:
                    heads[t - 2] = []
                    for (e, inv), (_, _, v) in zip(prob.pop(t - 2), qkv.pop(t - 2)):
                        o = by_head(t - 2 == n_grp - 1, _dot, e, v.astype(BF16)) * inv
                        heads[t - 2] += [o[:L], o[L:]]
                if 0 <= t - 1 < n_grp:
                    prob[t - 1] = [softmax(t == 1, q, k) for q, k, _ in qkv[t - 1]]
                if first and 1 <= t <= PERIOD:
                    load_next(jnp.minimum(s + PERIOD - 1 + t, n_seg - 1), t - 1)
                if first and t == n_grp:
                    load_left()
                if t == n_grp - 1:
                    load_own(jnp.minimum(s + 1, n_seg - 1))
            run_ahead((r, n_grp))
            if last:
                y, y_held = [jnp.concatenate(half, axis=1) for half in _HK.result(acc)]
                load_left(y[:M])
            else:
                y = acc
            base = x_rows(s * seg, seg) + _GELU_OUT * part_v[_at(s * seg, seg), :]
            x_v[_at(s * (seg // 2), 8), :] = _words(base[:16] + y[M:M + 16])
            tail = jnp.concatenate([base[16:24] + y[M + 16:], base[24:]], axis=0)
            if not last:
                part_v[_at(s * seg + 16, 16), :] = tail
            else:
                for q in range(PERIOD):
                    r0 = (s - r + q) * seg + 16
                    rest = part_v[_at(r0, 16), :] if q < r else tail
                    x_v[_at(r0 // 2, 8), :] = _words(jnp.concatenate(
                        [rest[:8], rest[8:] + y_held[8 * q:8 * q + 8]], axis=0))
            return y[:M]

        def period(p, _):
            mem = None
            for r in range(PERIOD):
                mem = step(p * PERIOD + r, r, mem)
            out_copy(_at(p * (PERIOD * seg // 2), PERIOD * seg // 2)).start()
            return 0

        mem0_copy.wait()
        for q in range(PERIOD):
            load_next(q, q)
        load_left()
        run_ahead(*AHEAD)
        load_own(0)
        load_left(mem0_v[...].astype(F32))
        lax.fori_loop(0, n_seg // PERIOD, period, 0)

    def with_attention_sums(sums_v):
        pl.run_scoped(
            functools.partial(channel_mlp, sums_v),
            *[pltpu.VMEM((n_prod, UNIT // 4, k // P), U32) for k in (D, D, FF, FF)])
        pl.run_scoped(
            functools.partial(recurrence, sums_v),
            pltpu.VMEM((seg - 8, D), F32),
            pltpu.VMEM((n_prod, (L - 8) // 2, D // P), U32),
            pltpu.VMEM((8 * PERIOD, D), F32),
            pltpu.VMEM((3 * H, 8 * (PERIOD - 1), Dh), F32),
            pltpu.VMEM((8 * (PERIOD - 1), H * Dh), F32),
            pltpu.VMEM((sum(AHEAD.values()), L - 8, Dh), F32))

    pl.run_scoped(
        token_mixing,
        pltpu.VMEM((D // LANE, S + 16, LANE), F32),
        pltpu.VMEM((2, D // 2, D), U32),
        pltpu.VMEM((2, D // 2 // LANE, D // 4, len(_HK2.summed) * LANE), U32),
        pltpu.VMEM((2, len(_HK2.products), UNIT // 4, D // 2), U32),
        pltpu.VMEM((len(_HK2.products), TM // 8, D // 2), U32))
    pl.run_scoped(with_attention_sums, pltpu.VMEM((4 * n_grp, kw, len(_HK.summed) * LANE), U32))
    out_copy(slice(0, S // 2)).wait()


@functools.partial(jax.jit, static_argnames=("A_seg_len",))
def pallas_parallel_sum__memory_aug_recurrent_mem_tr__mixer_s_mlp__prompt_kernel(
    A_x: jax.Array,
    A_mem0: jax.Array,
    A_Wq: jax.Array,
    A_Wk: jax.Array,
    A_Wv: jax.Array,
    A_Wo: jax.Array,
    A_seg_len: int,
    B_x: jax.Array,
    B_w1: jax.Array,
    B_w2: jax.Array,
    B_w3: jax.Array,
    B_w4: jax.Array,
):
    del B_x
    B, S, D = A_x.shape
    H, Dh = A_Wq.shape[1:]
    M = A_mem0.shape[1]
    FF = B_w3.shape[1]
    assert (B, S, D, H, Dh, M, A_seg_len) == (1, 2048, 1024, 32, 128, 8, 32)
    sums = len(_HK.summed) * LANE

    hbm = pl.BlockSpec(memory_space=pl.ANY)
    out = pl.pallas_call(
        functools.partial(_kernel, seg=A_seg_len),
        out_shape=jax.ShapeDtypeStruct((S, D), A_x.dtype),
        in_specs=[hbm] * 10,
        out_specs=hbm,
        scratch_shapes=[
            pltpu.VMEM(((S + UNIT) // 2, D), U32),
            pltpu.VMEM((S + UNIT, D), F32),
            pltpu.VMEM((M, D), A_mem0.dtype),
            pltpu.VMEM((3 * H, D // 2, Dh), U32),
            pltpu.VMEM((H * Dh // 2, D), U32),
            pltpu.VMEM((2, 3 * P, D // 2, Dh), U32),
            pltpu.VMEM((D // 2, FF), U32),
            pltpu.VMEM((FF // 2, D), U32),
            pltpu.VMEM((FF // P // LANE, D // 2 // P, sums), U32),
            pltpu.VMEM((D // P // LANE, FF // 2 // P, sums), U32),
            pltpu.SemaphoreType.DMA((S // TM + 1,)),
            pltpu.SemaphoreType.DMA((2, D // 2 // LANE)),
            pltpu.SemaphoreType.DMA((S // TM,)),
            pltpu.SemaphoreType.DMA((H // P,)),
            pltpu.SemaphoreType.DMA,
            pltpu.SemaphoreType.DMA,
        ],
        compiler_params=pltpu.CompilerParams(
            vmem_limit_bytes=127 * 1024 * 1024, disable_bounds_checks=True),
    )(A_x.reshape(S, D), A_mem0.reshape(M, D),
      *[w.reshape(D // 2, 2, H, Dh) for w in (A_Wq, A_Wk, A_Wv)],
      A_Wo.reshape(H * Dh, D), B_w1, B_w2, B_w3, B_w4)
    return out.reshape(B, S, D)
```

```python
import functools

import jax
import jax.numpy as jnp
import numpy as np
from jax import lax
import jax.experimental.pallas as pl
import jax.experimental.pallas.tpu as pltpu

F32 = jnp.float32
BF16 = jnp.bfloat16
U32 = jnp.uint32

_EPS = 1e-5
_MASKED = -1e9
_LOG2E = float(np.log2(np.e))
_GELU_C = float(np.sqrt(2.0 / np.pi))
_GELU_IN = float(np.cbrt(_GELU_C * 0.044715))
_GELU_OUT = 0.5 / _GELU_IN

LANE = 128
TM = 512
UNIT = 128
RC = 16
P = 4
PERIOD = 4
AHEAD = {(0, 8): 12, (1, 8): 10, (2, 8): 8, (3, 5): 2, (3, 6): 8, (3, 7): 8, (3, 8): 12}


def _dot(a, b):
    return lax.dot_general(a, b, (((1,), (0,)), ((), ())), preferred_element_type=F32)


def _dot_nt(a, b):
    return lax.dot_general(a, b, (((1,), (1,)), ((), ())), preferred_element_type=F32)


def _bf(words):
    return pltpu.bitcast(words, BF16)


def _words(x):
    return pltpu.bitcast(x.astype(BF16), U32)


def _at(start, n, align=None):
    return pl.ds(start if isinstance(start, int) else pl.multiple_of(start, align or n), n)


def _tile(j):
    return _at(j * LANE, LANE)


def _split(x, n):
    k = x.shape[1] // n
    return [x[:, i * k:(i + 1) * k] for i in range(n)]


def _same(v):
    return v


def _moments(x, note=_same):
    inv_n = 1.0 / x.shape[-1]
    xc = x - note(jnp.sum(x, axis=-1, keepdims=True)) * inv_n
    return xc, note(jnp.sum(xc * xc, axis=-1, keepdims=True)) * inv_n


def _ln(x):
    xc, var = _moments(x)
    return xc * lax.rsqrt(var + _EPS)


def _gelu(y):
    return y * (1.0 + jnp.tanh(y * (_GELU_C / _GELU_IN + y * y)))


def _signed_sum(terms):
    terms = sorted(terms, key=lambda t: -t[0])
    assert terms[0][0] > 0
    total = terms[0][1]
    for sign, value in terms[1:]:
        total = total + value if sign > 0 else total - value
    return total


class _HopcroftKerr:
    def __init__(self, p, order=None):
        own = {0: ((1, 2, 1), (2, 0, 1)), 1: ((2, 1, -1), (0, 2, 1)), 2: ((1, 1, 1), (0, 0, 1))}
        cross = {(0, 1): ((1, 0, 1, 0, 1, -1), (0, -1, 0, -1, 0, 1, -1), (-1, 0, 1, 0, 1, 0, 1)),
                 (0, 2): ((2, 0, 1, 2, 1, 1), (-1, 0, 0, -1, 0, 1, -1), (0, -1, -1, 0, -1, 0, 1)),
                 (1, 2): ((2, 1, -1, 2, 0, 1), (0, -1, -1, 0, 1, 0, 1), (1, 0, 0, -1, 0, 1, -1))}
        products, diag, uses = [], {}, {}

        def product(left, out):
            products.append((left, out))
            return len(products) - 1

        def diagonal(idx, kind):
            diag[idx] = [product([(i, f, 1) for i in idx], [(i, g, 1) for i in idx]) for f, g, _ in own[kind]]

        def pair(a, ka, b, kb):
            if ka > kb:
                return pair(b, kb, a, ka)[::-1]
            (f0, f1, s, g0, g1, t), ab, ba = cross[ka, kb]
            diagonal(a + b, 3 - ka - kb)
            used = diag[a] + diag[b] + diag[a + b] + [product(
                [(i, f0, 1) for i in a] + [(i, f1, s) for i in b],
                [(i, g0, 1) for i in a] + [(i, g1, t) for i in b])]
            return dict(zip(used, ab)), dict(zip(used, ba))

        for i in range(p):
            diagonal((i,), i % 3)
            uses[i, i] = {r: sign for r, (_, _, sign) in zip(diag[i,], own[i % 3])}
        for j in range(p):
            for i in range(j):
                if i % 3 != j % 3:
                    uses[i, j], uses[j, i] = pair((i,), i % 3, (j,), j % 3)
        for j in range(p):
            for i in range(j % 3, j, 3):
                k = i + 1
                both = (i, k) if (i, k) in diag else (k, i)
                uses[i, j], uses[j, i] = pair(both, 3 - i % 3 - k % 3, (j,), j % 3)
                for ij, kj in (((i, j), (k, j)), ((j, i), (j, k))):
                    for r, c in uses[kj].items():
                        uses[ij][r] = uses[ij].get(r, 0) - c
        self.p = p
        self.order = order or range(len(products))
        self.products = [(left, [(i, j, c[r]) for (i, j), c in sorted(uses.items()) if c.get(r)], out)
                         for r, (left, out) in enumerate(products)]
        self.summed = [r for r, (_, weight, _) in enumerate(self.products) if len(weight) > 1]
        self.lower = [r for r in self.order if all(f == 1 for _, f, _ in self.products[r][0])]

    def left(self, upper, lower):
        forms = [(u, l, u - l) for u, l in zip(upper, lower)]
        return [_signed_sum([(sign, forms[i][f]) for i, f, sign in left]) for left, _, _ in self.products]

    def right(self, n, block):
        def value(key):
            return block(*key).astype(F32) if isinstance(key[0], int) else value(key[0]) - value(key[1])

        terms = {(i, j): sign for i, j, sign in self.products[self.summed[n]][1]}
        for a, b in (((0, 3), (3, 0)), ((1, 0), (0, 3)), ((0, 1), (3, 0)), ((1, 3), ((0, 3), (3, 0)))):
            if terms.get(a, 0) * terms.get(b, 0) < 0:
                terms[a, b] = terms.pop(a)
                del terms[b]
        return _signed_sum([(sign, value(key)) for key, sign in terms.items()])

    def product(self, r, left, block, summed):
        w = summed(self.summed.index(r)) if r in self.summed else block(*self.products[r][1][0][:2])
        return _dot(left(r), w)

    def accumulate(self, left, block, summed, acc=(), known=()):
        acc = dict(acc)
        for r in self.order:
            _, weight, out = self.products[r]
            flip = 1 if r in self.summed else weight[0][2]
            m = known[r][...] if r in known else self.product(r, left, block, summed)
            for j, f, sign in out:
                if (j, f) in acc:
                    acc[j, f] = acc[j, f] + m if sign * flip > 0 else acc[j, f] - m
                else:
                    acc[j, f] = m if sign * flip > 0 else -m
        return acc

    def result(self, acc):
        return [[functools.reduce(jnp.add, [acc[j, g] for g in (f, 2) if (j, g) in acc])
                 for j in range(self.p)] for f in range(2)]


_HK = _HopcroftKerr(P, (9, 5, 18, 16, 3, 15, 1, 24, 7, 19, 10, 0, 13, 14, 2, 22, 21, 12, 11, 6, 20, 25, 23, 17, 4, 8))
_HKQ = _HopcroftKerr(P, (10, 19, 18, 7, 16, 1, 2, 9, 5, 15, 23, 20, 11, 17, 4, 8, 22, 25, 0, 13, 21, 14, 24, 3, 12, 6))
_HKO = _HopcroftKerr(P, (5, 18, 16, 9, 15, 1, 3, 24, 7, 19, 10, 0, 22, 13, 14, 2, 20, 21, 12, 6, 4, 25, 23, 17, 11, 8))
_HK12 = (_HopcroftKerr(2, (4, 0, 1, 2, 3, 5, 6)),
         _HopcroftKerr(P, (9, 3, 5, 18, 16, 15, 1, 24, 19, 7, 0, 10, 13, 14, 2, 8, 22, 12, 6, 21, 4, 20, 25, 17, 23, 11)))


class _Pace:
    def __init__(self, never):
        self.never, self.noted, self.due, self.pos = never, [], [], 0

    def note(self, v):
        u = pltpu.bitcast(jnp.broadcast_to(v, (v.shape[0], max(v.shape[1], LANE))), U32)
        self.noted.append(functools.reduce(jnp.bitwise_or, [
            u[r:r + 8, c:c + LANE] for r in range(0, u.shape[0], 8) for c in range(0, u.shape[1], LANE)]))
        return v

    def spread(self, first, last):
        n = len(self.noted)
        self.due += [(self.pos + first + (k + 1) * (last - first) / n, v) for k, v in enumerate(self.noted)]
        self.due.sort(key=lambda t: t[0])
        self.noted = []

    def load(self, words):
        self.pos += words.shape[0] // (LANE // 2)
        hints = []
        while self.due and self.due[0][0] <= self.pos:
            hints.append(self.due.pop(0)[1])
        if hints:
            hint, parts = functools.reduce(jnp.bitwise_or, hints), []
            for k in range(0, words.shape[0], LANE // 2):
                parts += [jnp.where(self.never, hint, words[k:k + 8]), words[k + 8:k + LANE // 2]]
            words = jnp.concatenate(parts, axis=0)
        return _bf(words)


def _kernel(x_hbm, mem0_hbm, wq_hbm, wk_hbm, wv_hbm, wo_hbm, w1_hbm, w2_hbm, w3_hbm, w4_hbm,
            out_hbm,
            x_v, part_v, mem0_v, wqkv_v, wo_v, raw_v, w3_v, w4_v, s3_v, s4_v,
            sem_x, sem_mix, sem_mlp, sem_attn, sem_mem, sem_out, *, seg):
    S, D = x_hbm.shape
    H, Dh = wq_hbm.shape[-2:]
    M = mem0_hbm.shape[0]
    FF = w3_hbm.shape[1]
    L = M + seg
    n_blk = S // TM
    n_seg = S // seg
    n_grp = H // P
    n_prod = len(_HK.products)
    kw = D // 2 // P
    fw = FF // 2 // P
    ft = FF // P // LANE
    dt = D // P // LANE
    grows = P * Dh // 2

    def copy(hbm, vmem, sem, *idx):
        return pltpu.make_async_copy(hbm.bitcast(U32).at[idx], vmem.at[idx], sem)

    def attn_copies(g):
        copies = [copy(wo_hbm, wo_v, sem_attn.at[g], _at(g * grows, grows))]
        for m, hbm in enumerate((wq_hbm, wk_hbm, wv_hbm)):
            for j in range(P // 2):
                for par in range(2):
                    copies.append(pltpu.make_async_copy(
                        hbm.bitcast(U32).at[:, par, g * (P // 2) + j, :],
                        raw_v.at[g % 2, m * P + 2 * j + par], sem_attn.at[g]))
        return copies

    def mlp_copies(q):
        return [copy(hbm, vmem, sem_mlp.at[q], _at(i * n + q * (n // n_blk), n // n_blk, 8))
                for hbm, vmem, n in ((w3_hbm, w3_v, kw), (w4_hbm, w4_v, fw)) for i in range(P)]

    def out_copy(rows):
        return pltpu.make_async_copy(x_v.at[rows], out_hbm.bitcast(U32).at[rows], sem_out)

    mem0_copy = pltpu.make_async_copy(mem0_hbm, mem0_v, sem_mem)

    def x_rows(r0, n):
        return _bf(x_v[_at(r0 // 2, n // 2), :]).astype(F32)

    def store_left(hk, ref, rows, size, note):
        for q in range(0, size // 2, RC):
            for n, v in enumerate(hk.left(_split(rows(q), hk.p), _split(rows(size // 2 + q), hk.p))):
                ref.at[n][q // 2:(q + RC) // 2, :] = _words(v)
                if n >= len(hk.products) - 2:
                    note(v)

    def store_right(hk, ref, rows, block):
        out, block = [], functools.cache(block)
        for n in range(len(hk.summed)):
            v = hk.right(n, block)
            ref[rows, _tile(n)] = _words(v)
            out.append(v[:8])
        return out

    def token_mixing(h_v, w_v, first_v, *buffers):
        sums_v, left_v = buffers[:2], buffers[2:]
        tiles = [D // hk.p // LANE for hk in _HK12]
        units = TM // UNIT
        loads = [t * t * len(hk.products) for t, hk in zip(tiles, _HK12)]

        def w_copies(n, j):
            return [copy((w1_hbm, w2_hbm)[n], w_v.at[n], sem_mix.at[n, j], slice(None), _tile(c * tiles[n] + j))
                    for c in range(_HK12[n].p)]

        def w2_copies(q):
            return [] if q * tiles[1] % n_blk else w_copies(1, q * tiles[1] // n_blk)

        def x_copy(i):
            return copy(x_hbm, x_v, sem_x.at[i + 1], slice((i * TM + UNIT) // 2, min(S, (i + 1) * TM + UNIT) // 2))

        def block(n, j, r=0, size=None):
            k = D // 2 // _HK12[n].p
            return lambda a, c: w_v.at[n][_at(a * k + r, size or k), _tile(c * tiles[n] + j)]

        def prepare(q, k, parts):
            size = D // 2 // _HK12[1].p * tiles[1] // n_blk // parts
            j, r = q // (n_blk // tiles[1]), (q % (n_blk // tiles[1]) * parts + k) * size
            store_right(_HK12[1], sums_v[1].at[j], _at(r, size), lambda a, c: _bf(block(1, j, r, size)(a, c)))

        def norm(r0, ref, size, note=_same):
            def rows(r):
                xc, var = _moments(x_rows(r0 + r, RC), note)
                inv = lax.rsqrt(var + _EPS)
                part_v[_at(r0 + r, RC), :] = xc * (inv * (1.0 / _GELU_OUT))
                return xc * (inv * lax.rsqrt(var * inv * inv + _EPS) * _GELU_IN)
            store_left(_HK12[0], ref, rows, size, note)

        def shift(r0, ref, note=_same):
            def rows(r):
                return jnp.concatenate(
                    [h_v.at[c][pl.ds(r0 + r + 8 + (-1, 1, -2, 2)[4 * c * LANE // D], RC), :]
                     for c in range(D // LANE)], axis=1)
            store_left(_HK12[1], ref, rows, UNIT, note)

        def matmul(n, left, r0, load=_bf, arriving=False):
            for j in range(tiles[n]):
                def summed(k):
                    if not arriving:
                        return load(sums_v[n].at[j][:, _tile(k)])
                    w = _HK12[n].right(k, lambda a, c: _bf(block(n, j)(a, c))).astype(BF16)
                    sums_v[n].at[j][:, _tile(k)] = pltpu.bitcast(w, U32)
                    return w

                if arriving:
                    for c in w_copies(n, j):
                        c.wait()
                halves = _HK12[n].result(_HK12[n].accumulate(
                    lambda r: _bf(left.at[r][...]), lambda a, c: load(block(n, j)(a, c)), summed))
                for f, half in enumerate(halves):
                    for c, v in enumerate(half):
                        size = v.shape[0]
                        if n == 0:
                            h_v.at[c * tiles[n] + j][_at(8 + r0 + f * size, size, 8), :] = _gelu(v)
                        else:
                            part_v[_at(r0 + f * size, size), _tile(c * tiles[n] + j)] += v

        def h_unit(r0, k, pace):
            norm(r0 + UNIT, left_v[0].at[(k + 1) % 2], UNIT, pace.note)
            pace.spread(0.15 * loads[0], loads[0])
            matmul(0, left_v[0].at[k % 2], r0, pace.load)

        def h_body(i, _):
            for n in range(1, n_blk):
                @pl.when(i == n)
                def _():
                    for later in range(2, n_blk) if n == 1 else ():
                        for c in [x_copy(later)] + w2_copies(later - 1):
                            c.start()
                    for c in w2_copies(n_blk - 1) if n == 2 else ():
                        c.start()
                    for c in [x_copy(n)] + w2_copies(n - 1):
                        c.wait()

            for c in mlp_copies(i - 1):
                c.start()
            pace = _Pace(i < 0)
            for k in range(units):
                h_unit(i * TM + k * UNIT, k, pace)
                prepare(i - 1, k, units)
            return 0

        def mix_body(i, _):
            @pl.when(i == 0)
            def _():
                for c in mlp_copies(n_blk - 1):
                    c.start()

            @pl.when(i == 1)
            def _():
                for c in attn_copies(0):
                    c.start()

            for c in mlp_copies(i):
                c.wait()

            def sums(w, ref, k, tiles, n, r):
                r += i * (k // n_blk)
                return jnp.concatenate(store_right(_HK, ref.at[n], _at(r, 8), lambda a, c: _bf(
                    w[_at(a * k + r, 8), _tile(c * tiles + n)])), axis=0)

            side = [functools.partial(sums, w, ref, k, tiles, n, r)
                    for w, ref, k, tiles in ((w3_v, s3_v, kw, ft), (w4_v, s4_v, fw, dt))
                    for n in range(tiles) for r in range(0, k // n_blk, 8)]
            pace = _Pace(i < 0)
            for k in range(units):
                r0 = i * TM + k * UNIT
                for task in side[k * len(side) // units:(k + 1) * len(side) // units]:
                    pace.note(task())
                pace.spread(0.05 * loads[1], 0.95 * loads[1])
                shift(jnp.minimum(r0 + UNIT, S - UNIT), left_v[1].at[(k + 1) % 2], pace.note)
                pace.spread(0, 0.9 * loads[1])
                matmul(1, left_v[1].at[k % 2], r0, pace.load)
            return 0

        first = [copy(x_hbm, x_v, sem_x.at[k], rows)
                 for k, rows in enumerate((slice(0, TM // 4), slice(TM // 4, (TM + UNIT) // 2)))]
        for c in ([first[0]] + sum((w_copies(0, j) for j in range(tiles[0])), [])
                  + [first[1], x_copy(1)] + w2_copies(0) + [mem0_copy]):
            c.start()
        h_v[:, 0:8, :] = jnp.zeros((D // LANE, 8, LANE), F32)
        h_v[:, S + 8:S + 16, :] = jnp.zeros((D // LANE, 8, LANE), F32)
        x_v[S // 2:, :] = jnp.zeros((UNIT // 2, D), U32)
        first[0].wait()
        norm(0, first_v, TM // 2)
        matmul(0, first_v, 0, arriving=True)
        first[1].wait()
        pace = _Pace(jnp.square(part_v[0:8, 0:LANE]) < 0)
        norm(TM // 2, left_v[0].at[units // 2 % 2], UNIT)
        for k in range(units // 2, units):
            h_unit(k * UNIT, k, pace)
        lax.fori_loop(1, n_blk, h_body, 0)
        shift(0, left_v[1].at[0])
        for c in w2_copies(n_blk - 1):
            c.wait()
        for k in range(8):
            prepare(n_blk - 1, k, 8)
        lax.fori_loop(0, n_blk, mix_body, 0)

    def channel_mlp(sums_v, *buffers):
        left_v, hidden_v = buffers[:2], buffers[2:]
        units = S // UNIT // n_grp

        def norm(r0, slot, note=_same):
            def rows(r):
                xc, var = _moments(part_v[_at(r0 + r, RC), :], note)
                return xc * (lax.rsqrt(var + _EPS / _GELU_OUT ** 2) * _GELU_IN)
            store_left(_HK, left_v[slot], rows, UNIT, note)

        def body(g, _):
            @pl.when(g + 1 < n_grp)
            def _():
                for c in attn_copies(g + 1):
                    c.start()

            for c in attn_copies(g):
                c.wait()
            pace = _Pace(g < 0)

            def prepare_qkv(m, r):
                blocks = {}
                for j in range(0, P, 2):
                    for i in range(P):
                        rows = slice(i * kw + r, i * kw + r + 8)
                        raw = [raw_v.at[g % 2, m * P + j + par][rows, :] for par in range(2)]
                        for n in range(2):
                            blocks[i, j + n] = [pltpu.unpack_elementwise(
                                w, index=n, packed_dtype=BF16, unpacked_dtype=F32) for w in raw]
                            wqkv_v[m * H + g * P + j + n, rows, :] = pltpu.pack_elementwise(
                                blocks[i, j + n], packed_dtype=BF16)
                out = []
                for n in range(len(_HK.summed)):
                    v = [_HK.right(n, lambda i, j: blocks[i, j][par]) for par in range(2)]
                    sums_v.at[m * n_grp + g][r:r + 8, _tile(n)] = pltpu.pack_elementwise(v, packed_dtype=BF16)
                    out.append(v[0])
                return out

            def prepare_out(r):
                return store_right(_HK, sums_v.at[3 * n_grp + g], slice(r, r + 8), lambda i, j: _bf(
                    wo_v[_at(g * grows + i * (Dh // 2) + r % (Dh // 2), 8), _tile(j * dt + r // (Dh // 2))]))

            def up(k):
                for n in range(ft):
                    upper, lower = _HK.result(_HK.accumulate(
                        lambda r: _bf(left_v[k % 2].at[r][...]),
                        lambda i, j: pace.load(w3_v[i * kw:(i + 1) * kw, _tile(j * ft + n)]),
                        lambda r: pace.load(s3_v.at[n][:, _tile(r)])))
                    for r, v in enumerate(_HK.left([_gelu(v) for v in upper], [_gelu(v) for v in lower])):
                        hidden_v[k % 2].at[r][:, _tile(n)] = _words(v)
                        if r < 2 * P and (n + 1 < ft or k):
                            pace.note(v)
                    pace.spread(20, 47)

            def down(k):
                for n in range(dt):
                    halves = _HK.result(_HK.accumulate(
                        lambda r: _bf(hidden_v[k % 2].at[r][...]),
                        lambda i, j: pace.load(w4_v[i * fw:(i + 1) * fw, _tile(j * dt + n)]),
                        lambda r: pace.load(s4_v.at[n][:, _tile(r)])))
                    for f, half in enumerate(halves):
                        for j, v in enumerate(half):
                            rows = _at((g * units + k) * UNIT + f * (UNIT // 2), UNIT // 2)
                            part_v[rows, _tile(j * dt + n)] += v

            for m in range(3):
                for r in range(0, kw, 8):
                    pace.note(prepare_qkv(m, r)[7])
            for r in range(0, kw, 8):
                pace.note(prepare_out(r)[7])
            loads = units * 2 * ft * dt * n_prod
            pace.spread(0.64 * loads, 0.99 * loads)
            for k in range(units):
                norm((g * units + k + 1) * UNIT, (k + 1) % 2, pace.note)
                pace.spread(0, 264)
                up(k)
                if k > 0:
                    down(k - 1)
            down(units - 1)
            return 0

        norm(0, 0)
        lax.fori_loop(0, n_grp, body, 0)

    def recurrence(sums_v, own_v, left_v, next_v, hq_v, ho_v, ahead_v):
        scale = float(Dh) ** -0.5
        row = lax.broadcasted_iota(jnp.int32, (2 * L, 2 * L), 0)
        col = lax.broadcasted_iota(jnp.int32, (2 * L, 2 * L), 1)
        r_in = jnp.where(row >= L, row - L, row)
        c_in = jnp.where(col >= L, col - L, col)
        same_head = (row >= L) == (col >= L)
        keep = same_head & ((r_in < M) | (r_in >= c_in))
        fill = jnp.where(same_head, _MASKED / scale, -jnp.inf).astype(F32)

        def load_own(s):
            own_v[...] = _ln(x_rows(s * seg, seg)[:seg - 8])

        def load_next(s, q):
            next_v[8 * q:8 * q + 8, :] = _ln(x_rows(s * seg + seg - 16, 16)[8:])

        def load_left(mem=None):
            lower = next_v[...]
            upper = lower if mem is None else jnp.concatenate([mem, own_v[...]], axis=0)
            for n, v in enumerate(_HK.left(_split(upper, P), _split(lower, P))):
                if (n in _HKQ.lower) == (mem is None):
                    left_v.at[n][...] = _words(v)

        def operands(g, m):
            return (lambda n: _bf(left_v.at[n][...]),
                    lambda i, j: _bf(wqkv_v.at[m * H + g * P + j][i * kw:(i + 1) * kw, :]),
                    lambda n: _bf(sums_v.at[m * n_grp + g][:, _tile(n)]))

        ahead = list(zip([when for when, n in AHEAD.items() for _ in range(n)],
                         [(k // 3, k % 3, n) for k in range(n_grp, 3 * n_grp) for n in _HKQ.lower]))

        def run_ahead(*now):
            for k, (when, (g, m, n)) in enumerate(ahead):
                if when in now:
                    ahead_v[k] = _HKQ.product(n, *operands(g, m))

        def by_head(apart, dot, a, b):
            return jnp.concatenate([dot(a[:L], b), dot(a[L:], b)], axis=0) if apart else dot(a, b)

        def softmax(apart, q, k):
            s = jnp.where(keep, by_head(apart, _dot_nt, q, k.astype(BF16)), fill)
            e = jnp.exp2((s - jnp.max(s, axis=-1, keepdims=True)) * (scale * _LOG2E))
            return e, pl.reciprocal(jnp.sum(e, axis=-1, keepdims=True), full_range=False)

        def step(s, r, mem):
            first, last = r == 0, r == PERIOD - 1
            if not first:
                upper = jnp.concatenate([mem, own_v[...]], axis=0)

            def project(g):
                res = []
                for m in range(3):
                    h0 = m * H + g * P
                    if first:
                        tops, rest = _HKQ.result(_HKQ.accumulate(*operands(g, m), known={
                            which[2]: ahead_v.at[k] for k, (_, which) in enumerate(ahead) if which[:2] == (g, m)}))
                        for j in range(P):
                            hq_v[h0 + j] = rest[j][8:]
                        held = [v[:8] for v in rest]
                    else:
                        tops = [_dot(upper.astype(BF16), _bf(wqkv_v[h0 + j])) for j in range(P)]
                        held = [hq_v[h0 + j, 8 * (r - 1):8 * r, :] for j in range(P)]
                    res.append([jnp.concatenate([tops[j], held[j], tops[j + 1], held[j + 1]], axis=0)
                                for j in range(0, P, 2)])
                return list(zip(*res))

            def merge(g, heads, acc):
                tops, held = [o[:L - 8] for o in heads], [o[L - 8:] for o in heads]
                if last:
                    waiting[g] = _HK.left(tops, [jnp.concatenate([ho_v[:, _tile(g * P + j)], held[j]], axis=0)
                                                 for j in range(P)])
                    if g not in (1, 4, 5, n_grp - 1):
                        return acc
                    left = {a: waiting.pop(a) for a in sorted(waiting)}
                    k = Dh // 2
                    return _HKO.accumulate(
                        lambda n: jnp.concatenate([v[n].astype(BF16) for v in left.values()], axis=1),
                        lambda i, j: jnp.concatenate([
                            _bf(wo_v[a * grows + i * k:a * grows + (i + 1) * k, j * dt * LANE:(j + 1) * dt * LANE])
                            for a in left], axis=0),
                        lambda n: jnp.concatenate([
                            jnp.concatenate([_bf(sums_v.at[3 * n_grp + a][c * k:(c + 1) * k, _tile(n)])
                                             for c in range(dt)], axis=1) for a in left], axis=0),
                        acc or ())
                for j in range(P):
                    ho_v[8 * r:8 * r + 8, _tile(g * P + j)] = held[j]
                y = _dot(jnp.concatenate(tops, axis=1).astype(BF16), _bf(wo_v[g * grows:(g + 1) * grows, :]))
                return y if acc is None else acc + y

            lag, late = (4, (5, 6)) if last else (5, (4, 6)) if first else (5, (4, 5))
            qkv, prob, heads, waiting = {}, {}, {}, {}
            acc, done = None, 0
            for t in range(n_grp + 3):
                if t < n_grp:
                    qkv[t] = project(t)
                while done < (t - lag + 1 if t < n_grp else (late + (n_grp,))[t - n_grp]):
                    run_ahead((r, done))
                    acc = merge(done, heads.pop(done), acc)
                    done += 1
                if 0 <= t - 2 < n_grp:
                    heads[t - 2] = []
                    for (e, inv), (_, _, v) in zip(prob.pop(t - 2), qkv.pop(t - 2)):
                        o = by_head(t - 2 == n_grp - 1, _dot, e, v.astype(BF16)) * inv
                        heads[t - 2] += [o[:L], o[L:]]
                if 0 <= t - 1 < n_grp:
                    prob[t - 1] = [softmax(t == 1, q, k) for q, k, _ in qkv[t - 1]]
                if first and 1 <= t <= PERIOD:
                    load_next(jnp.minimum(s + PERIOD - 1 + t, n_seg - 1), t - 1)
                if first and t == n_grp:
                    load_left()
                if t == n_grp - 1:
                    load_own(jnp.minimum(s + 1, n_seg - 1))
            run_ahead((r, n_grp))
            if last:
                y, y_held = [jnp.concatenate(half, axis=1) for half in _HK.result(acc)]
                load_left(y[:M])
            else:
                y = acc
            base = x_rows(s * seg, seg) + _GELU_OUT * part_v[_at(s * seg, seg), :]
            x_v[_at(s * (seg // 2), 8), :] = _words(base[:16] + y[M:M + 16])
            tail = jnp.concatenate([base[16:24] + y[M + 16:], base[24:]], axis=0)
            if not last:
                part_v[_at(s * seg + 16, 16), :] = tail
            else:
                for q in range(PERIOD):
                    r0 = (s - r + q) * seg + 16
                    rest = part_v[_at(r0, 16), :] if q < r else tail
                    x_v[_at(r0 // 2, 8), :] = _words(jnp.concatenate(
                        [rest[:8], rest[8:] + y_held[8 * q:8 * q + 8]], axis=0))
            return y[:M]

        def period(p, _):
            mem = None
            for r in range(PERIOD):
                mem = step(p * PERIOD + r, r, mem)
            out_copy(_at(p * (PERIOD * seg // 2), PERIOD * seg // 2)).start()
            return 0

        mem0_copy.wait()
        for q in range(PERIOD):
            load_next(q, q)
        load_left()
        run_ahead(*AHEAD)
        load_own(0)
        load_left(mem0_v[...].astype(F32))
        lax.fori_loop(0, n_seg // PERIOD, period, 0)

    def with_attention_sums(sums_v):
        pl.run_scoped(
            functools.partial(channel_mlp, sums_v),
            *[pltpu.VMEM((n_prod, UNIT // 4, k // P), U32) for k in (D, D, FF, FF)])
        pl.run_scoped(
            functools.partial(recurrence, sums_v),
            pltpu.VMEM((seg - 8, D), F32),
            pltpu.VMEM((n_prod, (L - 8) // 2, D // P), U32),
            pltpu.VMEM((8 * PERIOD, D), F32),
            pltpu.VMEM((3 * H, 8 * (PERIOD - 1), Dh), F32),
            pltpu.VMEM((8 * (PERIOD - 1), H * Dh), F32),
            pltpu.VMEM((sum(AHEAD.values()), L - 8, Dh), F32))

    pl.run_scoped(
        token_mixing,
        pltpu.VMEM((D // LANE, S + 16, LANE), F32),
        pltpu.VMEM((2, D // 2, D), U32),
        pltpu.VMEM((len(_HK12[0].products), TM // 8, D // _HK12[0].p), U32),
        *[pltpu.VMEM((D // hk.p // LANE, D // 2 // hk.p, len(hk.summed) * LANE), U32) for hk in _HK12],
        *[pltpu.VMEM((2, len(hk.products), UNIT // 4, D // hk.p), U32) for hk in _HK12])
    pl.run_scoped(with_attention_sums, pltpu.VMEM((4 * n_grp, kw, len(_HK.summed) * LANE), U32))
    out_copy(slice(0, S // 2)).wait()


@functools.partial(jax.jit, static_argnames=("A_seg_len",))
def pallas_parallel_sum__memory_aug_recurrent_mem_tr__mixer_s_mlp__prompt_kernel(
    A_x: jax.Array,
    A_mem0: jax.Array,
    A_Wq: jax.Array,
    A_Wk: jax.Array,
    A_Wv: jax.Array,
    A_Wo: jax.Array,
    A_seg_len: int,
    B_x: jax.Array,
    B_w1: jax.Array,
    B_w2: jax.Array,
    B_w3: jax.Array,
    B_w4: jax.Array,
):
    del B_x
    B, S, D = A_x.shape
    H, Dh = A_Wq.shape[1:]
    M = A_mem0.shape[1]
    FF = B_w3.shape[1]
    assert (B, S, D, H, Dh, M, A_seg_len) == (1, 2048, 1024, 32, 128, 8, 32)
    sums = len(_HK.summed) * LANE

    hbm = pl.BlockSpec(memory_space=pl.ANY)
    out = pl.pallas_call(
        functools.partial(_kernel, seg=A_seg_len),
        out_shape=jax.ShapeDtypeStruct((S, D), A_x.dtype),
        in_specs=[hbm] * 10,
        out_specs=hbm,
        scratch_shapes=[
            pltpu.VMEM(((S + UNIT) // 2, D), U32),
            pltpu.VMEM((S + UNIT, D), F32),
            pltpu.VMEM((M, D), A_mem0.dtype),
            pltpu.VMEM((3 * H, D // 2, Dh), U32),
            pltpu.VMEM((H * Dh // 2, D), U32),
            pltpu.VMEM((2, 3 * P, D // 2, Dh), U32),
            pltpu.VMEM((D // 2, FF), U32),
            pltpu.VMEM((FF // 2, D), U32),
            pltpu.VMEM((FF // P // LANE, D // 2 // P, sums), U32),
            pltpu.VMEM((D // P // LANE, FF // 2 // P, sums), U32),
            pltpu.SemaphoreType.DMA((S // TM + 1,)),
            pltpu.SemaphoreType.DMA((2, D // 2 // LANE)),
            pltpu.SemaphoreType.DMA((S // TM,)),
            pltpu.SemaphoreType.DMA((H // P,)),
            pltpu.SemaphoreType.DMA,
            pltpu.SemaphoreType.DMA,
        ],
        compiler_params=pltpu.CompilerParams(
            vmem_limit_bytes=127 * 1024 * 1024, disable_bounds_checks=True),
    )(A_x.reshape(S, D), A_mem0.reshape(M, D),
      *[w.reshape(D // 2, 2, H, Dh) for w in (A_Wq, A_Wk, A_Wv)],
      A_Wo.reshape(H * Dh, D), B_w1, B_w2, B_w3, B_w4)
    return out.reshape(B, S, D)
```

```python
import functools

import jax
import jax.numpy as jnp
import numpy as np
from jax import lax
import jax.experimental.pallas as pl
import jax.experimental.pallas.tpu as pltpu

F32 = jnp.float32
BF16 = jnp.bfloat16
U32 = jnp.uint32

_EPS = 1e-5
_MASKED = -1e9
_LOG2E = float(np.log2(np.e))
_GELU_C = float(np.sqrt(2.0 / np.pi))
_GELU_IN = float(np.cbrt(_GELU_C * 0.044715))
_GELU_OUT = 0.5 / _GELU_IN

LANE = 128
TM = 512
UNIT = 128
RC = 16
P = 4
PERIOD = 4
AHEAD = {(0, 8): 12, (1, 8): 10, (2, 8): 8, (3, 5): 2, (3, 6): 8, (3, 7): 8, (3, 8): 12}


def _dot(a, b):
    return lax.dot_general(a, b, (((1,), (0,)), ((), ())), preferred_element_type=F32)


def _dot_nt(a, b):
    return lax.dot_general(a, b, (((1,), (1,)), ((), ())), preferred_element_type=F32)


def _bf(words):
    return pltpu.bitcast(words, BF16)


def _words(x):
    return pltpu.bitcast(x.astype(BF16), U32)


def _at(start, n, align=None):
    return pl.ds(start if isinstance(start, int) else pl.multiple_of(start, align or n), n)


def _tile(j):
    return _at(j * LANE, LANE)


def _split(x, n):
    k = x.shape[1] // n
    return [x[:, i * k:(i + 1) * k] for i in range(n)]


def _same(v):
    return v


def _moments(x, note=_same):
    inv_n = 1.0 / x.shape[-1]
    xc = x - note(jnp.sum(x, axis=-1, keepdims=True)) * inv_n
    return xc, note(jnp.sum(xc * xc, axis=-1, keepdims=True)) * inv_n


def _ln(x):
    xc, var = _moments(x)
    return xc * lax.rsqrt(var + _EPS)


def _gelu(y):
    return y * (1.0 + jnp.tanh(y * (_GELU_C / _GELU_IN + y * y)))


def _signed_sum(terms):
    terms = sorted(terms, key=lambda t: -t[0])
    assert terms[0][0] > 0
    total = terms[0][1]
    for sign, value in terms[1:]:
        total = total + value if sign > 0 else total - value
    return total


class _HopcroftKerr:
    def __init__(self, p, order=None):
        own = {0: ((1, 2, 1), (2, 0, 1)), 1: ((2, 1, -1), (0, 2, 1)), 2: ((1, 1, 1), (0, 0, 1))}
        cross = {(0, 1): ((1, 0, 1, 0, 1, -1), (0, -1, 0, -1, 0, 1, -1), (-1, 0, 1, 0, 1, 0, 1)),
                 (0, 2): ((2, 0, 1, 2, 1, 1), (-1, 0, 0, -1, 0, 1, -1), (0, -1, -1, 0, -1, 0, 1)),
                 (1, 2): ((2, 1, -1, 2, 0, 1), (0, -1, -1, 0, 1, 0, 1), (1, 0, 0, -1, 0, 1, -1))}
        products, diag, uses = [], {}, {}

        def product(left, out):
            products.append((left, out))
            return len(products) - 1

        def diagonal(idx, kind):
            diag[idx] = [product([(i, f, 1) for i in idx], [(i, g, 1) for i in idx]) for f, g, _ in own[kind]]

        def pair(a, ka, b, kb):
            if ka > kb:
                return pair(b, kb, a, ka)[::-1]
            (f0, f1, s, g0, g1, t), ab, ba = cross[ka, kb]
            diagonal(a + b, 3 - ka - kb)
            used = diag[a] + diag[b] + diag[a + b] + [product(
                [(i, f0, 1) for i in a] + [(i, f1, s) for i in b],
                [(i, g0, 1) for i in a] + [(i, g1, t) for i in b])]
            return dict(zip(used, ab)), dict(zip(used, ba))

        for i in range(p):
            diagonal((i,), i % 3)
            uses[i, i] = {r: sign for r, (_, _, sign) in zip(diag[i,], own[i % 3])}
        for j in range(p):
            for i in range(j):
                if i % 3 != j % 3:
                    uses[i, j], uses[j, i] = pair((i,), i % 3, (j,), j % 3)
        for j in range(p):
            for i in range(j % 3, j, 3):
                k = i + 1
                both = (i, k) if (i, k) in diag else (k, i)
                uses[i, j], uses[j, i] = pair(both, 3 - i % 3 - k % 3, (j,), j % 3)
                for ij, kj in (((i, j), (k, j)), ((j, i), (j, k))):
                    for r, c in uses[kj].items():
                        uses[ij][r] = uses[ij].get(r, 0) - c
        self.p = p
        self.order = order or range(len(products))
        self.products = [(left, [(i, j, c[r]) for (i, j), c in sorted(uses.items()) if c.get(r)], out)
                         for r, (left, out) in enumerate(products)]
        self.summed = [r for r, (_, weight, _) in enumerate(self.products) if len(weight) > 1]
        self.lower = [r for r in self.order if all(f == 1 for _, f, _ in self.products[r][0])]

    def left(self, upper, lower):
        forms = [(u, l, u - l) for u, l in zip(upper, lower)]
        return [_signed_sum([(sign, forms[i][f]) for i, f, sign in left]) for left, _, _ in self.products]

    def right(self, n, block):
        def value(key):
            return block(*key).astype(F32) if isinstance(key[0], int) else value(key[0]) - value(key[1])

        terms = {(i, j): sign for i, j, sign in self.products[self.summed[n]][1]}
        for a, b in (((0, 3), (3, 0)), ((1, 0), (0, 3)), ((0, 1), (3, 0)), ((1, 3), ((0, 3), (3, 0)))):
            if terms.get(a, 0) * terms.get(b, 0) < 0:
                terms[a, b] = terms.pop(a)
                del terms[b]
        return _signed_sum([(sign, value(key)) for key, sign in terms.items()])

    def product(self, r, left, block, summed):
        w = summed(self.summed.index(r)) if r in self.summed else block(*self.products[r][1][0][:2])
        return _dot(left(r), w)

    def accumulate(self, left, block, summed, acc=(), known=()):
        acc = dict(acc)
        for r in self.order:
            _, weight, out = self.products[r]
            flip = 1 if r in self.summed else weight[0][2]
            m = known[r][...] if r in known else self.product(r, left, block, summed)
            for j, f, sign in out:
                if (j, f) in acc:
                    acc[j, f] = acc[j, f] + m if sign * flip > 0 else acc[j, f] - m
                else:
                    acc[j, f] = m if sign * flip > 0 else -m
        return acc

    def result(self, acc):
        return [[functools.reduce(jnp.add, [acc[j, g] for g in (f, 2) if (j, g) in acc])
                 for j in range(self.p)] for f in range(2)]


_HK = _HopcroftKerr(P, (9, 5, 18, 16, 3, 15, 1, 24, 7, 19, 10, 0, 13, 14, 2, 22, 21, 12, 11, 6, 20, 25, 23, 17, 4, 8))
_HKQ = _HopcroftKerr(P, (10, 19, 18, 7, 16, 1, 2, 9, 5, 15, 23, 20, 11, 17, 4, 8, 22, 25, 0, 13, 21, 14, 24, 3, 12, 6))
_HKO = _HopcroftKerr(P, (5, 18, 16, 9, 15, 1, 3, 24, 7, 19, 10, 0, 22, 13, 14, 2, 20, 21, 12, 6, 4, 25, 23, 17, 11, 8))
_HK12 = (_HopcroftKerr(2, (4, 0, 1, 2, 3, 5, 6)),
         _HopcroftKerr(P, (9, 3, 5, 18, 16, 15, 1, 24, 19, 7, 0, 10, 13, 14, 2, 8, 22, 12, 6, 21, 4, 20, 25, 17, 23, 11)))


class _Pace:
    def __init__(self, never):
        self.never, self.noted, self.due, self.pos = never, [], [], 0

    def note(self, v):
        u = pltpu.bitcast(jnp.broadcast_to(v, (v.shape[0], max(v.shape[1], LANE))), U32)
        self.noted.append(functools.reduce(jnp.bitwise_or, [
            u[r:r + 8, c:c + LANE] for r in range(0, u.shape[0], 8) for c in range(0, u.shape[1], LANE)]))
        return v

    def spread(self, first, last):
        n = len(self.noted)
        self.due += [(self.pos + first + (k + 1) * (last - first) / n, v) for k, v in enumerate(self.noted)]
        self.due.sort(key=lambda t: t[0])
        self.noted = []

    def load(self, words):
        self.pos += words.shape[0] // (LANE // 2)
        hints = []
        while self.due and self.due[0][0] <= self.pos:
            hints.append(self.due.pop(0)[1])
        if hints:
            hint, parts = functools.reduce(jnp.bitwise_or, hints), []
            for k in range(0, words.shape[0], LANE // 2):
                parts += [jnp.where(self.never, hint, words[k:k + 8]), words[k + 8:k + LANE // 2]]
            words = jnp.concatenate(parts, axis=0)
        return _bf(words)


def _kernel(x_hbm, mem0_hbm, wq_hbm, wk_hbm, wv_hbm, wo_hbm, w1_hbm, w2_hbm, w3_hbm, w4_hbm,
            out_hbm,
            x_v, part_v, mem0_v, wqkv_v, wo_v, raw_v, w3_v, w4_v, s3_v, s4_v,
            sem_x, sem_mix, sem_mlp, sem_attn, sem_mem, sem_out, *, seg):
    S, D = x_hbm.shape
    H, Dh = wq_hbm.shape[-2:]
    M = mem0_hbm.shape[0]
    FF = w3_hbm.shape[1]
    L = M + seg
    n_blk = S // TM
    n_seg = S // seg
    n_grp = H // P
    n_prod = len(_HK.products)
    kw = D // 2 // P
    fw = FF // 2 // P
    ft = FF // P // LANE
    dt = D // P // LANE
    grows = P * Dh // 2

    def copy(hbm, vmem, sem, *idx):
        return pltpu.make_async_copy(hbm.bitcast(U32).at[idx], vmem.at[idx], sem)

    def attn_copies(g):
        copies = [copy(wo_hbm, wo_v, sem_attn.at[g], _at(g * grows, grows))]
        for m, hbm in enumerate((wq_hbm, wk_hbm, wv_hbm)):
            for j in range(P // 2):
                for par in range(2):
                    copies.append(pltpu.make_async_copy(
                        hbm.bitcast(U32).at[:, par, g * (P // 2) + j, :],
                        raw_v.at[g % 2, m * P + 2 * j + par], sem_attn.at[g]))
        return copies

    def mlp_copies(q):
        return [copy(hbm, vmem, sem_mlp.at[q], _at(i * n + q * (n // n_blk), n // n_blk, 8))
                for hbm, vmem, n in ((w3_hbm, w3_v, kw), (w4_hbm, w4_v, fw)) for i in range(P)]

    def out_copy(rows):
        return pltpu.make_async_copy(x_v.at[rows], out_hbm.bitcast(U32).at[rows], sem_out)

    mem0_copy = pltpu.make_async_copy(mem0_hbm, mem0_v, sem_mem)

    def x_rows(r0, n):
        return _bf(x_v[_at(r0 // 2, n // 2), :]).astype(F32)

    def store_left(hk, ref, rows, size, note):
        for q in range(0, size // 2, RC):
            for n, v in enumerate(hk.left(_split(rows(q), hk.p), _split(rows(size // 2 + q), hk.p))):
                ref.at[n][q // 2:(q + RC) // 2, :] = _words(v)
                if n >= len(hk.products) - 2:
                    note(v)

    def store_right(hk, ref, rows, block):
        out, block = [], functools.cache(block)
        for n in range(len(hk.summed)):
            v = hk.right(n, block)
            ref[rows, _tile(n)] = _words(v)
            out.append(v[:8])
        return out

    def token_mixing(h_v, w_v, first_v, *buffers):
        sums_v, left_v = buffers[:2], buffers[2:]
        tiles = [D // hk.p // LANE for hk in _HK12]
        units = TM // UNIT
        loads = [t * t * len(hk.products) for t, hk in zip(tiles, _HK12)]

        def w_copies(n, j):
            return [copy((w1_hbm, w2_hbm)[n], w_v.at[n], sem_mix.at[n, j], slice(None), _tile(c * tiles[n] + j))
                    for c in range(_HK12[n].p)]

        def w2_copies(q):
            return [] if q * tiles[1] % n_blk else w_copies(1, q * tiles[1] // n_blk)

        def x_copy(i):
            return copy(x_hbm, x_v, sem_x.at[i + 2], slice((i * TM + UNIT) // 2, min(S, (i + 1) * TM + UNIT) // 2))

        def block(n, j, r=0, size=None):
            k = D // 2 // _HK12[n].p
            return lambda a, c: w_v.at[n][_at(a * k + r, size or k), _tile(c * tiles[n] + j)]

        def prepare(q, k, parts):
            size = D // 2 // _HK12[1].p * tiles[1] // n_blk // parts
            j, r = q // (n_blk // tiles[1]), (q % (n_blk // tiles[1]) * parts + k) * size
            store_right(_HK12[1], sums_v[1].at[j], _at(r, size), lambda a, c: _bf(block(1, j, r, size)(a, c)))

        def norm(r0, ref, size, note=_same):
            def rows(r):
                xc, var = _moments(x_rows(r0 + r, RC), note)
                inv = lax.rsqrt(var + _EPS)
                part_v[_at(r0 + r, RC), :] = xc * (inv * (1.0 / _GELU_OUT))
                return xc * (inv * lax.rsqrt(var * inv * inv + _EPS) * _GELU_IN)
            store_left(_HK12[0], ref, rows, size, note)

        def shift(r0, ref, note=_same):
            def rows(r):
                return jnp.concatenate(
                    [h_v.at[c][pl.ds(r0 + r + 8 + (-1, 1, -2, 2)[4 * c * LANE // D], RC), :]
                     for c in range(D // LANE)], axis=1)
            store_left(_HK12[1], ref, rows, UNIT, note)

        def matmul(n, left, r0, load, arriving=None):
            for j in range(tiles[n]):
                def summed(k):
                    if not arriving:
                        return load(sums_v[n].at[j][:, _tile(k)])
                    w = _HK12[n].right(k, lambda a, c: _bf(block(n, j)(a, c))).astype(BF16)
                    sums_v[n].at[j][:, _tile(k)] = pltpu.bitcast(w, U32)
                    return w

                if arriving:
                    arriving(j)
                halves = _HK12[n].result(_HK12[n].accumulate(
                    lambda r: _bf(left.at[r][...]), lambda a, c: load(block(n, j)(a, c)), summed))
                for f, half in enumerate(halves):
                    for c, v in enumerate(half):
                        size = v.shape[0]
                        if n == 0:
                            h_v.at[c * tiles[n] + j][_at(8 + r0 + f * size, size, 8), :] = _gelu(v)
                        else:
                            part_v[_at(r0 + f * size, size), _tile(c * tiles[n] + j)] += v

        def h_unit(r0, k, pace):
            norm(r0 + UNIT, left_v[0].at[(k + 1) % 2], UNIT, pace.note)
            pace.spread(0.15 * loads[0], loads[0])
            matmul(0, left_v[0].at[k % 2], r0, pace.load)

        def h_body(i, _):
            for n in range(1, n_blk):
                @pl.when(i == n)
                def _():
                    for later in range(2, n_blk) if n == 1 else ():
                        for c in [x_copy(later)] + w2_copies(later - 1):
                            c.start()
                    for c in w2_copies(n_blk - 1) if n == 2 else ():
                        c.start()
                    for c in [x_copy(n)] + w2_copies(n - 1):
                        c.wait()

            for c in mlp_copies(i - 1):
                c.start()
            pace = _Pace(i < 0)
            for k in range(units):
                h_unit(i * TM + k * UNIT, k, pace)
                prepare(i - 1, k, units)
            return 0

        def mix_body(i, _):
            @pl.when(i == 0)
            def _():
                for c in mlp_copies(n_blk - 1):
                    c.start()

            @pl.when(i == 1)
            def _():
                for c in attn_copies(0):
                    c.start()

            for c in mlp_copies(i):
                c.wait()

            def sums(w, ref, k, tiles, n, r):
                r += i * (k // n_blk)
                return jnp.concatenate(store_right(_HK, ref.at[n], _at(r, 8), lambda a, c: _bf(
                    w[_at(a * k + r, 8), _tile(c * tiles + n)])), axis=0)

            side = [functools.partial(sums, w, ref, k, tiles, n, r)
                    for w, ref, k, tiles in ((w3_v, s3_v, kw, ft), (w4_v, s4_v, fw, dt))
                    for n in range(tiles) for r in range(0, k // n_blk, 8)]
            pace = _Pace(i < 0)
            for k in range(units):
                r0 = i * TM + k * UNIT
                for task in side[k * len(side) // units:(k + 1) * len(side) // units]:
                    pace.note(task())
                pace.spread(0.05 * loads[1], 0.95 * loads[1])
                shift(jnp.minimum(r0 + UNIT, S - UNIT), left_v[1].at[(k + 1) % 2], pace.note)
                pace.spread(0, 0.9 * loads[1])
                matmul(1, left_v[1].at[k % 2], r0, pace.load)
            return 0

        cuts = (0, TM // 4, TM // 4 + UNIT // 2, (TM + UNIT) // 2)
        first = [copy(x_hbm, x_v, sem_x.at[k], slice(*cuts[k:k + 2])) for k in range(3)]
        columns = [w_copies(0, j) for j in range(tiles[0])]
        columns[1].append(first[1])
        for c in [first[0]] + sum(columns, []) + [first[2], x_copy(1)] + w2_copies(0) + [mem0_copy]:
            c.start()
        h_v[:, 0:8, :] = jnp.zeros((D // LANE, 8, LANE), F32)
        h_v[:, S + 8:S + 16, :] = jnp.zeros((D // LANE, 8, LANE), F32)
        x_v[S // 2:, :] = jnp.zeros((UNIT // 2, D), U32)
        first[0].wait()
        norm(0, first_v, TM // 2)
        pace = _Pace(jnp.square(part_v[0:8, 0:LANE]) < 0)

        def arriving(j):
            for c in columns[j]:
                c.wait()
            if j == 1:
                norm(TM // 2, left_v[0].at[units // 2 % 2], UNIT, pace.note)
                pace.spread(0, 2 * tiles[0])

        matmul(0, first_v, 0, pace.load, arriving)
        first[2].wait()
        for k in range(units // 2, units):
            h_unit(k * UNIT, k, pace)
        lax.fori_loop(1, n_blk, h_body, 0)
        shift(0, left_v[1].at[0])
        for c in w2_copies(n_blk - 1):
            c.wait()
        for k in range(8):
            prepare(n_blk - 1, k, 8)
        lax.fori_loop(0, n_blk, mix_body, 0)

    def channel_mlp(sums_v, *buffers):
        left_v, hidden_v = buffers[:2], buffers[2:]
        units = S // UNIT // n_grp

        def norm(r0, slot, note=_same):
            def rows(r):
                xc, var = _moments(part_v[_at(r0 + r, RC), :], note)
                return xc * (lax.rsqrt(var + _EPS / _GELU_OUT ** 2) * _GELU_IN)
            store_left(_HK, left_v[slot], rows, UNIT, note)

        def body(g, _):
            @pl.when(g + 1 < n_grp)
            def _():
                for c in attn_copies(g + 1):
                    c.start()

            for c in attn_copies(g):
                c.wait()
            pace = _Pace(g < 0)

            def prepare_qkv(m, r):
                blocks = {}
                for j in range(0, P, 2):
                    for i in range(P):
                        rows = slice(i * kw + r, i * kw + r + 8)
                        raw = [raw_v.at[g % 2, m * P + j + par][rows, :] for par in range(2)]
                        for n in range(2):
                            blocks[i, j + n] = [pltpu.unpack_elementwise(
                                w, index=n, packed_dtype=BF16, unpacked_dtype=F32) for w in raw]
                            wqkv_v[m * H + g * P + j + n, rows, :] = pltpu.pack_elementwise(
                                blocks[i, j + n], packed_dtype=BF16)
                out = []
                for n in range(len(_HK.summed)):
                    v = [_HK.right(n, lambda i, j: blocks[i, j][par]) for par in range(2)]
                    sums_v.at[m * n_grp + g][r:r + 8, _tile(n)] = pltpu.pack_elementwise(v, packed_dtype=BF16)
                    out.append(v[0])
                return out

            def prepare_out(r):
                return store_right(_HK, sums_v.at[3 * n_grp + g], slice(r, r + 8), lambda i, j: _bf(
                    wo_v[_at(g * grows + i * (Dh // 2) + r % (Dh // 2), 8), _tile(j * dt + r // (Dh // 2))]))

            def up(k):
                for n in range(ft):
                    upper, lower = _HK.result(_HK.accumulate(
                        lambda r: _bf(left_v[k % 2].at[r][...]),
                        lambda i, j: pace.load(w3_v[i * kw:(i + 1) * kw, _tile(j * ft + n)]),
                        lambda r: pace.load(s3_v.at[n][:, _tile(r)])))
                    for r, v in enumerate(_HK.left([_gelu(v) for v in upper], [_gelu(v) for v in lower])):
                        hidden_v[k % 2].at[r][:, _tile(n)] = _words(v)
                        if r < 2 * P and (n + 1 < ft or k):
                            pace.note(v)
                    pace.spread(20, 47)

            def down(k):
                for n in range(dt):
                    halves = _HK.result(_HK.accumulate(
                        lambda r: _bf(hidden_v[k % 2].at[r][...]),
                        lambda i, j: pace.load(w4_v[i * fw:(i + 1) * fw, _tile(j * dt + n)]),
                        lambda r: pace.load(s4_v.at[n][:, _tile(r)])))
                    for f, half in enumerate(halves):
                        for j, v in enumerate(half):
                            rows = _at((g * units + k) * UNIT + f * (UNIT // 2), UNIT // 2)
                            part_v[rows, _tile(j * dt + n)] += v

            for m in range(3):
                for r in range(0, kw, 8):
                    pace.note(prepare_qkv(m, r)[7])
            for r in range(0, kw, 8):
                pace.note(prepare_out(r)[7])
            loads = units * 2 * ft * dt * n_prod
            pace.spread(0.64 * loads, 0.99 * loads)
            for k in range(units):
                norm((g * units + k + 1) * UNIT, (k + 1) % 2, pace.note)
                pace.spread(0, 264)
                up(k)
                if k > 0:
                    down(k - 1)
            down(units - 1)
            return 0

        norm(0, 0)
        lax.fori_loop(0, n_grp, body, 0)

    def recurrence(sums_v, own_v, left_v, next_v, hq_v, ho_v, ahead_v):
        scale = float(Dh) ** -0.5
        row = lax.broadcasted_iota(jnp.int32, (2 * L, 2 * L), 0)
        col = lax.broadcasted_iota(jnp.int32, (2 * L, 2 * L), 1)
        r_in = jnp.where(row >= L, row - L, row)
        c_in = jnp.where(col >= L, col - L, col)
        same_head = (row >= L) == (col >= L)
        keep = same_head & ((r_in < M) | (r_in >= c_in))
        fill = jnp.where(same_head, _MASKED / scale, -jnp.inf).astype(F32)

        def load_own(s):
            own_v[...] = _ln(x_rows(s * seg, seg)[:seg - 8])

        def load_next(s, q):
            next_v[8 * q:8 * q + 8, :] = _ln(x_rows(s * seg + seg - 16, 16)[8:])

        def load_left(mem=None):
            lower = next_v[...]
            upper = lower if mem is None else jnp.concatenate([mem, own_v[...]], axis=0)
            for n, v in enumerate(_HK.left(_split(upper, P), _split(lower, P))):
                if (n in _HKQ.lower) == (mem is None):
                    left_v.at[n][...] = _words(v)

        def operands(g, m):
            return (lambda n: _bf(left_v.at[n][...]),
                    lambda i, j: _bf(wqkv_v.at[m * H + g * P + j][i * kw:(i + 1) * kw, :]),
                    lambda n: _bf(sums_v.at[m * n_grp + g][:, _tile(n)]))

        ahead = list(zip([when for when, n in AHEAD.items() for _ in range(n)],
                         [(k // 3, k % 3, n) for k in range(n_grp, 3 * n_grp) for n in _HKQ.lower]))

        def run_ahead(*now):
            for k, (when, (g, m, n)) in enumerate(ahead):
                if when in now:
                    ahead_v[k] = _HKQ.product(n, *operands(g, m))

        def by_head(apart, dot, a, b):
            return jnp.concatenate([dot(a[:L], b), dot(a[L:], b)], axis=0) if apart else dot(a, b)

        def softmax(apart, q, k):
            s = jnp.where(keep, by_head(apart, _dot_nt, q, k.astype(BF16)), fill)
            e = jnp.exp2((s - jnp.max(s, axis=-1, keepdims=True)) * (scale * _LOG2E))
            return e, pl.reciprocal(jnp.sum(e, axis=-1, keepdims=True), full_range=False)

        def step(s, r, mem):
            first, last = r == 0, r == PERIOD - 1
            if not first:
                upper = jnp.concatenate([mem, own_v[...]], axis=0)

            def project(g):
                res = []
                for m in range(3):
                    h0 = m * H + g * P
                    if first:
                        tops, rest = _HKQ.result(_HKQ.accumulate(*operands(g, m), known={
                            which[2]: ahead_v.at[k] for k, (_, which) in enumerate(ahead) if which[:2] == (g, m)}))
                        for j in range(P):
                            hq_v[h0 + j] = rest[j][8:]
                        held = [v[:8] for v in rest]
                    else:
                        tops = [_dot(upper.astype(BF16), _bf(wqkv_v[h0 + j])) for j in range(P)]
                        held = [hq_v[h0 + j, 8 * (r - 1):8 * r, :] for j in range(P)]
                    res.append([jnp.concatenate([tops[j], held[j], tops[j + 1], held[j + 1]], axis=0)
                                for j in range(0, P, 2)])
                return list(zip(*res))

            def merge(g, heads, acc):
                tops, held = [o[:L - 8] for o in heads], [o[L - 8:] for o in heads]
                if last:
                    waiting[g] = _HK.left(tops, [jnp.concatenate([ho_v[:, _tile(g * P + j)], held[j]], axis=0)
                                                 for j in range(P)])
                    if g not in (1, 4, 5, n_grp - 1):
                        return acc
                    left = {a: waiting.pop(a) for a in sorted(waiting)}
                    k = Dh // 2
                    return _HKO.accumulate(
                        lambda n: jnp.concatenate([v[n].astype(BF16) for v in left.values()], axis=1),
                        lambda i, j: jnp.concatenate([
                            _bf(wo_v[a * grows + i * k:a * grows + (i + 1) * k, j * dt * LANE:(j + 1) * dt * LANE])
                            for a in left], axis=0),
                        lambda n: jnp.concatenate([
                            jnp.concatenate([_bf(sums_v.at[3 * n_grp + a][c * k:(c + 1) * k, _tile(n)])
                                             for c in range(dt)], axis=1) for a in left], axis=0),
                        acc or ())
                for j in range(P):
                    ho_v[8 * r:8 * r + 8, _tile(g * P + j)] = held[j]
                y = _dot(jnp.concatenate(tops, axis=1).astype(BF16), _bf(wo_v[g * grows:(g + 1) * grows, :]))
                return y if acc is None else acc + y

            lag, late = (4, (5, 6)) if last else (5, (4, 6)) if first else (5, (4, 5))
            qkv, prob, heads, waiting = {}, {}, {}, {}
            acc, done = None, 0
            for t in range(n_grp + 3):
                if t < n_grp:
                    qkv[t] = project(t)
                while done < (t - lag + 1 if t < n_grp else (late + (n_grp,))[t - n_grp]):
                    run_ahead((r, done))
                    acc = merge(done, heads.pop(done), acc)
                    done += 1
                if 0 <= t - 2 < n_grp:
                    heads[t - 2] = []
                    for (e, inv), (_, _, v) in zip(prob.pop(t - 2), qkv.pop(t - 2)):
                        o = by_head(t - 2 == n_grp - 1, _dot, e, v.astype(BF16)) * inv
                        heads[t - 2] += [o[:L], o[L:]]
                if 0 <= t - 1 < n_grp:
                    prob[t - 1] = [softmax(t == 1, q, k) for q, k, _ in qkv[t - 1]]
                if first and 1 <= t <= PERIOD:
                    load_next(jnp.minimum(s + PERIOD - 1 + t, n_seg - 1), t - 1)
                if first and t == n_grp:
                    load_left()
                if t == n_grp - 1:
                    load_own(jnp.minimum(s + 1, n_seg - 1))
            run_ahead((r, n_grp))
            if last:
                y, y_held = [jnp.concatenate(half, axis=1) for half in _HK.result(acc)]
                load_left(y[:M])
            else:
                y = acc
            base = x_rows(s * seg, seg) + _GELU_OUT * part_v[_at(s * seg, seg), :]
            x_v[_at(s * (seg // 2), 8), :] = _words(base[:16] + y[M:M + 16])
            tail = jnp.concatenate([base[16:24] + y[M + 16:], base[24:]], axis=0)
            if not last:
                part_v[_at(s * seg + 16, 16), :] = tail
            else:
                for q in range(PERIOD):
                    r0 = (s - r + q) * seg + 16
                    rest = part_v[_at(r0, 16), :] if q < r else tail
                    x_v[_at(r0 // 2, 8), :] = _words(jnp.concatenate(
                        [rest[:8], rest[8:] + y_held[8 * q:8 * q + 8]], axis=0))
            return y[:M]

        def period(p, _):
            mem = None
            for r in range(PERIOD):
                mem = step(p * PERIOD + r, r, mem)
            out_copy(_at(p * (PERIOD * seg // 2), PERIOD * seg // 2)).start()
            return 0

        mem0_copy.wait()
        for q in range(PERIOD):
            load_next(q, q)
        load_left()
        run_ahead(*AHEAD)
        load_own(0)
        load_left(mem0_v[...].astype(F32))
        lax.fori_loop(0, n_seg // PERIOD, period, 0)

    def with_attention_sums(sums_v):
        pl.run_scoped(
            functools.partial(channel_mlp, sums_v),
            *[pltpu.VMEM((n_prod, UNIT // 4, k // P), U32) for k in (D, D, FF, FF)])
        pl.run_scoped(
            functools.partial(recurrence, sums_v),
            pltpu.VMEM((seg - 8, D), F32),
            pltpu.VMEM((n_prod, (L - 8) // 2, D // P), U32),
            pltpu.VMEM((8 * PERIOD, D), F32),
            pltpu.VMEM((3 * H, 8 * (PERIOD - 1), Dh), F32),
            pltpu.VMEM((8 * (PERIOD - 1), H * Dh), F32),
            pltpu.VMEM((sum(AHEAD.values()), L - 8, Dh), F32))

    pl.run_scoped(
        token_mixing,
        pltpu.VMEM((D // LANE, S + 16, LANE), F32),
        pltpu.VMEM((2, D // 2, D), U32),
        pltpu.VMEM((len(_HK12[0].products), TM // 8, D // _HK12[0].p), U32),
        *[pltpu.VMEM((D // hk.p // LANE, D // 2 // hk.p, len(hk.summed) * LANE), U32) for hk in _HK12],
        *[pltpu.VMEM((2, len(hk.products), UNIT // 4, D // hk.p), U32) for hk in _HK12])
    pl.run_scoped(with_attention_sums, pltpu.VMEM((4 * n_grp, kw, len(_HK.summed) * LANE), U32))
    out_copy(slice(0, S // 2)).wait()


@functools.partial(jax.jit, static_argnames=("A_seg_len",))
def pallas_parallel_sum__memory_aug_recurrent_mem_tr__mixer_s_mlp__prompt_kernel(
    A_x: jax.Array,
    A_mem0: jax.Array,
    A_Wq: jax.Array,
    A_Wk: jax.Array,
    A_Wv: jax.Array,
    A_Wo: jax.Array,
    A_seg_len: int,
    B_x: jax.Array,
    B_w1: jax.Array,
    B_w2: jax.Array,
    B_w3: jax.Array,
    B_w4: jax.Array,
):
    del B_x
    B, S, D = A_x.shape
    H, Dh = A_Wq.shape[1:]
    M = A_mem0.shape[1]
    FF = B_w3.shape[1]
    assert (B, S, D, H, Dh, M, A_seg_len) == (1, 2048, 1024, 32, 128, 8, 32)
    sums = len(_HK.summed) * LANE

    hbm = pl.BlockSpec(memory_space=pl.ANY)
    out = pl.pallas_call(
        functools.partial(_kernel, seg=A_seg_len),
        out_shape=jax.ShapeDtypeStruct((S, D), A_x.dtype),
        in_specs=[hbm] * 10,
        out_specs=hbm,
        scratch_shapes=[
            pltpu.VMEM(((S + UNIT) // 2, D), U32),
            pltpu.VMEM((S + UNIT, D), F32),
            pltpu.VMEM((M, D), A_mem0.dtype),
            pltpu.VMEM((3 * H, D // 2, Dh), U32),
            pltpu.VMEM((H * Dh // 2, D), U32),
            pltpu.VMEM((2, 3 * P, D // 2, Dh), U32),
            pltpu.VMEM((D // 2, FF), U32),
            pltpu.VMEM((FF // 2, D), U32),
            pltpu.VMEM((FF // P // LANE, D // 2 // P, sums), U32),
            pltpu.VMEM((D // P // LANE, FF // 2 // P, sums), U32),
            pltpu.SemaphoreType.DMA((S // TM + 2,)),
            pltpu.SemaphoreType.DMA((2, D // 2 // LANE)),
            pltpu.SemaphoreType.DMA((S // TM,)),
            pltpu.SemaphoreType.DMA((H // P,)),
            pltpu.SemaphoreType.DMA,
            pltpu.SemaphoreType.DMA,
        ],
        compiler_params=pltpu.CompilerParams(
            vmem_limit_bytes=127 * 1024 * 1024, disable_bounds_checks=True),
    )(A_x.reshape(S, D), A_mem0.reshape(M, D),
      *[w.reshape(D // 2, 2, H, Dh) for w in (A_Wq, A_Wk, A_Wv)],
      A_Wo.reshape(H * Dh, D), B_w1, B_w2, B_w3, B_w4)
    return out.reshape(B, S, D)
```

```python
import functools

import jax
import jax.numpy as jnp
import numpy as np
from jax import lax
import jax.experimental.pallas as pl
import jax.experimental.pallas.tpu as pltpu

F32 = jnp.float32
BF16 = jnp.bfloat16
U32 = jnp.uint32

_EPS = 1e-5
_MASKED = -1e9
_LOG2E = float(np.log2(np.e))
_GELU_C = float(np.sqrt(2.0 / np.pi))
_GELU_IN = float(np.cbrt(_GELU_C * 0.044715))
_GELU_OUT = 0.5 / _GELU_IN

LANE = 128
TM = 512
UNIT = 128
RC = 16
P = 4
PERIOD = 4
AHEAD = {(0, 8): 12, (1, 8): 10, (2, 8): 8, (3, 5): 2, (3, 6): 8, (3, 7): 8, (3, 8): 12}


def _dot(a, b):
    return lax.dot_general(a, b, (((1,), (0,)), ((), ())), preferred_element_type=F32)


def _dot_nt(a, b):
    return lax.dot_general(a, b, (((1,), (1,)), ((), ())), preferred_element_type=F32)


def _bf(words):
    return pltpu.bitcast(words, BF16)


def _words(x):
    return pltpu.bitcast(x.astype(BF16), U32)


def _at(start, n, align=None):
    return pl.ds(start if isinstance(start, int) else pl.multiple_of(start, align or n), n)


def _tile(j):
    return _at(j * LANE, LANE)


def _split(x, n):
    k = x.shape[1] // n
    return [x[:, i * k:(i + 1) * k] for i in range(n)]


def _same(v):
    return v


def _moments(x, note=_same):
    inv_n = 1.0 / x.shape[-1]
    xc = x - note(jnp.sum(x, axis=-1, keepdims=True)) * inv_n
    return xc, note(jnp.sum(xc * xc, axis=-1, keepdims=True)) * inv_n


def _ln(x):
    xc, var = _moments(x)
    return xc * lax.rsqrt(var + _EPS)


def _gelu(y):
    return y * (1.0 + jnp.tanh(y * (_GELU_C / _GELU_IN + y * y)))


def _signed_sum(terms):
    terms = sorted(terms, key=lambda t: -t[0])
    assert terms[0][0] > 0
    total = terms[0][1]
    for sign, value in terms[1:]:
        total = total + value if sign > 0 else total - value
    return total


class _HopcroftKerr:
    def __init__(self, p, order=None):
        own = {0: ((1, 2, 1), (2, 0, 1)), 1: ((2, 1, -1), (0, 2, 1)), 2: ((1, 1, 1), (0, 0, 1))}
        cross = {(0, 1): ((1, 0, 1, 0, 1, -1), (0, -1, 0, -1, 0, 1, -1), (-1, 0, 1, 0, 1, 0, 1)),
                 (0, 2): ((2, 0, 1, 2, 1, 1), (-1, 0, 0, -1, 0, 1, -1), (0, -1, -1, 0, -1, 0, 1)),
                 (1, 2): ((2, 1, -1, 2, 0, 1), (0, -1, -1, 0, 1, 0, 1), (1, 0, 0, -1, 0, 1, -1))}
        products, diag, uses = [], {}, {}

        def product(left, out):
            products.append((left, out))
            return len(products) - 1

        def diagonal(idx, kind):
            diag[idx] = [product([(i, f, 1) for i in idx], [(i, g, 1) for i in idx]) for f, g, _ in own[kind]]

        def pair(a, ka, b, kb):
            if ka > kb:
                return pair(b, kb, a, ka)[::-1]
            (f0, f1, s, g0, g1, t), ab, ba = cross[ka, kb]
            diagonal(a + b, 3 - ka - kb)
            used = diag[a] + diag[b] + diag[a + b] + [product(
                [(i, f0, 1) for i in a] + [(i, f1, s) for i in b],
                [(i, g0, 1) for i in a] + [(i, g1, t) for i in b])]
            return dict(zip(used, ab)), dict(zip(used, ba))

        for i in range(p):
            diagonal((i,), i % 3)
            uses[i, i] = {r: sign for r, (_, _, sign) in zip(diag[i,], own[i % 3])}
        for j in range(p):
            for i in range(j):
                if i % 3 != j % 3:
                    uses[i, j], uses[j, i] = pair((i,), i % 3, (j,), j % 3)
        for j in range(p):
            for i in range(j % 3, j, 3):
                k = i + 1
                both = (i, k) if (i, k) in diag else (k, i)
                uses[i, j], uses[j, i] = pair(both, 3 - i % 3 - k % 3, (j,), j % 3)
                for ij, kj in (((i, j), (k, j)), ((j, i), (j, k))):
                    for r, c in uses[kj].items():
                        uses[ij][r] = uses[ij].get(r, 0) - c
        self.p = p
        self.order = order or range(len(products))
        self.products = [(left, [(i, j, c[r]) for (i, j), c in sorted(uses.items()) if c.get(r)], out)
                         for r, (left, out) in enumerate(products)]
        self.summed = [r for r, (_, weight, _) in enumerate(self.products) if len(weight) > 1]
        self.lower = [r for r in self.order if all(f == 1 for _, f, _ in self.products[r][0])]

    def left(self, upper, lower):
        forms = [(u, l, u - l) for u, l in zip(upper, lower)]
        return [_signed_sum([(sign, forms[i][f]) for i, f, sign in left]) for left, _, _ in self.products]

    def right(self, n, block):
        def value(key):
            return block(*key).astype(F32) if isinstance(key[0], int) else value(key[0]) - value(key[1])

        terms = {(i, j): sign for i, j, sign in self.products[self.summed[n]][1]}
        for a, b in (((0, 3), (3, 0)), ((1, 0), (0, 3)), ((0, 1), (3, 0)), ((1, 3), ((0, 3), (3, 0)))):
            if terms.get(a, 0) * terms.get(b, 0) < 0:
                terms[a, b] = terms.pop(a)
                del terms[b]
        return _signed_sum([(sign, value(key)) for key, sign in terms.items()])

    def product(self, r, left, block, summed):
        w = summed(self.summed.index(r)) if r in self.summed else block(*self.products[r][1][0][:2])
        return _dot(left(r), w)

    def accumulate(self, left, block, summed, acc=(), known=()):
        acc = dict(acc)
        for r in self.order:
            _, weight, out = self.products[r]
            flip = 1 if r in self.summed else weight[0][2]
            m = known[r][...] if r in known else self.product(r, left, block, summed)
            for j, f, sign in out:
                if (j, f) in acc:
                    acc[j, f] = acc[j, f] + m if sign * flip > 0 else acc[j, f] - m
                else:
                    acc[j, f] = m if sign * flip > 0 else -m
        return acc

    def result(self, acc):
        return [[functools.reduce(jnp.add, [acc[j, g] for g in (f, 2) if (j, g) in acc])
                 for j in range(self.p)] for f in range(2)]


_HK = _HopcroftKerr(P, (9, 5, 18, 16, 3, 15, 1, 24, 7, 19, 10, 0, 13, 14, 2, 22, 21, 12, 11, 6, 20, 25, 23, 17, 4, 8))
_HKQ = _HopcroftKerr(P, (10, 19, 18, 7, 16, 1, 2, 9, 5, 15, 23, 20, 11, 17, 4, 8, 22, 25, 0, 13, 21, 14, 24, 3, 12, 6))
_HKO = _HopcroftKerr(P, (5, 18, 16, 9, 15, 1, 3, 24, 7, 19, 10, 0, 22, 13, 14, 2, 20, 21, 12, 6, 4, 25, 23, 17, 11, 8))
_HK12 = (_HopcroftKerr(2, (4, 0, 1, 2, 3, 5, 6)),
         _HopcroftKerr(P, (9, 3, 5, 18, 16, 15, 1, 24, 19, 7, 0, 10, 13, 14, 2, 8, 22, 12, 6, 21, 4, 20, 25, 17, 23, 11)))


class _Pace:
    def __init__(self, never):
        self.never, self.noted, self.due, self.pos = never, [], [], 0

    def note(self, v):
        u = pltpu.bitcast(jnp.broadcast_to(v, (v.shape[0], max(v.shape[1], LANE))), U32)
        self.noted.append(functools.reduce(jnp.bitwise_or, [
            u[r:r + 8, c:c + LANE] for r in range(0, u.shape[0], 8) for c in range(0, u.shape[1], LANE)]))
        return v

    def spread(self, first, last):
        n = len(self.noted)
        self.due += [(self.pos + first + (k + 1) * (last - first) / n, v) for k, v in enumerate(self.noted)]
        self.due.sort(key=lambda t: t[0])
        self.noted = []

    def load(self, words):
        self.pos += words.shape[0] // (LANE // 2)
        hints = []
        while self.due and self.due[0][0] <= self.pos:
            hints.append(self.due.pop(0)[1])
        if hints:
            hint, parts = functools.reduce(jnp.bitwise_or, hints), []
            for k in range(0, words.shape[0], LANE // 2):
                parts += [jnp.where(self.never, hint, words[k:k + 8]), words[k + 8:k + LANE // 2]]
            words = jnp.concatenate(parts, axis=0)
        return _bf(words)


def _kernel(x_hbm, mem0_hbm, wq_hbm, wk_hbm, wv_hbm, wo_hbm, w1_hbm, w2_hbm, w3_hbm, w4_hbm,
            out_hbm,
            x_v, part_v, mem0_v, wqkv_v, wo_v, raw_v, w3_v, w4_v, s3_v, s4_v,
            sem_x, sem_mix, sem_mlp, sem_attn, sem_mem, sem_out, *, seg):
    S, D = x_hbm.shape
    H, Dh = wq_hbm.shape[-2:]
    M = mem0_hbm.shape[0]
    FF = w3_hbm.shape[1]
    L = M + seg
    n_blk = S // TM
    n_seg = S // seg
    n_grp = H // P
    n_prod = len(_HK.products)
    kw = D // 2 // P
    fw = FF // 2 // P
    ft = FF // P // LANE
    dt = D // P // LANE
    grows = P * Dh // 2

    def copy(hbm, vmem, sem, *idx):
        return pltpu.make_async_copy(hbm.bitcast(U32).at[idx], vmem.at[idx], sem)

    def attn_copies(g):
        copies = [copy(wo_hbm, wo_v, sem_attn.at[g], _at(g * grows, grows))]
        for m, hbm in enumerate((wq_hbm, wk_hbm, wv_hbm)):
            for j in range(P // 2):
                for par in range(2):
                    copies.append(pltpu.make_async_copy(
                        hbm.bitcast(U32).at[:, par, g * (P // 2) + j, :],
                        raw_v.at[g % 2, m * P + 2 * j + par], sem_attn.at[g]))
        return copies

    def mlp_copies(q):
        return [copy(hbm, vmem, sem_mlp.at[q], _at(i * n + q * (n // n_blk), n // n_blk, 8))
                for hbm, vmem, n in ((w3_hbm, w3_v, kw), (w4_hbm, w4_v, fw)) for i in range(P)]

    def out_copy(rows):
        return pltpu.make_async_copy(x_v.at[rows], out_hbm.bitcast(U32).at[rows], sem_out)

    mem0_copy = pltpu.make_async_copy(mem0_hbm, mem0_v, sem_mem)

    def x_rows(r0, n):
        return _bf(x_v[_at(r0 // 2, n // 2), :]).astype(F32)

    def store_left(hk, ref, rows, size, note):
        for q in range(0, size // 2, RC):
            for n, v in enumerate(hk.left(_split(rows(q), hk.p), _split(rows(size // 2 + q), hk.p))):
                ref.at[n][q // 2:(q + RC) // 2, :] = _words(v)
                if n >= len(hk.products) - 2:
                    note(v)

    def store_right(hk, ref, rows, block):
        out, block = [], functools.cache(block)
        for n in range(len(hk.summed)):
            v = hk.right(n, block)
            ref[rows, _tile(n)] = _words(v)
            out.append(v[:8])
        return out

    def token_mixing(h_v, w_v, first_v, *buffers):
        sums_v, left_v = buffers[:2], buffers[2:]
        tiles = [D // hk.p // LANE for hk in _HK12]
        units = TM // UNIT
        loads = [t * t * len(hk.products) for t, hk in zip(tiles, _HK12)]

        def w_copies(n, j):
            return [copy((w1_hbm, w2_hbm)[n], w_v.at[n], sem_mix.at[n, j], slice(None), _tile(c * tiles[n] + j))
                    for c in range(_HK12[n].p)]

        def w2_copies(q):
            return [] if q * tiles[1] % n_blk else w_copies(1, q * tiles[1] // n_blk)

        def x_copy(i):
            return copy(x_hbm, x_v, sem_x.at[i + 2], slice((i * TM + UNIT) // 2, min(S, (i + 1) * TM + UNIT) // 2))

        def block(n, j, r=0, size=None):
            k = D // 2 // _HK12[n].p
            return lambda a, c: w_v.at[n][_at(a * k + r, size or k), _tile(c * tiles[n] + j)]

        def prepare(q, k, parts):
            size = D // 2 // _HK12[1].p * tiles[1] // n_blk // parts
            j, r = q // (n_blk // tiles[1]), (q % (n_blk // tiles[1]) * parts + k) * size
            store_right(_HK12[1], sums_v[1].at[j], _at(r, size), lambda a, c: _bf(block(1, j, r, size)(a, c)))

        def norm(r0, ref, size, note=_same):
            def rows(r):
                xc, var = _moments(x_rows(r0 + r, RC), note)
                inv = lax.rsqrt(var + _EPS)
                part_v[_at(r0 + r, RC), :] = xc * (inv * (1.0 / _GELU_OUT))
                return xc * (inv * lax.rsqrt(var * inv * inv + _EPS) * _GELU_IN)
            store_left(_HK12[0], ref, rows, size, note)

        def shift(r0, ref, note=_same):
            def rows(r):
                return jnp.concatenate(
                    [h_v.at[c][pl.ds(r0 + r + 8 + (-1, 1, -2, 2)[4 * c * LANE // D], RC), :]
                     for c in range(D // LANE)], axis=1)
            store_left(_HK12[1], ref, rows, UNIT, note)

        def matmul(n, left, r0, load, arriving=None):
            for j in range(tiles[n]):
                def summed(k):
                    if not arriving:
                        return load(sums_v[n].at[j][:, _tile(k)])
                    w = _HK12[n].right(k, lambda a, c: _bf(block(n, j)(a, c))).astype(BF16)
                    sums_v[n].at[j][:, _tile(k)] = pltpu.bitcast(w, U32)
                    return w

                if arriving:
                    arriving(j)
                halves = _HK12[n].result(_HK12[n].accumulate(
                    lambda r: _bf(left.at[r][...]), lambda a, c: load(block(n, j)(a, c)), summed))
                for f, half in enumerate(halves):
                    for c, v in enumerate(half):
                        size = v.shape[0]
                        if n == 0:
                            h_v.at[c * tiles[n] + j][_at(8 + r0 + f * size, size, 8), :] = _gelu(v)
                        else:
                            part_v[_at(r0 + f * size, size), _tile(c * tiles[n] + j)] += v

        def h_unit(r0, k, pace):
            norm(r0 + UNIT, left_v[0].at[(k + 1) % 2], UNIT, pace.note)
            pace.spread(0.15 * loads[0], loads[0])
            matmul(0, left_v[0].at[k % 2], r0, pace.load)

        def h_body(i, _):
            for n in range(1, n_blk):
                @pl.when(i == n)
                def _():
                    for later in range(2, n_blk) if n == 1 else ():
                        for c in [x_copy(later)] + w2_copies(later - 1):
                            c.start()
                    for c in w2_copies(n_blk - 1) if n == 2 else ():
                        c.start()
                    for c in [x_copy(n)] + w2_copies(n - 1):
                        c.wait()

            for c in mlp_copies(i - 1):
                c.start()
            pace = _Pace(i < 0)
            for k in range(units):
                h_unit(i * TM + k * UNIT, k, pace)
                prepare(i - 1, k, units)
            return 0

        def mix_body(i, _):
            @pl.when(i == 0)
            def _():
                for c in mlp_copies(n_blk - 1):
                    c.start()

            @pl.when(i == 1)
            def _():
                for c in attn_copies(0):
                    c.start()

            for c in mlp_copies(i):
                c.wait()

            def sums(w, ref, k, tiles, n, r):
                r += i * (k // n_blk)
                return jnp.concatenate(store_right(_HK, ref.at[n], _at(r, 8), lambda a, c: _bf(
                    w[_at(a * k + r, 8), _tile(c * tiles + n)])), axis=0)

            side = [functools.partial(sums, w, ref, k, tiles, n, r)
                    for w, ref, k, tiles in ((w3_v, s3_v, kw, ft), (w4_v, s4_v, fw, dt))
                    for n in range(tiles) for r in range(0, k // n_blk, 8)]
            pace = _Pace(i < 0)
            for k in range(units):
                r0 = i * TM + k * UNIT
                for task in side[k * len(side) // units:(k + 1) * len(side) // units]:
                    pace.note(task())
                pace.spread(0.05 * loads[1], 0.95 * loads[1])
                shift(jnp.minimum(r0 + UNIT, S - UNIT), left_v[1].at[(k + 1) % 2], pace.note)
                pace.spread(0, 0.9 * loads[1])
                matmul(1, left_v[1].at[k % 2], r0, pace.load)
            return 0

        cuts = (0, TM // 4, TM // 4 + UNIT // 2, (TM + UNIT) // 2)
        first = [copy(x_hbm, x_v, sem_x.at[k], slice(*cuts[k:k + 2])) for k in range(3)]
        columns = [w_copies(0, j) for j in range(tiles[0])]
        columns[1].append(first[1])
        for c in [first[0]] + sum(columns, []) + [first[2], x_copy(1)] + w2_copies(0) + [mem0_copy]:
            c.start()
        h_v[:, 0:8, :] = jnp.zeros((D // LANE, 8, LANE), F32)
        h_v[:, S + 8:S + 16, :] = jnp.zeros((D // LANE, 8, LANE), F32)
        x_v[S // 2:, :] = jnp.zeros((UNIT // 2, D), U32)
        first[0].wait()
        norm(0, first_v, TM // 2)
        pace = _Pace(jnp.square(part_v[0:8, 0:LANE]) < 0)

        def arriving(j):
            for c in columns[j]:
                c.wait()
            if j == 1:
                norm(TM // 2, left_v[0].at[units // 2 % 2], UNIT, pace.note)
                pace.spread(0, 2 * tiles[0])

        matmul(0, first_v, 0, pace.load, arriving)
        first[2].wait()
        for k in range(units // 2, units):
            h_unit(k * UNIT, k, pace)
        lax.fori_loop(1, n_blk, h_body, 0)
        shift(0, left_v[1].at[0])
        for c in w2_copies(n_blk - 1):
            c.wait()
        for k in range(8):
            prepare(n_blk - 1, k, 8)
        lax.fori_loop(0, n_blk, mix_body, 0)

    def channel_mlp(sums_v, *buffers):
        left_v, hidden_v = buffers[:2], buffers[2:]
        units = S // UNIT // n_grp

        def norm(r0, slot, note=_same):
            def rows(r):
                xc, var = _moments(part_v[_at(r0 + r, RC), :], note)
                return xc * (lax.rsqrt(var + _EPS / _GELU_OUT ** 2) * _GELU_IN)
            store_left(_HK, left_v[slot], rows, UNIT, note)

        def body(g, _):
            @pl.when(g + 1 < n_grp)
            def _():
                for c in attn_copies(g + 1):
                    c.start()

            for c in attn_copies(g):
                c.wait()
            pace = _Pace(g < 0)

            def prepare_qkv(m, r):
                blocks = {}
                for j in range(0, P, 2):
                    for i in range(P):
                        rows = slice(i * kw + r, i * kw + r + 8)
                        even, odd = raw_v.at[g % 2, m * P + j][rows, :], raw_v.at[g % 2, m * P + j + 1][rows, :]
                        for n, w in enumerate(((even & jnp.uint32(0xFFFF)) | (odd << 16),
                                               (even >> 16) | (odd & jnp.uint32(0xFFFF0000)))):
                            wqkv_v[m * H + g * P + j + n, rows, :] = w
                            blocks[i, j + n] = _bf(w)
                return store_right(_HK, sums_v.at[m * n_grp + g], slice(r, r + 8), lambda i, j: blocks[i, j])

            def prepare_out(r):
                return store_right(_HK, sums_v.at[3 * n_grp + g], slice(r, r + 8), lambda i, j: _bf(
                    wo_v[_at(g * grows + i * (Dh // 2) + r % (Dh // 2), 8), _tile(j * dt + r // (Dh // 2))]))

            def up(k):
                for n in range(ft):
                    upper, lower = _HK.result(_HK.accumulate(
                        lambda r: _bf(left_v[k % 2].at[r][...]),
                        lambda i, j: pace.load(w3_v[i * kw:(i + 1) * kw, _tile(j * ft + n)]),
                        lambda r: pace.load(s3_v.at[n][:, _tile(r)])))
                    for r, v in enumerate(_HK.left([_gelu(v) for v in upper], [_gelu(v) for v in lower])):
                        hidden_v[k % 2].at[r][:, _tile(n)] = _words(v)
                        if r < 2 * P and (n + 1 < ft or k):
                            pace.note(v)
                    pace.spread(20, 47)

            def down(k):
                for n in range(dt):
                    halves = _HK.result(_HK.accumulate(
                        lambda r: _bf(hidden_v[k % 2].at[r][...]),
                        lambda i, j: pace.load(w4_v[i * fw:(i + 1) * fw, _tile(j * dt + n)]),
                        lambda r: pace.load(s4_v.at[n][:, _tile(r)])))
                    for f, half in enumerate(halves):
                        for j, v in enumerate(half):
                            rows = _at((g * units + k) * UNIT + f * (UNIT // 2), UNIT // 2)
                            part_v[rows, _tile(j * dt + n)] += v

            for m in range(3):
                for r in range(0, kw, 8):
                    pace.note(prepare_qkv(m, r)[7])
            for r in range(0, kw, 8):
                pace.note(prepare_out(r)[7])
            loads = units * 2 * ft * dt * n_prod
            pace.spread(0.64 * loads, 0.99 * loads)
            for k in range(units):
                norm((g * units + k + 1) * UNIT, (k + 1) % 2, pace.note)
                pace.spread(0, 264)
                up(k)
                if k > 0:
                    down(k - 1)
            down(units - 1)
            return 0

        norm(0, 0)
        lax.fori_loop(0, n_grp, body, 0)

    def recurrence(sums_v, own_v, left_v, next_v, hq_v, ho_v, ahead_v):
        scale = float(Dh) ** -0.5
        row = lax.broadcasted_iota(jnp.int32, (2 * L, 2 * L), 0)
        col = lax.broadcasted_iota(jnp.int32, (2 * L, 2 * L), 1)
        r_in = jnp.where(row >= L, row - L, row)
        c_in = jnp.where(col >= L, col - L, col)
        same_head = (row >= L) == (col >= L)
        keep = same_head & ((r_in < M) | (r_in >= c_in))
        fill = jnp.where(same_head, _MASKED / scale, -jnp.inf).astype(F32)

        def load_own(s):
            own_v[...] = _ln(x_rows(s * seg, seg)[:seg - 8])

        def load_next(s, q):
            next_v[8 * q:8 * q + 8, :] = _ln(x_rows(s * seg + seg - 16, 16)[8:])

        def load_left(mem=None):
            lower = next_v[...]
            upper = lower if mem is None else jnp.concatenate([mem, own_v[...]], axis=0)
            for n, v in enumerate(_HK.left(_split(upper, P), _split(lower, P))):
                if (n in _HKQ.lower) == (mem is None):
                    left_v.at[n][...] = _words(v)

        def operands(g, m):
            return (lambda n: _bf(left_v.at[n][...]),
                    lambda i, j: _bf(wqkv_v.at[m * H + g * P + j][i * kw:(i + 1) * kw, :]),
                    lambda n: _bf(sums_v.at[m * n_grp + g][:, _tile(n)]))

        ahead = list(zip([when for when, n in AHEAD.items() for _ in range(n)],
                         [(k // 3, k % 3, n) for k in range(n_grp, 3 * n_grp) for n in _HKQ.lower]))

        def run_ahead(*now):
            for k, (when, (g, m, n)) in enumerate(ahead):
                if when in now:
                    ahead_v[k] = _HKQ.product(n, *operands(g, m))

        def by_head(apart, dot, a, b):
            return jnp.concatenate([dot(a[:L], b), dot(a[L:], b)], axis=0) if apart else dot(a, b)

        def softmax(apart, q, k):
            s = jnp.where(keep, by_head(apart, _dot_nt, q, k.astype(BF16)), fill)
            e = jnp.exp2((s - jnp.max(s, axis=-1, keepdims=True)) * (scale * _LOG2E))
            return e, pl.reciprocal(jnp.sum(e, axis=-1, keepdims=True), full_range=False)

        def step(s, r, mem):
            first, last = r == 0, r == PERIOD - 1
            if not first:
                upper = jnp.concatenate([mem, own_v[...]], axis=0)

            def project(g):
                res = []
                for m in range(3):
                    h0 = m * H + g * P
                    if first:
                        tops, rest = _HKQ.result(_HKQ.accumulate(*operands(g, m), known={
                            which[2]: ahead_v.at[k] for k, (_, which) in enumerate(ahead) if which[:2] == (g, m)}))
                        for j in range(P):
                            hq_v[h0 + j] = rest[j][8:]
                        held = [v[:8] for v in rest]
                    else:
                        tops = [_dot(upper.astype(BF16), _bf(wqkv_v[h0 + j])) for j in range(P)]
                        held = [hq_v[h0 + j, 8 * (r - 1):8 * r, :] for j in range(P)]
                    res.append([jnp.concatenate([tops[j], held[j], tops[j + 1], held[j + 1]], axis=0)
                                for j in range(0, P, 2)])
                return list(zip(*res))

            def merge(g, heads, acc):
                tops, held = [o[:L - 8] for o in heads], [o[L - 8:] for o in heads]
                if last:
                    waiting[g] = _HK.left(tops, [jnp.concatenate([ho_v[:, _tile(g * P + j)], held[j]], axis=0)
                                                 for j in range(P)])
                    if g not in (1, 4, 5, n_grp - 1):
                        return acc
                    left = {a: waiting.pop(a) for a in sorted(waiting)}
                    k = Dh // 2
                    return _HKO.accumulate(
                        lambda n: jnp.concatenate([v[n].astype(BF16) for v in left.values()], axis=1),
                        lambda i, j: jnp.concatenate([
                            _bf(wo_v[a * grows + i * k:a * grows + (i + 1) * k, j * dt * LANE:(j + 1) * dt * LANE])
                            for a in left], axis=0),
                        lambda n: jnp.concatenate([
                            jnp.concatenate([_bf(sums_v.at[3 * n_grp + a][c * k:(c + 1) * k, _tile(n)])
                                             for c in range(dt)], axis=1) for a in left], axis=0),
                        acc or ())
                for j in range(P):
                    ho_v[8 * r:8 * r + 8, _tile(g * P + j)] = held[j]
                y = _dot(jnp.concatenate(tops, axis=1).astype(BF16), _bf(wo_v[g * grows:(g + 1) * grows, :]))
                return y if acc is None else acc + y

            lag, late = (4, (5, 6)) if last else (5, (4, 6)) if first else (5, (4, 5))
            qkv, prob, heads, waiting = {}, {}, {}, {}
            acc, done = None, 0
            for t in range(n_grp + 3):
                if t < n_grp:
                    qkv[t] = project(t)
                while done < (t - lag + 1 if t < n_grp else (late + (n_grp,))[t - n_grp]):
                    run_ahead((r, done))
                    acc = merge(done, heads.pop(done), acc)
                    done += 1
                if 0 <= t - 2 < n_grp:
                    heads[t - 2] = []
                    for (e, inv), (_, _, v) in zip(prob.pop(t - 2), qkv.pop(t - 2)):
                        o = by_head(t - 2 == n_grp - 1, _dot, e, v.astype(BF16)) * inv
                        heads[t - 2] += [o[:L], o[L:]]
                if 0 <= t - 1 < n_grp:
                    prob[t - 1] = [softmax(t == 1, q, k) for q, k, _ in qkv[t - 1]]
                if first and 1 <= t <= PERIOD:
                    load_next(jnp.minimum(s + PERIOD - 1 + t, n_seg - 1), t - 1)
                if first and t == n_grp:
                    load_left()
                if t == n_grp - 1:
                    load_own(jnp.minimum(s + 1, n_seg - 1))
            run_ahead((r, n_grp))
            if last:
                y, y_held = [jnp.concatenate(half, axis=1) for half in _HK.result(acc)]
                load_left(y[:M])
            else:
                y = acc
            base = x_rows(s * seg, seg) + _GELU_OUT * part_v[_at(s * seg, seg), :]
            x_v[_at(s * (seg // 2), 8), :] = _words(base[:16] + y[M:M + 16])
            tail = jnp.concatenate([base[16:24] + y[M + 16:], base[24:]], axis=0)
            if not last:
                part_v[_at(s * seg + 16, 16), :] = tail
            else:
                for q in range(PERIOD):
                    r0 = (s - r + q) * seg + 16
                    rest = part_v[_at(r0, 16), :] if q < r else tail
                    x_v[_at(r0 // 2, 8), :] = _words(jnp.concatenate(
                        [rest[:8], rest[8:] + y_held[8 * q:8 * q + 8]], axis=0))
            return y[:M]

        def period(p, _):
            mem = None
            for r in range(PERIOD):
                mem = step(p * PERIOD + r, r, mem)
            out_copy(_at(p * (PERIOD * seg // 2), PERIOD * seg // 2)).start()
            return 0

        mem0_copy.wait()
        for q in range(PERIOD):
            load_next(q, q)
        load_left()
        run_ahead(*AHEAD)
        load_own(0)
        load_left(mem0_v[...].astype(F32))
        lax.fori_loop(0, n_seg // PERIOD, period, 0)

    def with_attention_sums(sums_v):
        pl.run_scoped(
            functools.partial(channel_mlp, sums_v),
            *[pltpu.VMEM((n_prod, UNIT // 4, k // P), U32) for k in (D, D, FF, FF)])
        pl.run_scoped(
            functools.partial(recurrence, sums_v),
            pltpu.VMEM((seg - 8, D), F32),
            pltpu.VMEM((n_prod, (L - 8) // 2, D // P), U32),
            pltpu.VMEM((8 * PERIOD, D), F32),
            pltpu.VMEM((3 * H, 8 * (PERIOD - 1), Dh), F32),
            pltpu.VMEM((8 * (PERIOD - 1), H * Dh), F32),
            pltpu.VMEM((sum(AHEAD.values()), L - 8, Dh), F32))

    pl.run_scoped(
        token_mixing,
        pltpu.VMEM((D // LANE, S + 16, LANE), F32),
        pltpu.VMEM((2, D // 2, D), U32),
        pltpu.VMEM((len(_HK12[0].products), TM // 8, D // _HK12[0].p), U32),
        *[pltpu.VMEM((D // hk.p // LANE, D // 2 // hk.p, len(hk.summed) * LANE), U32) for hk in _HK12],
        *[pltpu.VMEM((2, len(hk.products), UNIT // 4, D // hk.p), U32) for hk in _HK12])
    pl.run_scoped(with_attention_sums, pltpu.VMEM((4 * n_grp, kw, len(_HK.summed) * LANE), U32))
    out_copy(slice(0, S // 2)).wait()


@functools.partial(jax.jit, static_argnames=("A_seg_len",))
def pallas_parallel_sum__memory_aug_recurrent_mem_tr__mixer_s_mlp__prompt_kernel(
    A_x: jax.Array,
    A_mem0: jax.Array,
    A_Wq: jax.Array,
    A_Wk: jax.Array,
    A_Wv: jax.Array,
    A_Wo: jax.Array,
    A_seg_len: int,
    B_x: jax.Array,
    B_w1: jax.Array,
    B_w2: jax.Array,
    B_w3: jax.Array,
    B_w4: jax.Array,
):
    del B_x
    B, S, D = A_x.shape
    H, Dh = A_Wq.shape[1:]
    M = A_mem0.shape[1]
    FF = B_w3.shape[1]
    assert (B, S, D, H, Dh, M, A_seg_len) == (1, 2048, 1024, 32, 128, 8, 32)
    sums = len(_HK.summed) * LANE

    hbm = pl.BlockSpec(memory_space=pl.ANY)
    out = pl.pallas_call(
        functools.partial(_kernel, seg=A_seg_len),
        out_shape=jax.ShapeDtypeStruct((S, D), A_x.dtype),
        in_specs=[hbm] * 10,
        out_specs=hbm,
        scratch_shapes=[
            pltpu.VMEM(((S + UNIT) // 2, D), U32),
            pltpu.VMEM((S + UNIT, D), F32),
            pltpu.VMEM((M, D), A_mem0.dtype),
            pltpu.VMEM((3 * H, D // 2, Dh), U32),
            pltpu.VMEM((H * Dh // 2, D), U32),
            pltpu.VMEM((2, 3 * P, D // 2, Dh), U32),
            pltpu.VMEM((D // 2, FF), U32),
            pltpu.VMEM((FF // 2, D), U32),
            pltpu.VMEM((FF // P // LANE, D // 2 // P, sums), U32),
            pltpu.VMEM((D // P // LANE, FF // 2 // P, sums), U32),
            pltpu.SemaphoreType.DMA((S // TM + 2,)),
            pltpu.SemaphoreType.DMA((2, D // 2 // LANE)),
            pltpu.SemaphoreType.DMA((S // TM,)),
            pltpu.SemaphoreType.DMA((H // P,)),
            pltpu.SemaphoreType.DMA,
            pltpu.SemaphoreType.DMA,
        ],
        compiler_params=pltpu.CompilerParams(
            vmem_limit_bytes=127 * 1024 * 1024, disable_bounds_checks=True),
    )(A_x.reshape(S, D), A_mem0.reshape(M, D),
      *[w.reshape(D // 2, 2, H, Dh) for w in (A_Wq, A_Wk, A_Wv)],
      A_Wo.reshape(H * Dh, D), B_w1, B_w2, B_w3, B_w4)
    return out.reshape(B, S, D)
```

```python
import functools

import jax
import jax.numpy as jnp
import numpy as np
from jax import lax
import jax.experimental.pallas as pl
import jax.experimental.pallas.tpu as pltpu

F32 = jnp.float32
BF16 = jnp.bfloat16
U32 = jnp.uint32

_EPS = 1e-5
_MASKED = -1e9
_LOG2E = float(np.log2(np.e))
_GELU_C = float(np.sqrt(2.0 / np.pi))
_GELU_IN = float(np.cbrt(_GELU_C * 0.044715))
_GELU_OUT = 0.5 / _GELU_IN

LANE = 128
TM = 512
UNIT = 128
RC = 16
P = 4
PERIOD = 4
AHEAD = {(0, 8): 12, (1, 8): 10, (2, 8): 8, (3, 5): 2, (3, 6): 8, (3, 7): 8, (3, 8): 12}


def _dot(a, b):
    return lax.dot_general(a, b, (((1,), (0,)), ((), ())), preferred_element_type=F32)


def _dot_nt(a, b):
    return lax.dot_general(a, b, (((1,), (1,)), ((), ())), preferred_element_type=F32)


def _bf(words):
    return pltpu.bitcast(words, BF16)


def _words(x):
    return pltpu.bitcast(x.astype(BF16), U32)


def _at(start, n, align=None):
    return pl.ds(start if isinstance(start, int) else pl.multiple_of(start, align or n), n)


def _tile(j):
    return _at(j * LANE, LANE)


def _split(x, n):
    k = x.shape[1] // n
    return [x[:, i * k:(i + 1) * k] for i in range(n)]


def _same(v):
    return v


def _moments(x, note=_same):
    inv_n = 1.0 / x.shape[-1]
    xc = x - note(jnp.sum(x, axis=-1, keepdims=True)) * inv_n
    return xc, note(jnp.sum(xc * xc, axis=-1, keepdims=True)) * inv_n


def _ln(x):
    xc, var = _moments(x)
    return xc * lax.rsqrt(var + _EPS)


def _gelu(y):
    return y * (1.0 + jnp.tanh(y * (_GELU_C / _GELU_IN + y * y)))


def _signed_sum(terms):
    terms = sorted(terms, key=lambda t: -t[0])
    assert terms[0][0] > 0
    total = terms[0][1]
    for sign, value in terms[1:]:
        total = total + value if sign > 0 else total - value
    return total


class _HopcroftKerr:
    def __init__(self, p, order=None):
        own = {0: ((1, 2, 1), (2, 0, 1)), 1: ((2, 1, -1), (0, 2, 1)), 2: ((1, 1, 1), (0, 0, 1))}
        cross = {(0, 1): ((1, 0, 1, 0, 1, -1), (0, -1, 0, -1, 0, 1, -1), (-1, 0, 1, 0, 1, 0, 1)),
                 (0, 2): ((2, 0, 1, 2, 1, 1), (-1, 0, 0, -1, 0, 1, -1), (0, -1, -1, 0, -1, 0, 1)),
                 (1, 2): ((2, 1, -1, 2, 0, 1), (0, -1, -1, 0, 1, 0, 1), (1, 0, 0, -1, 0, 1, -1))}
        products, diag, uses = [], {}, {}

        def product(left, out):
            products.append((left, out))
            return len(products) - 1

        def diagonal(idx, kind):
            diag[idx] = [product([(i, f, 1) for i in idx], [(i, g, 1) for i in idx]) for f, g, _ in own[kind]]

        def pair(a, ka, b, kb):
            if ka > kb:
                return pair(b, kb, a, ka)[::-1]
            (f0, f1, s, g0, g1, t), ab, ba = cross[ka, kb]
            diagonal(a + b, 3 - ka - kb)
            used = diag[a] + diag[b] + diag[a + b] + [product(
                [(i, f0, 1) for i in a] + [(i, f1, s) for i in b],
                [(i, g0, 1) for i in a] + [(i, g1, t) for i in b])]
            return dict(zip(used, ab)), dict(zip(used, ba))

        for i in range(p):
            diagonal((i,), i % 3)
            uses[i, i] = {r: sign for r, (_, _, sign) in zip(diag[i,], own[i % 3])}
        for j in range(p):
            for i in range(j):
                if i % 3 != j % 3:
                    uses[i, j], uses[j, i] = pair((i,), i % 3, (j,), j % 3)
        for j in range(p):
            for i in range(j % 3, j, 3):
                k = i + 1
                both = (i, k) if (i, k) in diag else (k, i)
                uses[i, j], uses[j, i] = pair(both, 3 - i % 3 - k % 3, (j,), j % 3)
                for ij, kj in (((i, j), (k, j)), ((j, i), (j, k))):
                    for r, c in uses[kj].items():
                        uses[ij][r] = uses[ij].get(r, 0) - c
        self.p = p
        self.order = order or range(len(products))
        self.products = [(left, [(i, j, c[r]) for (i, j), c in sorted(uses.items()) if c.get(r)], out)
                         for r, (left, out) in enumerate(products)]
        self.summed = [r for r, (_, weight, _) in enumerate(self.products) if len(weight) > 1]
        self.lower = [r for r in self.order if all(f == 1 for _, f, _ in self.products[r][0])]

    def left(self, upper, lower):
        forms = [(u, l, u - l) for u, l in zip(upper, lower)]
        return [_signed_sum([(sign, forms[i][f]) for i, f, sign in left]) for left, _, _ in self.products]

    def right(self, n, block):
        def value(key):
            return block(*key).astype(F32) if isinstance(key[0], int) else value(key[0]) - value(key[1])

        terms = {(i, j): sign for i, j, sign in self.products[self.summed[n]][1]}
        for a, b in (((0, 3), (3, 0)), ((1, 0), (0, 3)), ((0, 1), (3, 0)), ((1, 3), ((0, 3), (3, 0)))):
            if terms.get(a, 0) * terms.get(b, 0) < 0:
                terms[a, b] = terms.pop(a)
                del terms[b]
        return _signed_sum([(sign, value(key)) for key, sign in terms.items()])

    def product(self, r, left, block, summed):
        w = summed(self.summed.index(r)) if r in self.summed else block(*self.products[r][1][0][:2])
        return _dot(left(r), w)

    def accumulate(self, left, block, summed, acc=(), known=()):
        acc = dict(acc)
        for r in self.order:
            _, weight, out = self.products[r]
            flip = 1 if r in self.summed else weight[0][2]
            m = known[r][...] if r in known else self.product(r, left, block, summed)
            for j, f, sign in out:
                if (j, f) in acc:
                    acc[j, f] = acc[j, f] + m if sign * flip > 0 else acc[j, f] - m
                else:
                    acc[j, f] = m if sign * flip > 0 else -m
        return acc

    def result(self, acc):
        return [[functools.reduce(jnp.add, [acc[j, g] for g in (f, 2) if (j, g) in acc])
                 for j in range(self.p)] for f in range(2)]


_HK = _HopcroftKerr(P, (9, 5, 18, 16, 3, 15, 1, 24, 7, 19, 0, 10, 13, 14, 2, 22, 21, 12, 11, 6, 20, 25, 23, 17, 4, 8))
_HKQ = _HopcroftKerr(P, (10, 18, 19, 7, 16, 1, 2, 9, 5, 15, 23, 20, 11, 17, 4, 8, 22, 25, 0, 13, 21, 14, 24, 3, 12, 6))
_HKO = _HopcroftKerr(P, (5, 18, 16, 9, 15, 1, 24, 7, 19, 10, 0, 22, 3, 13, 14, 2, 20, 21, 12, 6, 4, 25, 23, 17, 11, 8))
_HK12 = (_HopcroftKerr(2, (4, 0, 1, 3, 2, 5, 6)),
         _HopcroftKerr(P, (3, 9, 5, 18, 16, 15, 24, 1, 19, 7, 0, 10, 13, 14, 2, 8, 22, 6, 12, 4, 21, 20, 25, 17, 23, 11)))


class _Pace:
    def __init__(self, never):
        self.never, self.noted, self.due, self.pos = never, [], [], 0

    def note(self, v):
        u = pltpu.bitcast(jnp.broadcast_to(v, (v.shape[0], max(v.shape[1], LANE))), U32)
        self.noted.append(functools.reduce(jnp.bitwise_or, [
            u[r:r + 8, c:c + LANE] for r in range(0, u.shape[0], 8) for c in range(0, u.shape[1], LANE)]))
        return v

    def spread(self, first, last):
        n = len(self.noted)
        self.due += [(self.pos + first + (k + 1) * (last - first) / n, v) for k, v in enumerate(self.noted)]
        self.due.sort(key=lambda t: t[0])
        self.noted = []

    def load(self, words):
        self.pos += words.shape[0] // (LANE // 2)
        hints = []
        while self.due and self.due[0][0] <= self.pos:
            hints.append(self.due.pop(0)[1])
        if hints:
            hint, parts = functools.reduce(jnp.bitwise_or, hints), []
            for k in range(0, words.shape[0], LANE // 2):
                parts += [jnp.where(self.never, hint, words[k:k + 8]), words[k + 8:k + LANE // 2]]
            words = jnp.concatenate(parts, axis=0)
        return _bf(words)


def _kernel(x_hbm, mem0_hbm, wq_hbm, wk_hbm, wv_hbm, wo_hbm, w1_hbm, w2_hbm, w3_hbm, w4_hbm,
            out_hbm,
            x_v, part_v, mem0_v, wqkv_v, wo_v, raw_v, w3_v, w4_v, s3_v, s4_v,
            sem_x, sem_mix, sem_mlp, sem_attn, sem_mem, sem_out, *, seg):
    S, D = x_hbm.shape
    H, Dh = wq_hbm.shape[-2:]
    M = mem0_hbm.shape[0]
    FF = w3_hbm.shape[1]
    L = M + seg
    n_blk = S // TM
    n_seg = S // seg
    n_grp = H // P
    n_prod = len(_HK.products)
    kw = D // 2 // P
    fw = FF // 2 // P
    ft = FF // P // LANE
    dt = D // P // LANE
    grows = P * Dh // 2

    def copy(hbm, vmem, sem, *idx):
        return pltpu.make_async_copy(hbm.bitcast(U32).at[idx], vmem.at[idx], sem)

    def attn_copies(g):
        copies = [copy(wo_hbm, wo_v, sem_attn.at[g], _at(g * grows, grows))]
        for m, hbm in enumerate((wq_hbm, wk_hbm, wv_hbm)):
            for j in range(P // 2):
                for par in range(2):
                    copies.append(pltpu.make_async_copy(
                        hbm.bitcast(U32).at[:, par, g * (P // 2) + j, :],
                        raw_v.at[g % 2, m * P + 2 * j + par], sem_attn.at[g]))
        return copies

    def mlp_copies(q):
        return [copy(hbm, vmem, sem_mlp.at[q], _at(i * n + q * (n // n_blk), n // n_blk, 8))
                for hbm, vmem, n in ((w3_hbm, w3_v, kw), (w4_hbm, w4_v, fw)) for i in range(P)]

    def out_copy(rows):
        return pltpu.make_async_copy(x_v.at[rows], out_hbm.bitcast(U32).at[rows], sem_out)

    mem0_copy = pltpu.make_async_copy(mem0_hbm, mem0_v, sem_mem)

    def x_rows(r0, n):
        return _bf(x_v[_at(r0 // 2, n // 2), :]).astype(F32)

    def store_left(hk, ref, rows, size, note):
        for q in range(0, size // 2, RC):
            for n, v in enumerate(hk.left(_split(rows(q), hk.p), _split(rows(size // 2 + q), hk.p))):
                ref.at[n][q // 2:(q + RC) // 2, :] = _words(v)
                if n >= len(hk.products) - 2:
                    note(v)

    def store_right(hk, ref, rows, block):
        out, block = [], functools.cache(block)
        for n in range(len(hk.summed)):
            v = hk.right(n, block)
            ref[rows, _tile(n)] = _words(v)
            out.append(v[:8])
        return out

    def token_mixing(h_v, w_v, first_v, *buffers):
        sums_v, left_v = buffers[:2], buffers[2:]
        tiles = [D // hk.p // LANE for hk in _HK12]
        units = TM // UNIT
        loads = [t * t * len(hk.products) for t, hk in zip(tiles, _HK12)]

        def w_copies(n, j):
            return [copy((w1_hbm, w2_hbm)[n], w_v.at[n], sem_mix.at[n, j], slice(None), _tile(c * tiles[n] + j))
                    for c in range(_HK12[n].p)]

        def w2_copies(q):
            return [] if q * tiles[1] % n_blk else w_copies(1, q * tiles[1] // n_blk)

        def x_copy(i):
            return copy(x_hbm, x_v, sem_x.at[i + 2], slice((i * TM + UNIT) // 2, min(S, (i + 1) * TM + UNIT) // 2))

        def block(n, j, r=0, size=None):
            k = D // 2 // _HK12[n].p
            return lambda a, c: w_v.at[n][_at(a * k + r, size or k), _tile(c * tiles[n] + j)]

        def prepare(q, k, parts):
            size = D // 2 // _HK12[1].p * tiles[1] // n_blk // parts
            j, r = q // (n_blk // tiles[1]), (q % (n_blk // tiles[1]) * parts + k) * size
            store_right(_HK12[1], sums_v[1].at[j], _at(r, size), lambda a, c: _bf(block(1, j, r, size)(a, c)))

        def norm(r0, ref, size, note=_same):
            def rows(r):
                xc, var = _moments(x_rows(r0 + r, RC), note)
                inv = lax.rsqrt(var + _EPS)
                part_v[_at(r0 + r, RC), :] = xc * (inv * (1.0 / _GELU_OUT))
                return xc * (inv * lax.rsqrt(var * inv * inv + _EPS) * _GELU_IN)
            store_left(_HK12[0], ref, rows, size, note)

        def shift(r0, ref, note=_same):
            def rows(r):
                return jnp.concatenate(
                    [h_v.at[c][pl.ds(r0 + r + 8 + (-1, 1, -2, 2)[4 * c * LANE // D], RC), :]
                     for c in range(D // LANE)], axis=1)
            store_left(_HK12[1], ref, rows, UNIT, note)

        def matmul(n, left, r0, load, arriving=None):
            for j in range(tiles[n]):
                def summed(k):
                    if not arriving:
                        return load(sums_v[n].at[j][:, _tile(k)])
                    w = _HK12[n].right(k, lambda a, c: _bf(block(n, j)(a, c))).astype(BF16)
                    sums_v[n].at[j][:, _tile(k)] = pltpu.bitcast(w, U32)
                    return w

                if arriving:
                    arriving(j)
                halves = _HK12[n].result(_HK12[n].accumulate(
                    lambda r: _bf(left.at[r][...]), lambda a, c: load(block(n, j)(a, c)), summed))
                for f, half in enumerate(halves):
                    for c, v in enumerate(half):
                        size = v.shape[0]
                        if n == 0:
                            h_v.at[c * tiles[n] + j][_at(8 + r0 + f * size, size, 8), :] = _gelu(v)
                        else:
                            part_v[_at(r0 + f * size, size), _tile(c * tiles[n] + j)] += v

        def h_unit(r0, k, pace):
            norm(r0 + UNIT, left_v[0].at[(k + 1) % 2], UNIT, pace.note)
            pace.spread(0.15 * loads[0], loads[0])
            matmul(0, left_v[0].at[k % 2], r0, pace.load)

        def h_body(i, _):
            for n in range(1, n_blk):
                @pl.when(i == n)
                def _():
                    for later in range(2, n_blk) if n == 1 else ():
                        for c in [x_copy(later)] + w2_copies(later - 1):
                            c.start()
                    for c in w2_copies(n_blk - 1) if n == 2 else ():
                        c.start()
                    for c in [x_copy(n)] + w2_copies(n - 1):
                        c.wait()

            for c in mlp_copies(i - 1):
                c.start()
            pace = _Pace(i < 0)
            for k in range(units):
                h_unit(i * TM + k * UNIT, k, pace)
                prepare(i - 1, k, units)
            return 0

        def mix_body(i, _):
            @pl.when(i == 0)
            def _():
                for c in mlp_copies(n_blk - 1):
                    c.start()

            @pl.when(i == 1)
            def _():
                for c in attn_copies(0):
                    c.start()

            for c in mlp_copies(i):
                c.wait()

            def sums(w, ref, k, tiles, n, r):
                r += i * (k // n_blk)
                return jnp.concatenate(store_right(_HK, ref.at[n], _at(r, 8), lambda a, c: _bf(
                    w[_at(a * k + r, 8), _tile(c * tiles + n)])), axis=0)

            side = [functools.partial(sums, w, ref, k, tiles, n, r)
                    for w, ref, k, tiles in ((w3_v, s3_v, kw, ft), (w4_v, s4_v, fw, dt))
                    for n in range(tiles) for r in range(0, k // n_blk, 8)]
            pace = _Pace(i < 0)
            for k in range(units):
                r0 = i * TM + k * UNIT
                for task in side[k * len(side) // units:(k + 1) * len(side) // units]:
                    pace.note(task())
                pace.spread(0.05 * loads[1], 0.95 * loads[1])
                shift(jnp.minimum(r0 + UNIT, S - UNIT), left_v[1].at[(k + 1) % 2], pace.note)
                pace.spread(0, 0.9 * loads[1])
                matmul(1, left_v[1].at[k % 2], r0, pace.load)
            return 0

        cuts = (0, TM // 4, TM // 4 + UNIT // 2, (TM + UNIT) // 2)
        first = [copy(x_hbm, x_v, sem_x.at[k], slice(*cuts[k:k + 2])) for k in range(3)]
        columns = [w_copies(0, j) for j in range(tiles[0])]
        columns[1].append(first[1])
        for c in [first[0]] + sum(columns, []) + [first[2], x_copy(1)] + w2_copies(0) + [mem0_copy]:
            c.start()
        h_v[:, 0:8, :] = jnp.zeros((D // LANE, 8, LANE), F32)
        h_v[:, S + 8:S + 16, :] = jnp.zeros((D // LANE, 8, LANE), F32)
        x_v[S // 2:, :] = jnp.zeros((UNIT // 2, D), U32)
        first[0].wait()
        norm(0, first_v, TM // 2)
        pace = _Pace(jnp.square(part_v[0:8, 0:LANE]) < 0)

        def arriving(j):
            for c in columns[j]:
                c.wait()
            if j == 1:
                norm(TM // 2, left_v[0].at[units // 2 % 2], UNIT, pace.note)
                pace.spread(0, 2 * tiles[0])

        matmul(0, first_v, 0, pace.load, arriving)
        first[2].wait()
        for k in range(units // 2, units):
            h_unit(k * UNIT, k, pace)
        lax.fori_loop(1, n_blk, h_body, 0)
        shift(0, left_v[1].at[0])
        for c in w2_copies(n_blk - 1):
            c.wait()
        for k in range(8):
            prepare(n_blk - 1, k, 8)
        lax.fori_loop(0, n_blk, mix_body, 0)

    def channel_mlp(sums_v, *buffers):
        left_v, hidden_v = buffers[:2], buffers[2:]
        units = S // UNIT // n_grp

        def norm(r0, slot, note=_same):
            def rows(r):
                xc, var = _moments(part_v[_at(r0 + r, RC), :], note)
                return xc * (lax.rsqrt(var + _EPS / _GELU_OUT ** 2) * _GELU_IN)
            store_left(_HK, left_v[slot], rows, UNIT, note)

        def body(g, _):
            @pl.when(g + 1 < n_grp)
            def _():
                for c in attn_copies(g + 1):
                    c.start()

            for c in attn_copies(g):
                c.wait()
            pace = _Pace(g < 0)

            def prepare_qkv(m, r):
                blocks = {}
                for j in range(0, P, 2):
                    for i in range(P):
                        rows = slice(i * kw + r, i * kw + r + 8)
                        even, odd = raw_v.at[g % 2, m * P + j][rows, :], raw_v.at[g % 2, m * P + j + 1][rows, :]
                        for n, w in enumerate(((even & jnp.uint32(0xFFFF)) | (odd << 16),
                                               (even >> 16) | (odd & jnp.uint32(0xFFFF0000)))):
                            wqkv_v[m * H + g * P + j + n, rows, :] = w
                            blocks[i, j + n] = _bf(w)
                return store_right(_HK, sums_v.at[m * n_grp + g], slice(r, r + 8), lambda i, j: blocks[i, j])

            def prepare_out(r):
                return store_right(_HK, sums_v.at[3 * n_grp + g], slice(r, r + 8), lambda i, j: _bf(
                    wo_v[_at(g * grows + i * (Dh // 2) + r % (Dh // 2), 8), _tile(j * dt + r // (Dh // 2))]))

            def up(k):
                for n in range(ft):
                    upper, lower = _HK.result(_HK.accumulate(
                        lambda r: _bf(left_v[k % 2].at[r][...]),
                        lambda i, j: pace.load(w3_v[i * kw:(i + 1) * kw, _tile(j * ft + n)]),
                        lambda r: pace.load(s3_v.at[n][:, _tile(r)])))
                    for r, v in enumerate(_HK.left([_gelu(v) for v in upper], [_gelu(v) for v in lower])):
                        hidden_v[k % 2].at[r][:, _tile(n)] = _words(v)
                        if r < 2 * P and (n + 1 < ft or k):
                            pace.note(v)
                    pace.spread(20, 47)

            def down(k):
                for n in range(dt):
                    halves = _HK.result(_HK.accumulate(
                        lambda r: _bf(hidden_v[k % 2].at[r][...]),
                        lambda i, j: pace.load(w4_v[i * fw:(i + 1) * fw, _tile(j * dt + n)]),
                        lambda r: pace.load(s4_v.at[n][:, _tile(r)])))
                    for f, half in enumerate(halves):
                        for j, v in enumerate(half):
                            rows = _at((g * units + k) * UNIT + f * (UNIT // 2), UNIT // 2)
                            part_v[rows, _tile(j * dt + n)] += v

            for m in range(3):
                for r in range(0, kw, 8):
                    pace.note(prepare_qkv(m, r)[9])
            for r in range(0, kw, 8):
                pace.note(prepare_out(r)[9])
            loads = units * 2 * ft * dt * n_prod
            pace.spread(0.63 * loads, 0.99 * loads)
            for k in range(units):
                norm((g * units + k + 1) * UNIT, (k + 1) % 2, pace.note)
                pace.spread(0, 264)
                up(k)
                if k > 0:
                    down(k - 1)
            down(units - 1)
            return 0

        norm(0, 0)
        lax.fori_loop(0, n_grp, body, 0)

    def recurrence(sums_v, own_v, left_v, next_v, hq_v, ho_v, ahead_v):
        scale = float(Dh) ** -0.5
        row = lax.broadcasted_iota(jnp.int32, (2 * L, 2 * L), 0)
        col = lax.broadcasted_iota(jnp.int32, (2 * L, 2 * L), 1)
        r_in = jnp.where(row >= L, row - L, row)
        c_in = jnp.where(col >= L, col - L, col)
        same_head = (row >= L) == (col >= L)
        keep = same_head & ((r_in < M) | (r_in >= c_in))
        fill = jnp.where(same_head, _MASKED / scale, -jnp.inf).astype(F32)

        def load_own(s):
            own_v[...] = _ln(x_rows(s * seg, seg)[:seg - 8])

        def load_next(s, q):
            next_v[8 * q:8 * q + 8, :] = _ln(x_rows(s * seg + seg - 16, 16)[8:])

        def load_left(mem=None):
            lower = next_v[...]
            upper = lower if mem is None else jnp.concatenate([mem, own_v[...]], axis=0)
            for n, v in enumerate(_HK.left(_split(upper, P), _split(lower, P))):
                if (n in _HKQ.lower) == (mem is None):
                    left_v.at[n][...] = _words(v)

        def operands(g, m):
            return (lambda n: _bf(left_v.at[n][...]),
                    lambda i, j: _bf(wqkv_v.at[m * H + g * P + j][i * kw:(i + 1) * kw, :]),
                    lambda n: _bf(sums_v.at[m * n_grp + g][:, _tile(n)]))

        ahead = list(zip([when for when, n in AHEAD.items() for _ in range(n)],
                         [(k // 3, k % 3, n) for k in range(n_grp, 3 * n_grp) for n in _HKQ.lower]))

        def run_ahead(*now):
            for k, (when, (g, m, n)) in enumerate(ahead):
                if when in now:
                    ahead_v[k] = _HKQ.product(n, *operands(g, m))

        def by_head(apart, dot, a, b):
            return jnp.concatenate([dot(a[:L], b), dot(a[L:], b)], axis=0) if apart else dot(a, b)

        def softmax(apart, q, k):
            s = jnp.where(keep, by_head(apart, _dot_nt, q, k.astype(BF16)), fill)
            e = jnp.exp2((s - jnp.max(s, axis=-1, keepdims=True)) * (scale * _LOG2E))
            return e, pl.reciprocal(jnp.sum(e, axis=-1, keepdims=True), full_range=False)

        def step(s, r, mem):
            first, last = r == 0, r == PERIOD - 1
            if not first:
                upper = jnp.concatenate([mem, own_v[...]], axis=0)

            def project(g):
                res = []
                for m in range(3):
                    h0 = m * H + g * P
                    if first:
                        tops, rest = _HKQ.result(_HKQ.accumulate(*operands(g, m), known={
                            which[2]: ahead_v.at[k] for k, (_, which) in enumerate(ahead) if which[:2] == (g, m)}))
                        for j in range(P):
                            hq_v[h0 + j] = rest[j][8:]
                        held = [v[:8] for v in rest]
                    else:
                        tops = [_dot(upper.astype(BF16), _bf(wqkv_v[h0 + j])) for j in range(P)]
                        held = [hq_v[h0 + j, 8 * (r - 1):8 * r, :] for j in range(P)]
                    res.append([jnp.concatenate([tops[j], held[j], tops[j + 1], held[j + 1]], axis=0)
                                for j in range(0, P, 2)])
                return list(zip(*res))

            def merge(g, heads, acc):
                tops, held = [o[:L - 8] for o in heads], [o[L - 8:] for o in heads]
                if last:
                    waiting[g] = _HK.left(tops, [jnp.concatenate([ho_v[:, _tile(g * P + j)], held[j]], axis=0)
                                                 for j in range(P)])
                    if g not in (1, 4, 5, n_grp - 1):
                        return acc
                    left = {a: waiting.pop(a) for a in sorted(waiting)}
                    k = Dh // 2
                    return _HKO.accumulate(
                        lambda n: jnp.concatenate([v[n].astype(BF16) for v in left.values()], axis=1),
                        lambda i, j: jnp.concatenate([
                            _bf(wo_v[a * grows + i * k:a * grows + (i + 1) * k, j * dt * LANE:(j + 1) * dt * LANE])
                            for a in left], axis=0),
                        lambda n: jnp.concatenate([
                            jnp.concatenate([_bf(sums_v.at[3 * n_grp + a][c * k:(c + 1) * k, _tile(n)])
                                             for c in range(dt)], axis=1) for a in left], axis=0),
                        acc or ())
                for j in range(P):
                    ho_v[8 * r:8 * r + 8, _tile(g * P + j)] = held[j]
                y = _dot(jnp.concatenate(tops, axis=1).astype(BF16), _bf(wo_v[g * grows:(g + 1) * grows, :]))
                return y if acc is None else acc + y

            lag, late = (4, (5, 6)) if last else (5, (4, 6)) if first else (5, (4, 5))
            qkv, prob, heads, waiting = {}, {}, {}, {}
            acc, done = None, 0
            for t in range(n_grp + 3):
                if t < n_grp:
                    qkv[t] = project(t)
                while done < (t - lag + 1 if t < n_grp else (late + (n_grp,))[t - n_grp]):
                    run_ahead((r, done))
                    acc = merge(done, heads.pop(done), acc)
                    done += 1
                if 0 <= t - 2 < n_grp:
                    heads[t - 2] = []
                    for (e, inv), (_, _, v) in zip(prob.pop(t - 2), qkv.pop(t - 2)):
                        o = by_head(t - 2 == n_grp - 1, _dot, e, v.astype(BF16)) * inv
                        heads[t - 2] += [o[:L], o[L:]]
                if 0 <= t - 1 < n_grp:
                    prob[t - 1] = [softmax(t == 1, q, k) for q, k, _ in qkv[t - 1]]
                if first and 1 <= t <= PERIOD:
                    load_next(jnp.minimum(s + PERIOD - 1 + t, n_seg - 1), t - 1)
                if first and t == n_grp:
                    load_left()
                if t == n_grp - 1:
                    load_own(jnp.minimum(s + 1, n_seg - 1))
            run_ahead((r, n_grp))
            if last:
                y, y_held = [jnp.concatenate(half, axis=1) for half in _HK.result(acc)]
                load_left(y[:M])
            else:
                y = acc
            base = x_rows(s * seg, seg) + _GELU_OUT * part_v[_at(s * seg, seg), :]
            x_v[_at(s * (seg // 2), 8), :] = _words(base[:16] + y[M:M + 16])
            tail = jnp.concatenate([base[16:24] + y[M + 16:], base[24:]], axis=0)
            if not last:
                part_v[_at(s * seg + 16, 16), :] = tail
            else:
                for q in range(PERIOD):
                    r0 = (s - r + q) * seg + 16
                    rest = part_v[_at(r0, 16), :] if q < r else tail
                    x_v[_at(r0 // 2, 8), :] = _words(jnp.concatenate(
                        [rest[:8], rest[8:] + y_held[8 * q:8 * q + 8]], axis=0))
            return y[:M]

        def period(p, _):
            mem = None
            for r in range(PERIOD):
                mem = step(p * PERIOD + r, r, mem)
            out_copy(_at(p * (PERIOD * seg // 2), PERIOD * seg // 2)).start()
            return 0

        mem0_copy.wait()
        for q in range(PERIOD):
            load_next(q, q)
        load_left()
        run_ahead(*AHEAD)
        load_own(0)
        load_left(mem0_v[...].astype(F32))
        lax.fori_loop(0, n_seg // PERIOD, period, 0)

    def with_attention_sums(sums_v):
        pl.run_scoped(
            functools.partial(channel_mlp, sums_v),
            *[pltpu.VMEM((n_prod, UNIT // 4, k // P), U32) for k in (D, D, FF, FF)])
        pl.run_scoped(
            functools.partial(recurrence, sums_v),
            pltpu.VMEM((seg - 8, D), F32),
            pltpu.VMEM((n_prod, (L - 8) // 2, D // P), U32),
            pltpu.VMEM((8 * PERIOD, D), F32),
            pltpu.VMEM((3 * H, 8 * (PERIOD - 1), Dh), F32),
            pltpu.VMEM((8 * (PERIOD - 1), H * Dh), F32),
            pltpu.VMEM((sum(AHEAD.values()), L - 8, Dh), F32))

    pl.run_scoped(
        token_mixing,
        pltpu.VMEM((D // LANE, S + 16, LANE), F32),
        pltpu.VMEM((2, D // 2, D), U32),
        pltpu.VMEM((len(_HK12[0].products), TM // 8, D // _HK12[0].p), U32),
        *[pltpu.VMEM((D // hk.p // LANE, D // 2 // hk.p, len(hk.summed) * LANE), U32) for hk in _HK12],
        *[pltpu.VMEM((2, len(hk.products), UNIT // 4, D // hk.p), U32) for hk in _HK12])
    pl.run_scoped(with_attention_sums, pltpu.VMEM((4 * n_grp, kw, len(_HK.summed) * LANE), U32))
    out_copy(slice(0, S // 2)).wait()


@functools.partial(jax.jit, static_argnames=("A_seg_len",))
def pallas_parallel_sum__memory_aug_recurrent_mem_tr__mixer_s_mlp__prompt_kernel(
    A_x: jax.Array,
    A_mem0: jax.Array,
    A_Wq: jax.Array,
    A_Wk: jax.Array,
    A_Wv: jax.Array,
    A_Wo: jax.Array,
    A_seg_len: int,
    B_x: jax.Array,
    B_w1: jax.Array,
    B_w2: jax.Array,
    B_w3: jax.Array,
    B_w4: jax.Array,
):
    del B_x
    B, S, D = A_x.shape
    H, Dh = A_Wq.shape[1:]
    M = A_mem0.shape[1]
    FF = B_w3.shape[1]
    assert (B, S, D, H, Dh, M, A_seg_len) == (1, 2048, 1024, 32, 128, 8, 32)
    sums = len(_HK.summed) * LANE

    hbm = pl.BlockSpec(memory_space=pl.ANY)
    out = pl.pallas_call(
        functools.partial(_kernel, seg=A_seg_len),
        out_shape=jax.ShapeDtypeStruct((S, D), A_x.dtype),
        in_specs=[hbm] * 10,
        out_specs=hbm,
        scratch_shapes=[
            pltpu.VMEM(((S + UNIT) // 2, D), U32),
            pltpu.VMEM((S + UNIT, D), F32),
            pltpu.VMEM((M, D), A_mem0.dtype),
            pltpu.VMEM((3 * H, D // 2, Dh), U32),
            pltpu.VMEM((H * Dh // 2, D), U32),
            pltpu.VMEM((2, 3 * P, D // 2, Dh), U32),
            pltpu.VMEM((D // 2, FF), U32),
            pltpu.VMEM((FF // 2, D), U32),
            pltpu.VMEM((FF // P // LANE, D // 2 // P, sums), U32),
            pltpu.VMEM((D // P // LANE, FF // 2 // P, sums), U32),
            pltpu.SemaphoreType.DMA((S // TM + 2,)),
            pltpu.SemaphoreType.DMA((2, D // 2 // LANE)),
            pltpu.SemaphoreType.DMA((S // TM,)),
            pltpu.SemaphoreType.DMA((H // P,)),
            pltpu.SemaphoreType.DMA,
            pltpu.SemaphoreType.DMA,
        ],
        compiler_params=pltpu.CompilerParams(
            vmem_limit_bytes=127 * 1024 * 1024, disable_bounds_checks=True),
    )(A_x.reshape(S, D), A_mem0.reshape(M, D),
      *[w.reshape(D // 2, 2, H, Dh) for w in (A_Wq, A_Wk, A_Wv)],
      A_Wo.reshape(H * Dh, D), B_w1, B_w2, B_w3, B_w4)
    return out.reshape(B, S, D)
```

```python
import functools

import jax
import jax.numpy as jnp
import numpy as np
from jax import lax
import jax.experimental.pallas as pl
import jax.experimental.pallas.tpu as pltpu

F32 = jnp.float32
BF16 = jnp.bfloat16
U32 = jnp.uint32

_EPS = 1e-5
_MASKED = -1e9
_LOG2E = float(np.log2(np.e))
_GELU_C = float(np.sqrt(2.0 / np.pi))
_GELU_IN = float(np.cbrt(_GELU_C * 0.044715))
_GELU_OUT = 0.5 / _GELU_IN

LANE = 128
TM = 512
UNIT = 128
RC = 16
P = 4
PERIOD = 4
AHEAD = {(0, 8): 12, (1, 8): 10, (2, 8): 8, (3, 5): 2, (3, 6): 8, (3, 7): 8, (3, 8): 12}


def _dot(a, b):
    return lax.dot_general(a, b, (((1,), (0,)), ((), ())), preferred_element_type=F32)


def _dot_nt(a, b):
    return lax.dot_general(a, b, (((1,), (1,)), ((), ())), preferred_element_type=F32)


def _bf(words):
    return pltpu.bitcast(words, BF16)


def _words(x):
    return pltpu.bitcast(x.astype(BF16), U32)


def _at(start, n, align=None):
    return pl.ds(start if isinstance(start, int) else pl.multiple_of(start, align or n), n)


def _tile(j):
    return _at(j * LANE, LANE)


def _split(x, n):
    k = x.shape[1] // n
    return [x[:, i * k:(i + 1) * k] for i in range(n)]


def _same(v):
    return v


def _moments(x, note=_same):
    inv_n = 1.0 / x.shape[-1]
    xc = x - note(jnp.sum(x, axis=-1, keepdims=True)) * inv_n
    return xc, note(jnp.sum(xc * xc, axis=-1, keepdims=True)) * inv_n


def _ln(x):
    xc, var = _moments(x)
    return xc * lax.rsqrt(var + _EPS)


def _gelu(y):
    return y * (1.0 + jnp.tanh(y * (_GELU_C / _GELU_IN + y * y)))


def _signed_sum(terms):
    terms = sorted(terms, key=lambda t: -t[0])
    assert terms[0][0] > 0
    total = terms[0][1]
    for sign, value in terms[1:]:
        total = total + value if sign > 0 else total - value
    return total


class _HopcroftKerr:
    def __init__(self, p, order=None):
        own = {0: ((1, 2, 1), (2, 0, 1)), 1: ((2, 1, -1), (0, 2, 1)), 2: ((1, 1, 1), (0, 0, 1))}
        cross = {(0, 1): ((1, 0, 1, 0, 1, -1), (0, -1, 0, -1, 0, 1, -1), (-1, 0, 1, 0, 1, 0, 1)),
                 (0, 2): ((2, 0, 1, 2, 1, 1), (-1, 0, 0, -1, 0, 1, -1), (0, -1, -1, 0, -1, 0, 1)),
                 (1, 2): ((2, 1, -1, 2, 0, 1), (0, -1, -1, 0, 1, 0, 1), (1, 0, 0, -1, 0, 1, -1))}
        products, diag, uses = [], {}, {}

        def product(left, out):
            products.append((left, out))
            return len(products) - 1

        def diagonal(idx, kind):
            diag[idx] = [product([(i, f, 1) for i in idx], [(i, g, 1) for i in idx]) for f, g, _ in own[kind]]

        def pair(a, ka, b, kb):
            if ka > kb:
                return pair(b, kb, a, ka)[::-1]
            (f0, f1, s, g0, g1, t), ab, ba = cross[ka, kb]
            diagonal(a + b, 3 - ka - kb)
            used = diag[a] + diag[b] + diag[a + b] + [product(
                [(i, f0, 1) for i in a] + [(i, f1, s) for i in b],
                [(i, g0, 1) for i in a] + [(i, g1, t) for i in b])]
            return dict(zip(used, ab)), dict(zip(used, ba))

        for i in range(p):
            diagonal((i,), i % 3)
            uses[i, i] = {r: sign for r, (_, _, sign) in zip(diag[i,], own[i % 3])}
        for j in range(p):
            for i in range(j):
                if i % 3 != j % 3:
                    uses[i, j], uses[j, i] = pair((i,), i % 3, (j,), j % 3)
        for j in range(p):
            for i in range(j % 3, j, 3):
                k = i + 1
                both = (i, k) if (i, k) in diag else (k, i)
                uses[i, j], uses[j, i] = pair(both, 3 - i % 3 - k % 3, (j,), j % 3)
                for ij, kj in (((i, j), (k, j)), ((j, i), (j, k))):
                    for r, c in uses[kj].items():
                        uses[ij][r] = uses[ij].get(r, 0) - c
        self.p = p
        self.order = order or range(len(products))
        self.products = [(left, [(i, j, c[r]) for (i, j), c in sorted(uses.items()) if c.get(r)], out)
                         for r, (left, out) in enumerate(products)]
        self.summed = [r for r, (_, weight, _) in enumerate(self.products) if len(weight) > 1]
        self.lower = [r for r in self.order if all(f == 1 for _, f, _ in self.products[r][0])]

    def left(self, upper, lower):
        forms = [(u, l, u - l) for u, l in zip(upper, lower)]
        return [_signed_sum([(sign, forms[i][f]) for i, f, sign in left]) for left, _, _ in self.products]

    def right(self, n, block):
        def value(key):
            return block(*key).astype(F32) if isinstance(key[0], int) else value(key[0]) - value(key[1])

        terms = {(i, j): sign for i, j, sign in self.products[self.summed[n]][1]}
        for a, b in (((0, 3), (3, 0)), ((1, 0), (0, 3)), ((0, 1), (3, 0)), ((1, 3), ((0, 3), (3, 0)))):
            if terms.get(a, 0) * terms.get(b, 0) < 0:
                terms[a, b] = terms.pop(a)
                del terms[b]
        return _signed_sum([(sign, value(key)) for key, sign in terms.items()])

    def product(self, r, left, block, summed):
        w = summed(self.summed.index(r)) if r in self.summed else block(*self.products[r][1][0][:2])
        return _dot(left(r), w)

    def accumulate(self, left, block, summed, acc=(), known=()):
        acc = dict(acc)
        for r in self.order:
            _, weight, out = self.products[r]
            flip = 1 if r in self.summed else weight[0][2]
            m = known[r][...] if r in known else self.product(r, left, block, summed)
            for j, f, sign in out:
                if (j, f) in acc:
                    acc[j, f] = acc[j, f] + m if sign * flip > 0 else acc[j, f] - m
                else:
                    acc[j, f] = m if sign * flip > 0 else -m
        return acc

    def result(self, acc):
        return [[functools.reduce(jnp.add, [acc[j, g] for g in (f, 2) if (j, g) in acc])
                 for j in range(self.p)] for f in range(2)]


_HK = _HopcroftKerr(P, (9, 5, 18, 16, 3, 15, 1, 24, 7, 19, 0, 10, 13, 14, 2, 22, 21, 12, 11, 6, 20, 25, 23, 17, 4, 8))
_HKQ = _HopcroftKerr(P, (10, 18, 19, 7, 16, 1, 2, 9, 5, 15, 23, 20, 11, 17, 4, 8, 22, 25, 0, 13, 21, 14, 24, 3, 12, 6))
_HKO = _HopcroftKerr(P, (5, 18, 16, 9, 15, 1, 24, 7, 19, 10, 0, 22, 3, 13, 14, 2, 20, 21, 12, 6, 4, 25, 23, 17, 11, 8))
_HK12 = (_HopcroftKerr(2, (4, 0, 1, 3, 2, 5, 6)),
         _HopcroftKerr(P, (3, 9, 5, 18, 16, 15, 24, 1, 19, 7, 0, 10, 13, 14, 2, 8, 22, 6, 12, 4, 21, 20, 25, 17, 23, 11)))


class _Pace:
    def __init__(self, never):
        self.never, self.noted, self.due, self.pos = never, [], [], 0

    def note(self, v):
        u = pltpu.bitcast(jnp.broadcast_to(v, (v.shape[0], max(v.shape[1], LANE))), U32)
        self.noted.append(functools.reduce(jnp.bitwise_or, [
            u[r:r + 8, c:c + LANE] for r in range(0, u.shape[0], 8) for c in range(0, u.shape[1], LANE)]))
        return v

    def spread(self, first, last):
        n = len(self.noted)
        self.due += [(self.pos + first + (k + 1) * (last - first) / n, v) for k, v in enumerate(self.noted)]
        self.due.sort(key=lambda t: t[0])
        self.noted = []

    def load(self, words):
        self.pos += words.shape[0] // (LANE // 2)
        hints = []
        while self.due and self.due[0][0] <= self.pos:
            hints.append(self.due.pop(0)[1])
        if hints:
            hint, parts = functools.reduce(jnp.bitwise_or, hints), []
            for k in range(0, words.shape[0], LANE // 2):
                parts += [jnp.where(self.never, hint, words[k:k + 8]), words[k + 8:k + LANE // 2]]
            words = jnp.concatenate(parts, axis=0)
        return _bf(words)


def _kernel(x_hbm, mem0_hbm, wq_hbm, wk_hbm, wv_hbm, wo_hbm, w1_hbm, w2_hbm, w3_hbm, w4_hbm,
            out_hbm,
            x_v, part_v, mem0_v, wqkv_v, wo_v, raw_v, w3_v, w4_v, s3_v, s4_v,
            sem_x, sem_mix, sem_mlp, sem_attn, sem_mem, sem_out, *, seg):
    S, D = x_hbm.shape
    H, Dh = wq_hbm.shape[-2:]
    M = mem0_hbm.shape[0]
    FF = w3_hbm.shape[1]
    L = M + seg
    n_blk = S // TM
    n_seg = S // seg
    n_grp = H // P
    n_prod = len(_HK.products)
    kw = D // 2 // P
    fw = FF // 2 // P
    ft = FF // P // LANE
    dt = D // P // LANE
    grows = P * Dh // 2

    def copy(hbm, vmem, sem, *idx):
        return pltpu.make_async_copy(hbm.bitcast(U32).at[idx], vmem.at[idx], sem)

    def attn_copies(g):
        copies = [copy(wo_hbm, wo_v, sem_attn.at[g], _at(g * grows, grows))]
        for m, hbm in enumerate((wq_hbm, wk_hbm, wv_hbm)):
            for j in range(P // 2):
                for par in range(2):
                    copies.append(pltpu.make_async_copy(
                        hbm.bitcast(U32).at[:, par, g * (P // 2) + j, :],
                        raw_v.at[g % 2, m * P + 2 * j + par], sem_attn.at[g]))
        return copies

    def mlp_copies(q):
        return [copy(hbm, vmem, sem_mlp.at[q], _at(i * n + q * (n // n_blk), n // n_blk, 8))
                for hbm, vmem, n in ((w3_hbm, w3_v, kw), (w4_hbm, w4_v, fw)) for i in range(P)]

    def out_copy(rows):
        return pltpu.make_async_copy(x_v.at[rows], out_hbm.bitcast(U32).at[rows], sem_out)

    mem0_copy = pltpu.make_async_copy(mem0_hbm, mem0_v, sem_mem)

    def x_rows(r0, n):
        return _bf(x_v[_at(r0 // 2, n // 2), :]).astype(F32)

    def store_left(hk, ref, rows, size, note):
        for q in range(0, size // 2, RC):
            for n, v in enumerate(hk.left(_split(rows(q), hk.p), _split(rows(size // 2 + q), hk.p))):
                ref.at[n][q // 2:(q + RC) // 2, :] = _words(v)
                if n >= len(hk.products) - 2:
                    note(v)

    def store_right(hk, ref, rows, block):
        out, block = [], functools.cache(block)
        for n in range(len(hk.summed)):
            v = hk.right(n, block)
            ref[rows, _tile(n)] = _words(v)
            out.append(v[:8])
        return out

    def token_mixing(h_v, w_v, first_v, *buffers):
        sums_v, left_v = buffers[:2], buffers[2:]
        tiles = [D // hk.p // LANE for hk in _HK12]
        units = TM // UNIT
        loads = [t * t * len(hk.products) for t, hk in zip(tiles, _HK12)]

        def w_copies(n, j):
            return [copy((w1_hbm, w2_hbm)[n], w_v.at[n], sem_mix.at[n, j], slice(None), _tile(c * tiles[n] + j))
                    for c in range(_HK12[n].p)]

        def w2_copies(q):
            return [] if q * tiles[1] % n_blk else w_copies(1, q * tiles[1] // n_blk)

        def x_copy(i):
            return copy(x_hbm, x_v, sem_x.at[i + 2], slice((i * TM + UNIT) // 2, min(S, (i + 1) * TM + UNIT) // 2))

        def block(n, j, r=0, size=None):
            k = D // 2 // _HK12[n].p
            return lambda a, c: w_v.at[n][_at(a * k + r, size or k), _tile(c * tiles[n] + j)]

        def prepare(q, k, parts):
            size = D // 2 // _HK12[1].p * tiles[1] // n_blk // parts
            j, r = q // (n_blk // tiles[1]), (q % (n_blk // tiles[1]) * parts + k) * size
            return store_right(_HK12[1], sums_v[1].at[j], _at(r, size), lambda a, c: _bf(block(1, j, r, size)(a, c)))

        def norm(r0, ref, size, note=_same):
            def rows(r):
                xc, var = _moments(x_rows(r0 + r, RC), note)
                inv = lax.rsqrt(var + _EPS)
                part_v[_at(r0 + r, RC), :] = xc * (inv * (1.0 / _GELU_OUT))
                return xc * (inv * lax.rsqrt(var * inv * inv + _EPS) * _GELU_IN)
            store_left(_HK12[0], ref, rows, size, note)

        def shift(r0, ref, note=_same):
            def rows(r):
                return jnp.concatenate(
                    [h_v.at[c][pl.ds(r0 + r + 8 + (-1, 1, -2, 2)[4 * c * LANE // D], RC), :]
                     for c in range(D // LANE)], axis=1)
            store_left(_HK12[1], ref, rows, UNIT, note)

        def matmul(n, left, r0, load, arriving=None):
            for j in range(tiles[n]):
                def summed(k):
                    if not arriving:
                        return load(sums_v[n].at[j][:, _tile(k)])
                    w = _HK12[n].right(k, lambda a, c: _bf(block(n, j)(a, c))).astype(BF16)
                    sums_v[n].at[j][:, _tile(k)] = pltpu.bitcast(w, U32)
                    return w

                if arriving:
                    arriving(j)
                halves = _HK12[n].result(_HK12[n].accumulate(
                    lambda r: _bf(left.at[r][...]), lambda a, c: load(block(n, j)(a, c)), summed))
                for f, half in enumerate(halves):
                    for c, v in enumerate(half):
                        size = v.shape[0]
                        if n == 0:
                            h_v.at[c * tiles[n] + j][_at(8 + r0 + f * size, size, 8), :] = _gelu(v)
                        else:
                            part_v[_at(r0 + f * size, size), _tile(c * tiles[n] + j)] += v

        def h_unit(r0, k, pace):
            norm(r0 + UNIT, left_v[0].at[(k + 1) % 2], UNIT, pace.note)
            pace.spread(0.15 * loads[0], loads[0])
            matmul(0, left_v[0].at[k % 2], r0, pace.load)

        def h_body(i, _):
            for n in range(1, n_blk):
                @pl.when(i == n)
                def _():
                    for later in range(2, n_blk) if n == 1 else ():
                        for c in [x_copy(later)] + w2_copies(later - 1):
                            c.start()
                    for c in w2_copies(n_blk - 1) if n == 2 else ():
                        c.start()
                    for c in [x_copy(n)] + w2_copies(n - 1):
                        c.wait()

            for c in mlp_copies(i - 1):
                c.start()
            pace = _Pace(i < 0)
            for k in range(units):
                for v in prepare(i - 1, k, units)[::6]:
                    pace.note(v)
                pace.spread(0.65 * loads[0], loads[0])
                h_unit(i * TM + k * UNIT, k, pace)
            return 0

        def mix_body(i, _):
            @pl.when(i == 0)
            def _():
                for c in mlp_copies(n_blk - 1):
                    c.start()

            @pl.when(i == 1)
            def _():
                for c in attn_copies(0):
                    c.start()

            for c in mlp_copies(i):
                c.wait()

            def sums(w, ref, k, tiles, n, r):
                r += i * (k // n_blk)
                return jnp.concatenate(store_right(_HK, ref.at[n], _at(r, 8), lambda a, c: _bf(
                    w[_at(a * k + r, 8), _tile(c * tiles + n)])), axis=0)

            side = [functools.partial(sums, w, ref, k, tiles, n, r)
                    for w, ref, k, tiles in ((w3_v, s3_v, kw, ft), (w4_v, s4_v, fw, dt))
                    for n in range(tiles) for r in range(0, k // n_blk, 8)]
            pace = _Pace(i < 0)
            for k in range(units):
                r0 = i * TM + k * UNIT
                for task in side[k * len(side) // units:(k + 1) * len(side) // units]:
                    pace.note(task())
                pace.spread(0.05 * loads[1], 0.95 * loads[1])
                shift(jnp.minimum(r0 + UNIT, S - UNIT), left_v[1].at[(k + 1) % 2], pace.note)
                pace.spread(0, 0.9 * loads[1])
                matmul(1, left_v[1].at[k % 2], r0, pace.load)
            return 0

        cuts = (0, TM // 4, TM // 4 + UNIT // 2, (TM + UNIT) // 2)
        first = [copy(x_hbm, x_v, sem_x.at[k], slice(*cuts[k:k + 2])) for k in range(3)]
        columns = [w_copies(0, j) for j in range(tiles[0])]
        columns[1].append(first[1])
        for c in [first[0]] + sum(columns, []) + [first[2], x_copy(1)] + w2_copies(0) + [mem0_copy]:
            c.start()
        h_v[:, 0:8, :] = jnp.zeros((D // LANE, 8, LANE), F32)
        h_v[:, S + 8:S + 16, :] = jnp.zeros((D // LANE, 8, LANE), F32)
        x_v[S // 2:, :] = jnp.zeros((UNIT // 2, D), U32)
        first[0].wait()
        norm(0, first_v, TM // 2)
        pace = _Pace(jnp.square(part_v[0:8, 0:LANE]) < 0)

        def arriving(j):
            for c in columns[j]:
                c.wait()
            if j == 1:
                norm(TM // 2, left_v[0].at[units // 2 % 2], UNIT, pace.note)
                pace.spread(0, 2 * tiles[0])

        matmul(0, first_v, 0, pace.load, arriving)
        first[2].wait()
        for k in range(units // 2, units):
            h_unit(k * UNIT, k, pace)
        lax.fori_loop(1, n_blk, h_body, 0)
        shift(0, left_v[1].at[0])
        for c in w2_copies(n_blk - 1):
            c.wait()
        for k in range(8):
            prepare(n_blk - 1, k, 8)
        lax.fori_loop(0, n_blk, mix_body, 0)

    def channel_mlp(sums_v, *buffers):
        left_v, hidden_v = buffers[:2], buffers[2:]
        units = S // UNIT // n_grp

        def norm(r0, slot, note=_same):
            def rows(r):
                xc, var = _moments(part_v[_at(r0 + r, RC), :], note)
                return xc * (lax.rsqrt(var + _EPS / _GELU_OUT ** 2) * _GELU_IN)
            store_left(_HK, left_v[slot], rows, UNIT, note)

        def body(g, _):
            @pl.when(g + 1 < n_grp)
            def _():
                for c in attn_copies(g + 1):
                    c.start()

            for c in attn_copies(g):
                c.wait()
            pace = _Pace(g < 0)

            def prepare_qkv(m, r):
                blocks = {}
                for j in range(0, P, 2):
                    for i in range(P):
                        rows = slice(i * kw + r, i * kw + r + 8)
                        even, odd = raw_v.at[g % 2, m * P + j][rows, :], raw_v.at[g % 2, m * P + j + 1][rows, :]
                        for n, w in enumerate(((even & jnp.uint32(0xFFFF)) | (odd << 16),
                                               (even >> 16) | (odd & jnp.uint32(0xFFFF0000)))):
                            wqkv_v[m * H + g * P + j + n, rows, :] = w
                            blocks[i, j + n] = _bf(w)
                return store_right(_HK, sums_v.at[m * n_grp + g], slice(r, r + 8), lambda i, j: blocks[i, j])

            def prepare_out(r):
                return store_right(_HK, sums_v.at[3 * n_grp + g], slice(r, r + 8), lambda i, j: _bf(
                    wo_v[_at(g * grows + i * (Dh // 2) + r % (Dh // 2), 8), _tile(j * dt + r // (Dh // 2))]))

            def up(k):
                for n in range(ft):
                    upper, lower = _HK.result(_HK.accumulate(
                        lambda r: _bf(left_v[k % 2].at[r][...]),
                        lambda i, j: pace.load(w3_v[i * kw:(i + 1) * kw, _tile(j * ft + n)]),
                        lambda r: pace.load(s3_v.at[n][:, _tile(r)])))
                    for r, v in enumerate(_HK.left([_gelu(v) for v in upper], [_gelu(v) for v in lower])):
                        hidden_v[k % 2].at[r][:, _tile(n)] = _words(v)
                        if r < 2 * P and (n + 1 < ft or k):
                            pace.note(v)
                    pace.spread(20, 47)

            def down(k):
                for n in range(dt):
                    halves = _HK.result(_HK.accumulate(
                        lambda r: _bf(hidden_v[k % 2].at[r][...]),
                        lambda i, j: pace.load(w4_v[i * fw:(i + 1) * fw, _tile(j * dt + n)]),
                        lambda r: pace.load(s4_v.at[n][:, _tile(r)])))
                    for f, half in enumerate(halves):
                        for j, v in enumerate(half):
                            rows = _at((g * units + k) * UNIT + f * (UNIT // 2), UNIT // 2)
                            part_v[rows, _tile(j * dt + n)] += v

            for m in range(3):
                for r in range(0, kw, 8):
                    pace.note(prepare_qkv(m, r)[9])
            for r in range(0, kw, 8):
                pace.note(prepare_out(r)[9])
            loads = units * 2 * ft * dt * n_prod
            pace.spread(0.63 * loads, 0.99 * loads)
            for k in range(units):
                norm((g * units + k + 1) * UNIT, (k + 1) % 2, pace.note)
                pace.spread(0, 264)
                up(k)
                if k > 0:
                    down(k - 1)
            down(units - 1)
            return 0

        norm(0, 0)
        lax.fori_loop(0, n_grp, body, 0)

    def recurrence(sums_v, own_v, left_v, next_v, hq_v, ho_v, ahead_v):
        scale = float(Dh) ** -0.5
        row = lax.broadcasted_iota(jnp.int32, (2 * L, 2 * L), 0)
        col = lax.broadcasted_iota(jnp.int32, (2 * L, 2 * L), 1)
        r_in = jnp.where(row >= L, row - L, row)
        c_in = jnp.where(col >= L, col - L, col)
        same_head = (row >= L) == (col >= L)
        keep = same_head & ((r_in < M) | (r_in >= c_in))
        fill = jnp.where(same_head, _MASKED / scale, -jnp.inf).astype(F32)

        def load_own(s):
            own_v[...] = _ln(x_rows(s * seg, seg)[:seg - 8])

        def load_next(s, q):
            next_v[8 * q:8 * q + 8, :] = _ln(x_rows(s * seg + seg - 16, 16)[8:])

        def load_left(mem=None):
            lower = next_v[...]
            upper = lower if mem is None else jnp.concatenate([mem, own_v[...]], axis=0)
            for n, v in enumerate(_HK.left(_split(upper, P), _split(lower, P))):
                if (n in _HKQ.lower) == (mem is None):
                    left_v.at[n][...] = _words(v)

        def operands(g, m):
            return (lambda n: _bf(left_v.at[n][...]),
                    lambda i, j: _bf(wqkv_v.at[m * H + g * P + j][i * kw:(i + 1) * kw, :]),
                    lambda n: _bf(sums_v.at[m * n_grp + g][:, _tile(n)]))

        ahead = list(zip([when for when, n in AHEAD.items() for _ in range(n)],
                         [(k // 3, k % 3, n) for k in range(n_grp, 3 * n_grp) for n in _HKQ.lower]))

        def run_ahead(*now):
            for k, (when, (g, m, n)) in enumerate(ahead):
                if when in now:
                    ahead_v[k] = _HKQ.product(n, *operands(g, m))

        def by_head(apart, dot, a, b):
            return jnp.concatenate([dot(a[:L], b), dot(a[L:], b)], axis=0) if apart else dot(a, b)

        def softmax(apart, q, k):
            s = jnp.where(keep, by_head(apart, _dot_nt, q, k.astype(BF16)), fill)
            e = jnp.exp2((s - jnp.max(s, axis=-1, keepdims=True)) * (scale * _LOG2E))
            return e, pl.reciprocal(jnp.sum(e, axis=-1, keepdims=True), full_range=False)

        def step(s, r, mem):
            first, last = r == 0, r == PERIOD - 1
            if not first:
                upper = jnp.concatenate([mem, own_v[...]], axis=0)

            def project(g):
                res = []
                for m in range(3):
                    h0 = m * H + g * P
                    if first:
                        tops, rest = _HKQ.result(_HKQ.accumulate(*operands(g, m), known={
                            which[2]: ahead_v.at[k] for k, (_, which) in enumerate(ahead) if which[:2] == (g, m)}))
                        for j in range(P):
                            hq_v[h0 + j] = rest[j][8:]
                        held = [v[:8] for v in rest]
                    else:
                        tops = [_dot(upper.astype(BF16), _bf(wqkv_v[h0 + j])) for j in range(P)]
                        held = [hq_v[h0 + j, 8 * (r - 1):8 * r, :] for j in range(P)]
                    res.append([jnp.concatenate([tops[j], held[j], tops[j + 1], held[j + 1]], axis=0)
                                for j in range(0, P, 2)])
                return list(zip(*res))

            def merge(g, heads, acc):
                tops, held = [o[:L - 8] for o in heads], [o[L - 8:] for o in heads]
                if last:
                    waiting[g] = _HK.left(tops, [jnp.concatenate([ho_v[:, _tile(g * P + j)], held[j]], axis=0)
                                                 for j in range(P)])
                    if g not in (1, 4, 5, n_grp - 1):
                        return acc
                    left = {a: waiting.pop(a) for a in sorted(waiting)}
                    k = Dh // 2
                    return _HKO.accumulate(
                        lambda n: jnp.concatenate([v[n].astype(BF16) for v in left.values()], axis=1),
                        lambda i, j: jnp.concatenate([
                            _bf(wo_v[a * grows + i * k:a * grows + (i + 1) * k, j * dt * LANE:(j + 1) * dt * LANE])
                            for a in left], axis=0),
                        lambda n: jnp.concatenate([
                            jnp.concatenate([_bf(sums_v.at[3 * n_grp + a][c * k:(c + 1) * k, _tile(n)])
                                             for c in range(dt)], axis=1) for a in left], axis=0),
                        acc or ())
                for j in range(P):
                    ho_v[8 * r:8 * r + 8, _tile(g * P + j)] = held[j]
                y = _dot(jnp.concatenate(tops, axis=1).astype(BF16), _bf(wo_v[g * grows:(g + 1) * grows, :]))
                return y if acc is None else acc + y

            lag, late = (4, (5, 6)) if last else (5, (4, 6)) if first else (5, (4, 5))
            qkv, prob, heads, waiting = {}, {}, {}, {}
            acc, done = None, 0
            for t in range(n_grp + 3):
                if t < n_grp:
                    qkv[t] = project(t)
                while done < (t - lag + 1 if t < n_grp else (late + (n_grp,))[t - n_grp]):
                    run_ahead((r, done))
                    acc = merge(done, heads.pop(done), acc)
                    done += 1
                if 0 <= t - 2 < n_grp:
                    heads[t - 2] = []
                    for (e, inv), (_, _, v) in zip(prob.pop(t - 2), qkv.pop(t - 2)):
                        o = by_head(t - 2 == n_grp - 1, _dot, e, v.astype(BF16)) * inv
                        heads[t - 2] += [o[:L], o[L:]]
                if 0 <= t - 1 < n_grp:
                    prob[t - 1] = [softmax(t == 1, q, k) for q, k, _ in qkv[t - 1]]
                if first and 1 <= t <= PERIOD:
                    load_next(jnp.minimum(s + PERIOD - 1 + t, n_seg - 1), t - 1)
                if first and t == n_grp:
                    load_left()
                if t == n_grp - 1:
                    load_own(jnp.minimum(s + 1, n_seg - 1))
            run_ahead((r, n_grp))
            if last:
                y, y_held = [jnp.concatenate(half, axis=1) for half in _HK.result(acc)]
                load_left(y[:M])
            else:
                y = acc
            base = x_rows(s * seg, seg) + _GELU_OUT * part_v[_at(s * seg, seg), :]
            x_v[_at(s * (seg // 2), 8), :] = _words(base[:16] + y[M:M + 16])
            tail = jnp.concatenate([base[16:24] + y[M + 16:], base[24:]], axis=0)
            if not last:
                part_v[_at(s * seg + 16, 16), :] = tail
            else:
                for q in range(PERIOD):
                    r0 = (s - r + q) * seg + 16
                    rest = part_v[_at(r0, 16), :] if q < r else tail
                    x_v[_at(r0 // 2, 8), :] = _words(jnp.concatenate(
                        [rest[:8], rest[8:] + y_held[8 * q:8 * q + 8]], axis=0))
            return y[:M]

        def period(p, _):
            mem = None
            for r in range(PERIOD):
                mem = step(p * PERIOD + r, r, mem)
            out_copy(_at(p * (PERIOD * seg // 2), PERIOD * seg // 2)).start()
            return 0

        mem0_copy.wait()
        for q in range(PERIOD):
            load_next(q, q)
        load_left()
        run_ahead(*AHEAD)
        load_own(0)
        load_left(mem0_v[...].astype(F32))
        lax.fori_loop(0, n_seg // PERIOD, period, 0)

    def with_attention_sums(sums_v):
        pl.run_scoped(
            functools.partial(channel_mlp, sums_v),
            *[pltpu.VMEM((n_prod, UNIT // 4, k // P), U32) for k in (D, D, FF, FF)])
        pl.run_scoped(
            functools.partial(recurrence, sums_v),
            pltpu.VMEM((seg - 8, D), F32),
            pltpu.VMEM((n_prod, (L - 8) // 2, D // P), U32),
            pltpu.VMEM((8 * PERIOD, D), F32),
            pltpu.VMEM((3 * H, 8 * (PERIOD - 1), Dh), F32),
            pltpu.VMEM((8 * (PERIOD - 1), H * Dh), F32),
            pltpu.VMEM((sum(AHEAD.values()), L - 8, Dh), F32))

    pl.run_scoped(
        token_mixing,
        pltpu.VMEM((D // LANE, S + 16, LANE), F32),
        pltpu.VMEM((2, D // 2, D), U32),
        pltpu.VMEM((len(_HK12[0].products), TM // 8, D // _HK12[0].p), U32),
        *[pltpu.VMEM((D // hk.p // LANE, D // 2 // hk.p, len(hk.summed) * LANE), U32) for hk in _HK12],
        *[pltpu.VMEM((2, len(hk.products), UNIT // 4, D // hk.p), U32) for hk in _HK12])
    pl.run_scoped(with_attention_sums, pltpu.VMEM((4 * n_grp, kw, len(_HK.summed) * LANE), U32))
    out_copy(slice(0, S // 2)).wait()


@functools.partial(jax.jit, static_argnames=("A_seg_len",))
def pallas_parallel_sum__memory_aug_recurrent_mem_tr__mixer_s_mlp__prompt_kernel(
    A_x: jax.Array,
    A_mem0: jax.Array,
    A_Wq: jax.Array,
    A_Wk: jax.Array,
    A_Wv: jax.Array,
    A_Wo: jax.Array,
    A_seg_len: int,
    B_x: jax.Array,
    B_w1: jax.Array,
    B_w2: jax.Array,
    B_w3: jax.Array,
    B_w4: jax.Array,
):
    del B_x
    B, S, D = A_x.shape
    H, Dh = A_Wq.shape[1:]
    M = A_mem0.shape[1]
    FF = B_w3.shape[1]
    assert (B, S, D, H, Dh, M, A_seg_len) == (1, 2048, 1024, 32, 128, 8, 32)
    sums = len(_HK.summed) * LANE

    hbm = pl.BlockSpec(memory_space=pl.ANY)
    out = pl.pallas_call(
        functools.partial(_kernel, seg=A_seg_len),
        out_shape=jax.ShapeDtypeStruct((S, D), A_x.dtype),
        in_specs=[hbm] * 10,
        out_specs=hbm,
        scratch_shapes=[
            pltpu.VMEM(((S + UNIT) // 2, D), U32),
            pltpu.VMEM((S + UNIT, D), F32),
            pltpu.VMEM((M, D), A_mem0.dtype),
            pltpu.VMEM((3 * H, D // 2, Dh), U32),
            pltpu.VMEM((H * Dh // 2, D), U32),
            pltpu.VMEM((2, 3 * P, D // 2, Dh), U32),
            pltpu.VMEM((D // 2, FF), U32),
            pltpu.VMEM((FF // 2, D), U32),
            pltpu.VMEM((FF // P // LANE, D // 2 // P, sums), U32),
            pltpu.VMEM((D // P // LANE, FF // 2 // P, sums), U32),
            pltpu.SemaphoreType.DMA((S // TM + 2,)),
            pltpu.SemaphoreType.DMA((2, D // 2 // LANE)),
            pltpu.SemaphoreType.DMA((S // TM,)),
            pltpu.SemaphoreType.DMA((H // P,)),
            pltpu.SemaphoreType.DMA,
            pltpu.SemaphoreType.DMA,
        ],
        compiler_params=pltpu.CompilerParams(
            vmem_limit_bytes=127 * 1024 * 1024, disable_bounds_checks=True),
    )(A_x.reshape(S, D), A_mem0.reshape(M, D),
      *[w.reshape(D // 2, 2, H, Dh) for w in (A_Wq, A_Wk, A_Wv)],
      A_Wo.reshape(H * Dh, D), B_w1, B_w2, B_w3, B_w4)
    return out.reshape(B, S, D)
```
